```python
import jax
import jax.numpy as jnp

def _softmax(x, axis=-1):
    return jax.nn.softmax(x, axis=axis)
def _gelu(x):
    return jax.nn.gelu(x, approximate=True)
def _silu(x):
    return jax.nn.silu(x)
def _sigmoid(x):
    return jax.nn.sigmoid(x)
def _layernorm(x, axis=-1, eps=1e-5):
    m = jnp.mean(x, axis=axis, keepdims=True)
    v = jnp.var(x, axis=axis, keepdims=True)
    return (x - m) / jnp.sqrt(v + eps)
def _scatter_add(tgt, idx, src, axis=0):
    return tgt.at[idx].add(src)
def _segment_sum(src, seg, n):
    return jax.ops.segment_sum(src, seg, n)
class _Rng:
    def __init__(self, key):
        self._k = key
    def _next(self):
        self._k, sub = jax.random.split(self._k)
        return sub
    def normal(self, shape):
        return jax.random.normal(self._next(), shape, dtype=jnp.bfloat16)
    def randint(self, lo, hi, shape):
        return jax.random.randint(self._next(), shape, lo, hi, dtype=jnp.int32)
    def uniform(self, shape, lo=0.0, hi=1.0):
        return jax.random.uniform(self._next(), shape, jnp.bfloat16, lo, hi)
    def permutation(self, n):
        return jax.random.permutation(self._next(), n)


kernel_name = 'sequential_preLN__linear_kernel_hedgehog__moe_arch_mod__prompt'

def setup_inputs():
    _rng = _Rng(jax.random.key(int.from_bytes(__import__("os").urandom(4), "little")))
    _w = (lambda a: (lambda t: t.astype(jnp.bfloat16) if jnp.issubdtype(t.dtype, jnp.floating) else t)(jnp.asarray(a)))
    def _A_setup():
        B, S, D, H = 1, 2048, 1024, 32
        Dh = D // H
        return {
            "x": _w((lambda *s: _rng.normal(s) * 0.05)(B, S, D)),
            "wqkv": _w((lambda *s: _rng.normal(s) * 0.05)(D, 3 * D)),
            "w_phi": _w((lambda *s: _rng.normal(s) * 0.05)(H, Dh, Dh) * (Dh ** -0.5)),
            "wo": _w((lambda *s: _rng.normal(s) * 0.05)(D, D)),
        }
    _A_in = _A_setup()

    def _B_setup():
        B, S, D, F, C = 1, 2048, 1024, 3584, 1
        return {
            "x": _w((lambda *s: _rng.normal(s) * 0.05)(B, S, D)),
            "w_r": _w((lambda *s: _rng.normal(s) * 0.05)(D)),
            "w_gate": _w((lambda *s: _rng.normal(s) * 0.05)(D, F)),
            "w_up": _w((lambda *s: _rng.normal(s) * 0.05)(D, F)),
            "w_down": _w((lambda *s: _rng.normal(s) * 0.05)(F, D)),
        }
    _B_in = _B_setup()

    return {
        "A_x": _A_in["x"],
        "A_wqkv": _A_in["wqkv"],
        "A_w_phi": _A_in["w_phi"],
        "A_wo": _A_in["wo"],
        "B_x": _B_in["x"],
        "B_w_r": _B_in["w_r"],
        "B_w_gate": _B_in["w_gate"],
        "B_w_up": _B_in["w_up"],
        "B_w_down": _B_in["w_down"],
    }

def reference(A_x, A_wqkv, A_w_phi, A_wo, B_x, B_w_r, B_w_gate, B_w_up, B_w_down):
    def _A_ref(x, wqkv, w_phi, wo):
        B, S, D = x.shape
        H = 32; Dh = D // H
        qkv = (lambda x, *d: x.transpose(*d))((x @ wqkv).reshape(B, S, 3, H, Dh), 2, 0, 3, 1, 4)
        q, k, v = qkv[0], qkv[1], qkv[2]
        pq = jnp.einsum("bhsd,hdf->bhsf", q, w_phi)
        pk = jnp.einsum("bhsd,hdf->bhsf", k, w_phi)
        phi_q = jnp.concatenate([_softmax(pq, axis=-1), _softmax(-pq, axis=-1)], axis=-1)
        phi_k = jnp.concatenate([_softmax(pk, axis=-1), _softmax(-pk, axis=-1)], axis=-1)
        kv = jnp.einsum("bhsf,bhsd->bhfd", phi_k, v)
        z  = jnp.einsum("bhsf->bhf", phi_k)
        num = jnp.einsum("bhqf,bhfd->bhqd", phi_q, kv)
        den = jnp.einsum("bhqf,bhf->bhq", phi_q, z)[..., None] + 1e-6
        o = num / den
        return (lambda x, *d: x.transpose(*d))(o, 0, 2, 1, 3).reshape(B, S, D) @ wo

    def _B_ref(x, w_r, w_gate, w_up, w_down):
        B, S, D = x.shape
        C = 1
        r = x @ w_r
        idx = jnp.argsort(-r, axis=-1)[:, :C]
        idx_e = jnp.repeat(idx.reshape(B, C, 1), D, axis=2)
        x_sel = jnp.take_along_axis(x, idx_e, axis=1)
        g = _silu(x_sel @ w_gate)
        u = x_sel @ w_up
        y = (g * u) @ w_down
        r_sel = _sigmoid(jnp.take_along_axis(r, idx, axis=1))
        y = y * r_sel.reshape(B, C, 1)
        b_off = (jnp.arange(B) * S).reshape(B, 1)
        flat_idx = (idx + b_off).reshape(B * C)
        zero = (x * 0.0).reshape(B * S, D)
        upd = _scatter_add(zero, flat_idx, y.reshape(B * C, D), axis=0)
        return x + upd.reshape(B, S, D)

    x = A_x
    h = x + _A_ref(_layernorm(x, axis=-1), A_wqkv, A_w_phi, A_wo)
    h2 = h + _B_ref(_layernorm(h, axis=-1), B_w_r, B_w_gate, B_w_up, B_w_down)
    return h2
```

```python
import functools

import jax
import jax.numpy as jnp
from jax import lax
import jax.experimental.pallas as pl
import jax.experimental.pallas.tpu as pltpu

S = 2048
D = 1024
H = 32
DH = 32
F = 3584
NP = H // 2
T = 256
NT = S // T
LOG2E = 1.4426950408889634
EPS = 1e-5

f32 = jnp.float32
bf16 = jnp.bfloat16


def _dot_nt(a, b):
    return lax.dot_general(a, b, (((1,), (1,)), ((), ())), preferred_element_type=f32)


def _dot_tn(a, b):
    return lax.dot_general(a, b, (((0,), (0,)), ((), ())), preferred_element_type=f32)


def _dot(a, b):
    return jnp.dot(a, b, preferred_element_type=f32)


def _allred(v, op):
    v = op(v, pltpu.roll(v, 2, 0))
    return op(v, pltpu.roll(v, 4, 0))


def _phi(x):
    L = x.shape[1]
    x3 = x.reshape(8, 8, L)
    mx = _allred(jnp.max(x3, axis=0), jnp.maximum)
    mn = _allred(jnp.min(x3, axis=0), jnp.minimum)
    ep = jnp.exp2(x3 - mx[None])
    en = jnp.exp2(mn[None] - x3)
    rp = 1.0 / _allred(jnp.sum(ep, axis=0), jnp.add)
    rn = 1.0 / _allred(jnp.sum(en, axis=0), jnp.add)
    pp = (ep * rp[None]).reshape(64, L).astype(bf16)
    pn = (en * rn[None]).reshape(64, L).astype(bf16)
    return jnp.concatenate([pp, pn], axis=0)


def _ln(x):
    m = jnp.mean(x, axis=-1, keepdims=True)
    xc = x - m
    v = jnp.mean(xc * xc, axis=-1, keepdims=True)
    return xc * lax.rsqrt(v + EPS)


def _kernel(x_hbm, wqkv_hbm, wphi_hbm, wo_hbm, wr_hbm, wg_hbm, wu_hbm, wd_hbm, out_hbm,
            x_v, wqkv_v, wphi_v, wo_v, wr_v, wg_v, wu_v, wd_v,
            wt_v, xn_v, kv_acc, kvz_v, out_v, r_v, sems, xsems, osems):
    cp_phi = pltpu.make_async_copy(wphi_hbm, wphi_v, sems.at[0])
    cp_wk = pltpu.make_async_copy(wqkv_hbm.at[:, D:2 * D], wqkv_v.at[:, D:2 * D], sems.at[1])
    cp_wv = pltpu.make_async_copy(wqkv_hbm.at[:, 2 * D:3 * D], wqkv_v.at[:, 2 * D:3 * D], sems.at[2])
    cp_wq = pltpu.make_async_copy(wqkv_hbm.at[:, 0:D], wqkv_v.at[:, 0:D], sems.at[3])
    cp_wo = pltpu.make_async_copy(wo_hbm, wo_v, sems.at[4])
    cp_wr = pltpu.make_async_copy(wr_hbm, wr_v, sems.at[5])
    cp_wg = pltpu.make_async_copy(wg_hbm, wg_v, sems.at[6])
    cp_wu = pltpu.make_async_copy(wu_hbm, wu_v, sems.at[7])
    cp_wd = pltpu.make_async_copy(wd_hbm, wd_v, sems.at[8])

    def cp_x(i):
        return pltpu.make_async_copy(x_hbm.at[0, pl.ds(i * T, T)], x_v.at[pl.ds(i * T, T)], xsems.at[i])

    def cp_out(i):
        return pltpu.make_async_copy(out_v.at[pl.ds(i * T, T)], out_hbm.at[0, pl.ds(i * T, T)], osems.at[i])

    cp_phi.start()
    cp_wk.start()
    cp_x(0).start()
    cp_wv.start()
    cp_wq.start()
    for i in range(1, NT):
        cp_x(i).start()
    cp_wo.start()
    cp_wr.start()

    cp_phi.wait()
    w2 = wphi_v[...].reshape(H * DH, DH)
    r_i = lax.broadcasted_iota(jnp.int32, (128, DH), 0)
    f_i = lax.broadcasted_iota(jnp.int32, (128, DH), 1)
    sel = jnp.where(f_i == (r_i % 64) // 2, 1.0, 0.0).astype(bf16)
    a_full = _dot_nt(sel, w2)
    r_i = lax.broadcasted_iota(jnp.int32, (128, D), 0)
    c_i = lax.broadcasted_iota(jnp.int32, (128, D), 1)
    a_full = jnp.where((c_i % 128) // 32 == 2 * (r_i // 64) + r_i % 2, a_full, 0.0).astype(bf16)

    def fold(base):
        for g in range(8):
            w = wqkv_v[:, base + 128 * g: base + 128 * (g + 1)]
            wt_v[base + 128 * g: base + 128 * (g + 1), :] = (
                _dot_nt(a_full[:, 128 * g:128 * (g + 1)], w) * LOG2E).astype(bf16)

    cp_wk.wait()
    fold(D)
    cp_wv.wait()
    for g in range(8):
        wt_v[2 * D + 128 * g: 2 * D + 128 * (g + 1), :] = wqkv_v[:, 2 * D + 128 * g: 2 * D + 128 * (g + 1)].T
    cp_wq.wait()
    fold(0)
    cp_wg.start()
    cp_wu.start()
    cp_wd.start()

    kv_acc[...] = jnp.zeros(kv_acc.shape, f32)
    ones16 = jnp.ones((16, T), bf16)

    def phase1(i, c):
        s = pl.multiple_of(i * T, T)
        cp_x(i).wait()
        xn = _ln(x_v[pl.ds(s, T), :].astype(f32)).astype(bf16)
        xn_v[pl.ds(s, T), :] = xn
        y = _dot_nt(wt_v[D:3 * D, :], xn)
        for p in range(NP):
            phi = _phi(y[64 * p:64 * (p + 1)])
            lhs = jnp.concatenate([y[D + 64 * p: D + 64 * (p + 1)].astype(bf16), ones16], axis=0)
            kv_acc[p] += _dot_nt(lhs, phi)
        return c

    lax.fori_loop(0, NT, phase1, 0)

    r_i = lax.broadcasted_iota(jnp.int32, (80, 128), 0)
    c_i = lax.broadcasted_iota(jnp.int32, (80, 128), 1)
    hl_row = jnp.where(r_i < 64, r_i // 32, (r_i - 64) // 8)
    kmask = hl_row == c_i % 2
    for p in range(NP):
        kvz_v[p] = jnp.where(kmask, kv_acc[p], 0.0).astype(bf16)

    cp_wo.wait()
    cp_wr.wait()
    wr = wr_v[...].astype(f32)

    def phase2(i, c):
        s = pl.multiple_of(i * T, T)
        xn = xn_v[pl.ds(s, T), :]
        y = _dot_nt(wt_v[0:D, :], xn)
        os = []
        for p in range(NP):
            phi = _phi(y[64 * p:64 * (p + 1)])
            nd = _dot(kvz_v[p], phi)
            inv0 = 1.0 / (nd[64:72] + 1e-6)
            inv1 = 1.0 / (nd[72:80] + 1e-6)
            o0 = (nd[0:32].reshape(4, 8, T) * inv0[None]).reshape(32, T)
            o1 = (nd[32:64].reshape(4, 8, T) * inv1[None]).reshape(32, T)
            os.append(o0.astype(bf16))
            os.append(o1.astype(bf16))
        ot = jnp.concatenate(os, axis=0)
        h = x_v[pl.ds(s, T), :].astype(f32) + _dot_tn(ot, wo_v[...])
        hn = _ln(h)
        r_v[pl.ds(s, T), :] = jnp.sum(hn * wr, axis=-1, keepdims=True)
        xn_v[pl.ds(s, T), :] = hn.astype(bf16)
        out_v[pl.ds(s, T), :] = (h + hn).astype(bf16)
        cp_out(i).start()
        return c

    lax.fori_loop(0, NT, phase2, 0)

    r = r_v[...]
    rmax = jnp.max(r, axis=0, keepdims=True)
    t_i = lax.broadcasted_iota(jnp.int32, (S, 1), 0)
    idx = jnp.min(jnp.where(r == rmax, t_i, S - 1))
    base = pl.multiple_of((idx // 16) * 16, 16)
    xs = xn_v[pl.ds(base, 16), :]
    cp_wg.wait()
    cp_wu.wait()
    g = _dot(xs, wg_v[...])
    u = _dot(xs, wu_v[...])
    a = (g * jax.nn.sigmoid(g) * u).astype(bf16)
    cp_wd.wait()
    yv = _dot(a, wd_v[...]) * jax.nn.sigmoid(rmax)
    for i in range(NT):
        cp_out(i).wait()
    row = lax.broadcasted_iota(jnp.int32, (16, D), 0)
    cur = out_v[pl.ds(base, 16), :].astype(f32)
    out_v[pl.ds(base, 16), :] = jnp.where(row == idx - base, cur + yv, cur).astype(bf16)
    cp_fin = pltpu.make_async_copy(out_v.at[pl.ds(base, 16)], out_hbm.at[0, pl.ds(base, 16)], sems.at[9])
    cp_fin.start()
    cp_fin.wait()


@jax.jit
def pallas_sequential_preLN__linear_kernel_hedgehog__moe_arch_mod__prompt_kernel(
    A_x: jax.Array,
    A_wqkv: jax.Array,
    A_w_phi: jax.Array,
    A_wo: jax.Array,
    B_x: jax.Array,
    B_w_r: jax.Array,
    B_w_gate: jax.Array,
    B_w_up: jax.Array,
    B_w_down: jax.Array,
):
    del B_x
    any_spec = pl.BlockSpec(memory_space=pl.ANY)
    return pl.pallas_call(
        _kernel,
        out_shape=jax.ShapeDtypeStruct((1, S, D), bf16),
        in_specs=[any_spec] * 8,
        out_specs=any_spec,
        scratch_shapes=[
            pltpu.VMEM((S, D), bf16),
            pltpu.VMEM((D, 3 * D), bf16),
            pltpu.VMEM((H, DH, DH), bf16),
            pltpu.VMEM((D, D), bf16),
            pltpu.VMEM((1, D), bf16),
            pltpu.VMEM((D, F), bf16),
            pltpu.VMEM((D, F), bf16),
            pltpu.VMEM((F, D), bf16),
            pltpu.VMEM((3 * D, D), bf16),
            pltpu.VMEM((S, D), bf16),
            pltpu.VMEM((NP, 80, 128), f32),
            pltpu.VMEM((NP, 80, 128), bf16),
            pltpu.VMEM((S, D), bf16),
            pltpu.VMEM((S, 1), f32),
            pltpu.SemaphoreType.DMA((10,)),
            pltpu.SemaphoreType.DMA((NT,)),
            pltpu.SemaphoreType.DMA((NT,)),
        ],
        compiler_params=pltpu.CompilerParams(vmem_limit_bytes=100 * 1024 * 1024),
        name="hedgehog_mod",
    )(A_x, A_wqkv, A_w_phi, A_wo, B_w_r.reshape(1, D), B_w_gate, B_w_up, B_w_down)
```

```python
import jax
import jax.numpy as jnp
from jax import lax
import jax.experimental.pallas as pl
import jax.experimental.pallas.tpu as pltpu

S = 2048
D = 1024
H = 32
DH = 32
F = 3584
NP = H // 2
T = 512
NT = S // T
CHUNKS = [int(c) for c in '128,128,128,128'.split(",")]
CL = CHUNKS[-1]
SCHED = 'M5,V2,M3,V2,M3,V2,M3,V2,D6,V2,D6,V2,D2,V2'.split(",")
NBM = sum(int(t[1:]) for t in SCHED if t[0] == 'M')
NB = F // 128
FM = NBM * 128
RAWG = 3
RAWD = 2
FD = F - 128 * RAWD
REL = 2 * (NBM - RAWG) * D + 8 * FD
RELG = REL // (NT - 1)
assert REL % (NT - 1) == 0 and RELG % 256 == 0
ONLY1 = 0; ONLY2 = 0
K0 = 256; K1 = 512; V0 = 512; PH0 = 32
ORDER = 0
G = 16; NREL = 6
NXR = 1536; NXJ = 2
RLO = 1280; RB = 256; RJ = 3
LOG2E = 1.4426950408889634
EPS = 1e-5

f32 = jnp.float32
bf16 = jnp.bfloat16
u32 = jnp.uint32


def _dot_nt(a, b):
    return lax.dot_general(a, b, (((1,), (1,)), ((), ())), preferred_element_type=f32)


def _dot(a, b):
    return jnp.dot(a, b, preferred_element_type=f32)


def _pk(x):
    return pltpu.bitcast(x, u32)


def _un(x):
    return pltpu.bitcast(x, bf16)


def _rcp(x):
    r = pl.reciprocal(x, approx=True)
    return r * (2.0 - x * r)


def _allred(v, op):
    v = op(v, pltpu.roll(v, 2, 0))
    return op(v, pltpu.roll(v, 4, 0))


def _allred8(v, op):
    return _allred(op(v, pltpu.roll(v, 1, 0)), op)


def _exps(x):
    L = x.shape[1]
    x3 = x.reshape(8, 8, L)
    mx = _allred(jnp.max(x3, axis=0), jnp.maximum)
    mn = _allred(jnp.min(x3, axis=0), jnp.minimum)
    ep = jnp.exp2(x3 - mx[None])
    en = jnp.exp2(mn[None] - x3)
    rp = _rcp(_allred(jnp.sum(ep, axis=0), jnp.add))
    rn = _rcp(_allred(jnp.sum(en, axis=0), jnp.add))
    return ep, en, rp, rn


def _phi_k(x):
    L = x.shape[1]
    ep, en, rp, rn = _exps(x)
    phi = jnp.concatenate([(ep * rp[None]).reshape(64, L), (en * rn[None]).reshape(64, L)], axis=0)
    z = phi[:, 0:128]
    for c in range(128, L, 128):
        z = z + phi[:, c:c + 128]
    return phi.astype(bf16), z


def _phi_q(x, zb):
    L = x.shape[1]
    ep, en, rp, rn = _exps(x)
    zb = jnp.concatenate([zb] * (L // 128), axis=1).reshape(16, 8, L)
    den = rp * jnp.sum(ep * zb[0:8], axis=0) + rn * jnp.sum(en * zb[8:16], axis=0)
    inv = _rcp(_allred(den, jnp.add) + 1e-6)
    cp = rp * inv
    cn = rn * inv
    phi = jnp.concatenate([(ep * cp[None]).reshape(64, L), (en * cn[None]).reshape(64, L)], axis=0)
    return phi.astype(bf16)


def _ln(x, deps=None, zm=None):
    if deps is None:
        tot = jnp.sum(x, axis=-1, keepdims=True)
    else:
        g = x.shape[0] // len(deps)
        gate = jnp.concatenate(
            [jnp.zeros((8, 128), f32) if d is None else pltpu.bitcast(pltpu.bitcast(d, u32) & zm, f32)
             for d in deps for _ in range(g // 8)], axis=0)
        acc = x[:, 0:128] + gate
        for c in range(128, D, 128):
            acc = acc + x[:, c:c + 128]
        tot = jnp.sum(acc, axis=-1, keepdims=True)
    xc = x - tot * (1.0 / D)
    return xc * lax.rsqrt(jnp.sum(xc * xc, axis=-1, keepdims=True) * (1.0 / D) + EPS)


def _gated_pk(w, dep, zm):
    w = _pk(w)
    z = pltpu.bitcast(dep, u32) & zm
    return (w.reshape(w.shape[0] // 8, 8, 128) | z[None]).reshape(w.shape)


def _kernel(x_hbm, wqkv_hbm, wphi_hbm, wo_hbm, wr_hbm, wg_hbm, wu_hbm, wd_hbm, out_hbm,
            x_v, wqkv_v, wphi_v, wo_v, wo32, wr_v, graw_v, draw_v, gv_v, uv_v, rel_v, rel32,
            wt_v, a_v, xn_v, hn_v, kv_acc, z_acc, kvt_v, hbuf, out_v, zv, zs, xc_v, r_v, sems):
    nsem = [0]

    def newsem():
        nsem[0] += 1
        return nsem[0] - 1

    def cp(src, dst, sem=None):
        return pltpu.make_async_copy(src, dst, sems.at[newsem() if sem is None else sem])

    def cp_w(lo, hi):
        return cp(wqkv_hbm.at[:, lo:hi], wqkv_v.at[:, lo:hi])

    def cp_xr(lo, hi):
        return cp(x_hbm.at[0, lo:hi], x_v.at[lo:hi])

    cp_x0a = cp_xr(0, 256)
    cp_ph0 = cp(wphi_hbm.at[0:PH0], wphi_v.at[0:PH0])
    cp_ph1 = [cp(wphi_hbm.at[PH0:H], wphi_v.at[PH0:H])] if PH0 < H else []
    cp_wk0 = cp_w(D, D + K0)
    cp_x0b = cp_xr(256, 512)
    cp_wk1 = cp_w(D + K0, D + K1)
    cp_wk2 = cp_w(D + K1, 2 * D)
    cp_wv0 = cp_w(2 * D, 2 * D + V0)
    cp_wv1 = cp_w(2 * D + V0, 3 * D)
    cp_x1 = cp_xr(T, 2 * T + 128)
    cp_x2 = cp_xr(2 * T + 128, S)
    rsem0 = nsem[0]
    nsem[0] += NT - 1
    pieces = []
    for j in range(RAWG, NBM):
        pieces += [(wg_hbm, j, D), (wu_hbm, j, D)]
    pieces += [(wd_hbm, j, FD) for j in range(D // 128)]
    cp_rel = [[] for _ in range(NT - 1)]
    pos = 0
    for ref, j, n in pieces:
        r = 0
        while r < n:
            m = min(n - r, RELG - pos % RELG)
            cp_rel[pos // RELG].append(cp(ref.at[r:r + m, j * 128:(j + 1) * 128], rel_v.at[pos:pos + m],
                                          rsem0 + pos // RELG))
            r += m
            pos += m
    late = [cp_w(0, D), cp(wr_hbm, wr_v)]
    late += [cp(wo_hbm.at[:, j * 128:(j + 1) * 128], wo_v.at[j]) for j in range(D // 128)]
    for j in range(RAWG):
        late.append(cp(wg_hbm.at[:, j * 128:(j + 1) * 128], graw_v.at[2 * j]))
        late.append(cp(wu_hbm.at[:, j * 128:(j + 1) * 128], graw_v.at[2 * j + 1]))
    late += [cp(wd_hbm.at[FD:F, j * 128:(j + 1) * 128], draw_v.at[j]) for j in range(D // 128)]
    late += [cp(wg_hbm.at[:, FM:F], gv_v), cp(wu_hbm.at[:, FM:F], uv_v)]
    first = [cp_x0a, cp_ph0, cp_wk0] if ORDER == 0 else [cp_ph0, cp_wk0, cp_x0a]
    for c in first + [cp_x0b, cp_wk1] + cp_ph1 + [cp_wk2, cp_wv0, cp_wv1, cp_x1]:
        c.start()
    osem0 = nsem[0]
    nsem[0] += NT
    cp_last = [cp(out_v.at[(i + 1) * T:(i + 1) * T + CL], out_hbm.at[0, (i + 1) * T - CL:(i + 1) * T])
               for i in range(NT)]

    def cp_out(i):
        s = i * T if isinstance(i, int) else pl.multiple_of(i * T, T)
        return pltpu.make_async_copy(out_v.at[pl.ds(s + CL, T - CL)], out_hbm.at[0, pl.ds(s, T - CL)],
                                     sems.at[osem0 + i])

    def ln1(lo, hi):
        xn_v[lo:hi, :] = _ln(x_v[lo:hi, :].astype(f32)).astype(bf16)

    def fold(base, lo, hi):
        res = []
        for g in range(lo // 128, hi // 128):
            w = _dot_nt(_un(a_v[g]), wqkv_v[:, base + 128 * g: base + 128 * (g + 1)])
            wt_v[(base + 128 * g) // 2: (base + 128 * (g + 1)) // 2, :] = _pk((w * LOG2E).astype(bf16))
            res.append(w)
        return res

    def vtrans(lo, hi):
        for g in range(lo // 128, hi // 128):
            wt_v[(2 * D + 128 * g) // 2: (2 * D + 128 * (g + 1)) // 2, :] = _pk(
                wqkv_v[:, 2 * D + 128 * g: 2 * D + 128 * (g + 1)].T)

    def wt(lo, hi):
        return _un(wt_v[lo // 2:hi // 2, :])

    def build_a(h0, h1):
        w2 = wphi_v[h0:h1].reshape((h1 - h0) * DH, DH)
        r_i = lax.broadcasted_iota(jnp.int32, (128, DH), 0)
        f_i = lax.broadcasted_iota(jnp.int32, (128, DH), 1)
        sel = jnp.where(f_i == (r_i % 64) // 2, 1.0, 0.0).astype(bf16)
        a_full = _dot_nt(sel, w2)
        r_i = lax.broadcasted_iota(jnp.int32, (128, 128), 0)
        c_i = lax.broadcasted_iota(jnp.int32, (128, 128), 1)
        amask = c_i // 32 == 2 * (r_i // 64) + r_i % 2
        for g in range((h1 - h0) // 4):
            a_v[h0 // 4 + g] = _pk(jnp.where(amask, a_full[:, 128 * g:128 * (g + 1)], 0.0).astype(bf16))

    zv[...] = jnp.zeros((8, 128), u32)
    cp_z = cp(zv, zs)
    cp_z.start()
    for c in cp_rel[0] + [cp_x2] + sum(cp_rel[1:], []) + late:
        c.start()
    hbuf[...] = jnp.zeros(hbuf.shape, f32)
    r_v[...] = jnp.full(r_v.shape, -jnp.inf, f32)

    def rel_wait(g):
        rows = pl.ds(g * RELG if isinstance(g, int) else pl.multiple_of(g * RELG, RELG), RELG)
        pltpu.make_async_copy(rel_v.at[rows], rel_v.at[rows], sems.at[rsem0 + g]).wait()

    phis = {}

    def phis_of(y, p0, half):
        for p in range(y.shape[0] // 64):
            phi, z = _phi_k(y[64 * p:64 * (p + 1)])
            if half == 1:
                z_acc[p0 + p] += z
            else:
                z_acc[p0 + p] = z
            phis[(p0 + p, half)] = phi

    def kv_first(p, vt):
        if (p, 2) in phis:
            kv_acc[p] = _dot_nt(vt.astype(bf16), phis[(p, 2)])
        else:
            kv_acc[p] = (_dot_nt(vt[:, 0:256].astype(bf16), phis[(p, 0)])
                         + _dot_nt(vt[:, 256:512].astype(bf16), phis[(p, 1)]))

    if ONLY2:
        for c in first + [cp_x0b, cp_wk1] + cp_ph1 + [cp_wk2, cp_wv0, cp_wv1, cp_x1, cp_x2, cp_z]:
            c.wait()
        for g in range(NT - 1):
            rel_wait(g)
    else:
        if ORDER == 0:
            cp_x0a.wait()
            ln1(0, 256)
            cp_ph0.wait()
            build_a(0, PH0)
            cp_wk0.wait()
            fold(D, 0, K0)
        else:
            cp_ph0.wait()
            build_a(0, PH0)
            cp_wk0.wait()
            fold(D, 0, K0)
            cp_x0a.wait()
            ln1(0, 256)
        phis_of(_dot_nt(wt(D, D + K0), xn_v[0:256, :]), 0, 0)
        cp_x0b.wait()
        cp_wk1.wait()
        fold(D, K0, K1)
        ln1(256, 512)
        phis_of(_dot_nt(wt(D + K0, D + K1), xn_v[0:256, :]), K0 // 64, 0)
        phis_of(_dot_nt(wt(D, D + K1), xn_v[256:512, :]), 0, 1)
        for c in cp_ph1:
            c.wait()
        cp_wk2.wait()
        cp_wv0.wait()
        if PH0 < H:
            build_a(PH0, H)
        fold(D, K1, D)
        vtrans(0, V0)
        phis_of(_dot_nt(wt(D + K1, 2 * D), xn_v[0:T, :]), K1 // 64, 2)
        yv0 = _dot_nt(wt(2 * D, 2 * D + V0), xn_v[0:T, :])
        cp_wv1.wait()
        cp_x1.wait()
        cp_z.wait()
        vtrans(V0, D)
        for p in range(V0 // 64):
            kv_first(p, yv0[64 * p:64 * (p + 1)])
        yv1 = _dot_nt(wt(2 * D + V0, 3 * D), xn_v[0:T, :])
        nr = yv1.shape[0]
        deps = [yv1[(nr // 8) * k:(nr // 8) * k + 8, 128:256] for k in range(8)]
        xn_v[T:T + 128, :] = _ln(x_v[T:T + 128, :].astype(f32), deps, zv[...]).astype(bf16)
        for p in range((D - V0) // 64):
            kv_first(V0 // 64 + p, yv1[64 * p:64 * (p + 1)])

        def phase1(i, c):
            s = pl.multiple_of(i * T, T)
            rel_wait(i - 1)

            @pl.when(i == 2)
            def _():
                cp_x2.wait()

            zm = zv[...]
            xa = xn_v[pl.ds(s, 128), :]
            rest = pl.ds(pl.multiple_of(s + 128, 128), T - 128)
            xb = _ln(x_v[rest, :].astype(f32)).astype(bf16)
            xn_v[rest, :] = xb
            y = _dot_nt(wt(D, 3 * D), jnp.concatenate([xa, xb], axis=0))
            nxt = pl.multiple_of(jnp.where(i + 1 < NT, s + T, 0), 128)
            deps = [y[NXR + 64 * k:NXR + 64 * k + 8, 128 * NXJ:128 * NXJ + 128] for k in range(8)]
            xn_v[pl.ds(pl.multiple_of(s + T, 128), 128), :] = _ln(
                x_v[pl.ds(nxt, 128), :].astype(f32), deps, zm).astype(bf16)
            r0 = (i - 1) * RELG
            npc = RELG // RB
            for k in range(npc):
                jt = k * RJ // npc
                kk = k - (jt * npc + RJ - 1) // RJ
                per = (npc + RJ - 1) // RJ
                row = RLO + ((2 * D - RLO) * kk // per) // 8 * 8
                rel32[pl.ds(pl.multiple_of((r0 + k * RB) // 2, RB // 2), RB // 2), :] = _gated_pk(
                    rel_v[pl.ds(pl.multiple_of(r0 + k * RB, RB), RB), :],
                    y[row:row + 8, 128 * jt:128 * jt + 128], zm)
            for p in range(NP):
                phi, z = _phi_k(y[64 * p:64 * (p + 1)])
                z_acc[p] += z
                kv_acc[p] += _dot_nt(y[D + 64 * p: D + 64 * (p + 1)].astype(bf16), phi)
            return c
        lax.fori_loop(1, NT, phase1, 0)
    for c in late:
        c.wait()
    wq = fold(0, 0, D)
    for j in range(D // 128):
        for k in range(4):
            wo32[j, 128 * k:128 * (k + 1), :] = _gated_pk(
                wo_v[j, 256 * k:256 * (k + 1), :], wq[j * 7 // 8][32 * k:32 * k + 8, 0:128], zv[...])
    r_i = lax.broadcasted_iota(jnp.int32, (64, 128), 0)
    c_i = lax.broadcasted_iota(jnp.int32, (64, 128), 1)
    kmask = r_i // 32 == c_i % 2
    for p in range(NP):
        kvt_v[p] = _pk(jnp.where(kmask, kv_acc[p], 0.0).astype(bf16))
        z_acc[p] = jnp.broadcast_to(jnp.sum(z_acc[p], axis=1, keepdims=True), (128, 128))

    def ln2(h, row0, onepass=False, deps=None):
        wr = wr_v[...].reshape(1, D).astype(f32)
        if onepass:
            m = jnp.sum(h, axis=-1, keepdims=True) * (1.0 / D)
            v = jnp.sum(h * h, axis=-1, keepdims=True) * (1.0 / D) - m * m
            rs = lax.rsqrt(jnp.maximum(v, 0.0) + EPS)
            r = (jnp.sum(h * wr, axis=-1, keepdims=True) - m * jnp.sum(wr, axis=-1, keepdims=True)) * rs
            hn = (h - m) * rs
        else:
            hn = _ln(h, deps, zv[...])
            r = jnp.sum(hn * wr, axis=-1, keepdims=True)
        rows = pl.ds(row0, h.shape[0])
        hn_v[rows, :] = hn.astype(bf16)
        out_v[rows, :] = (h + hn).astype(bf16)
        return r

    def gates(nx, ngr):
        deps = [None]
        for j in range(1, ngr):
            t = (j * NREL * 2) // ngr - 1
            r0 = (nx.shape[0] - 8) * (t % 2)
            deps.append(nx[r0:r0 + 8, 128 * (t // 2):128 * (t // 2) + 128] if t >= 0 else None)
        return deps

    def phase2(i, c_):
        s = pl.multiple_of(i * T, T)

        @pl.when(i > 0)
        def _():
            cp_out(i - 1).start()

        hprev = hbuf[...]
        y = _dot_nt(wt(0, D), xn_v[pl.ds(s, T), :])
        os_ = []
        for p in range(NP):
            phi = _phi_q(y[64 * p:64 * (p + 1)], z_acc[p])
            os_.append(_dot(_un(kvt_v[p]), phi))
        o = jnp.concatenate(os_, axis=0).astype(bf16).T
        atts = []
        c = 0
        for k, ch in enumerate(CHUNKS):
            wo = jnp.concatenate([_un(wo32[j]) for j in range(D // 128)], axis=1)
            atts.append(_dot(o[c:c + ch], wo))
            c += ch
        rs_ = [jnp.where(i > 0, ln2(hprev, s, deps=gates(atts[0], CL // G)), -jnp.inf)]
        c = 0
        for k, ch in enumerate(CHUNKS):
            h = x_v[pl.ds(pl.multiple_of(s + c, 16), ch), :].astype(f32) + atts[k]
            if k == len(CHUNKS) - 1:
                hbuf[...] = h
            else:
                rs_.append(ln2(h, pl.multiple_of(s + c + CL, 16), deps=gates(atts[k + 1], ch // G)))
            c += ch
        j = 0
        for r in rs_:
            for k in range(0, r.shape[0], 8):
                r_v[i, :, j:j + 1] = r[k:k + 8]
                j += 1
        return c_
    lax.fori_loop(0, 0 if ONLY1 else NT, phase2, 0)
    if not ONLY1:
        cp_out(NT - 1).start()
    tok = (lax.broadcasted_iota(jnp.int32, (8, 128), 1) * 8
           + lax.broadcasted_iota(jnp.int32, (8, 128), 0) - CL).astype(f32)
    pv, pt = r_v[0], tok
    for i in range(1, NT):
        gt = r_v[i] > pv
        pv = jnp.where(gt, r_v[i], pv)
        pt = jnp.where(gt, tok + float(i * T), pt)
    pm = jnp.max(_allred8(pv, jnp.maximum), axis=1, keepdims=True)
    pi = jnp.min(_allred8(jnp.where(pv == pm, pt, float(S)), jnp.minimum), axis=1, keepdims=True)
    r = ln2(hbuf[...], S, onepass=True)
    for c in cp_last:
        c.start()
    sub = lax.broadcasted_iota(jnp.int32, (8, 1), 0).astype(f32)
    cands = [(r[k:k + 8], sub + float(S - CL + k)) for k in range(0, CL, 8)]
    while len(cands) > 1:
        nxt = []
        for k in range(0, len(cands), 2):
            (va, ia), (vb, ib) = cands[k], cands[k + 1]
            gt = vb > va
            nxt.append((jnp.where(gt, vb, va), jnp.where(gt, ib, ia)))
        cands = nxt
    lv, lt = cands[0]
    gt = lv > pm
    bv = jnp.broadcast_to(jnp.where(gt, lv, pm), (8, 128))
    bt = jnp.broadcast_to(jnp.where(gt, lt, pi), (8, 128))
    rmax = _allred8(bv, jnp.maximum)
    idxv = _allred8(jnp.where(bv == rmax, bt, float(S)), jnp.minimum).astype(jnp.int32)
    idx = jnp.clip(idxv[0, 0], 0, S - 1)
    base = pl.multiple_of(lax.shift_left(lax.shift_right_logical(idx, 4), 4), 16)
    baseq = pl.multiple_of(base + CL, 16)
    hit16 = lax.broadcasted_iota(jnp.int32, (16, D), 0) == idx - base
    slab = jnp.where(hit16, hn_v[pl.ds(baseq, 16), :].astype(f32), 0.0)
    x8 = _allred8(slab[0:8] + slab[8:16], jnp.add)
    xs = jnp.concatenate([x8, x8], axis=0).astype(bf16)
    xcol0 = jnp.concatenate([x8] * 16, axis=0).astype(bf16).T.astype(f32)
    xc_v[...] = xcol0

    def act(g, u):
        a8 = g * jax.nn.sigmoid(g) * u
        return jnp.concatenate([a8, a8], axis=0).astype(bf16)

    def w_down(k0, k1):
        if k0 >= NB - RAWD:
            return jnp.concatenate([draw_v[j, (k0 - NB + RAWD) * 128:(k1 - NB + RAWD) * 128] for j in range(8)], axis=1)
        assert k1 <= NB - RAWD
        b = (NBM - RAWG) * D
        return jnp.concatenate([_un(rel32[b + j * (FD // 2) + k0 * 64:b + j * (FD // 2) + k1 * 64])
                                for j in range(8)], axis=1)

    def w_gu(j0, j1, t):
        return jnp.concatenate(
            [graw_v[2 * j + t] if j < RAWG else
             _un(rel32[(2 * (j - RAWG) + t) * (D // 2):(2 * (j - RAWG) + t + 1) * (D // 2)])
             for j in range(j0, j1)], axis=1)

    def vpu_gu(j0, j1):
        nb = j1 - j0
        c0, c1 = (j0 - NBM) * 128, (j1 - NBM) * 128
        xcol = xcol0 if j0 == NBM else xc_v[pl.ds(pl.multiple_of(zs[1, j0].astype(jnp.int32), 8), D), :]
        accg = accu = None
        for k in range(0, D, 8):
            xk = jnp.concatenate([xcol[k:k + 8]] * nb, axis=1)
            pg = gv_v[k:k + 8, c0:c1].astype(f32) * xk
            pu = uv_v[k:k + 8, c0:c1].astype(f32) * xk
            accg = pg if accg is None else accg + pg
            accu = pu if accu is None else accu + pu
        return act(_allred8(accg, jnp.add), _allred8(accu, jnp.add))

    yv = None
    mpos = dpos = 0
    vpos = NBM
    am = []
    for tk in SCHED:
        n = int(tk[1:])
        y_ = None
        if tk[0] == 'M':
            a_ = act(_dot(xs, w_gu(mpos, mpos + n, 0))[0:8], _dot(xs, w_gu(mpos, mpos + n, 1))[0:8])
            am += [a_[:, c * 128:c * 128 + 128] for c in range(n)]
            mpos += n
        elif tk[0] == 'D':
            y_ = _dot(jnp.concatenate(am[dpos:dpos + n], axis=1), w_down(dpos, dpos + n))
            dpos += n
        else:
            y_ = _dot(vpu_gu(vpos, vpos + n), w_down(vpos, vpos + n))
            vpos += n
        if y_ is not None:
            yv = y_ if yv is None else yv + y_
    assert mpos == dpos == NBM and vpos == NB
    sg = jax.nn.sigmoid(rmax)
    yv = yv * jnp.concatenate([jnp.concatenate([sg, sg], axis=0)] * (D // 128), axis=1)
    for i in range(NT):
        if not ONLY1:
            cp_out(i).wait()
        cp_last[i].wait()
    cur = out_v[pl.ds(baseq, 16), :].astype(f32)
    out_v[pl.ds(baseq, 16), :] = jnp.where(hit16, cur + yv, cur).astype(bf16)
    cp_fin = cp(out_v.at[pl.ds(baseq, 16)], out_hbm.at[0, pl.ds(base, 16)])
    cp_fin.start()
    cp_fin.wait()


@jax.jit
def pallas_sequential_preLN__linear_kernel_hedgehog__moe_arch_mod__prompt_kernel(
    A_x, A_wqkv, A_w_phi, A_wo, B_x, B_w_r, B_w_gate, B_w_up, B_w_down):
    del B_x
    any_spec = pl.BlockSpec(memory_space=pl.ANY)
    return pl.pallas_call(
        _kernel,
        out_shape=jax.ShapeDtypeStruct((1, S, D), bf16),
        in_specs=[any_spec] * 8,
        out_specs=any_spec,
        scratch_shapes=[
            pltpu.VMEM((S, D), bf16),
            pltpu.VMEM((D, 3 * D), bf16),
            pltpu.VMEM((H, DH, DH), bf16),
            pltpu.VMEM((D // 128, D, 128), bf16),
            pltpu.VMEM((D // 128, D // 2, 128), u32),
            pltpu.VMEM((D,), bf16),
            pltpu.VMEM((2 * RAWG, D, 128), bf16),
            pltpu.VMEM((D // 128, 128 * RAWD, 128), bf16),
            pltpu.VMEM((D, F - FM), bf16),
            pltpu.VMEM((D, F - FM), bf16),
            pltpu.VMEM((REL, 128), bf16),
            pltpu.VMEM((REL // 2, 128), u32),
            pltpu.VMEM((3 * D // 2, D), u32),
            pltpu.VMEM((8, 64, 128), u32),
            pltpu.VMEM((S + 128, D), bf16),
            pltpu.VMEM((S + CL, D), bf16),
            pltpu.VMEM((NP, 64, 128), f32),
            pltpu.VMEM((NP, 128, 128), f32),
            pltpu.VMEM((NP, 32, 128), u32),
            pltpu.VMEM((CL, D), f32),
            pltpu.VMEM((S + CL, D), bf16),
            pltpu.VMEM((8, 128), u32),
            pltpu.SMEM((8, 128), u32),
            pltpu.VMEM((D, 128), f32),
            pltpu.VMEM((NT, 8, 128), f32),
            pltpu.SemaphoreType.DMA((64,)),
        ],
        compiler_params=pltpu.CompilerParams(vmem_limit_bytes=120 * 1024 * 1024,
                                             disable_bounds_checks=True,
                                             disable_semaphore_checks=True),
        name="hedgehog_mod",
    )(A_x, A_wqkv, A_w_phi, A_wo, B_w_r, B_w_gate, B_w_up, B_w_down)
```

```python
import jax
import jax.numpy as jnp
from jax import lax
import jax.experimental.pallas as pl
import jax.experimental.pallas.tpu as pltpu

S = 2048
D = 1024
H = 32
DH = 32
F = 3584
NP = H // 2
T = 512
NT = S // T
CHUNKS = [int(c) for c in '128,128,128,128'.split(",")]
CL = CHUNKS[-1]
NB = F // 128
NV = 2
NM = NB - NV
ND = 2
NDV = NM - ND
MB = 2
LAG = 3; VD = 3
RAWG = 2
REL = 2 * (NM - RAWG) * D
RELG = REL // (NT - 1)
assert REL % (NT - 1) == 0 and RELG % 256 == 0
ONLY1 = 0; ONLY2 = 0
K0 = 256; K1 = 512; V0 = 512; PH0 = 32
ORDER = 0
G = 16; NREL = 6
NXR = 1536; NXJ = 2
RLO = 1280; RB = 256; RJ = 3
X0 = 1
MO = 8
TST = 0
LOG2E = 1.4426950408889634
EPS = 1e-5

f32 = jnp.float32
bf16 = jnp.bfloat16
u32 = jnp.uint32


def _dot_nt(a, b):
    return lax.dot_general(a, b, (((1,), (1,)), ((), ())), preferred_element_type=f32)


def _dot(a, b):
    return jnp.dot(a, b, preferred_element_type=f32)


def _pk(x):
    return pltpu.bitcast(x, u32)


def _un(x):
    return pltpu.bitcast(x, bf16)


def _rcp(x):
    r = pl.reciprocal(x, approx=True)
    return r * (2.0 - x * r)


def _allred(v, op):
    v = op(v, pltpu.roll(v, 2, 0))
    return op(v, pltpu.roll(v, 4, 0))


def _allred8(v, op):
    return _allred(op(v, pltpu.roll(v, 1, 0)), op)


def _exps(x):
    L = x.shape[1]
    x3 = x.reshape(8, 8, L)
    mx = _allred(jnp.max(x3, axis=0), jnp.maximum)
    mn = _allred(jnp.min(x3, axis=0), jnp.minimum)
    ep = jnp.exp2(x3 - mx[None])
    en = jnp.exp2(mn[None] - x3)
    rp = _rcp(_allred(jnp.sum(ep, axis=0), jnp.add))
    rn = _rcp(_allred(jnp.sum(en, axis=0), jnp.add))
    return ep, en, rp, rn


def _phi_k(x):
    L = x.shape[1]
    ep, en, rp, rn = _exps(x)
    phi = jnp.concatenate([(ep * rp[None]).reshape(64, L), (en * rn[None]).reshape(64, L)], axis=0)
    z = phi[:, 0:128]
    for c in range(128, L, 128):
        z = z + phi[:, c:c + 128]
    return phi.astype(bf16), z


def _phi_q(x, zb):
    L = x.shape[1]
    ep, en, rp, rn = _exps(x)
    zb = jnp.concatenate([zb] * (L // 128), axis=1).reshape(16, 8, L)
    den = rp * jnp.sum(ep * zb[0:8], axis=0) + rn * jnp.sum(en * zb[8:16], axis=0)
    inv = _rcp(_allred(den, jnp.add) + 1e-6)
    cp = rp * inv
    cn = rn * inv
    phi = jnp.concatenate([(ep * cp[None]).reshape(64, L), (en * cn[None]).reshape(64, L)], axis=0)
    return phi.astype(bf16)


def _ln(x, deps=None, zm=None):
    if deps is None:
        tot = jnp.sum(x, axis=-1, keepdims=True)
    else:
        g = x.shape[0] // len(deps)
        gate = jnp.concatenate(
            [jnp.zeros((8, 128), f32) if d is None else pltpu.bitcast(pltpu.bitcast(d, u32) & zm, f32)
             for d in deps for _ in range(g // 8)], axis=0)
        acc = x[:, 0:128] + gate
        for c in range(128, D, 128):
            acc = acc + x[:, c:c + 128]
        tot = jnp.sum(acc, axis=-1, keepdims=True)
    xc = x - tot * (1.0 / D)
    return xc * lax.rsqrt(jnp.sum(xc * xc, axis=-1, keepdims=True) * (1.0 / D) + EPS)


def _gated_pk(w, dep, zm):
    w = _pk(w)
    z = pltpu.bitcast(dep, u32) & zm
    return (w.reshape(w.shape[0] // 8, 8, 128) | z[None]).reshape(w.shape)


def _kernel(x_hbm, wqkv_hbm, wphi_hbm, wo_hbm, wr_hbm, wg_hbm, wu_hbm, wd_hbm, out_hbm,
            x_v, wqkv_v, wphi_v, wo_v, wo32, wr_v, graw_v, draw_v, guv_v, wd_v, rel_v, rel32,
            wt_v, a_v, xn_v, hn_v, kv_acc, z_acc, kvt_v, hbuf, out_v, zv, zs, r_v, sems):
    nsem = [0]

    def newsem():
        nsem[0] += 1
        return nsem[0] - 1

    def cp(src, dst, sem=None):
        return pltpu.make_async_copy(src, dst, sems.at[newsem() if sem is None else sem])

    def cp_w(lo, hi):
        return cp(wqkv_hbm.at[:, lo:hi], wqkv_v.at[:, lo:hi])

    def cp_xr(lo, hi):
        return cp(x_hbm.at[0, lo:hi], x_v.at[lo:hi])

    cp_x0a = cp_xr(0, 256)
    cp_ph0 = cp(wphi_hbm.at[0:PH0], wphi_v.at[0:PH0])
    cp_ph1 = [cp(wphi_hbm.at[PH0:H], wphi_v.at[PH0:H])] if PH0 < H else []
    cp_wk0 = cp_w(D, D + K0)
    cp_x0b = cp_xr(256, 512)
    cp_wk1 = cp_w(D + K0, D + K1)
    cp_wk2 = cp_w(D + K1, 2 * D)
    cp_wv0 = cp_w(2 * D, 2 * D + V0)
    cp_wv1 = cp_w(2 * D + V0, 3 * D)
    cp_x1 = cp_xr(T, 2 * T + 128)
    cp_x2 = cp_xr(2 * T + 128, S)
    rsem0 = nsem[0]
    nsem[0] += NT - 1
    pieces = []
    for j in range(RAWG, NM):
        pieces += [(wg_hbm, j, D), (wu_hbm, j, D)]
    cp_rel = [[] for _ in range(NT - 1)]
    pos = 0
    for ref, j, n in pieces:
        r = 0
        while r < n:
            m = min(n - r, RELG - pos % RELG)
            cp_rel[pos // RELG].append(cp(ref.at[r:r + m, j * 128:(j + 1) * 128], rel_v.at[pos:pos + m],
                                          rsem0 + pos // RELG))
            r += m
            pos += m
    late = [cp_w(0, D), cp(wr_hbm, wr_v)]
    late += [cp(wo_hbm.at[:, j * 128:(j + 1) * 128], wo_v.at[j]) for j in range(D // 128)]
    late2 = []
    for j in range(RAWG):
        late2.append(cp(wg_hbm.at[:, j * 128:(j + 1) * 128], graw_v.at[2 * j]))
        late2.append(cp(wu_hbm.at[:, j * 128:(j + 1) * 128], graw_v.at[2 * j + 1]))
    late2 += [cp(wd_hbm.at[NDV * 128:F, j * 128:(j + 1) * 128], draw_v.at[j]) for j in range(D // 128)]
    for j in range(NV):
        late2.append(cp(wg_hbm.at[:, (NM + j) * 128:(NM + j + 1) * 128], guv_v.at[:, j * 256:j * 256 + 128]))
        late2.append(cp(wu_hbm.at[:, (NM + j) * 128:(NM + j + 1) * 128], guv_v.at[:, j * 256 + 128:j * 256 + 256]))
    cp_wd = cp(wd_hbm.at[0:NDV * 128], wd_v)
    first = [cp_x0a, cp_ph0, cp_wk0] if ORDER == 0 else [cp_ph0, cp_wk0, cp_x0a]
    for c in first + [cp_x0b, cp_wk1] + cp_ph1 + [cp_wk2, cp_wv0, cp_wv1, cp_x1]:
        c.start()
    osem0 = nsem[0]
    nsem[0] += NT
    cp_last = cp(out_v.at[S:S + CL], out_hbm.at[0, S - CL:S])
    cp_out0 = cp(out_v.at[CL:T], out_hbm.at[0, 0:T - CL])

    def cp_out(i):
        s = i * T if isinstance(i, int) else pl.multiple_of(i * T, T)
        return pltpu.make_async_copy(out_v.at[pl.ds(s, T)], out_hbm.at[0, pl.ds(s - CL, T)], sems.at[osem0 + i])

    def ln1(lo, hi):
        xn_v[lo:hi, :] = _ln(x_v[lo:hi, :].astype(f32)).astype(bf16)

    def fold(base, lo, hi):
        res = []
        for g in range(lo // 128, hi // 128):
            w = _dot_nt(_un(a_v[g]), wqkv_v[:, base + 128 * g: base + 128 * (g + 1)])
            wt_v[(base + 128 * g) // 2: (base + 128 * (g + 1)) // 2, :] = _pk((w * LOG2E).astype(bf16))
            res.append(w)
        return res

    def vtrans(lo, hi):
        for g in range(lo // 128, hi // 128):
            wt_v[(2 * D + 128 * g) // 2: (2 * D + 128 * (g + 1)) // 2, :] = _pk(
                wqkv_v[:, 2 * D + 128 * g: 2 * D + 128 * (g + 1)].T)

    def wt(lo, hi):
        return _un(wt_v[lo // 2:hi // 2, :])

    def build_a(h0, h1):
        w2 = wphi_v[h0:h1].reshape((h1 - h0) * DH, DH)
        r_i = lax.broadcasted_iota(jnp.int32, (128, DH), 0)
        f_i = lax.broadcasted_iota(jnp.int32, (128, DH), 1)
        sel = jnp.where(f_i == (r_i % 64) // 2, 1.0, 0.0).astype(bf16)
        a_full = _dot_nt(sel, w2)
        r_i = lax.broadcasted_iota(jnp.int32, (128, 128), 0)
        c_i = lax.broadcasted_iota(jnp.int32, (128, 128), 1)
        amask = c_i // 32 == 2 * (r_i // 64) + r_i % 2
        for g in range((h1 - h0) // 4):
            a_v[h0 // 4 + g] = _pk(jnp.where(amask, a_full[:, 128 * g:128 * (g + 1)], 0.0).astype(bf16))

    zv[...] = jnp.zeros((8, 128), u32)
    cp_z = cp(zv, zs)
    cp_z.start()
    for c in cp_rel[0] + [cp_x2] + cp_rel[1] + (cp_rel[2] + late + late2 + [cp_wd] if ONLY2 else []):
        c.start()
    hbuf[...] = jnp.zeros(hbuf.shape, f32)
    r_v[...] = jnp.full(r_v.shape, -jnp.inf, f32)

    def rel_wait(g):
        rows = pl.ds(g * RELG if isinstance(g, int) else pl.multiple_of(g * RELG, RELG), RELG)
        pltpu.make_async_copy(rel_v.at[rows], rel_v.at[rows], sems.at[rsem0 + g]).wait()

    phis = {}

    def phis_of(y, p0, half):
        for p in range(y.shape[0] // 64):
            phi, z = _phi_k(y[64 * p:64 * (p + 1)])
            if half == 1:
                z_acc[p0 + p] += z
            else:
                z_acc[p0 + p] = z
            phis[(p0 + p, half)] = phi

    def kv_first(p, vt):
        if (p, 2) in phis:
            kv_acc[p] = _dot_nt(vt.astype(bf16), phis[(p, 2)])
        else:
            kv_acc[p] = (_dot_nt(vt[:, 0:256].astype(bf16), phis[(p, 0)])
                         + _dot_nt(vt[:, 256:512].astype(bf16), phis[(p, 1)]))

    if ONLY2:
        for c in first + [cp_x0b, cp_wk1] + cp_ph1 + [cp_wk2, cp_wv0, cp_wv1, cp_x1, cp_x2, cp_z]:
            c.wait()
        for g in range(NT - 1):
            rel_wait(g)
    else:
        if ORDER == 0:
            cp_x0a.wait()
            ln1(0, 256)
            cp_ph0.wait()
            build_a(0, PH0)
            cp_wk0.wait()
            fold(D, 0, K0)
        else:
            cp_ph0.wait()
            build_a(0, PH0)
            cp_wk0.wait()
            fold(D, 0, K0)
            cp_x0a.wait()
            ln1(0, 256)
        phis_of(_dot_nt(wt(D, D + K0), xn_v[0:256, :]), 0, 0)
        cp_x0b.wait()
        cp_wk1.wait()
        fold(D, K0, K1)
        ln1(256, 512)
        phis_of(_dot_nt(wt(D + K0, D + K1), xn_v[0:256, :]), K0 // 64, 0)
        phis_of(_dot_nt(wt(D, D + K1), xn_v[256:512, :]), 0, 1)
        for c in cp_ph1:
            c.wait()
        cp_wk2.wait()
        cp_wv0.wait()
        if PH0 < H:
            build_a(PH0, H)
        fold(D, K1, D)
        vtrans(0, V0)
        phis_of(_dot_nt(wt(D + K1, 2 * D), xn_v[0:T, :]), K1 // 64, 2)
        yv0 = _dot_nt(wt(2 * D, 2 * D + V0), xn_v[0:T, :])
        cp_wv1.wait()
        cp_x1.wait()
        cp_z.wait()
        for c in cp_rel[2] + late:
            c.start()
        vtrans(V0, D)
        for p in range(V0 // 64):
            kv_first(p, yv0[64 * p:64 * (p + 1)])
        yv1 = _dot_nt(wt(2 * D + V0, 3 * D), xn_v[0:T, :])
        nr = yv1.shape[0]
        deps = [yv1[(nr // 8) * k:(nr // 8) * k + 8, 128:256] for k in range(8)]
        xn_v[T:T + 128, :] = _ln(x_v[T:T + 128, :].astype(f32), deps, zv[...]).astype(bf16)
        for p in range((D - V0) // 64):
            kv_first(V0 // 64 + p, yv1[64 * p:64 * (p + 1)])

        def phase1(i, c):
            s = pl.multiple_of(i * T, T)
            rel_wait(i - 1)

            @pl.when(i == 2)
            def _():
                cp_x2.wait()
                for c in late2 + [cp_wd]:
                    c.start()

            zm = zv[...]
            xa = xn_v[pl.ds(s, 128), :]
            rest = pl.ds(pl.multiple_of(s + 128, 128), T - 128)
            xb = _ln(x_v[rest, :].astype(f32)).astype(bf16)
            xn_v[rest, :] = xb
            y = _dot_nt(wt(D, 3 * D), jnp.concatenate([xa, xb], axis=0))
            nxt = pl.multiple_of(jnp.where(i + 1 < NT, s + T, 0), 128)
            deps = [y[NXR + 64 * k:NXR + 64 * k + 8, 128 * NXJ:128 * NXJ + 128] for k in range(8)]
            xn_v[pl.ds(pl.multiple_of(s + T, 128), 128), :] = _ln(
                x_v[pl.ds(nxt, 128), :].astype(f32), deps, zm).astype(bf16)
            r0 = (i - 1) * RELG
            npc = RELG // RB
            for k in range(npc):
                jt = k * RJ // npc
                kk = k - (jt * npc + RJ - 1) // RJ
                per = (npc + RJ - 1) // RJ
                row = RLO + ((2 * D - RLO) * kk // per) // 8 * 8
                rel32[pl.ds(pl.multiple_of((r0 + k * RB) // 2, RB // 2), RB // 2), :] = _gated_pk(
                    rel_v[pl.ds(pl.multiple_of(r0 + k * RB, RB), RB), :],
                    y[row:row + 8, 128 * jt:128 * jt + 128], zm)
            for p in range(NP):
                phi, z = _phi_k(y[64 * p:64 * (p + 1)])
                z_acc[p] += z
                kv_acc[p] += _dot_nt(y[D + 64 * p: D + 64 * (p + 1)].astype(bf16), phi)
            return c
        lax.fori_loop(1, NT, phase1, 0)
    for c in late + late2:
        c.wait()
    wq = fold(0, 0, D)
    for j in range(D // 128):
        for k in range(4):
            wo32[j, 128 * k:128 * (k + 1), :] = _gated_pk(
                wo_v[j, 256 * k:256 * (k + 1), :], wq[j * 7 // 8][32 * k:32 * k + 8, 0:128], zv[...])
    r_i = lax.broadcasted_iota(jnp.int32, (64, 128), 0)
    c_i = lax.broadcasted_iota(jnp.int32, (64, 128), 1)
    kmask = r_i // 32 == c_i % 2
    for p in range(NP):
        kvt_v[p] = _pk(jnp.where(kmask, kv_acc[p], 0.0).astype(bf16))
        z_acc[p] = jnp.broadcast_to(jnp.sum(z_acc[p], axis=1, keepdims=True), (128, 128))

    def ln2(h, row0, onepass=False, deps=None):
        wr = wr_v[...].reshape(1, D).astype(f32)
        if onepass:
            m = jnp.sum(h, axis=-1, keepdims=True) * (1.0 / D)
            v = jnp.sum(h * h, axis=-1, keepdims=True) * (1.0 / D) - m * m
            rs = lax.rsqrt(jnp.maximum(v, 0.0) + EPS)
            r = (jnp.sum(h * wr, axis=-1, keepdims=True) - m * jnp.sum(wr, axis=-1, keepdims=True)) * rs
            hn = (h - m) * rs
        else:
            hn = _ln(h, deps, zv[...])
            r = jnp.sum(hn * wr, axis=-1, keepdims=True)
        rows = pl.ds(row0, h.shape[0])
        hn_v[rows, :] = hn.astype(bf16)
        out_v[rows, :] = (h + hn).astype(bf16)
        return r

    def gates(nx, ngr):
        deps = [None]
        for j in range(1, ngr):
            t = (j * NREL * 2) // ngr - 1
            r0 = (nx.shape[0] - 8) * (t % 2)
            deps.append(nx[r0:r0 + 8, 128 * (t // 2):128 * (t // 2) + 128] if t >= 0 else None)
        return deps

    def phase2(i, c_):
        s = pl.multiple_of(i * T, T)

        @pl.when(i == 1)
        def _():
            cp_out0.start()

        @pl.when(i > 1)
        def _():
            cp_out(i - 1).start()

        hprev = hbuf[...]
        y = _dot_nt(wt(0, D), xn_v[pl.ds(s, T), :])
        os_ = []
        for p in range(NP):
            phi = _phi_q(y[64 * p:64 * (p + 1)], z_acc[p])
            os_.append(_dot(_un(kvt_v[p]), phi))
        o = jnp.concatenate(os_, axis=0).astype(bf16).T
        atts = []
        c = 0
        for k, ch in enumerate(CHUNKS):
            wo = jnp.concatenate([_un(wo32[j]) for j in range(D // 128)], axis=1)
            atts.append(_dot(o[c:c + ch], wo))
            c += ch
        rs_ = [jnp.where(i > 0, ln2(hprev, s, deps=gates(atts[0], CL // G)), -jnp.inf)]
        c = 0
        for k, ch in enumerate(CHUNKS):
            h = x_v[pl.ds(pl.multiple_of(s + c, 16), ch), :].astype(f32) + atts[k]
            if k == len(CHUNKS) - 1:
                hbuf[...] = h
            else:
                rs_.append(ln2(h, pl.multiple_of(s + c + CL, 16), deps=gates(atts[k + 1], ch // G)))
            c += ch
        j = 0
        for r in rs_:
            for k in range(0, r.shape[0], 8):
                r_v[i, :, j:j + 1] = r[k:k + 8]
                j += 1
        return c_
    lax.fori_loop(0, 0 if ONLY1 else NT, phase2, 0)
    cp_out(NT - 1).start()
    tok = (lax.broadcasted_iota(jnp.int32, (8, 128), 1) * 8
           + lax.broadcasted_iota(jnp.int32, (8, 128), 0) - CL).astype(f32)
    pv, pt = r_v[0], tok
    for i in range(1, NT):
        gt = r_v[i] > pv
        pv = jnp.where(gt, r_v[i], pv)
        pt = jnp.where(gt, tok + float(i * T), pt)
    pm = jnp.max(_allred8(pv, jnp.maximum), axis=1, keepdims=True)
    pi = jnp.min(_allred8(jnp.where(pv == pm, pt, float(S)), jnp.minimum), axis=1, keepdims=True)
    r = ln2(hbuf[...], S, onepass=True)
    cp_last.start()
    sub = lax.broadcasted_iota(jnp.int32, (8, 1), 0).astype(f32)
    cands = [(r[k:k + 8], sub + float(S - CL + k)) for k in range(0, CL, 8)]
    while len(cands) > 1:
        nxt = []
        for k in range(0, len(cands), 2):
            (va, ia), (vb, ib) = cands[k], cands[k + 1]
            gt = vb > va
            nxt.append((jnp.where(gt, vb, va), jnp.where(gt, ib, ia)))
        cands = nxt
    lv, lt = cands[0]
    gt = lv > pm
    bv = jnp.broadcast_to(jnp.where(gt, lv, pm), (8, 128))
    bt = jnp.broadcast_to(jnp.where(gt, lt, pi), (8, 128))
    rmax = _allred8(bv, jnp.maximum)
    idxv = _allred8(jnp.where(bv == rmax, bt, float(S)), jnp.minimum).astype(jnp.int32)
    idx = jnp.clip(idxv[0, 0], 0, S - 1)
    base = pl.multiple_of(lax.shift_left(lax.shift_right_logical(idx, 4), 4), 16)
    baseq = pl.multiple_of(base + CL, 16)
    hit16 = lax.broadcasted_iota(jnp.int32, (16, D), 0) == idx - base
    cp_wd.wait()
    slab = jnp.where(hit16, hn_v[pl.ds(baseq, 16), :].astype(f32), 0.0)
    x8 = _allred8(slab[0:8] + slab[8:16], jnp.add)
    xs32 = _pk(jnp.concatenate([x8, x8], axis=0).astype(bf16))
    zm8 = jnp.concatenate([zv[...]] * 8, axis=1)

    def col(a8):
        return jnp.concatenate([a8] * 16, axis=0).astype(bf16).T.astype(f32)

    def act(r):
        n = r.shape[1] // 256
        g = jnp.concatenate([r[:, t * 256:t * 256 + 128] for t in range(n)], axis=1)
        u = jnp.concatenate([r[:, t * 256 + 128:t * 256 + 256] for t in range(n)], axis=1)
        return g * jax.nn.sigmoid(g) * u

    xcol = col(x8)
    av = None
    for k in range(0, D, 8):
        p = guv_v[k:k + 8, :].astype(f32) * jnp.concatenate([xcol[k:k + 8]] * (2 * NV), axis=1)
        av = p if av is None else av + p
    acc = None
    hist = []
    tail = []
    for cnt, j in enumerate(range(0, NM, MB)):
        w = jnp.concatenate(
            [graw_v[t] if t < 2 * RAWG else _un(rel32[(t - 2 * RAWG) * (D // 2):(t - 2 * RAWG + 1) * (D // 2)])
             for t in range(2 * j, 2 * (j + MB))], axis=1)
        xl = xs32
        if LAG <= cnt < LAG + len(hist) and cnt - LAG < len(hist):
            xl = xl | (pltpu.bitcast(hist[cnt - LAG], u32) & zm8)
        if cnt == VD:
            xl = xl | (pltpu.bitcast(jnp.concatenate([av] * (4 // NV), axis=1), u32) & zm8)
        a8 = act(_dot(_un(xl), w)[0:8])
        if j >= NDV:
            tail.append((a8, j, j + MB))
        else:
            ac = col(a8)
            for k in range(0, MB * 128, 8):
                p = wd_v[j * 128 + k:j * 128 + k + 8, :].astype(f32) * jnp.concatenate([ac[k:k + 8]] * 8, axis=1)
                acc = p if acc is None else acc + p
            hist.append(acc)
    tail = tail[:-1] + [(act(_allred8(av, jnp.add)), NM, NB)] + tail[-1:]
    yv = _allred8(acc, jnp.add)
    for a8, k0, k1 in tail:
        wdm = jnp.concatenate([draw_v[t, (k0 - NDV) * 128:(k1 - NDV) * 128] for t in range(8)], axis=1)
        yv = yv + _dot(jnp.concatenate([a8, a8], axis=0).astype(bf16), wdm)[0:8]
    sg = jax.nn.sigmoid(rmax)
    yv = yv * jnp.concatenate([sg] * (D // 128), axis=1)
    yv = jnp.concatenate([yv, yv], axis=0)
    if not ONLY1:
        cp_out0.wait()
        for i in range(1, NT - 1):
            cp_out(i).wait()
    cp_out(NT - 1).wait()
    cp_last.wait()
    cur = out_v[pl.ds(baseq, 16), :].astype(f32)
    out_v[pl.ds(baseq, 16), :] = jnp.where(hit16, cur + yv, cur).astype(bf16)
    cp_fin = cp(out_v.at[pl.ds(baseq, 16)], out_hbm.at[0, pl.ds(base, 16)])
    cp_fin.start()
    cp_fin.wait()


@jax.jit
def pallas_sequential_preLN__linear_kernel_hedgehog__moe_arch_mod__prompt_kernel(
    A_x, A_wqkv, A_w_phi, A_wo, B_x, B_w_r, B_w_gate, B_w_up, B_w_down):
    del B_x
    any_spec = pl.BlockSpec(memory_space=pl.ANY)
    return pl.pallas_call(
        _kernel,
        out_shape=jax.ShapeDtypeStruct((1, S, D), bf16),
        in_specs=[any_spec] * 8,
        out_specs=any_spec,
        scratch_shapes=[
            pltpu.VMEM((S, D), bf16),
            pltpu.VMEM((D, 3 * D), bf16),
            pltpu.VMEM((H, DH, DH), bf16),
            pltpu.VMEM((D // 128, D, 128), bf16),
            pltpu.VMEM((D // 128, D // 2, 128), u32),
            pltpu.VMEM((D,), bf16),
            pltpu.VMEM((2 * RAWG, D, 128), bf16),
            pltpu.VMEM((D // 128, F - NDV * 128, 128), bf16),
            pltpu.VMEM((D, NV * 256), bf16),
            pltpu.VMEM((NDV * 128, D), bf16),
            pltpu.VMEM((REL, 128), bf16),
            pltpu.VMEM((REL // 2, 128), u32),
            pltpu.VMEM((3 * D // 2, D), u32),
            pltpu.VMEM((8, 64, 128), u32),
            pltpu.VMEM((S + 128, D), bf16),
            pltpu.VMEM((S + CL, D), bf16),
            pltpu.VMEM((NP, 64, 128), f32),
            pltpu.VMEM((NP, 128, 128), f32),
            pltpu.VMEM((NP, 32, 128), u32),
            pltpu.VMEM((CL, D), f32),
            pltpu.VMEM((S + CL, D), bf16),
            pltpu.VMEM((8, 128), u32),
            pltpu.SMEM((8, 128), u32),
            pltpu.VMEM((NT, 8, 128), f32),
            pltpu.SemaphoreType.DMA((64,)),
        ],
        compiler_params=pltpu.CompilerParams(vmem_limit_bytes=120 * 1024 * 1024,
                                             disable_bounds_checks=True,
                                             disable_semaphore_checks=True),
        name="hedgehog_mod",
    )(A_x, A_wqkv, A_w_phi, A_wo, B_w_r, B_w_gate, B_w_up, B_w_down)
```

```python
import jax
import jax.numpy as jnp
from jax import lax
import jax.experimental.pallas as pl
import jax.experimental.pallas.tpu as pltpu

S = 2048
D = 1024
H = 32
DH = 32
F = 3584
NP = H // 2
T = 512
NT = S // T
CHUNKS = [int(c) for c in '128,128,128,128'.split(",")]
CL = CHUNKS[-1]
NB = F // 128
NV = 2
NM = NB - NV
ND = 2
NDV = NM - ND
MB = 2
LAG = 3; VD = 3
RAWG = 2
REL = 2 * (NM - RAWG) * D
RELG = REL // (NT - 1)
assert REL % (NT - 1) == 0 and RELG % 256 == 0
ONLY1 = 0; ONLY2 = 0
K0 = 256; K1 = 512; V0 = 512; PH0 = 32
ORDER = 0
G = 16; NREL = 6
NXR = 1536; NXJ = 2
RLO = 1280; RB = 256; RJ = 3
X0 = 1
MO = 8
TST = 0
SEGS = [tuple(128 * int(v) for v in t) for t in '22,12,14'.split(",")]
EARLY = 0
KEEP = 256; DEFER = 2
LOG2E = 1.4426950408889634
EPS = 1e-5

f32 = jnp.float32
bf16 = jnp.bfloat16
u32 = jnp.uint32


def _dot_nt(a, b):
    return lax.dot_general(a, b, (((1,), (1,)), ((), ())), preferred_element_type=f32)


def _dot(a, b):
    return jnp.dot(a, b, preferred_element_type=f32)


def _pk(x):
    return pltpu.bitcast(x, u32)


def _un(x):
    return pltpu.bitcast(x, bf16)


def _rcp(x):
    r = pl.reciprocal(x, approx=True)
    return r * (2.0 - x * r)


def _allred(v, op):
    v = op(v, pltpu.roll(v, 2, 0))
    return op(v, pltpu.roll(v, 4, 0))


def _allred8(v, op):
    return _allred(op(v, pltpu.roll(v, 1, 0)), op)


def _exps(x):
    L = x.shape[1]
    x3 = x.reshape(8, 8, L)
    mx = _allred(jnp.max(x3, axis=0), jnp.maximum)
    mn = _allred(jnp.min(x3, axis=0), jnp.minimum)
    ep = jnp.exp2(x3 - mx[None])
    en = jnp.exp2(mn[None] - x3)
    rp = _rcp(_allred(jnp.sum(ep, axis=0), jnp.add))
    rn = _rcp(_allred(jnp.sum(en, axis=0), jnp.add))
    return ep, en, rp, rn


def _phi_k(x):
    L = x.shape[1]
    ep, en, rp, rn = _exps(x)
    phi = jnp.concatenate([(ep * rp[None]).reshape(64, L), (en * rn[None]).reshape(64, L)], axis=0)
    z = phi[:, 0:128]
    for c in range(128, L, 128):
        z = z + phi[:, c:c + 128]
    return phi.astype(bf16), z


def _phi_q(x, zb):
    L = x.shape[1]
    ep, en, rp, rn = _exps(x)
    zb = jnp.concatenate([zb] * (L // 128), axis=1).reshape(16, 8, L)
    den = rp * jnp.sum(ep * zb[0:8], axis=0) + rn * jnp.sum(en * zb[8:16], axis=0)
    inv = _rcp(_allred(den, jnp.add) + 1e-6)
    cp = rp * inv
    cn = rn * inv
    phi = jnp.concatenate([(ep * cp[None]).reshape(64, L), (en * cn[None]).reshape(64, L)], axis=0)
    return phi.astype(bf16)


def _ln(x, deps=None, zm=None):
    if deps is None:
        tot = jnp.sum(x, axis=-1, keepdims=True)
    else:
        g = x.shape[0] // len(deps)
        gate = jnp.concatenate(
            [jnp.zeros((8, 128), f32) if d is None else pltpu.bitcast(pltpu.bitcast(d, u32) & zm, f32)
             for d in deps for _ in range(g // 8)], axis=0)
        acc = x[:, 0:128] + gate
        for c in range(128, D, 128):
            acc = acc + x[:, c:c + 128]
        tot = jnp.sum(acc, axis=-1, keepdims=True)
    xc = x - tot * (1.0 / D)
    return xc * lax.rsqrt(jnp.sum(xc * xc, axis=-1, keepdims=True) * (1.0 / D) + EPS)


def _gated_pk(w, dep, zm):
    w = _pk(w)
    z = pltpu.bitcast(dep, u32) & zm
    return (w.reshape(w.shape[0] // 8, 8, 128) | z[None]).reshape(w.shape)


def _kernel(x_hbm, wqkv_hbm, wphi_hbm, wo_hbm, wr_hbm, wg_hbm, wu_hbm, wd_hbm, out_hbm,
            x_v, wqkv_v, wphi_v, wo_v, wo32, wr_v, graw_v, draw_v, guv_v, wd_v, rel_v, rel32,
            wt_v, a_v, xn_v, hn_v, kv_acc, z_acc, kvt_v, hbuf, out_v, zv, zs, r_v, sems):
    nsem = [0]

    def newsem():
        nsem[0] += 1
        return nsem[0] - 1

    def cp(src, dst, sem=None):
        return pltpu.make_async_copy(src, dst, sems.at[newsem() if sem is None else sem])

    def cp_w(lo, hi):
        return cp(wqkv_hbm.at[:, lo:hi], wqkv_v.at[:, lo:hi])

    def cp_xr(lo, hi):
        return cp(x_hbm.at[0, lo:hi], x_v.at[lo:hi])

    def cp_ph(lo, hi):
        return cp(wphi_hbm.at[lo // DH:hi // DH], wphi_v.at[lo // DH:hi // DH])

    seg_cp = []
    x0 = k0 = 0
    kcum = [0]
    for dx, dk in SEGS:
        kcum.append(kcum[-1] + dk)
    arng = [(0 if si == 0 else kcum[si + 1], kcum[min(si + 2, len(SEGS))]) for si in range(len(SEGS))]
    for si, (dx, dk) in enumerate(SEGS):
        ph = [cp_ph(*arng[si])] if arng[si][1] > arng[si][0] else []
        seg_cp.append([cp_xr(x0, x0 + dx)] + ph + [cp_w(D + k0, D + k0 + dk)])
        x0 += dx
        k0 += dk
    cp_wv = cp_w(2 * D, 3 * D)
    cp_x1a = cp_xr(T, T + 128)
    cp_x1 = cp_xr(T + 128, 2 * T + 128)
    cp_x2 = cp_xr(2 * T + 128, S)
    rsem0 = nsem[0]
    nsem[0] += NT - 1
    pieces = []
    for j in range(RAWG, NM):
        pieces += [(wg_hbm, j, D), (wu_hbm, j, D)]
    cp_rel = [[] for _ in range(NT - 1)]
    pos = 0
    for ref, j, n in pieces:
        r = 0
        while r < n:
            m = min(n - r, RELG - pos % RELG)
            cp_rel[pos // RELG].append(cp(ref.at[r:r + m, j * 128:(j + 1) * 128], rel_v.at[pos:pos + m],
                                          rsem0 + pos // RELG))
            r += m
            pos += m
    late = [cp_w(0, D), cp(wr_hbm, wr_v)]
    late += [cp(wo_hbm.at[:, j * 128:(j + 1) * 128], wo_v.at[j]) for j in range(D // 128)]
    late2 = []
    for j in range(RAWG):
        late2.append(cp(wg_hbm.at[:, j * 128:(j + 1) * 128], graw_v.at[2 * j]))
        late2.append(cp(wu_hbm.at[:, j * 128:(j + 1) * 128], graw_v.at[2 * j + 1]))
    late2 += [cp(wd_hbm.at[NDV * 128:F, j * 128:(j + 1) * 128], draw_v.at[j]) for j in range(D // 128)]
    for j in range(NV):
        late2.append(cp(wg_hbm.at[:, (NM + j) * 128:(NM + j + 1) * 128], guv_v.at[:, j * 256:j * 256 + 128]))
        late2.append(cp(wu_hbm.at[:, (NM + j) * 128:(NM + j + 1) * 128], guv_v.at[:, j * 256 + 128:j * 256 + 256]))
    cp_wd = cp(wd_hbm.at[0:NDV * 128], wd_v)
    first = [c for t in seg_cp for c in t] + [cp_wv, cp_x1a, cp_x1]
    for c in first:
        c.start()
    osem0 = nsem[0]
    nsem[0] += NT
    cp_last = cp(out_v.at[S:S + CL], out_hbm.at[0, S - CL:S])
    cp_out0 = cp(out_v.at[CL:T], out_hbm.at[0, 0:T - CL])

    def cp_out(i):
        s = i * T if isinstance(i, int) else pl.multiple_of(i * T, T)
        return pltpu.make_async_copy(out_v.at[pl.ds(s, T)], out_hbm.at[0, pl.ds(s - CL, T)], sems.at[osem0 + i])

    def ln1(lo, hi):
        xn_v[lo:hi, :] = _ln(x_v[lo:hi, :].astype(f32)).astype(bf16)

    def fold(base, lo, hi):
        res = []
        for g in range(lo // 128, hi // 128):
            w = _dot_nt(_un(a_v[g]), wqkv_v[:, base + 128 * g: base + 128 * (g + 1)])
            wt_v[(base + 128 * g) // 2: (base + 128 * (g + 1)) // 2, :] = _pk((w * LOG2E).astype(bf16))
            res.append(w)
        return res

    def vtrans(lo, hi):
        for g in range(lo // 128, hi // 128):
            wt_v[(2 * D + 128 * g) // 2: (2 * D + 128 * (g + 1)) // 2, :] = _pk(
                wqkv_v[:, 2 * D + 128 * g: 2 * D + 128 * (g + 1)].T)

    def wt(lo, hi):
        return _un(wt_v[lo // 2:hi // 2, :])

    r_i = lax.broadcasted_iota(jnp.int32, (128, DH), 0)
    f_i = lax.broadcasted_iota(jnp.int32, (128, DH), 1)
    sel = jnp.where(f_i == (r_i % 64) // 2, 1.0, 0.0).astype(bf16)
    r_i = lax.broadcasted_iota(jnp.int32, (128, 128), 0)
    c_i = lax.broadcasted_iota(jnp.int32, (128, 128), 1)
    amask = jnp.where(c_i // 32 == 2 * (r_i // 64) + r_i % 2, jnp.uint32(0xFFFFFFFF), jnp.uint32(0))

    def build_a(lo, hi):
        a_full = _dot_nt(sel, wphi_v[lo // DH:hi // DH].reshape(hi - lo, DH))
        for g in range((hi - lo) // 128):
            blk = pltpu.bitcast(pltpu.bitcast(a_full[:, 128 * g:128 * (g + 1)], u32) & amask, f32)
            a_v[lo // 128 + g] = _pk(blk.astype(bf16))

    zv[...] = jnp.zeros((8, 128), u32)
    cp_z = cp(zv, zs)
    cp_z.start()
    for c in cp_rel[0] + [cp_x2] + cp_rel[1] + (cp_rel[2] + late + late2 + [cp_wd] if ONLY2 else []):
        c.start()
    hbuf[...] = jnp.zeros(hbuf.shape, f32)
    r_v[...] = jnp.full(r_v.shape, -jnp.inf, f32)

    def rel_wait(g):
        rows = pl.ds(g * RELG if isinstance(g, int) else pl.multiple_of(g * RELG, RELG), RELG)
        pltpu.make_async_copy(rel_v.at[rows], rel_v.at[rows], sems.at[rsem0 + g]).wait()

    phis = [[] for _ in range(NP)]
    pending = []

    def phi_piece(p, t0, yp, dep=None):
        if dep is not None:
            gate = pltpu.bitcast(pltpu.bitcast(dep, u32) & zv[...], f32)
            yp = jnp.concatenate([yp[0:8] + gate, yp[8:]], axis=0)
        phi, z = _phi_k(yp)
        if phis[p]:
            z_acc[p] += z
        else:
            z_acc[p] = z
        phis[p].append((t0, phi))

    def k_block(klo, khi, t0, t1, defer=0, early=None):
        w = wt_v[(D + klo) // 2:(D + khi) // 2, :]
        if early is not None:
            if EARLY == 1:
                e = pltpu.bitcast(early, u32) & jnp.concatenate(
                    [jnp.concatenate([zv[...]] * 8, axis=1)] * (early.shape[0] // 8), axis=0)
                w = (w | e) if e.shape[0] == w.shape[0] else jnp.concatenate([w[0:e.shape[0]] | e, w[e.shape[0]:]], axis=0)
            else:
                e = pltpu.bitcast(early[:, D - 128:D], u32) & jnp.concatenate([zv[...]] * (early.shape[0] // 8), axis=0)
                w0 = w[:, 0:128]
                w0 = (w0 | e) if e.shape[0] == w.shape[0] else jnp.concatenate([w0[0:e.shape[0]] | e, w0[e.shape[0]:]], axis=0)
                w = jnp.concatenate([w0, w[:, 128:]], axis=1)
        y = _dot_nt(_un(w), xn_v[t0:t1, :])
        npair = (khi - klo) // 64
        for p in range(npair):
            yp = y[64 * p:64 * (p + 1)]
            if p >= npair - defer:
                if t1 - t0 > 128:
                    phi_piece(klo // 64 + p, t0, yp[:, 0:t1 - t0 - 128])
                pending.append((klo // 64 + p, t1 - 128, yp[:, t1 - t0 - 128:]))
            else:
                phi_piece(klo // 64 + p, t0, yp)
        return y

    def flush(res):
        for k, (p, t0, yp) in enumerate(pending):
            phi_piece(p, t0, yp, res[32 * k:32 * k + 8, 0:128])
        del pending[:]

    if ONLY2:
        for c in first + [cp_x2, cp_z]:
            c.wait()
        for g in range(NT - 1):
            rel_wait(g)
    else:
        x0 = k0 = 0
        for si, (dx, dk) in enumerate(SEGS):
            if si == 0:
                seg_cp[0][0].wait()
                ln1(0, dx)
                seg_cp[0][1].wait()
                build_a(*arng[0])
                seg_cp[0][2].wait()
                res = fold(D, k0, k0 + dk)
                early = None
            else:
                for c in seg_cp[si]:
                    c.wait()
                res = fold(D, k0, k0 + dk)
                if arng[si][1] > arng[si][0]:
                    build_a(*arng[si])
                xn_new = _ln(x_v[x0:x0 + dx, :].astype(f32))
                xn_v[x0:x0 + dx, :] = xn_new.astype(bf16)
                early = xn_new if EARLY else None
            flush(res[0])
            keep = KEEP if si == len(SEGS) - 1 else 0
            if x0:
                k_block(k0, k0 + dk, 0, x0, early=early)
            k_block(0, k0 + dk - keep, x0, x0 + dx, DEFER)
            x0 += dx
            k0 += dk
        cp_wv.wait()
        cp_x1a.wait()
        cp_z.wait()
        for c in cp_rel[2] + late:
            c.start()
        vtrans(0, D)
        res = k_block(D - KEEP, D, T - SEGS[-1][0], T)
        flush(res)
        yv = _dot_nt(wt(2 * D, 3 * D), xn_v[0:T, :])
        deps = [yv[128 * k:128 * k + 8, 128:256] for k in range(8)]
        xn_v[T:T + 128, :] = _ln(x_v[T:T + 128, :].astype(f32), deps, zv[...]).astype(bf16)
        for p in range(NP):
            kv = None
            for t0, phi in phis[p]:
                d_ = _dot_nt(yv[64 * p:64 * (p + 1), t0:t0 + phi.shape[1]].astype(bf16), phi)
                kv = d_ if kv is None else kv + d_
            kv_acc[p] = kv
        cp_x1.wait()

        def phase1(i, c):
            s = pl.multiple_of(i * T, T)
            rel_wait(i - 1)

            @pl.when(i == 2)
            def _():
                cp_x2.wait()
                for c in late2 + [cp_wd]:
                    c.start()

            zm = zv[...]
            xa = xn_v[pl.ds(s, 128), :]
            rest = pl.ds(pl.multiple_of(s + 128, 128), T - 128)
            xb = _ln(x_v[rest, :].astype(f32)).astype(bf16)
            xn_v[rest, :] = xb
            y = _dot_nt(wt(D, 3 * D), jnp.concatenate([xa, xb], axis=0))
            nxt = pl.multiple_of(jnp.where(i + 1 < NT, s + T, 0), 128)
            deps = [y[NXR + 64 * k:NXR + 64 * k + 8, 128 * NXJ:128 * NXJ + 128] for k in range(8)]
            xn_v[pl.ds(pl.multiple_of(s + T, 128), 128), :] = _ln(
                x_v[pl.ds(nxt, 128), :].astype(f32), deps, zm).astype(bf16)
            r0 = (i - 1) * RELG
            npc = RELG // RB
            for k in range(npc):
                jt = k * RJ // npc
                kk = k - (jt * npc + RJ - 1) // RJ
                per = (npc + RJ - 1) // RJ
                row = RLO + ((2 * D - RLO) * kk // per) // 8 * 8
                rel32[pl.ds(pl.multiple_of((r0 + k * RB) // 2, RB // 2), RB // 2), :] = _gated_pk(
                    rel_v[pl.ds(pl.multiple_of(r0 + k * RB, RB), RB), :],
                    y[row:row + 8, 128 * jt:128 * jt + 128], zm)
            for p in range(NP):
                phi, z = _phi_k(y[64 * p:64 * (p + 1)])
                z_acc[p] += z
                kv_acc[p] += _dot_nt(y[D + 64 * p: D + 64 * (p + 1)].astype(bf16), phi)
            return c
        lax.fori_loop(1, NT, phase1, 0)
    for c in late + late2:
        c.wait()
    wq = fold(0, 0, D)
    for j in range(D // 128):
        for k in range(4):
            wo32[j, 128 * k:128 * (k + 1), :] = _gated_pk(
                wo_v[j, 256 * k:256 * (k + 1), :], wq[j * 7 // 8][32 * k:32 * k + 8, 0:128], zv[...])
    r_i = lax.broadcasted_iota(jnp.int32, (64, 128), 0)
    c_i = lax.broadcasted_iota(jnp.int32, (64, 128), 1)
    kmask = r_i // 32 == c_i % 2
    for p in range(NP):
        kvt_v[p] = _pk(jnp.where(kmask, kv_acc[p], 0.0).astype(bf16))
        z_acc[p] = jnp.broadcast_to(jnp.sum(z_acc[p], axis=1, keepdims=True), (128, 128))

    def ln2(h, row0, onepass=False, deps=None):
        wr = wr_v[...].reshape(1, D).astype(f32)
        if onepass:
            m = jnp.sum(h, axis=-1, keepdims=True) * (1.0 / D)
            v = jnp.sum(h * h, axis=-1, keepdims=True) * (1.0 / D) - m * m
            rs = lax.rsqrt(jnp.maximum(v, 0.0) + EPS)
            r = (jnp.sum(h * wr, axis=-1, keepdims=True) - m * jnp.sum(wr, axis=-1, keepdims=True)) * rs
            hn = (h - m) * rs
        else:
            hn = _ln(h, deps, zv[...])
            r = jnp.sum(hn * wr, axis=-1, keepdims=True)
        rows = pl.ds(row0, h.shape[0])
        hn_v[rows, :] = hn.astype(bf16)
        out_v[rows, :] = (h + hn).astype(bf16)
        return r

    def gates(nx, ngr):
        deps = [None]
        for j in range(1, ngr):
            t = (j * NREL * 2) // ngr - 1
            r0 = (nx.shape[0] - 8) * (t % 2)
            deps.append(nx[r0:r0 + 8, 128 * (t // 2):128 * (t // 2) + 128] if t >= 0 else None)
        return deps

    def phase2(i, c_):
        s = pl.multiple_of(i * T, T)

        @pl.when(i == 1)
        def _():
            cp_out0.start()

        @pl.when(i > 1)
        def _():
            cp_out(i - 1).start()

        hprev = hbuf[...]
        y = _dot_nt(wt(0, D), xn_v[pl.ds(s, T), :])
        os_ = []
        for p in range(NP):
            phi = _phi_q(y[64 * p:64 * (p + 1)], z_acc[p])
            os_.append(_dot(_un(kvt_v[p]), phi))
        o = jnp.concatenate(os_, axis=0).astype(bf16).T
        atts = []
        c = 0
        for k, ch in enumerate(CHUNKS):
            wo = jnp.concatenate([_un(wo32[j]) for j in range(D // 128)], axis=1)
            atts.append(_dot(o[c:c + ch], wo))
            c += ch
        rs_ = [jnp.where(i > 0, ln2(hprev, s, deps=gates(atts[0], CL // G)), -jnp.inf)]
        c = 0
        for k, ch in enumerate(CHUNKS):
            h = x_v[pl.ds(pl.multiple_of(s + c, 16), ch), :].astype(f32) + atts[k]
            if k == len(CHUNKS) - 1:
                hbuf[...] = h
            else:
                rs_.append(ln2(h, pl.multiple_of(s + c + CL, 16), deps=gates(atts[k + 1], ch // G)))
            c += ch
        j = 0
        for r in rs_:
            for k in range(0, r.shape[0], 8):
                r_v[i, :, j:j + 1] = r[k:k + 8]
                j += 1
        return c_
    lax.fori_loop(0, 0 if ONLY1 else NT, phase2, 0)
    cp_out(NT - 1).start()
    tok = (lax.broadcasted_iota(jnp.int32, (8, 128), 1) * 8
           + lax.broadcasted_iota(jnp.int32, (8, 128), 0) - CL).astype(f32)
    pv, pt = r_v[0], tok
    for i in range(1, NT):
        gt = r_v[i] > pv
        pv = jnp.where(gt, r_v[i], pv)
        pt = jnp.where(gt, tok + float(i * T), pt)
    pm = jnp.max(_allred8(pv, jnp.maximum), axis=1, keepdims=True)
    pi = jnp.min(_allred8(jnp.where(pv == pm, pt, float(S)), jnp.minimum), axis=1, keepdims=True)
    r = ln2(hbuf[...], S, onepass=True)
    cp_last.start()
    sub = lax.broadcasted_iota(jnp.int32, (8, 1), 0).astype(f32)
    cands = [(r[k:k + 8], sub + float(S - CL + k)) for k in range(0, CL, 8)]
    while len(cands) > 1:
        nxt = []
        for k in range(0, len(cands), 2):
            (va, ia), (vb, ib) = cands[k], cands[k + 1]
            gt = vb > va
            nxt.append((jnp.where(gt, vb, va), jnp.where(gt, ib, ia)))
        cands = nxt
    lv, lt = cands[0]
    gt = lv > pm
    bv = jnp.broadcast_to(jnp.where(gt, lv, pm), (8, 128))
    bt = jnp.broadcast_to(jnp.where(gt, lt, pi), (8, 128))
    rmax = _allred8(bv, jnp.maximum)
    idxv = _allred8(jnp.where(bv == rmax, bt, float(S)), jnp.minimum).astype(jnp.int32)
    idx = jnp.clip(idxv[0, 0], 0, S - 1)
    base = pl.multiple_of(lax.shift_left(lax.shift_right_logical(idx, 4), 4), 16)
    baseq = pl.multiple_of(base + CL, 16)
    hit16 = lax.broadcasted_iota(jnp.int32, (16, D), 0) == idx - base
    cp_wd.wait()
    slab = jnp.where(hit16, hn_v[pl.ds(baseq, 16), :].astype(f32), 0.0)
    x8 = _allred8(slab[0:8] + slab[8:16], jnp.add)
    xs32 = _pk(jnp.concatenate([x8, x8], axis=0).astype(bf16))
    zm8 = jnp.concatenate([zv[...]] * 8, axis=1)

    def col(a8):
        return jnp.concatenate([a8] * 16, axis=0).astype(bf16).T.astype(f32)

    def act(r):
        n = r.shape[1] // 256
        g = jnp.concatenate([r[:, t * 256:t * 256 + 128] for t in range(n)], axis=1)
        u = jnp.concatenate([r[:, t * 256 + 128:t * 256 + 256] for t in range(n)], axis=1)
        return g * jax.nn.sigmoid(g) * u

    xcol = col(x8)
    av = None
    for k in range(0, D, 8):
        p = guv_v[k:k + 8, :].astype(f32) * jnp.concatenate([xcol[k:k + 8]] * (2 * NV), axis=1)
        av = p if av is None else av + p
    acc = None
    hist = []
    tail = []
    for cnt, j in enumerate(range(0, NM, MB)):
        w = jnp.concatenate(
            [graw_v[t] if t < 2 * RAWG else _un(rel32[(t - 2 * RAWG) * (D // 2):(t - 2 * RAWG + 1) * (D // 2)])
             for t in range(2 * j, 2 * (j + MB))], axis=1)
        xl = xs32
        if LAG <= cnt < LAG + len(hist) and cnt - LAG < len(hist):
            xl = xl | (pltpu.bitcast(hist[cnt - LAG], u32) & zm8)
        if cnt == VD:
            xl = xl | (pltpu.bitcast(jnp.concatenate([av] * (4 // NV), axis=1), u32) & zm8)
        a8 = act(_dot(_un(xl), w)[0:8])
        if j >= NDV:
            tail.append((a8, j, j + MB))
        else:
            ac = col(a8)
            for k in range(0, MB * 128, 8):
                p = wd_v[j * 128 + k:j * 128 + k + 8, :].astype(f32) * jnp.concatenate([ac[k:k + 8]] * 8, axis=1)
                acc = p if acc is None else acc + p
            hist.append(acc)
    tail = tail[:-1] + [(act(_allred8(av, jnp.add)), NM, NB)] + tail[-1:]
    yv = _allred8(acc, jnp.add)
    for a8, k0, k1 in tail:
        wdm = jnp.concatenate([draw_v[t, (k0 - NDV) * 128:(k1 - NDV) * 128] for t in range(8)], axis=1)
        yv = yv + _dot(jnp.concatenate([a8, a8], axis=0).astype(bf16), wdm)[0:8]
    sg = jax.nn.sigmoid(rmax)
    yv = yv * jnp.concatenate([sg] * (D // 128), axis=1)
    yv = jnp.concatenate([yv, yv], axis=0)
    if not ONLY1:
        cp_out0.wait()
        for i in range(1, NT - 1):
            cp_out(i).wait()
    cp_out(NT - 1).wait()
    cp_last.wait()
    cur = out_v[pl.ds(baseq, 16), :].astype(f32)
    out_v[pl.ds(baseq, 16), :] = jnp.where(hit16, cur + yv, cur).astype(bf16)
    cp_fin = cp(out_v.at[pl.ds(baseq, 16)], out_hbm.at[0, pl.ds(base, 16)])
    cp_fin.start()
    cp_fin.wait()


@jax.jit
def pallas_sequential_preLN__linear_kernel_hedgehog__moe_arch_mod__prompt_kernel(
    A_x, A_wqkv, A_w_phi, A_wo, B_x, B_w_r, B_w_gate, B_w_up, B_w_down):
    del B_x
    any_spec = pl.BlockSpec(memory_space=pl.ANY)
    return pl.pallas_call(
        _kernel,
        out_shape=jax.ShapeDtypeStruct((1, S, D), bf16),
        in_specs=[any_spec] * 8,
        out_specs=any_spec,
        scratch_shapes=[
            pltpu.VMEM((S, D), bf16),
            pltpu.VMEM((D, 3 * D), bf16),
            pltpu.VMEM((H, DH, DH), bf16),
            pltpu.VMEM((D // 128, D, 128), bf16),
            pltpu.VMEM((D // 128, D // 2, 128), u32),
            pltpu.VMEM((D,), bf16),
            pltpu.VMEM((2 * RAWG, D, 128), bf16),
            pltpu.VMEM((D // 128, F - NDV * 128, 128), bf16),
            pltpu.VMEM((D, NV * 256), bf16),
            pltpu.VMEM((NDV * 128, D), bf16),
            pltpu.VMEM((REL, 128), bf16),
            pltpu.VMEM((REL // 2, 128), u32),
            pltpu.VMEM((3 * D // 2, D), u32),
            pltpu.VMEM((8, 64, 128), u32),
            pltpu.VMEM((S + 128, D), bf16),
            pltpu.VMEM((S + CL, D), bf16),
            pltpu.VMEM((NP, 64, 128), f32),
            pltpu.VMEM((NP, 128, 128), f32),
            pltpu.VMEM((NP, 32, 128), u32),
            pltpu.VMEM((CL, D), f32),
            pltpu.VMEM((S + CL, D), bf16),
            pltpu.VMEM((8, 128), u32),
            pltpu.SMEM((8, 128), u32),
            pltpu.VMEM((NT, 8, 128), f32),
            pltpu.SemaphoreType.DMA((64,)),
        ],
        compiler_params=pltpu.CompilerParams(vmem_limit_bytes=120 * 1024 * 1024,
                                             disable_bounds_checks=True,
                                             disable_semaphore_checks=True),
        name="hedgehog_mod",
    )(A_x, A_wqkv, A_w_phi, A_wo, B_w_r, B_w_gate, B_w_up, B_w_down)
```

```python
import jax
import jax.numpy as jnp
from jax import lax
import jax.experimental.pallas as pl
import jax.experimental.pallas.tpu as pltpu

S = 2048
D = 1024
H = 32
DH = 32
F = 3584
NP = H // 2
T = 512
NT = S // T
C = 128
NC = S // C
CPT = T // C
NB = F // 128
ONLY1 = 0; ONLY2 = 0
G = 16; NREL = 6
NXR = 1536; NXJ = 2
SEGS = [tuple(128 * int(v) for v in t) for t in '22,12,14'.split(",")]
KEEP = 256; DEFER = 2
NA = 10
SEG = 8; W0 = 0; W1 = 24
TD0 = 48; TD1 = 490
NCAND = 2
PR0 = 1408; DMID = 1; EPS_ = 2
FORCE = 0
LOG2E = 1.4426950408889634
EPS = 1e-5

f32 = jnp.float32
bf16 = jnp.bfloat16
u32 = jnp.uint32
i32 = jnp.int32


def _dot_nt(a, b):
    return lax.dot_general(a, b, (((1,), (1,)), ((), ())), preferred_element_type=f32)


def _dot(a, b):
    return jnp.dot(a, b, preferred_element_type=f32)


def _pk(x):
    return pltpu.bitcast(x, u32)


def _un(x):
    return pltpu.bitcast(x, bf16)


def _rcp(x):
    r = pl.reciprocal(x, approx=True)
    return r * (2.0 - x * r)


def _allred(v, op):
    v = op(v, pltpu.roll(v, 2, 0))
    return op(v, pltpu.roll(v, 4, 0))


def _allred8(v, op):
    return _allred(op(v, pltpu.roll(v, 1, 0)), op)


def _zero_after(dep, zm):
    return pltpu.bitcast(pltpu.bitcast(dep, u32) & zm, f32)


def _exps(x):
    L = x.shape[1]
    x3 = x.reshape(8, 8, L)
    mx = _allred(jnp.max(x3, axis=0), jnp.maximum)
    mn = _allred(jnp.min(x3, axis=0), jnp.minimum)
    ep = jnp.exp2(x3 - mx[None])
    en = jnp.exp2(mn[None] - x3)
    rp = _rcp(_allred(jnp.sum(ep, axis=0), jnp.add))
    rn = _rcp(_allred(jnp.sum(en, axis=0), jnp.add))
    return ep, en, rp, rn


def _phi_k(x):
    L = x.shape[1]
    ep, en, rp, rn = _exps(x)
    phi = jnp.concatenate([(ep * rp[None]).reshape(64, L), (en * rn[None]).reshape(64, L)], axis=0)
    z = phi[:, 0:128]
    for c in range(128, L, 128):
        z = z + phi[:, c:c + 128]
    return phi.astype(bf16), z


def _phi_q(x, zb):
    L = x.shape[1]
    ep, en, rp, rn = _exps(x)
    zb = jnp.concatenate([zb] * (L // 128), axis=1).reshape(16, 8, L)
    den = rp * jnp.sum(ep * zb[0:8], axis=0) + rn * jnp.sum(en * zb[8:16], axis=0)
    inv = _rcp(_allred(den, jnp.add) + 1e-6)
    cp = rp * inv
    cn = rn * inv
    phi = jnp.concatenate([(ep * cp[None]).reshape(64, L), (en * cn[None]).reshape(64, L)], axis=0)
    return phi.astype(bf16)


def _ln(x, deps=None, zm=None):
    if deps is None:
        tot = jnp.sum(x, axis=-1, keepdims=True)
    else:
        g = x.shape[0] // len(deps)
        gate = jnp.concatenate(
            [jnp.zeros((8, 128), f32) if d is None else _zero_after(d, zm)
             for d in deps for _ in range(g // 8)], axis=0)
        acc = x[:, 0:128] + gate
        for c in range(128, D, 128):
            acc = acc + x[:, c:c + 128]
        tot = jnp.sum(acc, axis=-1, keepdims=True)
    xc = x - tot * (1.0 / D)
    return xc * lax.rsqrt(jnp.sum(xc * xc, axis=-1, keepdims=True) * (1.0 / D) + EPS)


def _col(a8):
    return jnp.concatenate([a8] * 16, axis=0).astype(bf16).T.astype(f32)


def _first_max(v, t):
    m = jnp.max(_allred8(v, jnp.maximum), axis=1, keepdims=True)
    return m, jnp.min(_allred8(jnp.where(v == m, t, float(2 * S)), jnp.minimum), axis=1, keepdims=True)


def _kernel(x_hbm, wqkv_hbm, wphi_hbm, wo_hbm, wr_hbm, wg_hbm, wu_hbm, wd_hbm, out_hbm,
            x_v, wqkv_v, wphi_v, wo_v, wo32, wr_v, wg_v, wu_v, wd_v,
            wt_v, a_v, xn_v, hn_v, kv_acc, z_acc, kvt_v, hbuf, out_v, zv, zs, p_v, r_v,
            xc_v, pa_v, ac_v, y_v, ord_s, sems):
    nsem = [0]

    def cp(src, dst):
        nsem[0] += 1
        return pltpu.make_async_copy(src, dst, sems.at[nsem[0] - 1])

    def cp_w(lo, hi):
        return cp(wqkv_hbm.at[:, lo:hi], wqkv_v.at[:, lo:hi])

    def cp_xr(lo, hi):
        return cp(x_hbm.at[0, lo:hi], x_v.at[lo:hi])

    def cp_ph(lo, hi):
        return cp(wphi_hbm.at[lo // DH:hi // DH], wphi_v.at[lo // DH:hi // DH])

    cp_wr = cp(wr_hbm, wr_v)
    seg_cp = []
    x0 = k0 = 0
    kcum = [0]
    for dx, dk in SEGS:
        kcum.append(kcum[-1] + dk)
    arng = [(0 if si == 0 else kcum[si + 1], kcum[min(si + 2, len(SEGS))]) for si in range(len(SEGS))]
    for si, (dx, dk) in enumerate(SEGS):
        ph = [cp_ph(*arng[si])] if arng[si][1] > arng[si][0] else []
        seg_cp.append([cp_xr(x0, x0 + dx)] + ph + [cp_w(D + k0, D + k0 + dk)])
        x0 += dx
        k0 += dk
    cp_wv = cp_w(2 * D, 3 * D)
    cp_x1a = cp_xr(T, T + C)
    cp_x1 = cp_xr(T + C, S)
    late = [cp_w(0, D)] + [cp(wo_hbm.at[:, j * 128:(j + 1) * 128], wo_v.at[j]) for j in range(D // 128)]
    late += [cp(wg_hbm, wg_v), cp(wu_hbm, wu_v), cp(wd_hbm, wd_v)]
    first = [c for t in seg_cp for c in t] + [cp_wr, cp_wv, cp_x1a, cp_x1]
    for c in first + late:
        c.start()
    osem0 = nsem[0]
    nsem[0] += NC + 1

    def cp_out(q):
        rows = pl.ds(pl.multiple_of(ord_s[q], C), C)
        return pltpu.make_async_copy(out_v.at[rows], out_hbm.at[0, rows], sems.at[osem0 + q])

    def wr_row():
        return wr_v[...].reshape(1, D).astype(f32)

    def put_cols(ref, idx, col0, r):
        for k in range(0, r.shape[0], 8):
            ref[idx, :, col0 + k // 8:col0 + k // 8 + 1] = r[k:k + 8]

    def ln1(src, dst, deps=None):
        xb = _ln(x_v[src, :].astype(f32), deps, None if deps is None else zv[...]).astype(bf16)
        xn_v[dst, :] = xb
        return xb

    def predict(rows, c, deps):
        wr = wr_row()
        wc = wr - jnp.sum(wr, axis=-1, keepdims=True) * (1.0 / D)
        t = x_v[rows, :].astype(f32) * wc
        g = C // len(deps)
        acc = t[:, 0:128] + jnp.concatenate([_zero_after(d, zv[...]) for d in deps for _ in range(g // 8)], axis=0)
        for j in range(128, D, 128):
            acc = acc + t[:, j:j + 128]
        put_cols(p_v, c, 0, jnp.sum(acc, axis=-1, keepdims=True))

    def fold(base, lo, hi):
        res = []
        for g in range(lo // 128, hi // 128):
            w = _dot_nt(_un(a_v[g]), wqkv_v[:, base + 128 * g: base + 128 * (g + 1)])
            wt_v[(base + 128 * g) // 2: (base + 128 * (g + 1)) // 2, :] = _pk((w * LOG2E).astype(bf16))
            res.append(w)
        return res

    def wt(lo, hi):
        return _un(wt_v[lo // 2:hi // 2, :])

    r_i = lax.broadcasted_iota(i32, (128, DH), 0)
    f_i = lax.broadcasted_iota(i32, (128, DH), 1)
    sel = jnp.where(f_i == (r_i % 64) // 2, 1.0, 0.0).astype(bf16)
    r_i = lax.broadcasted_iota(i32, (128, 128), 0)
    c_i = lax.broadcasted_iota(i32, (128, 128), 1)
    amask = jnp.where(c_i // 32 == 2 * (r_i // 64) + r_i % 2, jnp.uint32(0xFFFFFFFF), jnp.uint32(0))

    def build_a(lo, hi):
        a_full = _dot_nt(sel, wphi_v[lo // DH:hi // DH].reshape(hi - lo, DH))
        for g in range((hi - lo) // 128):
            blk = pltpu.bitcast(pltpu.bitcast(a_full[:, 128 * g:128 * (g + 1)], u32) & amask, f32)
            a_v[lo // 128 + g] = _pk(blk.astype(bf16))

    zv[...] = jnp.zeros((8, 128), u32)
    cp_z = cp(zv, zs)
    cp_z.start()
    hbuf[...] = jnp.zeros(hbuf.shape, f32)
    xc_v[...] = jnp.zeros(xc_v.shape, f32)
    y_v[...] = jnp.zeros(y_v.shape, f32)
    r_v[...] = jnp.full(r_v.shape, -jnp.inf, f32)
    p_v[...] = jnp.full(p_v.shape, -jnp.inf, f32)

    phis = [[] for _ in range(NP)]
    pending = []

    def phi_piece(p, t0, yp, dep=None):
        if dep is not None:
            yp = jnp.concatenate([yp[0:8] + _zero_after(dep, zv[...]), yp[8:]], axis=0)
        phi, z = _phi_k(yp)
        if phis[p]:
            z_acc[p] += z
        else:
            z_acc[p] = z
        phis[p].append((t0, phi))

    def k_block(klo, khi, t0, t1, defer=0):
        y = _dot_nt(wt(D + klo, D + khi), xn_v[t0:t1, :])
        npair = (khi - klo) // 64
        for p in range(npair):
            yp = y[64 * p:64 * (p + 1)]
            if p >= npair - defer:
                if t1 - t0 > 128:
                    phi_piece(klo // 64 + p, t0, yp[:, 0:t1 - t0 - 128])
                pending.append((klo // 64 + p, t1 - 128, yp[:, t1 - t0 - 128:]))
            else:
                phi_piece(klo // 64 + p, t0, yp)
        return y

    def flush(res):
        for k, (p, t0, yp) in enumerate(pending):
            phi_piece(p, t0, yp, res[32 * k:32 * k + 8, 0:128])
        del pending[:]

    if ONLY2:
        for c in first + [cp_z]:
            c.wait()
    else:
        x0 = k0 = 0
        for si, (dx, dk) in enumerate(SEGS):
            rows = slice(x0, x0 + dx)
            if si == 0:
                seg_cp[0][0].wait()
                ln1(rows, rows)
                seg_cp[0][1].wait()
                build_a(*arng[0])
                seg_cp[0][2].wait()
                res = fold(D, k0, k0 + dk)
            else:
                for c in seg_cp[si]:
                    c.wait()
                res = fold(D, k0, k0 + dk)
                if arng[si][1] > arng[si][0]:
                    build_a(*arng[si])
                ln1(rows, rows)
            flush(res[0])
            keep = KEEP if si == len(SEGS) - 1 else 0
            if x0:
                k_block(k0, k0 + dk, 0, x0)
            k_block(0, k0 + dk - keep, x0, x0 + dx, DEFER)
            x0 += dx
            k0 += dk
        cp_wv.wait()
        cp_x1a.wait()
        cp_wr.wait()
        cp_z.wait()
        for g in range(D // 128):
            wt_v[(2 * D + 128 * g) // 2: (2 * D + 128 * (g + 1)) // 2, :] = _pk(
                wqkv_v[:, 2 * D + 128 * g: 2 * D + 128 * (g + 1)].T)
        flush(k_block(D - KEEP, D, T - SEGS[-1][0], T))
        yv = _dot_nt(wt(2 * D, 3 * D), xn_v[0:T, :])
        ln1(slice(T, T + C), slice(T, T + C), [yv[128 * k:128 * k + 8, 128:256] for k in range(8)])
        for c in range(CPT):
            predict(slice(C * c, C * (c + 1)), c,
                    [yv[256 * c + 32 * k:256 * c + 32 * k + 8, 256:384] for k in range(8)])
        for p in range(NP):
            kv = None
            for t0, phi in phis[p]:
                d_ = _dot_nt(yv[64 * p:64 * (p + 1), t0:t0 + phi.shape[1]].astype(bf16), phi)
                kv = d_ if kv is None else kv + d_
            kv_acc[p] = kv
        cp_x1.wait()

        def phase1(i, c):
            s = pl.multiple_of(i * T, T)
            xa = xn_v[pl.ds(s, C), :]
            rest = pl.ds(pl.multiple_of(s + C, C), T - C)
            xb = ln1(rest, rest)
            y = _dot_nt(wt(D, 3 * D), jnp.concatenate([xa, xb], axis=0))
            nxt = pl.multiple_of(jnp.where(i + 1 < NT, s + T, 0), C)
            ln1(pl.ds(nxt, C), pl.ds(pl.multiple_of(s + T, C), C),
                [y[NXR + 64 * k:NXR + 64 * k + 8, 128 * NXJ:128 * NXJ + 128] for k in range(8)])
            for c in range(CPT):
                r0 = PR0 + ((2 * D - PR0) // 2) * (c % 2)
                st = ((2 * D - PR0) // 16) // 8 * 8
                predict(pl.ds(pl.multiple_of(s + C * c, C), C), CPT * i + c,
                        [y[r0 + st * k:r0 + st * k + 8, 128 * (c // 2):128 * (c // 2) + 128] for k in range(8)])
            for p in range(NP):
                phi, z = _phi_k(y[64 * p:64 * (p + 1)])
                z_acc[p] += z
                kv_acc[p] += _dot_nt(y[D + 64 * p: D + 64 * (p + 1)].astype(bf16), phi)
            return c
        lax.fori_loop(1, NT, phase1, 0)
    for c in late:
        c.wait()
    keys = []
    for c in range(NC):
        m = jnp.max(_allred8(p_v[c], jnp.maximum), axis=1, keepdims=True)
        b = pltpu.bitcast(jnp.broadcast_to(m, (8, 128)), i32)
        keys.append((b ^ (lax.shift_right_arithmetic(b, 31) & 0x7FFFFFFF))[0, 0])
    rank = [jnp.int32(0)] * NC
    for a in range(NC):
        for b in range(a + 1, NC):
            ge = (keys[a] >= keys[b]).astype(i32)
            rank[b] = rank[b] + ge
            rank[a] = rank[a] + (1 - ge)
    ord_s[0] = S
    for c in range(NC):
        ord_s[1 + (NC - 1 - rank[c] if FORCE else rank[c])] = c * C
    wq = fold(0, 0, D)
    for j in range(D // 128):
        for k in range(4):
            w = _pk(wo_v[j, 256 * k:256 * (k + 1), :])
            z = pltpu.bitcast(wq[j * 7 // 8][32 * k:32 * k + 8, 0:128], u32) & zv[...]
            wo32[j, 128 * k:128 * (k + 1), :] = (w.reshape(16, 8, 128) | z[None]).reshape(128, 128)
    r_i = lax.broadcasted_iota(i32, (64, 128), 0)
    c_i = lax.broadcasted_iota(i32, (64, 128), 1)
    kmask = r_i // 32 == c_i % 2
    for p in range(NP):
        kvt_v[p] = _pk(jnp.where(kmask, kv_acc[p], 0.0).astype(bf16))
        z_acc[p] = jnp.broadcast_to(jnp.sum(z_acc[p], axis=1, keepdims=True), (128, 128))

    def ln2(h, row0, onepass=False, deps=None):
        wr = wr_row()
        if onepass:
            m = jnp.sum(h, axis=-1, keepdims=True) * (1.0 / D)
            v = jnp.sum(h * h, axis=-1, keepdims=True) * (1.0 / D) - m * m
            rs = lax.rsqrt(jnp.maximum(v, 0.0) + EPS)
            r = (jnp.sum(h * wr, axis=-1, keepdims=True) - m * jnp.sum(wr, axis=-1, keepdims=True)) * rs
            hn = (h - m) * rs
        else:
            hn = _ln(h, deps, zv[...])
            r = jnp.sum(hn * wr, axis=-1, keepdims=True)
        hn_v[pl.ds(row0, C), :] = hn.astype(bf16)
        out_v[pl.ds(row0, C), :] = (h + hn).astype(bf16)
        return r

    def gates(nx):
        deps = [None]
        ngr = C // G
        for j in range(1, ngr):
            t = (j * NREL * 2) // ngr - 1
            r0 = (C - 8) * (t % 2)
            deps.append(nx[r0:r0 + 8, 128 * (t // 2):128 * (t // 2) + 128] if t >= 0 else None)
        return deps

    lane = lax.broadcasted_iota(i32, (8, 128), 1)
    pos = (lane * 8 + lax.broadcasted_iota(i32, (8, 128), 0)).astype(f32)

    def token_at(posv, lo, hi):
        p = jnp.clip(jnp.broadcast_to(posv, (8, 128)).astype(i32)[0, 0], lo, hi - 1)
        return ord_s[lax.shift_right_logical(p, 7)] + (p & (C - 1))

    def token_row(tok):
        base = pl.multiple_of(lax.shift_left(lax.shift_right_logical(tok, 4), 4), 16)
        hit = lax.broadcasted_iota(i32, (16, D), 0) == tok - base
        slab = jnp.where(hit, hn_v[pl.ds(base, 16), :].astype(f32), 0.0)
        return _allred8(slab[0:8] + slab[8:16], jnp.add)

    def phase2(i, c_):
        q0 = CPT * i

        @pl.when(i > 0)
        def _():
            cp_out(q0 - 1).start()

        off = [pl.multiple_of(ord_s[q0 + k], C) for k in range(CPT + 1)]
        zm = zv[...]
        hprev = hbuf[...]
        ya, ys = [], []
        for n in range(CPT):
            xt = xn_v[pl.ds(off[n + 1], C), :]
            ya.append(_dot_nt(_un(wt_v[0:D // 2, 0:D // 2]), xt[:, 0:D // 2]))
            ys.append(ya[n] + _dot_nt(_un(wt_v[0:D // 2, D // 2:D]), xt[:, D // 2:D]))
        y = jnp.concatenate(ys, axis=1)
        os_ = []
        for p in range(NP):
            phi = _phi_q(y[64 * p:64 * (p + 1)], z_acc[p])
            os_.append(_dot(_un(kvt_v[p]), phi))
        o = jnp.concatenate(os_, axis=0).astype(bf16).T
        wo = jnp.concatenate([_un(wo32[j]) for j in range(D // 128)], axis=1)
        atts = [_dot(o[C * k:C * (k + 1)], wo) for k in range(CPT)]

        def qgate(v):
            lens = [128 - W0] + [128 - W1] * 3
            t = int(v * sum(lens))
            n = 0
            while t >= lens[n]:
                t -= lens[n]
                n += 1
            r0 = 8 * (t + 128 - lens[n])
            return _zero_after(ya[n][r0:r0 + 8], zm)

        def ogate(t):
            r0, j = 8 * (t % 16), (t % 128) // 16
            return _zero_after(atts[t // 128][r0:r0 + 8, 128 * j:128 * j + 128], zm)

        b0 = jnp.where(i < 2, 0, jnp.where(i == 2, NA, NB - NA))
        nsb = NA // 2
        for sb in range(nsb):
            c0 = pl.multiple_of((b0 + 2 * sb) * 128, 256)
            xcol = xc_v[pl.ds(pl.multiple_of(zs[1, sb].astype(i32), 8), D), :]
            acc = None
            for k in range(0, D, 8):
                xk = jnp.concatenate([xcol[k:k + 8]] * 2, axis=1)
                p = jnp.concatenate([wg_v[k:k + 8, pl.ds(c0, 256)].astype(f32) * xk,
                                     wu_v[k:k + 8, pl.ds(c0, 256)].astype(f32) * xk], axis=1)
                if (k // 8) % SEG == 0:
                    p = p + jnp.concatenate([qgate((sb * D + k) / (nsb * D))] * 4, axis=1)
                acc = p if acc is None else acc + p
            pa_v[:, 512 * sb:512 * (sb + 1)] = acc

        put_cols(r_v, i, 0, jnp.where(i > 0, ln2(hprev, off[0], deps=gates(atts[0])), -jnp.inf))

        @pl.when(i > 0)
        def _():
            cp_out(q0).start()

        acc = _allred8(pa_v[pl.ds(pl.multiple_of(zs[3, 0].astype(i32), 8), 8), :], jnp.add)
        g_ = jnp.concatenate([acc[:, 512 * t:512 * t + 256] for t in range(nsb)], axis=1)
        u_ = jnp.concatenate([acc[:, 512 * t + 256:512 * t + 512] for t in range(nsb)], axis=1)
        a8 = g_ * jax.nn.sigmoid(g_) * u_
        ndup = (3 * NA - NB) * 128
        a8 = jnp.concatenate([jnp.where(i == NT - 1, 0.0, a8[:, 0:ndup]), a8[:, ndup:]], axis=1)
        ac_v[...] = _col(a8)
        ac = ac_v[pl.ds(pl.multiple_of(zs[2, 0].astype(i32), 8), NA * 128), :]
        ysum = jnp.where(i > 1, y_v[...], 0.0)
        for k in range(0, NA * 128, 8):
            p = (wd_v[pl.ds(pl.multiple_of(b0 * 128 + k, 8), 8), :].astype(f32)
                 * jnp.concatenate([ac[k:k + 8]] * 8, axis=1))
            if (k // 8) % (SEG // 2) == 0:
                p = p + jnp.concatenate([ogate(TD0 + k * (TD1 - TD0) // (NA * 128))] * 8, axis=1)
            ysum = ysum + p
        y_v[...] = ysum

        for k in range(CPT):
            if k == NCAND:
                ok = (lane >= C // 8) & (lane < (NCAND + 1) * (C // 8))
                cand = token_at(_first_max(jnp.where(ok, r_v[0], -jnp.inf), pos)[1], C, (NCAND + 1) * C)
                ord_s[NC + 1] = cand
                xc_v[...] = _col(token_row(cand))
            h = x_v[pl.ds(off[k + 1], C), :].astype(f32) + atts[k]
            if k == CPT - 1:
                hbuf[...] = h
            else:
                put_cols(r_v, i, (k + 1) * (C // 8), ln2(h, off[k + 1], deps=gates(atts[k + 1])))
                if k < CPT - 2:
                    cp_out(q0 + k + 1).start()
        return c_
    lax.fori_loop(0, 0 if ONLY1 else NT, phase2, 0)
    cp_out(NC - 1).start()
    pv, pt = r_v[0], pos
    for i in range(1, NT):
        gt = r_v[i] > pv
        pv = jnp.where(gt, r_v[i], pv)
        pt = jnp.where(gt, pos + float(i * T), pt)
    pm, pi = _first_max(pv, pt)
    r = ln2(hbuf[...], pl.multiple_of(ord_s[NC], C), onepass=True)
    cp_out(NC).start()
    sub = lax.broadcasted_iota(i32, (8, 1), 0).astype(f32)
    cands = [(r[k:k + 8], sub + float(S + k)) for k in range(0, C, 8)]
    while len(cands) > 1:
        nxt = []
        for k in range(0, len(cands), 2):
            (va, ia), (vb, ib) = cands[k], cands[k + 1]
            gt = vb > va
            nxt.append((jnp.where(gt, vb, va), jnp.where(gt, ib, ia)))
        cands = nxt
    lv, lt = cands[0]
    gt = lv > pm
    bv = jnp.broadcast_to(jnp.where(gt, lv, pm), (8, 128))
    bt = jnp.broadcast_to(jnp.where(gt, lt, pi), (8, 128))
    rmax = _allred8(bv, jnp.maximum)
    idx = token_at(_allred8(jnp.where(bv == rmax, bt, float(2 * S)), jnp.minimum), C, S + C)
    y_v[...] = _allred8(y_v[...], jnp.add)

    miss = idx != ord_s[NC + 1]
    for q in range(1, NCAND + 1):
        cp_out(q).wait()

    def wait_rest():
        for q in range(NCAND + 1, NC + 1):
            cp_out(q).wait()

    @pl.when(miss)
    def _():
        x8 = token_row(idx)
        xs = jnp.concatenate([x8, x8], axis=0).astype(bf16)

        def step(j, acc):
            cols = pl.ds(pl.multiple_of(j * 512, 512), 512)
            g = _dot(xs, wg_v[:, cols])
            a = g * jax.nn.sigmoid(g) * _dot(xs, wu_v[:, cols])
            return acc + _dot(a.astype(bf16), wd_v[cols, :])[0:8]

        y_v[...] = lax.fori_loop(0, F // 512, step, jnp.zeros((8, D), f32))
        wait_rest()
    yv = y_v[...] * jnp.concatenate([jax.nn.sigmoid(rmax)] * (D // 128), axis=1)
    base = pl.multiple_of(lax.shift_left(lax.shift_right_logical(idx, 4), 4), 16)
    hit16 = lax.broadcasted_iota(i32, (16, D), 0) == idx - base
    cur = out_v[pl.ds(base, 16), :].astype(f32)
    out_v[pl.ds(base, 16), :] = jnp.where(hit16, cur + jnp.concatenate([yv, yv], axis=0), cur).astype(bf16)
    cp_fin = cp(out_v.at[pl.ds(base, 16)], out_hbm.at[0, pl.ds(base, 16)])
    cp_fin.start()

    @pl.when(jnp.logical_not(miss))
    def _():
        wait_rest()

    cp_fin.wait()


@jax.jit
def pallas_sequential_preLN__linear_kernel_hedgehog__moe_arch_mod__prompt_kernel(
    A_x, A_wqkv, A_w_phi, A_wo, B_x, B_w_r, B_w_gate, B_w_up, B_w_down):
    del B_x
    any_spec = pl.BlockSpec(memory_space=pl.ANY)
    return pl.pallas_call(
        _kernel,
        out_shape=jax.ShapeDtypeStruct((1, S, D), bf16),
        in_specs=[any_spec] * 8,
        out_specs=any_spec,
        scratch_shapes=[
            pltpu.VMEM((S, D), bf16),
            pltpu.VMEM((D, 3 * D), bf16),
            pltpu.VMEM((H, DH, DH), bf16),
            pltpu.VMEM((D // 128, D, 128), bf16),
            pltpu.VMEM((D // 128, D // 2, 128), u32),
            pltpu.VMEM((D,), bf16),
            pltpu.VMEM((D, F), bf16),
            pltpu.VMEM((D, F), bf16),
            pltpu.VMEM((F, D), bf16),
            pltpu.VMEM((3 * D // 2, D), u32),
            pltpu.VMEM((8, 64, 128), u32),
            pltpu.VMEM((S + C, D), bf16),
            pltpu.VMEM((S + C, D), bf16),
            pltpu.VMEM((NP, 64, 128), f32),
            pltpu.VMEM((NP, 128, 128), f32),
            pltpu.VMEM((NP, 32, 128), u32),
            pltpu.VMEM((C, D), f32),
            pltpu.VMEM((S + C, D), bf16),
            pltpu.VMEM((8, 128), u32),
            pltpu.SMEM((8, 128), u32),
            pltpu.VMEM((NC, 8, 128), f32),
            pltpu.VMEM((NT, 8, 128), f32),
            pltpu.VMEM((D, 128), f32),
            pltpu.VMEM((8, NA * 256), f32),
            pltpu.VMEM((NA * 128, 128), f32),
            pltpu.VMEM((8, D), f32),
            pltpu.SMEM((NC + 2,), i32),
            pltpu.SemaphoreType.DMA((64,)),
        ],
        compiler_params=pltpu.CompilerParams(vmem_limit_bytes=120 * 1024 * 1024,
                                             disable_bounds_checks=True,
                                             disable_semaphore_checks=True),
        name="hedgehog_mod",
    )(A_x, A_wqkv, A_w_phi, A_wo, B_w_r, B_w_gate, B_w_up, B_w_down)
```

```python
import jax
import jax.numpy as jnp
from jax import lax
import jax.experimental.pallas as pl
import jax.experimental.pallas.tpu as pltpu

S = 2048
D = 1024
H = 32
DH = 32
F = 3584
NP = H // 2
T = 512
NT = S // T
C = 128
NC = S // C
CPT = T // C
NB = F // 128
ONLY1 = 0; ONLY2 = 0
G = 16; NREL = 6
NXR = 1536; NXJ = 2
SEGS = [tuple(128 * int(v) for v in t) for t in '22,12,14'.split(",")]
KEEP = 256; DEFER = 2
NA = 10
SEG = 8; W0 = 0; W1 = 24
TD0 = 64; TD1 = 440
B0 = (0, NA, NB - NA)
NDUP = (3 * NA - NB) * 128
NCAND = 2
PR0 = 1408; DMID = 1; EPS_ = 2
NOC = 0; NOG = 0; NOD = 0
NH = 2; SEGD = 4
FORCE = 0
LOG2E = 1.4426950408889634
EPS = 1e-5

f32 = jnp.float32
bf16 = jnp.bfloat16
u32 = jnp.uint32
i32 = jnp.int32


def _dot_nt(a, b):
    return lax.dot_general(a, b, (((1,), (1,)), ((), ())), preferred_element_type=f32)


def _dot(a, b):
    return jnp.dot(a, b, preferred_element_type=f32)


def _pk(x):
    return pltpu.bitcast(x, u32)


def _un(x):
    return pltpu.bitcast(x, bf16)


def _rcp(x):
    r = pl.reciprocal(x, approx=True)
    return r * (2.0 - x * r)


def _allred(v, op):
    v = op(v, pltpu.roll(v, 2, 0))
    return op(v, pltpu.roll(v, 4, 0))


def _allred8(v, op):
    return _allred(op(v, pltpu.roll(v, 1, 0)), op)


def _zero_after(dep, zm):
    return pltpu.bitcast(pltpu.bitcast(dep, u32) & zm, f32)


def _exps(x):
    L = x.shape[1]
    x3 = x.reshape(8, 8, L)
    mx = _allred(jnp.max(x3, axis=0), jnp.maximum)
    mn = _allred(jnp.min(x3, axis=0), jnp.minimum)
    ep = jnp.exp2(x3 - mx[None])
    en = jnp.exp2(mn[None] - x3)
    rp = _rcp(_allred(jnp.sum(ep, axis=0), jnp.add))
    rn = _rcp(_allred(jnp.sum(en, axis=0), jnp.add))
    return ep, en, rp, rn


def _phi_k(x):
    L = x.shape[1]
    ep, en, rp, rn = _exps(x)
    phi = jnp.concatenate([(ep * rp[None]).reshape(64, L), (en * rn[None]).reshape(64, L)], axis=0)
    z = phi[:, 0:128]
    for c in range(128, L, 128):
        z = z + phi[:, c:c + 128]
    return phi.astype(bf16), z


def _phi_q(x, zb):
    L = x.shape[1]
    ep, en, rp, rn = _exps(x)
    zb = jnp.concatenate([zb] * (L // 128), axis=1).reshape(16, 8, L)
    den = rp * jnp.sum(ep * zb[0:8], axis=0) + rn * jnp.sum(en * zb[8:16], axis=0)
    inv = _rcp(_allred(den, jnp.add) + 1e-6)
    cp = rp * inv
    cn = rn * inv
    phi = jnp.concatenate([(ep * cp[None]).reshape(64, L), (en * cn[None]).reshape(64, L)], axis=0)
    return phi.astype(bf16)


def _ln(x, deps=None, zm=None):
    if deps is None:
        tot = jnp.sum(x, axis=-1, keepdims=True)
    else:
        g = x.shape[0] // len(deps)
        gate = jnp.concatenate(
            [jnp.zeros((8, 128), f32) if d is None else _zero_after(d, zm)
             for d in deps for _ in range(g // 8)], axis=0)
        acc = x[:, 0:128] + gate
        for c in range(128, D, 128):
            acc = acc + x[:, c:c + 128]
        tot = jnp.sum(acc, axis=-1, keepdims=True)
    xc = x - tot * (1.0 / D)
    return xc * lax.rsqrt(jnp.sum(xc * xc, axis=-1, keepdims=True) * (1.0 / D) + EPS)


def _col(a8):
    return jnp.concatenate([a8] * 16, axis=0).astype(bf16).T.astype(f32)


def _first_max(v, t):
    m = jnp.max(_allred8(v, jnp.maximum), axis=1, keepdims=True)
    return m, jnp.min(_allred8(jnp.where(v == m, t, float(2 * S)), jnp.minimum), axis=1, keepdims=True)


def _kernel(x_hbm, wqkv_hbm, wphi_hbm, wo_hbm, wr_hbm, wg_hbm, wu_hbm, wd_hbm, out_hbm,
            x_v, wqkv_v, wphi_v, wo_v, wo32, wr_v, wg_v, wu_v, wd_v,
            wt_v, a_v, xn_v, hn_v, kv_acc, z_acc, kvt_v, hbuf, out_v, zv, zs, p_v, r_v,
            xc_v, pa_v, y_v, ord_s, sems):
    nsem = [0]

    def cp(src, dst):
        nsem[0] += 1
        return pltpu.make_async_copy(src, dst, sems.at[nsem[0] - 1])

    def cp_w(lo, hi):
        return cp(wqkv_hbm.at[:, lo:hi], wqkv_v.at[:, lo:hi])

    def cp_xr(lo, hi):
        return cp(x_hbm.at[0, lo:hi], x_v.at[lo:hi])

    def cp_ph(lo, hi):
        return cp(wphi_hbm.at[lo // DH:hi // DH], wphi_v.at[lo // DH:hi // DH])

    cp_wr = cp(wr_hbm, wr_v)
    seg_cp = []
    x0 = k0 = 0
    kcum = [0]
    for dx, dk in SEGS:
        kcum.append(kcum[-1] + dk)
    arng = [(0 if si == 0 else kcum[si + 1], kcum[min(si + 2, len(SEGS))]) for si in range(len(SEGS))]
    for si, (dx, dk) in enumerate(SEGS):
        ph = [cp_ph(*arng[si])] if arng[si][1] > arng[si][0] else []
        seg_cp.append([cp_xr(x0, x0 + dx)] + ph + [cp_w(D + k0, D + k0 + dk)])
        x0 += dx
        k0 += dk
    cp_wv = cp_w(2 * D, 3 * D)
    cp_x1a = cp_xr(T, T + C)
    cp_x1 = cp_xr(T + C, S)
    late = [cp_w(0, D)] + [cp(wo_hbm.at[:, j * 128:(j + 1) * 128], wo_v.at[j]) for j in range(D // 128)]
    for t, b in enumerate(B0):
        late += [cp(wg_hbm.at[:, b * 128:(b + NA) * 128], wg_v.at[t]),
                 cp(wu_hbm.at[:, b * 128:(b + NA) * 128], wu_v.at[t]),
                 cp(wd_hbm.at[b * 128:(b + NA) * 128], wd_v.at[t])]
    first = [c for t in seg_cp for c in t] + [cp_wr, cp_wv, cp_x1a, cp_x1]
    for c in first + late:
        c.start()
    osem0 = nsem[0]
    nsem[0] += NC + 1

    def cp_out(q):
        rows = pl.ds(pl.multiple_of(ord_s[q], C), C)
        return pltpu.make_async_copy(out_v.at[rows], out_hbm.at[0, rows], sems.at[osem0 + q])

    def wr_row():
        return wr_v[...].reshape(1, D).astype(f32)

    def put_cols(ref, idx, col0, r):
        for k in range(0, r.shape[0], 8):
            ref[idx, :, col0 + k // 8:col0 + k // 8 + 1] = r[k:k + 8]

    def ln1(src, dst, deps=None):
        xb = _ln(x_v[src, :].astype(f32), deps, None if deps is None else zv[...]).astype(bf16)
        xn_v[dst, :] = xb
        return xb

    def predict(rows, c, deps):
        wr = wr_row()
        wc = wr - jnp.sum(wr, axis=-1, keepdims=True) * (1.0 / D)
        t = x_v[rows, :].astype(f32) * wc
        g = C // len(deps)
        acc = t[:, 0:128] + jnp.concatenate([_zero_after(d, zv[...]) for d in deps for _ in range(g // 8)], axis=0)
        for j in range(128, D, 128):
            acc = acc + t[:, j:j + 128]
        put_cols(p_v, c, 0, jnp.sum(acc, axis=-1, keepdims=True))

    def fold(base, lo, hi):
        res = []
        for g in range(lo // 128, hi // 128):
            w = _dot_nt(_un(a_v[g]), wqkv_v[:, base + 128 * g: base + 128 * (g + 1)])
            wt_v[(base + 128 * g) // 2: (base + 128 * (g + 1)) // 2, :] = _pk((w * LOG2E).astype(bf16))
            res.append(w)
        return res

    def wt(lo, hi):
        return _un(wt_v[lo // 2:hi // 2, :])

    r_i = lax.broadcasted_iota(i32, (128, DH), 0)
    f_i = lax.broadcasted_iota(i32, (128, DH), 1)
    sel = jnp.where(f_i == (r_i % 64) // 2, 1.0, 0.0).astype(bf16)
    r_i = lax.broadcasted_iota(i32, (128, 128), 0)
    c_i = lax.broadcasted_iota(i32, (128, 128), 1)
    amask = jnp.where(c_i // 32 == 2 * (r_i // 64) + r_i % 2, jnp.uint32(0xFFFFFFFF), jnp.uint32(0))

    def build_a(lo, hi):
        a_full = _dot_nt(sel, wphi_v[lo // DH:hi // DH].reshape(hi - lo, DH))
        for g in range((hi - lo) // 128):
            blk = pltpu.bitcast(pltpu.bitcast(a_full[:, 128 * g:128 * (g + 1)], u32) & amask, f32)
            a_v[lo // 128 + g] = _pk(blk.astype(bf16))

    zv[...] = jnp.zeros((8, 128), u32)
    cp_z = cp(zv, zs)
    cp_z.start()
    hbuf[...] = jnp.zeros(hbuf.shape, f32)
    xc_v[...] = jnp.zeros(xc_v.shape, f32)
    y_v[...] = jnp.zeros(y_v.shape, f32)
    r_v[...] = jnp.full(r_v.shape, -jnp.inf, f32)
    p_v[...] = jnp.full(p_v.shape, -jnp.inf, f32)

    phis = [[] for _ in range(NP)]
    pending = []

    def phi_piece(p, t0, yp, dep=None):
        if dep is not None:
            yp = jnp.concatenate([yp[0:8] + _zero_after(dep, zv[...]), yp[8:]], axis=0)
        phi, z = _phi_k(yp)
        if phis[p]:
            z_acc[p] += z
        else:
            z_acc[p] = z
        phis[p].append((t0, phi))

    def k_block(klo, khi, t0, t1, defer=0):
        y = _dot_nt(wt(D + klo, D + khi), xn_v[t0:t1, :])
        npair = (khi - klo) // 64
        for p in range(npair):
            yp = y[64 * p:64 * (p + 1)]
            if p >= npair - defer:
                if t1 - t0 > 128:
                    phi_piece(klo // 64 + p, t0, yp[:, 0:t1 - t0 - 128])
                pending.append((klo // 64 + p, t1 - 128, yp[:, t1 - t0 - 128:]))
            else:
                phi_piece(klo // 64 + p, t0, yp)
        return y

    def flush(res):
        for k, (p, t0, yp) in enumerate(pending):
            phi_piece(p, t0, yp, res[32 * k:32 * k + 8, 0:128])
        del pending[:]

    if ONLY2:
        for c in first + [cp_z]:
            c.wait()
    else:
        x0 = k0 = 0
        for si, (dx, dk) in enumerate(SEGS):
            rows = slice(x0, x0 + dx)
            if si == 0:
                seg_cp[0][0].wait()
                ln1(rows, rows)
                seg_cp[0][1].wait()
                build_a(*arng[0])
                seg_cp[0][2].wait()
                res = fold(D, k0, k0 + dk)
            else:
                for c in seg_cp[si]:
                    c.wait()
                res = fold(D, k0, k0 + dk)
                if arng[si][1] > arng[si][0]:
                    build_a(*arng[si])
                ln1(rows, rows)
            flush(res[0])
            keep = KEEP if si == len(SEGS) - 1 else 0
            if x0:
                k_block(k0, k0 + dk, 0, x0)
            k_block(0, k0 + dk - keep, x0, x0 + dx, DEFER)
            x0 += dx
            k0 += dk
        cp_wv.wait()
        cp_x1a.wait()
        cp_wr.wait()
        cp_z.wait()
        for g in range(D // 128):
            wt_v[(2 * D + 128 * g) // 2: (2 * D + 128 * (g + 1)) // 2, :] = _pk(
                wqkv_v[:, 2 * D + 128 * g: 2 * D + 128 * (g + 1)].T)
        flush(k_block(D - KEEP, D, T - SEGS[-1][0], T))
        yv = _dot_nt(wt(2 * D, 3 * D), xn_v[0:T, :])
        ln1(slice(T, T + C), slice(T, T + C), [yv[128 * k:128 * k + 8, 128:256] for k in range(8)])
        for c in range(CPT):
            predict(slice(C * c, C * (c + 1)), c,
                    [yv[256 * c + 32 * k:256 * c + 32 * k + 8, 256:384] for k in range(8)])
        for p in range(NP):
            kv = None
            for t0, phi in phis[p]:
                d_ = _dot_nt(yv[64 * p:64 * (p + 1), t0:t0 + phi.shape[1]].astype(bf16), phi)
                kv = d_ if kv is None else kv + d_
            kv_acc[p] = kv
        cp_x1.wait()

        def phase1(i, c):
            s = pl.multiple_of(i * T, T)
            xa = xn_v[pl.ds(s, C), :]
            rest = pl.ds(pl.multiple_of(s + C, C), T - C)
            xb = ln1(rest, rest)
            y = _dot_nt(wt(D, 3 * D), jnp.concatenate([xa, xb], axis=0))
            nxt = pl.multiple_of(jnp.where(i + 1 < NT, s + T, 0), C)
            ln1(pl.ds(nxt, C), pl.ds(pl.multiple_of(s + T, C), C),
                [y[NXR + 64 * k:NXR + 64 * k + 8, 128 * NXJ:128 * NXJ + 128] for k in range(8)])
            for c in range(CPT):
                r0 = PR0 + ((2 * D - PR0) // 2) * (c % 2)
                st = ((2 * D - PR0) // 16) // 8 * 8
                predict(pl.ds(pl.multiple_of(s + C * c, C), C), CPT * i + c,
                        [y[r0 + st * k:r0 + st * k + 8, 128 * (c // 2):128 * (c // 2) + 128] for k in range(8)])
            for p in range(NP):
                phi, z = _phi_k(y[64 * p:64 * (p + 1)])
                z_acc[p] += z
                kv_acc[p] += _dot_nt(y[D + 64 * p: D + 64 * (p + 1)].astype(bf16), phi)
            return c
        lax.fori_loop(1, NT, phase1, 0)
    for c in late:
        c.wait()
    keys = []
    for c in range(NC):
        m = jnp.max(_allred8(p_v[c], jnp.maximum), axis=1, keepdims=True)
        b = pltpu.bitcast(jnp.broadcast_to(m, (8, 128)), i32)
        keys.append((b ^ (lax.shift_right_arithmetic(b, 31) & 0x7FFFFFFF))[0, 0])
    rank = [jnp.int32(0)] * NC
    for a in range(NC):
        for b in range(a + 1, NC):
            ge = (keys[a] >= keys[b]).astype(i32)
            rank[b] = rank[b] + ge
            rank[a] = rank[a] + (1 - ge)
    ord_s[0] = S
    for c in range(NC):
        ord_s[1 + (NC - 1 - rank[c] if FORCE else rank[c])] = c * C
    wq = fold(0, 0, D)
    for j in range(D // 128):
        for k in range(4):
            w = _pk(wo_v[j, 256 * k:256 * (k + 1), :])
            z = pltpu.bitcast(wq[j * 7 // 8][32 * k:32 * k + 8, 0:128], u32) & zv[...]
            wo32[j, 128 * k:128 * (k + 1), :] = (w.reshape(16, 8, 128) | z[None]).reshape(128, 128)
    r_i = lax.broadcasted_iota(i32, (64, 128), 0)
    c_i = lax.broadcasted_iota(i32, (64, 128), 1)
    kmask = r_i // 32 == c_i % 2
    for p in range(NP):
        kvt_v[p] = _pk(jnp.where(kmask, kv_acc[p], 0.0).astype(bf16))
        z_acc[p] = jnp.broadcast_to(jnp.sum(z_acc[p], axis=1, keepdims=True), (128, 128))

    def ln2(h, row0, onepass=False, deps=None):
        wr = wr_row()
        if onepass:
            m = jnp.sum(h, axis=-1, keepdims=True) * (1.0 / D)
            v = jnp.sum(h * h, axis=-1, keepdims=True) * (1.0 / D) - m * m
            rs = lax.rsqrt(jnp.maximum(v, 0.0) + EPS)
            r = (jnp.sum(h * wr, axis=-1, keepdims=True) - m * jnp.sum(wr, axis=-1, keepdims=True)) * rs
            hn = (h - m) * rs
        else:
            hn = _ln(h, deps, zv[...])
            r = jnp.sum(hn * wr, axis=-1, keepdims=True)
        hn_v[pl.ds(row0, C), :] = hn.astype(bf16)
        out_v[pl.ds(row0, C), :] = (h + hn).astype(bf16)
        return r

    def gates(nx):
        deps = [None]
        ngr = C // G
        for j in range(1, ngr):
            t = (j * NREL * 2) // ngr - 1
            r0 = (C - 8) * (t % 2)
            deps.append(nx[r0:r0 + 8, 128 * (t // 2):128 * (t // 2) + 128] if t >= 0 else None)
        return deps

    lane = lax.broadcasted_iota(i32, (8, 128), 1)
    pos = (lane * 8 + lax.broadcasted_iota(i32, (8, 128), 0)).astype(f32)

    def token_at(posv, lo, hi):
        p = jnp.clip(jnp.broadcast_to(posv, (8, 128)).astype(i32)[0, 0], lo, hi - 1)
        return ord_s[lax.shift_right_logical(p, 7)] + (p & (C - 1))

    def token_row(tok):
        base = pl.multiple_of(lax.shift_left(lax.shift_right_logical(tok, 4), 4), 16)
        hit = lax.broadcasted_iota(i32, (16, D), 0) == tok - base
        slab = jnp.where(hit, hn_v[pl.ds(base, 16), :].astype(f32), 0.0)
        return _allred8(slab[0:8] + slab[8:16], jnp.add)

    def phase2(i, c_):
        q0 = CPT * i

        @pl.when(i > 0)
        def _():
            cp_out(q0 - 1).start()

        off = [pl.multiple_of(ord_s[q0 + k], C) for k in range(CPT + 1)]
        zm = zv[...]
        hprev = hbuf[...]
        ya, ys = [], []
        for n in range(CPT):
            xt = xn_v[pl.ds(off[n + 1], C), :]
            ya.append(_dot_nt(_un(wt_v[0:D // 2, 0:D // 2]), xt[:, 0:D // 2]))
            ys.append(ya[n] + _dot_nt(_un(wt_v[0:D // 2, D // 2:D]), xt[:, D // 2:D]))
        y = jnp.concatenate(ys, axis=1)
        os_ = []
        for p in range(NP):
            phi = _phi_q(y[64 * p:64 * (p + 1)], z_acc[p])
            os_.append(_dot(_un(kvt_v[p]), phi))
        o = jnp.concatenate(os_, axis=0).astype(bf16).T
        wo = jnp.concatenate([_un(wo32[j]) for j in range(D // 128)], axis=1)
        atts = [_dot(o[C * k:C * (k + 1)], wo) for k in range(CPT)]

        def qgate(v):
            lens = [128 - W0] + [128 - W1] * 3
            t = int(v * sum(lens))
            n = 0
            while t >= lens[n]:
                t -= lens[n]
                n += 1
            r0 = 8 * (t + 128 - lens[n])
            return _zero_after(ya[n][r0:r0 + 8], zm)

        def ogate(t):
            r0, j = 8 * (t % 16), (t % 128) // 16
            return _zero_after(atts[t // 128][r0:r0 + 8, 128 * j:128 * j + 128], zm)

        t3 = jnp.maximum(i - 1, 0)
        nsb = NA // 2
        for sb in range(0 if NOG else nsb):
            c0 = 256 * sb
            xcol = xc_v[...]
            acc = None
            for k in range(0, D, 8):
                xk = jnp.concatenate([xcol[k:k + 8]] * 2, axis=1)
                p = jnp.concatenate([wg_v[t3, k:k + 8, c0:c0 + 256].astype(f32) * xk,
                                     wu_v[t3, k:k + 8, c0:c0 + 256].astype(f32) * xk], axis=1)
                if (k // 8) % SEG == 0:
                    p = p + jnp.concatenate([qgate((sb * D + k) / (nsb * D))] * 4, axis=1)
                acc = p if acc is None else acc + p
            pa_v[:, 512 * sb:512 * (sb + 1)] = acc

        put_cols(r_v, i, 0, jnp.where(i > 0, ln2(hprev, off[0], deps=gates(atts[0])), -jnp.inf))

        @pl.when(i > 0)
        def _():
            cp_out(q0).start()

        acc = _allred8(pa_v[pl.ds(pl.multiple_of(zs[3, 0].astype(i32) * 32, 32), 8), :], jnp.add)
        g_ = jnp.concatenate([acc[:, 512 * t:512 * t + 256] for t in range(nsb)], axis=1)
        u_ = jnp.concatenate([acc[:, 512 * t + 256:512 * t + 512] for t in range(nsb)], axis=1)
        a8 = g_ * jax.nn.sigmoid(g_) * u_
        a8 = jnp.concatenate([jnp.where(t3 == 2, 0.0, a8[:, 0:NDUP]), a8[:, NDUP:]], axis=1)
        ac = _col(a8)
        wd_ = D // NH
        for q in range(NH):
            ysum = jnp.where(i > 1, y_v[:, wd_ * q:wd_ * (q + 1)], 0.0)
            for k in range(0, NA * 128, 8):
                p = (wd_v[t3, k:k + 8, wd_ * q:wd_ * (q + 1)].astype(f32)
                     * jnp.concatenate([ac[k:k + 8]] * (wd_ // 128), axis=1))
                if (k // 8) % SEGD == 0:
                    t = TD0 + (q * NA * 128 + k) * (TD1 - TD0) // (NH * NA * 128)
                    p = p + jnp.concatenate([ogate(t)] * (wd_ // 128), axis=1)
                ysum = ysum + p
            y_v[:, wd_ * q:wd_ * (q + 1)] = ysum

        for k in range(CPT):
            if k == NCAND and not NOC:
                ok = (lane >= C // 8) & (lane < (NCAND + 1) * (C // 8))
                cand = token_at(_first_max(jnp.where(ok, r_v[0], -jnp.inf), pos)[1], C, (NCAND + 1) * C)
                ord_s[NC + 1] = cand
                xc_v[...] = _col(token_row(cand))
            h = x_v[pl.ds(off[k + 1], C), :].astype(f32) + atts[k]
            if k == CPT - 1:
                hbuf[...] = h
            else:
                put_cols(r_v, i, (k + 1) * (C // 8), ln2(h, off[k + 1], deps=gates(atts[k + 1])))
                if k < CPT - 2:
                    cp_out(q0 + k + 1).start()
        return c_
    lax.fori_loop(0, 0 if ONLY1 else NT, phase2, 0)
    cp_out(NC - 1).start()
    pv, pt = r_v[0], pos
    for i in range(1, NT):
        gt = r_v[i] > pv
        pv = jnp.where(gt, r_v[i], pv)
        pt = jnp.where(gt, pos + float(i * T), pt)
    pm, pi = _first_max(pv, pt)
    r = ln2(hbuf[...], pl.multiple_of(ord_s[NC], C), onepass=True)
    cp_out(NC).start()
    sub = lax.broadcasted_iota(i32, (8, 1), 0).astype(f32)
    cands = [(r[k:k + 8], sub + float(S + k)) for k in range(0, C, 8)]
    while len(cands) > 1:
        nxt = []
        for k in range(0, len(cands), 2):
            (va, ia), (vb, ib) = cands[k], cands[k + 1]
            gt = vb > va
            nxt.append((jnp.where(gt, vb, va), jnp.where(gt, ib, ia)))
        cands = nxt
    lv, lt = cands[0]
    gt = lv > pm
    bv = jnp.broadcast_to(jnp.where(gt, lv, pm), (8, 128))
    bt = jnp.broadcast_to(jnp.where(gt, lt, pi), (8, 128))
    rmax = _allred8(bv, jnp.maximum)
    idx = token_at(_allred8(jnp.where(bv == rmax, bt, float(2 * S)), jnp.minimum), C, S + C)
    y_v[...] = _allred8(y_v[...], jnp.add)

    miss = idx != ord_s[NC + 1]
    for q in range(1, NCAND + 1):
        cp_out(q).wait()

    def wait_rest():
        for q in range(NCAND + 1, NC + 1):
            cp_out(q).wait()

    @pl.when(miss)
    def _():
        x8 = token_row(idx)
        xs = jnp.concatenate([x8, x8], axis=0).astype(bf16)

        def step(j, acc):
            t, hf = lax.shift_right_logical(j, 1), j & 1
            cols = pl.ds(pl.multiple_of(hf * (NA * 64), 128), NA * 64)
            g = _dot(xs, wg_v[t, :, cols])
            a = g * jax.nn.sigmoid(g) * _dot(xs, wu_v[t, :, cols])
            a = jnp.concatenate([jnp.where(j == 4, 0.0, a[:, 0:NDUP]), a[:, NDUP:]], axis=1)
            return acc + _dot(a.astype(bf16), wd_v[t, cols, :])[0:8]

        y_v[...] = lax.fori_loop(0, 6, step, jnp.zeros((8, D), f32))
        wait_rest()
    yv = y_v[...] * jnp.concatenate([jax.nn.sigmoid(rmax)] * (D // 128), axis=1)
    base = pl.multiple_of(lax.shift_left(lax.shift_right_logical(idx, 4), 4), 16)
    hit16 = lax.broadcasted_iota(i32, (16, D), 0) == idx - base
    cur = out_v[pl.ds(base, 16), :].astype(f32)
    out_v[pl.ds(base, 16), :] = jnp.where(hit16, cur + jnp.concatenate([yv, yv], axis=0), cur).astype(bf16)
    cp_fin = cp(out_v.at[pl.ds(base, 16)], out_hbm.at[0, pl.ds(base, 16)])
    cp_fin.start()

    @pl.when(jnp.logical_not(miss))
    def _():
        wait_rest()

    cp_fin.wait()


@jax.jit
def pallas_sequential_preLN__linear_kernel_hedgehog__moe_arch_mod__prompt_kernel(
    A_x, A_wqkv, A_w_phi, A_wo, B_x, B_w_r, B_w_gate, B_w_up, B_w_down):
    del B_x
    any_spec = pl.BlockSpec(memory_space=pl.ANY)
    return pl.pallas_call(
        _kernel,
        out_shape=jax.ShapeDtypeStruct((1, S, D), bf16),
        in_specs=[any_spec] * 8,
        out_specs=any_spec,
        scratch_shapes=[
            pltpu.VMEM((S, D), bf16),
            pltpu.VMEM((D, 3 * D), bf16),
            pltpu.VMEM((H, DH, DH), bf16),
            pltpu.VMEM((D // 128, D, 128), bf16),
            pltpu.VMEM((D // 128, D // 2, 128), u32),
            pltpu.VMEM((D,), bf16),
            pltpu.VMEM((3, D, NA * 128), bf16),
            pltpu.VMEM((3, D, NA * 128), bf16),
            pltpu.VMEM((3, NA * 128, D), bf16),
            pltpu.VMEM((3 * D // 2, D), u32),
            pltpu.VMEM((8, 64, 128), u32),
            pltpu.VMEM((S + C, D), bf16),
            pltpu.VMEM((S + C, D), bf16),
            pltpu.VMEM((NP, 64, 128), f32),
            pltpu.VMEM((NP, 128, 128), f32),
            pltpu.VMEM((NP, 32, 128), u32),
            pltpu.VMEM((C, D), f32),
            pltpu.VMEM((S + C, D), bf16),
            pltpu.VMEM((8, 128), u32),
            pltpu.SMEM((8, 128), u32),
            pltpu.VMEM((NC, 8, 128), f32),
            pltpu.VMEM((NT, 8, 128), f32),
            pltpu.VMEM((D, 128), f32),
            pltpu.VMEM((8, NA * 256), f32),
            pltpu.VMEM((8, D), f32),
            pltpu.SMEM((NC + 2,), i32),
            pltpu.SemaphoreType.DMA((64,)),
        ],
        compiler_params=pltpu.CompilerParams(vmem_limit_bytes=120 * 1024 * 1024,
                                             disable_bounds_checks=True,
                                             disable_semaphore_checks=True),
        name="hedgehog_mod",
    )(A_x, A_wqkv, A_w_phi, A_wo, B_w_r, B_w_gate, B_w_up, B_w_down)
```

```python
import jax
import jax.numpy as jnp
from jax import lax
import jax.experimental.pallas as pl
import jax.experimental.pallas.tpu as pltpu

S = 2048
D = 1024
H = 32
DH = 32
F = 3584
NP = H // 2
T = 512
NT = S // T
C = 128
NC = S // C
CPT = T // C
NB = F // 128
ONLY1 = 0; ONLY2 = 0
G = 16; NREL = 6
NXR = 1536; NXJ = 2
SEGS = [tuple(128 * int(v) for v in t) for t in '22,12,14'.split(",")]
KEEP = 256; DEFER = 2
NA = 10
SEG = 8; W0 = 0; W1 = 24
TD0 = 64; TD1 = 440
B0 = (0, NA, NB - NA)
NDUP = (3 * NA - NB) * 128
NCAND = 2
PR0 = 1408; DMID = 1; EPS_ = 2
NOC = 0; NOG = 0; NOD = 0
NH = 2; SEGD = 4
EG = 32; MG = 6; ZG = 1
DIN = 1; NREL2 = 5
ESER = 0
FORCE = 0
LOG2E = 1.4426950408889634
EPS = 1e-5

f32 = jnp.float32
bf16 = jnp.bfloat16
u32 = jnp.uint32
i32 = jnp.int32


def _dot_nt(a, b):
    return lax.dot_general(a, b, (((1,), (1,)), ((), ())), preferred_element_type=f32)


def _dot(a, b):
    return jnp.dot(a, b, preferred_element_type=f32)


def _pk(x):
    return pltpu.bitcast(x, u32)


def _un(x):
    return pltpu.bitcast(x, bf16)


def _rcp(x):
    r = pl.reciprocal(x, approx=True)
    return r * (2.0 - x * r)


def _allred(v, op):
    v = op(v, pltpu.roll(v, 2, 0))
    return op(v, pltpu.roll(v, 4, 0))


def _allred8(v, op):
    return _allred(op(v, pltpu.roll(v, 1, 0)), op)


def _zero_after(dep, zm):
    return pltpu.bitcast(pltpu.bitcast(dep, u32) & zm, f32)


def _exps(x):
    L = x.shape[1]
    x3 = x.reshape(8, 8, L)
    mx = _allred(jnp.max(x3, axis=0), jnp.maximum)
    mn = _allred(jnp.min(x3, axis=0), jnp.minimum)
    ep = jnp.exp2(x3 - mx[None])
    en = jnp.exp2(mn[None] - x3)
    rp = _rcp(_allred(jnp.sum(ep, axis=0), jnp.add))
    rn = _rcp(_allred(jnp.sum(en, axis=0), jnp.add))
    return ep, en, rp, rn


def _phi_k(x):
    L = x.shape[1]
    ep, en, rp, rn = _exps(x)
    phi = jnp.concatenate([(ep * rp[None]).reshape(64, L), (en * rn[None]).reshape(64, L)], axis=0)
    z = phi[:, 0:128]
    for c in range(128, L, 128):
        z = z + phi[:, c:c + 128]
    return phi.astype(bf16), z


def _phi_q(x, zb):
    L = x.shape[1]
    ep, en, rp, rn = _exps(x)
    zb = jnp.concatenate([zb] * (L // 128), axis=1).reshape(16, 8, L)
    den = rp * jnp.sum(ep * zb[0:8], axis=0) + rn * jnp.sum(en * zb[8:16], axis=0)
    inv = _rcp(_allred(den, jnp.add) + 1e-6)
    cp = rp * inv
    cn = rn * inv
    phi = jnp.concatenate([(ep * cp[None]).reshape(64, L), (en * cn[None]).reshape(64, L)], axis=0)
    return phi.astype(bf16)


def _ln(x, deps=None, zm=None):
    if deps is None:
        tot = jnp.sum(x, axis=-1, keepdims=True)
    else:
        g = x.shape[0] // len(deps)
        gate = jnp.concatenate(
            [jnp.zeros((8, 128), f32) if d is None else _zero_after(d, zm)
             for d in deps for _ in range(g // 8)], axis=0)
        acc = x[:, 0:128] + gate
        for c in range(128, D, 128):
            acc = acc + x[:, c:c + 128]
        tot = jnp.sum(acc, axis=-1, keepdims=True)
    xc = x - tot * (1.0 / D)
    return xc * lax.rsqrt(jnp.sum(xc * xc, axis=-1, keepdims=True) * (1.0 / D) + EPS)


def _col(a8):
    return jnp.concatenate([a8] * 16, axis=0).astype(bf16).T.astype(f32)


def _first_max(v, t):
    m = jnp.max(_allred8(v, jnp.maximum), axis=1, keepdims=True)
    return m, jnp.min(_allred8(jnp.where(v == m, t, float(2 * S)), jnp.minimum), axis=1, keepdims=True)


def _kernel(x_hbm, wqkv_hbm, wphi_hbm, wo_hbm, wr_hbm, wg_hbm, wu_hbm, wd_hbm, out_hbm,
            x_v, wqkv_v, wphi_v, wo_v, wo32, wr_v, wg_v, wu_v, wd_v,
            wt_v, a_v, xn_v, hn_v, kv_acc, z_acc, kvt_v, hbuf, out_v, zv, zs, p_v, r_v,
            xc_v, pa_v, y_v, sg_v, fix_v, ord_s, sems):
    nsem = [0]

    def cp(src, dst):
        nsem[0] += 1
        return pltpu.make_async_copy(src, dst, sems.at[nsem[0] - 1])

    def cp_w(lo, hi):
        return cp(wqkv_hbm.at[:, lo:hi], wqkv_v.at[:, lo:hi])

    def cp_xr(lo, hi):
        return cp(x_hbm.at[0, lo:hi], x_v.at[lo:hi])

    def cp_ph(lo, hi):
        return cp(wphi_hbm.at[lo // DH:hi // DH], wphi_v.at[lo // DH:hi // DH])

    cp_wr = cp(wr_hbm, wr_v)
    seg_cp = []
    x0 = k0 = 0
    kcum = [0]
    for dx, dk in SEGS:
        kcum.append(kcum[-1] + dk)
    arng = [(0 if si == 0 else kcum[si + 1], kcum[min(si + 2, len(SEGS))]) for si in range(len(SEGS))]
    for si, (dx, dk) in enumerate(SEGS):
        ph = [cp_ph(*arng[si])] if arng[si][1] > arng[si][0] else []
        seg_cp.append([cp_xr(x0, x0 + dx)] + ph + [cp_w(D + k0, D + k0 + dk)])
        x0 += dx
        k0 += dk
    cp_wv = cp_w(2 * D, 3 * D)
    cp_x1a = cp_xr(T, T + C)
    cp_x1 = cp_xr(T + C, S)
    late = [cp_w(0, D)] + [cp(wo_hbm.at[:, j * 128:(j + 1) * 128], wo_v.at[j]) for j in range(D // 128)]
    for t, b in enumerate(B0):
        late += [cp(wg_hbm.at[:, b * 128:(b + NA) * 128], wg_v.at[t]),
                 cp(wu_hbm.at[:, b * 128:(b + NA) * 128], wu_v.at[t]),
                 cp(wd_hbm.at[b * 128:(b + NA) * 128], wd_v.at[t])]
    first = [c for t in seg_cp for c in t] + [cp_wr, cp_wv, cp_x1a, cp_x1]
    for c in first + late:
        c.start()
    osem0 = nsem[0]
    nsem[0] += NC + 1

    def cp_out(q):
        rows = pl.ds(pl.multiple_of(ord_s[q], C), C)
        return pltpu.make_async_copy(out_v.at[rows], out_hbm.at[0, rows], sems.at[osem0 + q])

    def wr_row():
        return wr_v[...].reshape(1, D).astype(f32)

    def put_cols(ref, idx, col0, r):
        for k in range(0, r.shape[0], 8):
            ref[idx, :, col0 + k // 8:col0 + k // 8 + 1] = r[k:k + 8]

    def ln1(src, dst, deps=None):
        xb = _ln(x_v[src, :].astype(f32), deps, None if deps is None else zv[...]).astype(bf16)
        xn_v[dst, :] = xb
        return xb

    def predict(rows, c, deps):
        wr = wr_row()
        wc = wr - jnp.sum(wr, axis=-1, keepdims=True) * (1.0 / D)
        t = x_v[rows, :].astype(f32) * wc
        g = C // len(deps)
        acc = t[:, 0:128] + jnp.concatenate([_zero_after(d, zv[...]) for d in deps for _ in range(g // 8)], axis=0)
        for j in range(128, D, 128):
            acc = acc + t[:, j:j + 128]
        put_cols(p_v, c, 0, jnp.sum(acc, axis=-1, keepdims=True))

    def fold(base, lo, hi):
        res = []
        for g in range(lo // 128, hi // 128):
            w = _dot_nt(_un(a_v[g]), wqkv_v[:, base + 128 * g: base + 128 * (g + 1)])
            wt_v[(base + 128 * g) // 2: (base + 128 * (g + 1)) // 2, :] = _pk((w * LOG2E).astype(bf16))
            res.append(w)
        return res

    def wt(lo, hi):
        return _un(wt_v[lo // 2:hi // 2, :])

    r_i = lax.broadcasted_iota(i32, (128, DH), 0)
    f_i = lax.broadcasted_iota(i32, (128, DH), 1)
    sel = jnp.where(f_i == (r_i % 64) // 2, 1.0, 0.0).astype(bf16)
    r_i = lax.broadcasted_iota(i32, (128, 128), 0)
    c_i = lax.broadcasted_iota(i32, (128, 128), 1)
    amask = jnp.where(c_i // 32 == 2 * (r_i // 64) + r_i % 2, jnp.uint32(0xFFFFFFFF), jnp.uint32(0))

    def build_a(lo, hi):
        a_full = _dot_nt(sel, wphi_v[lo // DH:hi // DH].reshape(hi - lo, DH))
        for g in range((hi - lo) // 128):
            blk = pltpu.bitcast(pltpu.bitcast(a_full[:, 128 * g:128 * (g + 1)], u32) & amask, f32)
            a_v[lo // 128 + g] = _pk(blk.astype(bf16))

    zv[...] = jnp.zeros((8, 128), u32)
    cp_z = cp(zv, zs)
    cp_z.start()
    hbuf[...] = jnp.zeros(hbuf.shape, f32)
    xc_v[...] = jnp.zeros(xc_v.shape, f32)
    y_v[...] = jnp.zeros(y_v.shape, f32)
    r_v[...] = jnp.full(r_v.shape, -jnp.inf, f32)
    p_v[...] = jnp.full(p_v.shape, -jnp.inf, f32)

    phis = [[] for _ in range(NP)]
    pending = []

    def phi_piece(p, t0, yp, dep=None):
        if dep is not None:
            yp = jnp.concatenate([yp[0:8] + _zero_after(dep, zv[...]), yp[8:]], axis=0)
        phi, z = _phi_k(yp)
        if phis[p]:
            z_acc[p] += z
        else:
            z_acc[p] = z
        phis[p].append((t0, phi))

    def k_block(klo, khi, t0, t1, defer=0):
        y = _dot_nt(wt(D + klo, D + khi), xn_v[t0:t1, :])
        npair = (khi - klo) // 64
        for p in range(npair):
            yp = y[64 * p:64 * (p + 1)]
            if p >= npair - defer:
                if t1 - t0 > 128:
                    phi_piece(klo // 64 + p, t0, yp[:, 0:t1 - t0 - 128])
                pending.append((klo // 64 + p, t1 - 128, yp[:, t1 - t0 - 128:]))
            else:
                phi_piece(klo // 64 + p, t0, yp)
        return y

    def flush(res):
        for k, (p, t0, yp) in enumerate(pending):
            phi_piece(p, t0, yp, res[32 * k:32 * k + 8, 0:128])
        del pending[:]

    if ONLY2:
        for c in first + [cp_z]:
            c.wait()
    else:
        x0 = k0 = 0
        for si, (dx, dk) in enumerate(SEGS):
            rows = slice(x0, x0 + dx)
            if si == 0:
                seg_cp[0][0].wait()
                ln1(rows, rows)
                seg_cp[0][1].wait()
                build_a(*arng[0])
                seg_cp[0][2].wait()
                res = fold(D, k0, k0 + dk)
            else:
                for c in seg_cp[si]:
                    c.wait()
                res = fold(D, k0, k0 + dk)
                if arng[si][1] > arng[si][0]:
                    build_a(*arng[si])
                ln1(rows, rows)
            flush(res[0])
            keep = KEEP if si == len(SEGS) - 1 else 0
            if x0:
                k_block(k0, k0 + dk, 0, x0)
            k_block(0, k0 + dk - keep, x0, x0 + dx, DEFER)
            x0 += dx
            k0 += dk
        cp_wv.wait()
        cp_x1a.wait()
        cp_wr.wait()
        cp_z.wait()
        for g in range(D // 128):
            wt_v[(2 * D + 128 * g) // 2: (2 * D + 128 * (g + 1)) // 2, :] = _pk(
                wqkv_v[:, 2 * D + 128 * g: 2 * D + 128 * (g + 1)].T)
        flush(k_block(D - KEEP, D, T - SEGS[-1][0], T))
        yv = _dot_nt(wt(2 * D, 3 * D), xn_v[0:T, :])
        ln1(slice(T, T + C), slice(T, T + C), [yv[128 * k:128 * k + 8, 128:256] for k in range(8)])
        for c in range(CPT):
            predict(slice(C * c, C * (c + 1)), c,
                    [yv[256 * c + 32 * k:256 * c + 32 * k + 8, 256:384] for k in range(8)])
        for p in range(NP):
            kv = None
            for t0, phi in phis[p]:
                d_ = _dot_nt(yv[64 * p:64 * (p + 1), t0:t0 + phi.shape[1]].astype(bf16), phi)
                kv = d_ if kv is None else kv + d_
            kv_acc[p] = kv
        cp_x1.wait()

        def phase1(i, c):
            s = pl.multiple_of(i * T, T)
            xa = xn_v[pl.ds(s, C), :]
            rest = pl.ds(pl.multiple_of(s + C, C), T - C)
            xb = ln1(rest, rest)
            y = _dot_nt(wt(D, 3 * D), jnp.concatenate([xa, xb], axis=0))
            nxt = pl.multiple_of(jnp.where(i + 1 < NT, s + T, 0), C)
            ln1(pl.ds(nxt, C), pl.ds(pl.multiple_of(s + T, C), C),
                [y[NXR + 64 * k:NXR + 64 * k + 8, 128 * NXJ:128 * NXJ + 128] for k in range(8)])
            for c in range(CPT):
                r0 = PR0 + ((2 * D - PR0) // 2) * (c % 2)
                st = ((2 * D - PR0) // 16) // 8 * 8
                predict(pl.ds(pl.multiple_of(s + C * c, C), C), CPT * i + c,
                        [y[r0 + st * k:r0 + st * k + 8, 128 * (c // 2):128 * (c // 2) + 128] for k in range(8)])
            for p in range(NP):
                phi, z = _phi_k(y[64 * p:64 * (p + 1)])
                z_acc[p] += z
                kv_acc[p] += _dot_nt(y[D + 64 * p: D + 64 * (p + 1)].astype(bf16), phi)
            return c
        lax.fori_loop(1, NT, phase1, 0)
    for c in late:
        c.wait()
    keys = []
    for c in range(NC):
        m = jnp.max(_allred8(p_v[c], jnp.maximum), axis=1, keepdims=True)
        b = pltpu.bitcast(jnp.broadcast_to(m, (8, 128)), i32)
        keys.append((b ^ (lax.shift_right_arithmetic(b, 31) & 0x7FFFFFFF))[0, 0])
    rank = [jnp.int32(0)] * NC
    for a in range(NC):
        for b in range(a + 1, NC):
            ge = (keys[a] >= keys[b]).astype(i32)
            rank[b] = rank[b] + ge
            rank[a] = rank[a] + (1 - ge)
    ord_s[0] = S
    for c in range(NC):
        ord_s[1 + (NC - 1 - rank[c] if FORCE else rank[c])] = c * C
    wq = fold(0, 0, D)
    for j in range(D // 128):
        for k in range(4):
            w = _pk(wo_v[j, 256 * k:256 * (k + 1), :])
            z = pltpu.bitcast(wq[j * 7 // 8][32 * k:32 * k + 8, 0:128], u32) & zv[...]
            wo32[j, 128 * k:128 * (k + 1), :] = (w.reshape(16, 8, 128) | z[None]).reshape(128, 128)
    r_i = lax.broadcasted_iota(i32, (64, 128), 0)
    c_i = lax.broadcasted_iota(i32, (64, 128), 1)
    kmask = r_i // 32 == c_i % 2
    for p in range(NP):
        gz = _zero_after(wq[p * MG // NP][64 * (p % 2):64 * (p % 2) + 8, 512:640], zv[...])
        kvt_v[p] = _pk(jnp.where(kmask, kv_acc[p], jnp.concatenate([gz] * 8, axis=0)).astype(bf16))
        zp = z_acc[p] + jnp.concatenate([gz] * 16, axis=0) if ZG else z_acc[p]
        z_acc[p] = jnp.broadcast_to(jnp.sum(zp, axis=1, keepdims=True), (128, 128))

    def ln2(h, row0, deps):
        hn = _ln(h, deps, zv[...])
        r = jnp.sum(hn * wr_row(), axis=-1, keepdims=True)
        hn_v[pl.ds(row0, C), :] = hn.astype(bf16)
        out_v[pl.ds(row0, C), :] = (h + hn).astype(bf16)
        return r

    def gates(nx, nrel=NREL):
        deps = [None]
        ngr = C // G
        for j in range(1, ngr):
            t = (j * nrel * 2) // ngr - 1
            r0 = (C - 8) * (t % 2)
            deps.append(nx[r0:r0 + 8, 128 * (t // 2):128 * (t // 2) + 128] if t >= 0 else None)
        return deps

    lane = lax.broadcasted_iota(i32, (8, 128), 1)
    pos = (lane * 8 + lax.broadcasted_iota(i32, (8, 128), 0)).astype(f32)

    def token_at(posv, lo, hi):
        p = jnp.clip(jnp.broadcast_to(posv, (8, 128)).astype(i32)[0, 0], lo, hi - 1)
        return ord_s[lax.shift_right_logical(p, 7)] + (p & (C - 1))

    def token_row(tok):
        base = pl.multiple_of(lax.shift_left(lax.shift_right_logical(tok, 4), 4), 16)
        hit = lax.broadcasted_iota(i32, (16, D), 0) == tok - base
        slab = jnp.where(hit, hn_v[pl.ds(base, 16), :].astype(f32), 0.0)
        return _allred8(slab[0:8] + slab[8:16], jnp.add)

    def phase2(i, c_):
        q0 = CPT * i

        if not DIN:
            @pl.when(i > 0)
            def _():
                cp_out(q0 - 1).start()

        off = [pl.multiple_of(ord_s[q0 + k], C) for k in range(CPT + 1)]
        zm = zv[...]
        hprev = hbuf[...]
        ya, ys = [], []
        for n in range(CPT):
            xt = xn_v[pl.ds(off[n + 1], C), :]
            ya.append(_dot_nt(_un(wt_v[0:D // 2, 0:D // 2]), xt[:, 0:D // 2]))
            ys.append(ya[n] + _dot_nt(_un(wt_v[0:D // 2, D // 2:D]), xt[:, D // 2:D]))
        y = jnp.concatenate(ys, axis=1)
        os_ = []
        for p in range(NP):
            phi = _phi_q(y[64 * p:64 * (p + 1)], z_acc[p])
            os_.append(_dot(_un(kvt_v[p]), phi))
        o = jnp.concatenate(os_, axis=0).astype(bf16).T
        wo = jnp.concatenate([_un(wo32[j]) for j in range(D // 128)], axis=1)
        atts = [_dot(o[C * k:C * (k + 1)], wo) for k in range(CPT)]

        def qgate(v):
            lens = [128 - W0] + [128 - W1] * 3
            t = int(v * sum(lens))
            n = 0
            while t >= lens[n]:
                t -= lens[n]
                n += 1
            r0 = 8 * (t + 128 - lens[n])
            return _zero_after(ya[n][r0:r0 + 8], zm)

        def ogate(t):
            r0, j = 8 * (t % 16), (t % 128) // 16
            return _zero_after(atts[t // 128][r0:r0 + 8, 128 * j:128 * j + 128], zm)

        t3 = jnp.maximum(i - 1, 0)
        nsb = NA // 2
        for sb in range(0 if NOG else nsb):
            c0 = 256 * sb
            xcol = xc_v[...]
            acc = None
            for k in range(0, D, 8):
                xk = jnp.concatenate([xcol[k:k + 8]] * 2, axis=1)
                p = jnp.concatenate([wg_v[t3, k:k + 8, c0:c0 + 256].astype(f32) * xk,
                                     wu_v[t3, k:k + 8, c0:c0 + 256].astype(f32) * xk], axis=1)
                if (k // 8) % SEG == 0:
                    p = p + jnp.concatenate([qgate((sb * D + k) / (nsb * D))] * 4, axis=1)
                acc = p if acc is None else acc + p
            pa_v[:, 512 * sb:512 * (sb + 1)] = acc

        put_cols(r_v, i, 0, jnp.where(i > 0, ln2(hprev, off[0], deps=gates(atts[0])), -jnp.inf))

        @pl.when(i > 0)
        def _():
            cp_out(q0).start()

        acc = _allred8(pa_v[pl.ds(pl.multiple_of(zs[3, 0].astype(i32) * 32, 32), 8), :], jnp.add)
        g_ = jnp.concatenate([acc[:, 512 * t:512 * t + 256] for t in range(nsb)], axis=1)
        u_ = jnp.concatenate([acc[:, 512 * t + 256:512 * t + 512] for t in range(nsb)], axis=1)
        a8 = g_ * jax.nn.sigmoid(g_) * u_
        a8 = jnp.concatenate([jnp.where(t3 == 2, 0.0, a8[:, 0:NDUP]), a8[:, NDUP:]], axis=1)
        ac = _col(a8)
        wd_ = D // NH
        for q in range(NH):
            ysum = jnp.where(i > 1, y_v[:, wd_ * q:wd_ * (q + 1)], 0.0)
            for k in range(0, NA * 128, 8):
                p = (wd_v[t3, k:k + 8, wd_ * q:wd_ * (q + 1)].astype(f32)
                     * jnp.concatenate([ac[k:k + 8]] * (wd_ // 128), axis=1))
                if (k // 8) % SEGD == 0:
                    t = TD0 + (q * NA * 128 + k) * (TD1 - TD0) // (NH * NA * 128)
                    p = p + jnp.concatenate([ogate(t)] * (wd_ // 128), axis=1)
                ysum = ysum + p
            y_v[:, wd_ * q:wd_ * (q + 1)] = ysum

        for k in range(CPT):
            if k == NCAND and not NOC:
                ok = (lane >= C // 8) & (lane < (NCAND + 1) * (C // 8))
                cm, cpos = _first_max(jnp.where(ok, r_v[0], -jnp.inf), pos)
                cand = token_at(cpos, C, (NCAND + 1) * C)
                ord_s[NC + 1] = cand
                sg_v[...] = jax.nn.sigmoid(jnp.broadcast_to(cm, (8, 128)))
                xc_v[...] = _col(token_row(cand))
            h = x_v[pl.ds(off[k + 1], C), :].astype(f32) + atts[k]
            if k == CPT - 1:
                hbuf[...] = h
            else:
                put_cols(r_v, i, (k + 1) * (C // 8),
                         ln2(h, off[k + 1], deps=gates(atts[k + 1], NREL2 if k == CPT - 2 else NREL)))
                if k < CPT - 2 or DIN:
                    cp_out(q0 + k + 1).start()
        return c_
    lax.fori_loop(0, 0 if ONLY1 else NT, phase2, 0)
    if not DIN:
        cp_out(NC - 1).start()
    for q in range(1, NCAND + 1):
        cp_out(q).wait()
    fsem = nsem[0]
    nsem[0] += 1

    def slab_of(tok):
        return pl.multiple_of(lax.shift_left(lax.shift_right_logical(tok, 4), 4), 16)

    def patch(tok, y8, sg):
        base = slab_of(tok)
        yv = y8 * jnp.concatenate([sg] * (D // 128), axis=1)
        cur = out_v[pl.ds(base, 16), :].astype(f32)
        hit = lax.broadcasted_iota(i32, (16, D), 0) == tok - base
        fix_v[...] = jnp.where(hit, cur + jnp.concatenate([yv, yv], axis=0), cur).astype(bf16)
        return pltpu.make_async_copy(fix_v, out_hbm.at[0, pl.ds(base, 16)], sems.at[fsem])

    cand = ord_s[NC + 1]
    cp_fix = patch(cand, _allred8(y_v[...], jnp.add), sg_v[...])
    cp_fix.start()
    last = pl.multiple_of(ord_s[NC], C)
    sub = lax.broadcasted_iota(i32, (8, 1), 0).astype(f32)
    stats, cp_l = [], []
    gate = None
    for g in range(0, C, EG):
        h = hbuf[g:g + EG, :]
        s1, s2 = h[:, 0:128], None
        if gate is not None:
            s1 = s1 + jnp.concatenate([gate] * (EG // 8), axis=0)
        s2 = s1 * s1
        for j in range(128, D, 128):
            s1 = s1 + h[:, j:j + 128]
            s2 = s2 + h[:, j:j + 128] * h[:, j:j + 128]
        if ESER:
            gate = _zero_after(s2[EG - 8:EG], zv[...])
        m = jnp.sum(s1, axis=-1, keepdims=True) * (1.0 / D)
        v = jnp.sum(s2, axis=-1, keepdims=True) * (1.0 / D) - m * m
        rs = lax.rsqrt(jnp.maximum(v, 0.0) + EPS)
        stats.append((m, rs))
        rows = pl.ds(pl.multiple_of(last + g, EG), EG)
        out_v[rows, :] = (h * (1.0 + rs) - m * rs).astype(bf16)
        cp_l.append(cp(out_v.at[rows], out_hbm.at[0, rows]))
        cp_l[-1].start()
    for q in range(NCAND + 1, NC - 1):
        cp_out(q).wait()
    pv, pt = r_v[0], pos
    for i in range(1, NT):
        gt = r_v[i] > pv
        pv = jnp.where(gt, r_v[i], pv)
        pt = jnp.where(gt, pos + float(i * T), pt)
    pm, pi = _first_max(pv, pt)
    wr = wr_row()
    wsum = jnp.sum(wr, axis=-1, keepdims=True)
    cands = []
    for g, (m, rs) in zip(range(0, C, EG), stats):
        r = (jnp.sum(hbuf[g:g + EG, :] * wr, axis=-1, keepdims=True) - m * wsum) * rs
        cands += [(r[k:k + 8], sub + float(S + g + k)) for k in range(0, EG, 8)]
    while len(cands) > 1:
        nxt = []
        for k in range(0, len(cands), 2):
            (va, ia), (vb, ib) = cands[k], cands[k + 1]
            gt = vb > va
            nxt.append((jnp.where(gt, vb, va), jnp.where(gt, ib, ia)))
        cands = nxt
    lv, lt = cands[0]
    gt = lv > pm
    bv = jnp.broadcast_to(jnp.where(gt, lv, pm), (8, 128))
    bt = jnp.broadcast_to(jnp.where(gt, lt, pi), (8, 128))
    rmax = _allred8(bv, jnp.maximum)
    idx = token_at(_allred8(jnp.where(bv == rmax, bt, float(2 * S)), jnp.minimum), C, S + C)
    cp_out(NC - 1).wait()
    cp_fix.wait()
    for c in cp_l:
        c.wait()

    @pl.when(idx != cand)
    def _():
        rows = pl.ds(slab_of(cand), 16)
        undo = pltpu.make_async_copy(out_v.at[rows], out_hbm.at[0, rows], sems.at[fsem])
        undo.start()
        hn_v[pl.ds(last, C), :] = _ln(hbuf[...]).astype(bf16)
        x8 = token_row(idx)
        xs = jnp.concatenate([x8, x8], axis=0).astype(bf16)

        def step(j, acc):
            t, hf = lax.shift_right_logical(j, 1), j & 1
            cols = pl.ds(pl.multiple_of(hf * (NA * 64), 128), NA * 64)
            g = _dot(xs, wg_v[t, :, cols])
            a = g * jax.nn.sigmoid(g) * _dot(xs, wu_v[t, :, cols])
            a = jnp.concatenate([jnp.where(j == 4, 0.0, a[:, 0:NDUP]), a[:, NDUP:]], axis=1)
            return acc + _dot(a.astype(bf16), wd_v[t, cols, :])[0:8]

        y8 = lax.fori_loop(0, 6, step, jnp.zeros((8, D), f32))
        undo.wait()
        redo = patch(idx, y8, jax.nn.sigmoid(rmax))
        redo.start()
        redo.wait()


@jax.jit
def pallas_sequential_preLN__linear_kernel_hedgehog__moe_arch_mod__prompt_kernel(
    A_x, A_wqkv, A_w_phi, A_wo, B_x, B_w_r, B_w_gate, B_w_up, B_w_down):
    del B_x
    any_spec = pl.BlockSpec(memory_space=pl.ANY)
    return pl.pallas_call(
        _kernel,
        out_shape=jax.ShapeDtypeStruct((1, S, D), bf16),
        in_specs=[any_spec] * 8,
        out_specs=any_spec,
        scratch_shapes=[
            pltpu.VMEM((S, D), bf16),
            pltpu.VMEM((D, 3 * D), bf16),
            pltpu.VMEM((H, DH, DH), bf16),
            pltpu.VMEM((D // 128, D, 128), bf16),
            pltpu.VMEM((D // 128, D // 2, 128), u32),
            pltpu.VMEM((D,), bf16),
            pltpu.VMEM((3, D, NA * 128), bf16),
            pltpu.VMEM((3, D, NA * 128), bf16),
            pltpu.VMEM((3, NA * 128, D), bf16),
            pltpu.VMEM((3 * D // 2, D), u32),
            pltpu.VMEM((8, 64, 128), u32),
            pltpu.VMEM((S + C, D), bf16),
            pltpu.VMEM((S + C, D), bf16),
            pltpu.VMEM((NP, 64, 128), f32),
            pltpu.VMEM((NP, 128, 128), f32),
            pltpu.VMEM((NP, 32, 128), u32),
            pltpu.VMEM((C, D), f32),
            pltpu.VMEM((S + C, D), bf16),
            pltpu.VMEM((8, 128), u32),
            pltpu.SMEM((8, 128), u32),
            pltpu.VMEM((NC, 8, 128), f32),
            pltpu.VMEM((NT, 8, 128), f32),
            pltpu.VMEM((D, 128), f32),
            pltpu.VMEM((8, NA * 256), f32),
            pltpu.VMEM((8, D), f32),
            pltpu.VMEM((8, 128), f32),
            pltpu.VMEM((16, D), bf16),
            pltpu.SMEM((NC + 2,), i32),
            pltpu.SemaphoreType.DMA((64,)),
        ],
        compiler_params=pltpu.CompilerParams(vmem_limit_bytes=120 * 1024 * 1024,
                                             disable_bounds_checks=True,
                                             disable_semaphore_checks=True),
        name="hedgehog_mod",
    )(A_x, A_wqkv, A_w_phi, A_wo, B_w_r, B_w_gate, B_w_up, B_w_down)
```

```python
import jax
import jax.numpy as jnp
from jax import lax
import jax.experimental.pallas as pl
import jax.experimental.pallas.tpu as pltpu

S = 2048
D = 1024
H = 32
DH = 32
F = 3584
NP = H // 2
T = 512
NT = S // T
C = 128
NC = S // C
CPT = T // C
NB = F // 128
ONLY1 = 0; ONLY2 = 0
G = 16; NREL = 6
NXR = 1536; NXJ = 2
SEGS = [tuple(128 * int(v) for v in t) for t in '22,12,14'.split(",")]
KEEP = 256; DEFER = 2
NA = 10
SEG = 8; W0 = 0; W1 = 24
TD0 = 64; TD1 = 440
B0 = (0, NA, NB - NA)
NDUP = (3 * NA - NB) * 128
NCAND = 2
PR0 = 1408; DMID = 1; EPS_ = 2
NOC = 0; NOG = 0; NOD = 0
NH = 2; SEGD = 4
EG = 32; MG = 6; ZG = 1
DIN = 1; NREL2 = 5
ESER = 0
ZL = 4; ZP1 = 1
FORCE = 0
LOG2E = 1.4426950408889634
EPS = 1e-5

f32 = jnp.float32
bf16 = jnp.bfloat16
u32 = jnp.uint32
i32 = jnp.int32


def _dot_nt(a, b):
    return lax.dot_general(a, b, (((1,), (1,)), ((), ())), preferred_element_type=f32)


def _dot(a, b):
    return jnp.dot(a, b, preferred_element_type=f32)


def _pk(x):
    return pltpu.bitcast(x, u32)


def _un(x):
    return pltpu.bitcast(x, bf16)


def _rcp(x):
    r = pl.reciprocal(x, approx=True)
    return r * (2.0 - x * r)


def _allred(v, op):
    v = op(v, pltpu.roll(v, 2, 0))
    return op(v, pltpu.roll(v, 4, 0))


def _allred8(v, op):
    return _allred(op(v, pltpu.roll(v, 1, 0)), op)


def _zero_after(dep, zm):
    return pltpu.bitcast(pltpu.bitcast(dep, u32) & zm, f32)


def _exps(x):
    L = x.shape[1]
    x3 = x.reshape(8, 8, L)
    mx = _allred(jnp.max(x3, axis=0), jnp.maximum)
    mn = _allred(jnp.min(x3, axis=0), jnp.minimum)
    ep = jnp.exp2(x3 - mx[None])
    en = jnp.exp2(mn[None] - x3)
    rp = _rcp(_allred(jnp.sum(ep, axis=0), jnp.add))
    rn = _rcp(_allred(jnp.sum(en, axis=0), jnp.add))
    return ep, en, rp, rn


def _phi_k(x):
    L = x.shape[1]
    ep, en, rp, rn = _exps(x)
    return jnp.concatenate([(ep * rp[None]).reshape(64, L), (en * rn[None]).reshape(64, L)], axis=0)


def _lane_blocks_sum(phi, z):
    for c in range(0, phi.shape[1], 128):
        z = phi[:, c:c + 128] if z is None else z + phi[:, c:c + 128]
    return z


def _phi_q(x, zb):
    L = x.shape[1]
    ep, en, rp, rn = _exps(x)
    zb = jnp.concatenate([zb] * (L // 128), axis=1).reshape(16, 8, L)
    den = rp * jnp.sum(ep * zb[0:8], axis=0) + rn * jnp.sum(en * zb[8:16], axis=0)
    inv = _rcp(_allred(den, jnp.add) + 1e-6)
    cp = rp * inv
    cn = rn * inv
    phi = jnp.concatenate([(ep * cp[None]).reshape(64, L), (en * cn[None]).reshape(64, L)], axis=0)
    return phi.astype(bf16)


def _ln(x, deps=None, zm=None):
    if deps is None:
        tot = jnp.sum(x, axis=-1, keepdims=True)
    else:
        g = x.shape[0] // len(deps)
        gate = jnp.concatenate(
            [jnp.zeros((8, 128), f32) if d is None else _zero_after(d, zm)
             for d in deps for _ in range(g // 8)], axis=0)
        acc = x[:, 0:128] + gate
        for c in range(128, D, 128):
            acc = acc + x[:, c:c + 128]
        tot = jnp.sum(acc, axis=-1, keepdims=True)
    xc = x - tot * (1.0 / D)
    return xc * lax.rsqrt(jnp.sum(xc * xc, axis=-1, keepdims=True) * (1.0 / D) + EPS)


def _col(a8):
    return jnp.concatenate([a8] * 16, axis=0).astype(bf16).T.astype(f32)


def _first_max(v, t):
    m = jnp.max(_allred8(v, jnp.maximum), axis=1, keepdims=True)
    return m, jnp.min(_allred8(jnp.where(v == m, t, float(2 * S)), jnp.minimum), axis=1, keepdims=True)


def _kernel(x_hbm, wqkv_hbm, wphi_hbm, wo_hbm, wr_hbm, wg_hbm, wu_hbm, wd_hbm, out_hbm,
            x_v, wqkv_v, wphi_v, wo_v, wo32, wr_v, wg_v, wu_v, wd_v,
            wt_v, a_v, xn_v, hn_v, kv_acc, z_acc, kvt_v, hbuf, out_v, zv, zs, p_v, r_v,
            xc_v, pa_v, y_v, sg_v, fix_v, ord_s, sems):
    nsem = [0]

    def cp(src, dst):
        nsem[0] += 1
        return pltpu.make_async_copy(src, dst, sems.at[nsem[0] - 1])

    def cp_w(lo, hi):
        return cp(wqkv_hbm.at[:, lo:hi], wqkv_v.at[:, lo:hi])

    def cp_xr(lo, hi):
        return cp(x_hbm.at[0, lo:hi], x_v.at[lo:hi])

    def cp_ph(lo, hi):
        return cp(wphi_hbm.at[lo // DH:hi // DH], wphi_v.at[lo // DH:hi // DH])

    cp_wr = cp(wr_hbm, wr_v)
    seg_cp = []
    x0 = k0 = 0
    kcum = [0]
    for dx, dk in SEGS:
        kcum.append(kcum[-1] + dk)
    arng = [(0 if si == 0 else kcum[si + 1], kcum[min(si + 2, len(SEGS))]) for si in range(len(SEGS))]
    for si, (dx, dk) in enumerate(SEGS):
        ph = [cp_ph(*arng[si])] if arng[si][1] > arng[si][0] else []
        seg_cp.append([cp_xr(x0, x0 + dx)] + ph + [cp_w(D + k0, D + k0 + dk)])
        x0 += dx
        k0 += dk
    cp_wv = cp_w(2 * D, 3 * D)
    cp_x1a = cp_xr(T, T + C)
    cp_x1 = cp_xr(T + C, S)
    late = [cp_w(0, D)] + [cp(wo_hbm.at[:, j * 128:(j + 1) * 128], wo_v.at[j]) for j in range(D // 128)]
    for t, b in enumerate(B0):
        late += [cp(wg_hbm.at[:, b * 128:(b + NA) * 128], wg_v.at[t]),
                 cp(wu_hbm.at[:, b * 128:(b + NA) * 128], wu_v.at[t]),
                 cp(wd_hbm.at[b * 128:(b + NA) * 128], wd_v.at[t])]
    first = [c for t in seg_cp for c in t] + [cp_wr, cp_wv, cp_x1a, cp_x1]
    for c in first + late:
        c.start()
    osem0 = nsem[0]
    nsem[0] += NC + 1

    def cp_out(q):
        rows = pl.ds(pl.multiple_of(ord_s[q], C), C)
        return pltpu.make_async_copy(out_v.at[rows], out_hbm.at[0, rows], sems.at[osem0 + q])

    def wr_row():
        return wr_v[...].reshape(1, D).astype(f32)

    def put_cols(ref, idx, col0, r):
        for k in range(0, r.shape[0], 8):
            ref[idx, :, col0 + k // 8:col0 + k // 8 + 1] = r[k:k + 8]

    def ln1(src, dst, deps=None):
        xb = _ln(x_v[src, :].astype(f32), deps, None if deps is None else zv[...]).astype(bf16)
        xn_v[dst, :] = xb
        return xb

    def predict(rows, c, deps):
        wr = wr_row()
        wc = wr - jnp.sum(wr, axis=-1, keepdims=True) * (1.0 / D)
        t = x_v[rows, :].astype(f32) * wc
        g = C // len(deps)
        acc = t[:, 0:128] + jnp.concatenate([_zero_after(d, zv[...]) for d in deps for _ in range(g // 8)], axis=0)
        for j in range(128, D, 128):
            acc = acc + t[:, j:j + 128]
        put_cols(p_v, c, 0, jnp.sum(acc, axis=-1, keepdims=True))

    def fold(base, lo, hi):
        res = []
        for g in range(lo // 128, hi // 128):
            w = _dot_nt(_un(a_v[g]), wqkv_v[:, base + 128 * g: base + 128 * (g + 1)])
            wt_v[(base + 128 * g) // 2: (base + 128 * (g + 1)) // 2, :] = _pk((w * LOG2E).astype(bf16))
            res.append(w)
        return res

    def wt(lo, hi):
        return _un(wt_v[lo // 2:hi // 2, :])

    r_i = lax.broadcasted_iota(i32, (128, DH), 0)
    f_i = lax.broadcasted_iota(i32, (128, DH), 1)
    sel = jnp.where(f_i == (r_i % 64) // 2, 1.0, 0.0).astype(bf16)
    r_i = lax.broadcasted_iota(i32, (128, 128), 0)
    c_i = lax.broadcasted_iota(i32, (128, 128), 1)
    amask = jnp.where(c_i // 32 == 2 * (r_i // 64) + r_i % 2, jnp.uint32(0xFFFFFFFF), jnp.uint32(0))

    def build_a(lo, hi):
        a_full = _dot_nt(sel, wphi_v[lo // DH:hi // DH].reshape(hi - lo, DH))
        for g in range((hi - lo) // 128):
            blk = pltpu.bitcast(pltpu.bitcast(a_full[:, 128 * g:128 * (g + 1)], u32) & amask, f32)
            a_v[lo // 128 + g] = _pk(blk.astype(bf16))

    zv[...] = jnp.zeros((8, 128), u32)
    cp_z = cp(zv, zs)
    cp_z.start()
    hbuf[...] = jnp.zeros(hbuf.shape, f32)
    xc_v[...] = jnp.zeros(xc_v.shape, f32)
    y_v[...] = jnp.zeros(y_v.shape, f32)
    r_v[...] = jnp.full(r_v.shape, -jnp.inf, f32)
    p_v[...] = jnp.full(p_v.shape, -jnp.inf, f32)

    phis = [[] for _ in range(NP)]
    pending = []

    def phi_piece(p, t0, yp, dep=None):
        if dep is not None:
            yp = jnp.concatenate([yp[0:8] + _zero_after(dep, zv[...]), yp[8:]], axis=0)
        phis[p].append((t0, _phi_k(yp)))

    def k_block(klo, khi, t0, t1, defer=0):
        y = _dot_nt(wt(D + klo, D + khi), xn_v[t0:t1, :])
        npair = (khi - klo) // 64
        for p in range(npair):
            yp = y[64 * p:64 * (p + 1)]
            if p >= npair - defer:
                if t1 - t0 > 128:
                    phi_piece(klo // 64 + p, t0, yp[:, 0:t1 - t0 - 128])
                pending.append((klo // 64 + p, t1 - 128, yp[:, t1 - t0 - 128:]))
            else:
                phi_piece(klo // 64 + p, t0, yp)
        return y

    def flush(res):
        for k, (p, t0, yp) in enumerate(pending):
            phi_piece(p, t0, yp, res[32 * k:32 * k + 8, 0:128])
        del pending[:]

    if ONLY2:
        for c in first + [cp_z]:
            c.wait()
    else:
        x0 = k0 = 0
        for si, (dx, dk) in enumerate(SEGS):
            rows = slice(x0, x0 + dx)
            if si == 0:
                seg_cp[0][0].wait()
                ln1(rows, rows)
                seg_cp[0][1].wait()
                build_a(*arng[0])
                seg_cp[0][2].wait()
                res = fold(D, k0, k0 + dk)
            else:
                for c in seg_cp[si]:
                    c.wait()
                res = fold(D, k0, k0 + dk)
                if arng[si][1] > arng[si][0]:
                    build_a(*arng[si])
                ln1(rows, rows)
            flush(res[0])
            keep = KEEP if si == len(SEGS) - 1 else 0
            if x0:
                k_block(k0, k0 + dk, 0, x0)
            k_block(0, k0 + dk - keep, x0, x0 + dx, DEFER)
            x0 += dx
            k0 += dk
        cp_wv.wait()
        cp_x1a.wait()
        cp_wr.wait()
        cp_z.wait()
        for g in range(D // 128):
            wt_v[(2 * D + 128 * g) // 2: (2 * D + 128 * (g + 1)) // 2, :] = _pk(
                wqkv_v[:, 2 * D + 128 * g: 2 * D + 128 * (g + 1)].T)
        flush(k_block(D - KEEP, D, T - SEGS[-1][0], T))
        yv = _dot_nt(wt(2 * D, 3 * D), xn_v[0:T, :])
        ln1(slice(T, T + C), slice(T, T + C), [yv[128 * k:128 * k + 8, 128:256] for k in range(8)])
        for c in range(CPT):
            predict(slice(C * c, C * (c + 1)), c,
                    [yv[256 * c + 32 * k:256 * c + 32 * k + 8, 256:384] for k in range(8)])
        kvs = []
        for p in range(NP):
            phi = jnp.concatenate([ph for _, ph in sorted(phis[p], key=lambda tp: tp[0])], axis=1)
            kvs.append(_dot_nt(yv[64 * p:64 * (p + 1)].astype(bf16), phi.astype(bf16)))
            kv_acc[p] = kvs[p]
            dep = kvs[p - ZL][0:8] if p >= ZL else yv[D - 64 * (ZL - p):D - 64 * (ZL - p) + 8, T - 128:T]
            z_acc[p] = _lane_blocks_sum(phi, jnp.concatenate([_zero_after(dep, zv[...])] * 16, axis=0))
        cp_x1.wait()

        def phase1(i, c):
            s = pl.multiple_of(i * T, T)
            xa = xn_v[pl.ds(s, C), :]
            rest = pl.ds(pl.multiple_of(s + C, C), T - C)
            xb = ln1(rest, rest)
            y = _dot_nt(wt(D, 3 * D), jnp.concatenate([xa, xb], axis=0))
            nxt = pl.multiple_of(jnp.where(i + 1 < NT, s + T, 0), C)
            ln1(pl.ds(nxt, C), pl.ds(pl.multiple_of(s + T, C), C),
                [y[NXR + 64 * k:NXR + 64 * k + 8, 128 * NXJ:128 * NXJ + 128] for k in range(8)])
            for c in range(CPT):
                r0 = PR0 + ((2 * D - PR0) // 2) * (c % 2)
                st = ((2 * D - PR0) // 16) // 8 * 8
                predict(pl.ds(pl.multiple_of(s + C * c, C), C), CPT * i + c,
                        [y[r0 + st * k:r0 + st * k + 8, 128 * (c // 2):128 * (c // 2) + 128] for k in range(8)])
            kvs = []
            for p in range(NP):
                phi = _phi_k(y[64 * p:64 * (p + 1)])
                kvs.append(_dot_nt(y[D + 64 * p: D + 64 * (p + 1)].astype(bf16), phi.astype(bf16)))
                kv_acc[p] += kvs[p]
                if ZP1:
                    dep = kvs[p - ZL][0:8] if p >= ZL else y[2 * D - 64 * (ZL - p):2 * D - 64 * (ZL - p) + 8, T - 128:T]
                    z0 = z_acc[p] + jnp.concatenate([_zero_after(dep, zv[...])] * 16, axis=0)
                    z_acc[p] = _lane_blocks_sum(phi, z0)
                else:
                    z_acc[p] += _lane_blocks_sum(phi, None)
            return c
        lax.fori_loop(1, NT, phase1, 0)
    for c in late:
        c.wait()
    keys = []
    for c in range(NC):
        m = jnp.max(_allred8(p_v[c], jnp.maximum), axis=1, keepdims=True)
        b = pltpu.bitcast(jnp.broadcast_to(m, (8, 128)), i32)
        keys.append((b ^ (lax.shift_right_arithmetic(b, 31) & 0x7FFFFFFF))[0, 0])
    rank = [jnp.int32(0)] * NC
    for a in range(NC):
        for b in range(a + 1, NC):
            ge = (keys[a] >= keys[b]).astype(i32)
            rank[b] = rank[b] + ge
            rank[a] = rank[a] + (1 - ge)
    ord_s[0] = S
    for c in range(NC):
        ord_s[1 + (NC - 1 - rank[c] if FORCE else rank[c])] = c * C
    wq = fold(0, 0, D)
    for j in range(D // 128):
        for k in range(4):
            w = _pk(wo_v[j, 256 * k:256 * (k + 1), :])
            z = pltpu.bitcast(wq[j * 7 // 8][32 * k:32 * k + 8, 0:128], u32) & zv[...]
            wo32[j, 128 * k:128 * (k + 1), :] = (w.reshape(16, 8, 128) | z[None]).reshape(128, 128)
    r_i = lax.broadcasted_iota(i32, (64, 128), 0)
    c_i = lax.broadcasted_iota(i32, (64, 128), 1)
    kmask = r_i // 32 == c_i % 2
    for p in range(NP):
        gz = _zero_after(wq[p * MG // NP][64 * (p % 2):64 * (p % 2) + 8, 512:640], zv[...])
        kvt_v[p] = _pk(jnp.where(kmask, kv_acc[p], jnp.concatenate([gz] * 8, axis=0)).astype(bf16))
        zp = z_acc[p] + jnp.concatenate([gz] * 16, axis=0) if ZG else z_acc[p]
        z_acc[p] = jnp.broadcast_to(jnp.sum(zp, axis=1, keepdims=True), (128, 128))

    def ln2(h, row0, deps):
        hn = _ln(h, deps, zv[...])
        r = jnp.sum(hn * wr_row(), axis=-1, keepdims=True)
        hn_v[pl.ds(row0, C), :] = hn.astype(bf16)
        out_v[pl.ds(row0, C), :] = (h + hn).astype(bf16)
        return r

    def gates(nx, nrel=NREL):
        deps = [None]
        ngr = C // G
        for j in range(1, ngr):
            t = (j * nrel * 2) // ngr - 1
            r0 = (C - 8) * (t % 2)
            deps.append(nx[r0:r0 + 8, 128 * (t // 2):128 * (t // 2) + 128] if t >= 0 else None)
        return deps

    lane = lax.broadcasted_iota(i32, (8, 128), 1)
    pos = (lane * 8 + lax.broadcasted_iota(i32, (8, 128), 0)).astype(f32)

    def token_at(posv, lo, hi):
        p = jnp.clip(jnp.broadcast_to(posv, (8, 128)).astype(i32)[0, 0], lo, hi - 1)
        return ord_s[lax.shift_right_logical(p, 7)] + (p & (C - 1))

    def token_row(tok):
        base = pl.multiple_of(lax.shift_left(lax.shift_right_logical(tok, 4), 4), 16)
        hit = lax.broadcasted_iota(i32, (16, D), 0) == tok - base
        slab = jnp.where(hit, hn_v[pl.ds(base, 16), :].astype(f32), 0.0)
        return _allred8(slab[0:8] + slab[8:16], jnp.add)

    def phase2(i, c_):
        q0 = CPT * i

        if not DIN:
            @pl.when(i > 0)
            def _():
                cp_out(q0 - 1).start()

        off = [pl.multiple_of(ord_s[q0 + k], C) for k in range(CPT + 1)]
        zm = zv[...]
        hprev = hbuf[...]
        ya, ys = [], []
        for n in range(CPT):
            xt = xn_v[pl.ds(off[n + 1], C), :]
            ya.append(_dot_nt(_un(wt_v[0:D // 2, 0:D // 2]), xt[:, 0:D // 2]))
            ys.append(ya[n] + _dot_nt(_un(wt_v[0:D // 2, D // 2:D]), xt[:, D // 2:D]))
        y = jnp.concatenate(ys, axis=1)
        os_ = []
        for p in range(NP):
            phi = _phi_q(y[64 * p:64 * (p + 1)], z_acc[p])
            os_.append(_dot(_un(kvt_v[p]), phi))
        o = jnp.concatenate(os_, axis=0).astype(bf16).T
        wo = jnp.concatenate([_un(wo32[j]) for j in range(D // 128)], axis=1)
        atts = [_dot(o[C * k:C * (k + 1)], wo) for k in range(CPT)]

        def qgate(v):
            lens = [128 - W0] + [128 - W1] * 3
            t = int(v * sum(lens))
            n = 0
            while t >= lens[n]:
                t -= lens[n]
                n += 1
            r0 = 8 * (t + 128 - lens[n])
            return _zero_after(ya[n][r0:r0 + 8], zm)

        def ogate(t):
            r0, j = 8 * (t % 16), (t % 128) // 16
            return _zero_after(atts[t // 128][r0:r0 + 8, 128 * j:128 * j + 128], zm)

        t3 = jnp.maximum(i - 1, 0)
        nsb = NA // 2
        for sb in range(0 if NOG else nsb):
            c0 = 256 * sb
            xcol = xc_v[...]
            acc = None
            for k in range(0, D, 8):
                xk = jnp.concatenate([xcol[k:k + 8]] * 2, axis=1)
                p = jnp.concatenate([wg_v[t3, k:k + 8, c0:c0 + 256].astype(f32) * xk,
                                     wu_v[t3, k:k + 8, c0:c0 + 256].astype(f32) * xk], axis=1)
                if (k // 8) % SEG == 0:
                    p = p + jnp.concatenate([qgate((sb * D + k) / (nsb * D))] * 4, axis=1)
                acc = p if acc is None else acc + p
            pa_v[:, 512 * sb:512 * (sb + 1)] = acc

        put_cols(r_v, i, 0, jnp.where(i > 0, ln2(hprev, off[0], deps=gates(atts[0])), -jnp.inf))

        @pl.when(i > 0)
        def _():
            cp_out(q0).start()

        acc = _allred8(pa_v[pl.ds(pl.multiple_of(zs[3, 0].astype(i32) * 32, 32), 8), :], jnp.add)
        g_ = jnp.concatenate([acc[:, 512 * t:512 * t + 256] for t in range(nsb)], axis=1)
        u_ = jnp.concatenate([acc[:, 512 * t + 256:512 * t + 512] for t in range(nsb)], axis=1)
        a8 = g_ * jax.nn.sigmoid(g_) * u_
        a8 = jnp.concatenate([jnp.where(t3 == 2, 0.0, a8[:, 0:NDUP]), a8[:, NDUP:]], axis=1)
        ac = _col(a8)
        wd_ = D // NH
        for q in range(NH):
            ysum = jnp.where(i > 1, y_v[:, wd_ * q:wd_ * (q + 1)], 0.0)
            for k in range(0, NA * 128, 8):
                p = (wd_v[t3, k:k + 8, wd_ * q:wd_ * (q + 1)].astype(f32)
                     * jnp.concatenate([ac[k:k + 8]] * (wd_ // 128), axis=1))
                if (k // 8) % SEGD == 0:
                    t = TD0 + (q * NA * 128 + k) * (TD1 - TD0) // (NH * NA * 128)
                    p = p + jnp.concatenate([ogate(t)] * (wd_ // 128), axis=1)
                ysum = ysum + p
            y_v[:, wd_ * q:wd_ * (q + 1)] = ysum

        for k in range(CPT):
            if k == NCAND and not NOC:
                ok = (lane >= C // 8) & (lane < (NCAND + 1) * (C // 8))
                cm, cpos = _first_max(jnp.where(ok, r_v[0], -jnp.inf), pos)
                cand = token_at(cpos, C, (NCAND + 1) * C)
                ord_s[NC + 1] = cand
                sg_v[...] = jax.nn.sigmoid(jnp.broadcast_to(cm, (8, 128)))
                xc_v[...] = _col(token_row(cand))
            h = x_v[pl.ds(off[k + 1], C), :].astype(f32) + atts[k]
            if k == CPT - 1:
                hbuf[...] = h
            else:
                put_cols(r_v, i, (k + 1) * (C // 8),
                         ln2(h, off[k + 1], deps=gates(atts[k + 1], NREL2 if k == CPT - 2 else NREL)))
                if k < CPT - 2 or DIN:
                    cp_out(q0 + k + 1).start()
        return c_
    lax.fori_loop(0, 0 if ONLY1 else NT, phase2, 0)
    if not DIN:
        cp_out(NC - 1).start()
    for q in range(1, NCAND + 1):
        cp_out(q).wait()
    fsem = nsem[0]
    nsem[0] += 1

    def slab_of(tok):
        return pl.multiple_of(lax.shift_left(lax.shift_right_logical(tok, 4), 4), 16)

    def patch(tok, y8, sg):
        base = slab_of(tok)
        yv = y8 * jnp.concatenate([sg] * (D // 128), axis=1)
        cur = out_v[pl.ds(base, 16), :].astype(f32)
        hit = lax.broadcasted_iota(i32, (16, D), 0) == tok - base
        fix_v[...] = jnp.where(hit, cur + jnp.concatenate([yv, yv], axis=0), cur).astype(bf16)
        return pltpu.make_async_copy(fix_v, out_hbm.at[0, pl.ds(base, 16)], sems.at[fsem])

    cand = ord_s[NC + 1]
    cp_fix = patch(cand, _allred8(y_v[...], jnp.add), sg_v[...])
    cp_fix.start()
    last = pl.multiple_of(ord_s[NC], C)
    sub = lax.broadcasted_iota(i32, (8, 1), 0).astype(f32)
    stats, cp_l = [], []
    gate = None
    for g in range(0, C, EG):
        h = hbuf[g:g + EG, :]
        s1, s2 = h[:, 0:128], None
        if gate is not None:
            s1 = s1 + jnp.concatenate([gate] * (EG // 8), axis=0)
        s2 = s1 * s1
        for j in range(128, D, 128):
            s1 = s1 + h[:, j:j + 128]
            s2 = s2 + h[:, j:j + 128] * h[:, j:j + 128]
        if ESER:
            gate = _zero_after(s2[EG - 8:EG], zv[...])
        m = jnp.sum(s1, axis=-1, keepdims=True) * (1.0 / D)
        v = jnp.sum(s2, axis=-1, keepdims=True) * (1.0 / D) - m * m
        rs = lax.rsqrt(jnp.maximum(v, 0.0) + EPS)
        stats.append((m, rs))
        rows = pl.ds(pl.multiple_of(last + g, EG), EG)
        out_v[rows, :] = (h * (1.0 + rs) - m * rs).astype(bf16)
        cp_l.append(cp(out_v.at[rows], out_hbm.at[0, rows]))
        cp_l[-1].start()
    for q in range(NCAND + 1, NC - 1):
        cp_out(q).wait()
    pv, pt = r_v[0], pos
    for i in range(1, NT):
        gt = r_v[i] > pv
        pv = jnp.where(gt, r_v[i], pv)
        pt = jnp.where(gt, pos + float(i * T), pt)
    pm, pi = _first_max(pv, pt)
    wr = wr_row()
    wsum = jnp.sum(wr, axis=-1, keepdims=True)
    cands = []
    for g, (m, rs) in zip(range(0, C, EG), stats):
        r = (jnp.sum(hbuf[g:g + EG, :] * wr, axis=-1, keepdims=True) - m * wsum) * rs
        cands += [(r[k:k + 8], sub + float(S + g + k)) for k in range(0, EG, 8)]
    while len(cands) > 1:
        nxt = []
        for k in range(0, len(cands), 2):
            (va, ia), (vb, ib) = cands[k], cands[k + 1]
            gt = vb > va
            nxt.append((jnp.where(gt, vb, va), jnp.where(gt, ib, ia)))
        cands = nxt
    lv, lt = cands[0]
    gt = lv > pm
    bv = jnp.broadcast_to(jnp.where(gt, lv, pm), (8, 128))
    bt = jnp.broadcast_to(jnp.where(gt, lt, pi), (8, 128))
    rmax = _allred8(bv, jnp.maximum)
    idx = token_at(_allred8(jnp.where(bv == rmax, bt, float(2 * S)), jnp.minimum), C, S + C)
    cp_out(NC - 1).wait()
    cp_fix.wait()
    for c in cp_l:
        c.wait()

    @pl.when(idx != cand)
    def _():
        rows = pl.ds(slab_of(cand), 16)
        undo = pltpu.make_async_copy(out_v.at[rows], out_hbm.at[0, rows], sems.at[fsem])
        undo.start()
        hn_v[pl.ds(last, C), :] = _ln(hbuf[...]).astype(bf16)
        x8 = token_row(idx)
        xs = jnp.concatenate([x8, x8], axis=0).astype(bf16)

        def step(j, acc):
            t, hf = lax.shift_right_logical(j, 1), j & 1
            cols = pl.ds(pl.multiple_of(hf * (NA * 64), 128), NA * 64)
            g = _dot(xs, wg_v[t, :, cols])
            a = g * jax.nn.sigmoid(g) * _dot(xs, wu_v[t, :, cols])
            a = jnp.concatenate([jnp.where(j == 4, 0.0, a[:, 0:NDUP]), a[:, NDUP:]], axis=1)
            return acc + _dot(a.astype(bf16), wd_v[t, cols, :])[0:8]

        y8 = lax.fori_loop(0, 6, step, jnp.zeros((8, D), f32))
        undo.wait()
        redo = patch(idx, y8, jax.nn.sigmoid(rmax))
        redo.start()
        redo.wait()


@jax.jit
def pallas_sequential_preLN__linear_kernel_hedgehog__moe_arch_mod__prompt_kernel(
    A_x, A_wqkv, A_w_phi, A_wo, B_x, B_w_r, B_w_gate, B_w_up, B_w_down):
    del B_x
    any_spec = pl.BlockSpec(memory_space=pl.ANY)
    return pl.pallas_call(
        _kernel,
        out_shape=jax.ShapeDtypeStruct((1, S, D), bf16),
        in_specs=[any_spec] * 8,
        out_specs=any_spec,
        scratch_shapes=[
            pltpu.VMEM((S, D), bf16),
            pltpu.VMEM((D, 3 * D), bf16),
            pltpu.VMEM((H, DH, DH), bf16),
            pltpu.VMEM((D // 128, D, 128), bf16),
            pltpu.VMEM((D // 128, D // 2, 128), u32),
            pltpu.VMEM((D,), bf16),
            pltpu.VMEM((3, D, NA * 128), bf16),
            pltpu.VMEM((3, D, NA * 128), bf16),
            pltpu.VMEM((3, NA * 128, D), bf16),
            pltpu.VMEM((3 * D // 2, D), u32),
            pltpu.VMEM((8, 64, 128), u32),
            pltpu.VMEM((S + C, D), bf16),
            pltpu.VMEM((S + C, D), bf16),
            pltpu.VMEM((NP, 64, 128), f32),
            pltpu.VMEM((NP, 128, 128), f32),
            pltpu.VMEM((NP, 32, 128), u32),
            pltpu.VMEM((C, D), f32),
            pltpu.VMEM((S + C, D), bf16),
            pltpu.VMEM((8, 128), u32),
            pltpu.SMEM((8, 128), u32),
            pltpu.VMEM((NC, 8, 128), f32),
            pltpu.VMEM((NT, 8, 128), f32),
            pltpu.VMEM((D, 128), f32),
            pltpu.VMEM((8, NA * 256), f32),
            pltpu.VMEM((8, D), f32),
            pltpu.VMEM((8, 128), f32),
            pltpu.VMEM((16, D), bf16),
            pltpu.SMEM((NC + 2,), i32),
            pltpu.SemaphoreType.DMA((64,)),
        ],
        compiler_params=pltpu.CompilerParams(vmem_limit_bytes=120 * 1024 * 1024,
                                             disable_bounds_checks=True,
                                             disable_semaphore_checks=True),
        name="hedgehog_mod",
    )(A_x, A_wqkv, A_w_phi, A_wo, B_w_r, B_w_gate, B_w_up, B_w_down)
```

```python
import jax
import jax.numpy as jnp
from jax import lax
import jax.experimental.pallas as pl
import jax.experimental.pallas.tpu as pltpu

S = 2048
D = 1024
H = 32
DH = 32
F = 3584
NP = H // 2
C = 128
NC = S // C
T = 512
NT = S // T
CPT = T // C
T1 = 512
N1 = (S - T) // T1
CP1 = T1 // C
GQ = 6 // N1
GO = -(-8 // N1)
SEGS = ((256, 256), (128, 256), (128, 512))
PHI = ((0, 512), (512, 512), (512, 1024))
KEEP = 256
DEFER = 2
NB = F // 128
NA = 10
B0 = (0, NA, NB - NA)
NDUP = (3 * NA - NB) * 128
NCAND = 2
EG = 32
LOG2E = 1.4426950408889634
EPS = 1e-5

f32 = jnp.float32
bf16 = jnp.bfloat16
u32 = jnp.uint32
i32 = jnp.int32


def _dot_nt(a, b):
    return lax.dot_general(a, b, (((1,), (1,)), ((), ())), preferred_element_type=f32)


def _dot(a, b):
    return jnp.dot(a, b, preferred_element_type=f32)


def _pk(x):
    return pltpu.bitcast(x, u32)


def _un(x):
    return pltpu.bitcast(x, bf16)


def _rcp(x):
    r = pl.reciprocal(x, approx=True)
    return r * (2.0 - x * r)


def _allred(v, op):
    v = op(v, pltpu.roll(v, 2, 0))
    return op(v, pltpu.roll(v, 4, 0))


def _allred8(v, op):
    return _allred(op(v, pltpu.roll(v, 1, 0)), op)


def _rows(v, n):
    return jnp.concatenate([v] * n, axis=0)


def _lanes(v, n):
    return jnp.concatenate([v] * n, axis=1)


def _zero_after(dep, zm):
    return pltpu.bitcast(pltpu.bitcast(dep, u32) & zm, f32)


def _exps(x):
    x3 = x.reshape(8, 8, x.shape[1])
    mx = _allred(jnp.max(x3, axis=0), jnp.maximum)
    mn = _allred(jnp.min(x3, axis=0), jnp.minimum)
    ep = jnp.exp2(x3 - mx[None])
    en = jnp.exp2(mn[None] - x3)
    rp = _rcp(_allred(jnp.sum(ep, axis=0), jnp.add))
    rn = _rcp(_allred(jnp.sum(en, axis=0), jnp.add))
    return ep, en, rp, rn


def _phi_k(x):
    L = x.shape[1]
    ep, en, rp, rn = _exps(x)
    return jnp.concatenate([(ep * rp[None]).reshape(64, L), (en * rn[None]).reshape(64, L)], axis=0)


def _phi_q(x, zb):
    L = x.shape[1]
    ep, en, rp, rn = _exps(x)
    zb = _lanes(zb, L // 128).reshape(16, 8, L)
    den = rp * jnp.sum(ep * zb[0:8], axis=0) + rn * jnp.sum(en * zb[8:16], axis=0)
    inv = _rcp(_allred(den, jnp.add) + 1e-6)
    cp = rp * inv
    cn = rn * inv
    phi = jnp.concatenate([(ep * cp[None]).reshape(64, L), (en * cn[None]).reshape(64, L)], axis=0)
    return phi.astype(bf16)


def _lane_blocks_sum(v, acc):
    for c in range(0, v.shape[1], 128):
        acc = acc + v[:, c:c + 128]
    return acc


def _row_sum(x, deps, zm):
    g = x.shape[0] // len(deps)
    gate = jnp.concatenate([jnp.zeros((8, 128), f32) if d is None else _zero_after(d, zm)
                            for d in deps for _ in range(g // 8)], axis=0)
    return jnp.sum(_lane_blocks_sum(x[:, 128:], x[:, 0:128] + gate), axis=-1, keepdims=True)


def _ln(x, deps=None, zm=None):
    tot = jnp.sum(x, axis=-1, keepdims=True) if deps is None else _row_sum(x, deps, zm)
    xc = x - tot * (1.0 / D)
    return xc * lax.rsqrt(jnp.sum(xc * xc, axis=-1, keepdims=True) * (1.0 / D) + EPS)


def _col(a8):
    return _rows(a8, 16).astype(bf16).T.astype(f32)


def _first_max(v, t):
    m = jnp.max(_allred8(v, jnp.maximum), axis=1, keepdims=True)
    return m, jnp.min(_allred8(jnp.where(v == m, t, float(2 * S)), jnp.minimum), axis=1, keepdims=True)


def _merge_max(cands):
    v, t = cands[0]
    for v2, t2 in cands[1:]:
        gt = v2 > v
        v, t = jnp.where(gt, v2, v), jnp.where(gt, t2, t)
    return v, t


def _scalar(v, lo, hi):
    return jnp.clip(jnp.broadcast_to(v, (8, 128)).astype(i32)[0, 0], lo, hi)


class _Group:
    def __init__(self, parts, dst, sem):
        self.parts, self.dst, self.sem = parts, dst, sem

    def start(self):
        for src, dst in self.parts:
            pltpu.make_async_copy(src, dst, self.sem).start()

    def wait(self):
        pltpu.make_async_copy(self.dst, self.dst, self.sem).wait()


def _kernel(x_hbm, wqkv_hbm, wphi_hbm, wo_hbm, wr_hbm, wg_hbm, wu_hbm, wd_hbm, out_hbm,
            x_v, wkv_v, wqb_v, wphi_v, wo_v, wo32, wr_v, wg_v, wu_v, wd_v,
            wt_v, wq_v, a_v, xn_v, hn_v, kv_acc, z_acc, zb_v, hbuf, out_v, zv, zs, p_v, r_v,
            xc_v, pa_v, y_v, sg_v, fix_v, ord_s, sems):
    nsem = [0]

    def new_sems(n):
        nsem[0] += n
        return nsem[0] - n

    def cp(src, dst):
        return pltpu.make_async_copy(src, dst, sems.at[new_sems(1)])

    def cp_w(lo, hi):
        return cp(wqkv_hbm.at[:, lo:hi], wkv_v.at[:, lo:hi])

    def cp_x(lo, hi):
        return cp(x_hbm.at[0, lo:hi], x_v.at[lo:hi])

    cp_wr = cp(wr_hbm, wr_v)
    kcum = [0]
    for _, dk in SEGS:
        kcum.append(kcum[-1] + dk)
    seg_cp = []
    x0 = 0
    for si, (dx, dk) in enumerate(SEGS):
        lo, hi = PHI[si][0] // DH, PHI[si][1] // DH
        ph = [cp(wphi_hbm.at[lo:hi], wphi_v.at[lo:hi])] if hi > lo else []
        seg_cp.append([cp_x(x0, x0 + dx)] + ph + [cp_w(D + kcum[si], D + kcum[si + 1])])
        x0 += dx
    cp_wv = cp_w(2 * D, 3 * D)
    cp_x1a = cp_x(T, T + C)
    cp_x1 = cp_x(T + C, S)
    cp_q0 = _Group([(wqkv_hbm.at[:, 128 * g:128 * (g + 1)], wqb_v.at[g]) for g in range(2)],
                   wqb_v.at[0:2], sems.at[new_sems(1)])
    qsem0 = new_sems(2 * N1)

    def cp_step(j):
        pq = po = None
        if isinstance(j, int):
            pq = [(wqkv_hbm.at[:, 128 * g:128 * (g + 1)], wqb_v.at[g]) for g in range(2 + GQ * j, 2 + GQ * (j + 1))]
            po = [(wo_hbm.at[:, 128 * min(g, 7):128 * (min(g, 7) + 1)], wo_v.at[g])
                  for g in range(GO * j, GO * (j + 1))]
        return [_Group(pq, wqb_v.at[pl.ds(2 + GQ * j, GQ)], sems.at[qsem0 + 2 * j]),
                _Group(po, wo_v.at[pl.ds(GO * j, GO)], sems.at[qsem0 + 2 * j + 1])]

    cp_ffn = []
    for t, b in enumerate(B0):
        cp_ffn += [cp(wg_hbm.at[:, b * 128:(b + NA) * 128], wg_v.at[t]),
                   cp(wu_hbm.at[:, b * 128:(b + NA) * 128], wu_v.at[t]),
                   cp(wd_hbm.at[b * 128:(b + NA) * 128], wd_v.at[t])]
    for c in ([c for t in seg_cp for c in t] + [cp_wr, cp_wv, cp_x1a, cp_q0, cp_x1]
              + [c for j in range(N1) for c in cp_step(j)] + cp_ffn):
        c.start()
    osem0 = new_sems(NC + 1)

    def cp_out(q):
        rows = pl.ds(pl.multiple_of(ord_s[q], C), C)
        return pltpu.make_async_copy(out_v.at[rows], out_hbm.at[0, rows], sems.at[osem0 + q])

    def wr_row():
        return wr_v[...].reshape(1, D).astype(f32)

    def put_cols(ref, idx, col0, r):
        for k in range(0, r.shape[0], 8):
            ref[idx, :, col0 + k // 8:col0 + k // 8 + 1] = r[k:k + 8]

    def ln1(src, dst, deps=None):
        xb = _ln(x_v[src, :].astype(f32), deps, None if deps is None else zv[...]).astype(bf16)
        xn_v[dst, :] = xb
        return xb

    def predict(rows, t, c, deps):
        wr = wr_row()
        wc = wr - jnp.sum(wr, axis=-1, keepdims=True) * (1.0 / D)
        put_cols(p_v, t, c * (C // 8), _row_sum(x_v[rows, :].astype(f32) * wc, deps, zv[...]))

    def fold(dst, w, g):
        rows = pl.ds(64 * g if isinstance(g, int) else pl.multiple_of(64 * g, 64), 64)
        res = _dot_nt(_un(a_v[g]), w)
        dst[rows, :] = _pk((res * LOG2E).astype(bf16))
        return res

    def wt(lo, hi):
        return _un(wt_v[lo // 2:hi // 2, :])

    def kv_and_z(vt, phis, z_of, tail, zm):
        lag = 4
        kvs, zs_ = [], []
        for p in range(NP):
            kvs.append(_dot_nt(vt[64 * p:64 * (p + 1)].astype(bf16), phis[p].astype(bf16)))
            dep = kvs[p - lag][0:8] if p >= lag else tail[D - 64 * (lag - p):D - 64 * (lag - p) + 8]
            zs_.append(_lane_blocks_sum(phis[p], z_of(p, _rows(_zero_after(dep, zm), 16))))
        return kvs, zs_

    r_i = lax.broadcasted_iota(i32, (128, DH), 0)
    f_i = lax.broadcasted_iota(i32, (128, DH), 1)
    sel = jnp.where(f_i == (r_i % 64) // 2, 1.0, 0.0).astype(bf16)
    r_i = lax.broadcasted_iota(i32, (128, 128), 0)
    c_i = lax.broadcasted_iota(i32, (128, 128), 1)
    amask = jnp.where(c_i // 32 == 2 * (r_i // 64) + r_i % 2, jnp.uint32(0xFFFFFFFF), jnp.uint32(0))

    def build_a(lo, hi):
        a_full = _dot_nt(sel, wphi_v[lo // DH:hi // DH].reshape(hi - lo, DH))
        for g in range((hi - lo) // 128):
            blk = pltpu.bitcast(pltpu.bitcast(a_full[:, 128 * g:128 * (g + 1)], u32) & amask, f32)
            a_v[lo // 128 + g] = _pk(blk.astype(bf16))

    zv[...] = jnp.zeros((8, 128), u32)
    cp_z = cp(zv, zs)
    cp_z.start()
    hbuf[...] = jnp.zeros(hbuf.shape, f32)
    xc_v[...] = jnp.zeros(xc_v.shape, f32)
    y_v[...] = jnp.zeros(y_v.shape, f32)
    r_v[...] = jnp.full(r_v.shape, -jnp.inf, f32)
    p_v[...] = jnp.full(p_v.shape, -jnp.inf, f32)

    pieces = [[] for _ in range(NP)]
    pending = []

    def phi_piece(p, t0, yp, dep=None):
        if dep is not None:
            yp = jnp.concatenate([yp[0:8] + _zero_after(dep, zv[...]), yp[8:]], axis=0)
        pieces[p].append((t0, _phi_k(yp)))

    def k_block(klo, khi, t0, t1, defer=0):
        y = _dot_nt(wt(klo, khi), xn_v[t0:t1, :])
        npair = (khi - klo) // 64
        for p in range(npair):
            yp = y[64 * p:64 * (p + 1)]
            if p >= npair - defer:
                if t1 - t0 > C:
                    phi_piece(klo // 64 + p, t0, yp[:, 0:t1 - t0 - C])
                pending.append((klo // 64 + p, t1 - C, yp[:, t1 - t0 - C:]))
            else:
                phi_piece(klo // 64 + p, t0, yp)
        return y

    def flush(res):
        for k, (p, t0, yp) in enumerate(pending):
            phi_piece(p, t0, yp, res[32 * k:32 * k + 8, 0:128])
        del pending[:]

    x0 = 0
    for si, (dx, dk) in enumerate(SEGS):
        rows = slice(x0, x0 + dx)
        k0, k1 = kcum[si], kcum[si + 1]
        if si == 0:
            seg_cp[0][0].wait()
            ln1(rows, rows)
            seg_cp[0][1].wait()
            build_a(*PHI[0])
            seg_cp[0][2].wait()
        else:
            for c in seg_cp[si]:
                c.wait()
            if PHI[si][1] > PHI[si][0]:
                build_a(*PHI[si])
        res = [fold(wt_v, wkv_v[:, D + 128 * g:D + 128 * (g + 1)], g) for g in range(k0 // 128, k1 // 128)]
        flush(res[0])
        if si:
            ln1(rows, rows)
            k_block(k0, k1, 0, x0)
        k_block(0, k1 - (KEEP if k1 == D else 0), x0, x0 + dx, DEFER)
        x0 += dx
    for c in (cp_wv, cp_x1a, cp_q0, cp_wr, cp_z):
        c.wait()
    for g in range(D // 128):
        wt_v[(D + 128 * g) // 2:(D + 128 * (g + 1)) // 2, :] = _pk(wkv_v[:, 2 * D + 128 * g:2 * D + 128 * (g + 1)].T)
    flush(k_block(D - KEEP, D, T - SEGS[-1][0], T))
    yv = _dot_nt(wt(D, 2 * D), xn_v[0:T, :])
    ln1(slice(T, T + C), slice(T, T + C), [yv[128 * k:128 * k + 8, 128:256] for k in range(8)])
    for c in range(CPT):
        predict(slice(C * c, C * (c + 1)), 0, c,
                [yv[256 * c + 32 * k:256 * c + 32 * k + 8, 256:384] for k in range(8)])
    phis = [jnp.concatenate([ph for _, ph in sorted(pieces[p], key=lambda tp: tp[0])], axis=1) for p in range(NP)]
    kvs, zs_ = kv_and_z(yv, phis, lambda p, zero: zero, yv[:, T - C:T], zv[...])
    for p in range(NP):
        kv_acc[p] = kvs[p]
        z_acc[p] = zs_[p]
    fold(wq_v, wqb_v[0], 0)
    fold(wq_v, wqb_v[1], 1)
    cp_x1.wait()

    def order_chunks():
        lane16 = lax.shift_right_logical(lax.broadcasted_iota(i32, (8, 128), 1), 4).astype(f32)
        vals = [p_v[t] for t in range(1 + N1)]
        cids = [lane16 + float(0 if t == 0 else CPT + CP1 * (t - 1)) for t in range(1 + N1)]
        b1 = _first_max(*_merge_max(list(zip(vals, cids))))[1]
        b2 = _first_max(*_merge_max([(jnp.where(c == b1, -jnp.inf, v), c) for v, c in zip(vals, cids)]))[1]
        c1, c2 = _scalar(b1, 0, NC - 1), _scalar(b2, 0, NC - 1)
        c2 = jnp.where(c2 == c1, (c1 + 1) & (NC - 1), c2)
        ord_s[0] = S
        for c in range(NC):
            ord_s[1 + c] = c * C
        ord_s[1 + c1] = 0
        ord_s[1] = c1 * C
        ord_s[1 + jnp.where(c2 == 0, c1, c2)] = jnp.where(c1 == 1, 0, C)
        ord_s[2] = c2 * C

    def phase1(j, carry):
        for c in cp_step(j):
            c.wait()
        zm = zv[...]
        s = pl.multiple_of(T + j * T1, C)
        nxt = pl.multiple_of(jnp.where(j + 1 < N1, s + T1, 0), C)
        xt = xn_v[pl.ds(s, C), :]
        ys, ph = [], []
        for n in range(CP1):
            if n + 1 < CP1:
                rows = pl.ds(pl.multiple_of(s + C * (n + 1), C), C)
                xt1 = ln1(rows, rows)
                yn = _dot_nt(wt(0, 2 * D), xt)
                xt = xt1
            else:
                ya = _dot_nt(_un(wt_v[:, 0:D // 2]), xt[:, 0:D // 2])
                for c in range(CP1):
                    r0, st = 384 + 1280 * c // CP1 // 8 * 8, 1280 // CP1 // 64 * 8
                    predict(pl.ds(pl.multiple_of(s + C * c, C), C), 1 + j, c,
                            [ya[r0 + st * k:r0 + st * k + 8] for k in range(8)])
                order_chunks()
                yn = ya + _dot_nt(_un(wt_v[:, D // 2:D]), xt[:, D // 2:D])
            ys.append(yn)
            ph.append([_phi_k(yn[64 * p:64 * (p + 1)]) for p in range(NP)])
            if n == CP1 - 2:
                ln1(pl.ds(nxt, C), pl.ds(pl.multiple_of(s + T1, C), C),
                    [yn[1536 + 64 * k:1536 + 64 * k + 8] for k in range(8)])
        for t in range(GQ):
            fold(wq_v, wqb_v[2 + GQ * j + t], 2 + GQ * j + t)
        for e in range(4 * GO):
            row = 1408 + 640 * e // (4 * GO) // 8 * 8
            w = _pk(wo_v[GO * j + e // 4, 256 * (e % 4):256 * (e % 4 + 1), :])
            wo32[GO * j + e // 4, 128 * (e % 4):128 * (e % 4 + 1), :] = (
                w.reshape(16, 8, 128) | (_pk(ys[0][row:row + 8]) & zm)[None]).reshape(128, 128)
        vt = jnp.concatenate([yn[D:] for yn in ys], axis=1)
        phis = [jnp.concatenate([ph[n][p] for n in range(CP1)], axis=1) for p in range(NP)]
        kvs, zs_ = kv_and_z(vt, phis, lambda p, zero: z_acc[p] + zero, ys[-1][D:], zm)
        for p in range(NP):
            kv_acc[p] += kvs[p]
            z_acc[p] = zs_[p]
            zb_v[p] = jnp.broadcast_to(jnp.sum(zs_[p], axis=1, keepdims=True), (128, 128))
        return carry

    lax.fori_loop(0, N1, phase1, 0)
    for c in cp_ffn:
        c.wait()

    def ln2(h, row0, nx, nrel):
        deps = [None]
        for j in range(1, C // 8):
            t = (j * nrel * 2) // (C // 8) - 1
            r0 = (C - 8) * (t % 2)
            deps.append(nx[r0:r0 + 8, 128 * (t // 2):128 * (t // 2) + 128] if t >= 0 else None)
        hn = _ln(h, deps, zv[...])
        r = jnp.sum(hn * wr_row(), axis=-1, keepdims=True)
        hn_v[pl.ds(row0, C), :] = hn.astype(bf16)
        out_v[pl.ds(row0, C), :] = (h + hn).astype(bf16)
        return r

    lane = lax.broadcasted_iota(i32, (8, 128), 1)
    pos = (lane * 8 + lax.broadcasted_iota(i32, (8, 128), 0)).astype(f32)

    def token_at(posv, lo, hi):
        p = _scalar(posv, lo, hi - 1)
        return ord_s[lax.shift_right_logical(p, 7)] + (p & (C - 1))

    def slab_of(tok):
        base = pl.multiple_of(lax.shift_left(lax.shift_right_logical(tok, 4), 4), 16)
        return pl.ds(base, 16), lax.broadcasted_iota(i32, (16, D), 0) == tok - base

    def token_row(tok):
        rows, hit = slab_of(tok)
        slab = jnp.where(hit, hn_v[rows, :].astype(f32), 0.0)
        return _allred8(slab[0:8] + slab[8:16], jnp.add)

    def phase2(i, carry):
        q0 = CPT * i
        off = [pl.multiple_of(ord_s[q0 + k], C) for k in range(CPT + 1)]
        zm = zv[...]
        hprev = hbuf[...]
        kmask = lax.broadcasted_iota(i32, (64, 128), 0) // 32 == lax.broadcasted_iota(i32, (64, 128), 1) % 2

        def attend(y):
            os_ = []
            for p in range(NP):
                phi = _phi_q(y[64 * p:64 * (p + 1)], zb_v[p])
                os_.append(_dot(jnp.where(kmask, kv_acc[p], 0.0).astype(bf16), phi))
            return jnp.concatenate(os_, axis=0).astype(bf16).T

        ya, ys = [], []
        for n in range(CPT):
            xt = xn_v[pl.ds(off[n + 1], C), :]
            ya.append(_dot_nt(_un(wq_v[:, 0:D // 2]), xt[:, 0:D // 2]))
            if n == CPT - 1:
                o01 = attend(jnp.concatenate(ys[0:2], axis=1))
            ys.append(ya[n] + _dot_nt(_un(wq_v[:, D // 2:D]), xt[:, D // 2:D]))
        wo = jnp.concatenate([_un(wo32[j]) for j in range(D // 128)], axis=1)
        head = _dot(o01[0:C], wo[:, 0:256])
        o23 = attend(jnp.concatenate(ys[2:4], axis=1))
        atts = [jnp.concatenate([head, _dot(o01[0:C], wo[:, 256:])], axis=1),
                _dot(o01[C:2 * C], wo), _dot(o23[0:C], wo), _dot(o23[C:2 * C], wo)]

        def q_gate(v):
            lens = [128, 104, 104, 104]
            t, n = int(v * sum(lens)), 0
            while t >= lens[n]:
                t -= lens[n]
                n += 1
            r0 = 8 * (t + 128 - lens[n])
            return _zero_after(ya[n][r0:r0 + 8], zm)

        def o_gate(t):
            r0, j = 8 * (t % 16), (t % 128) // 16
            return _zero_after(atts[t // 128][r0:r0 + 8, 128 * j:128 * j + 128], zm)

        t3 = jnp.maximum(i - 1, 0)
        nsb = NA // 2
        for sb in range(nsb):
            cols = slice(256 * sb, 256 * (sb + 1))
            xcol = xc_v[...]
            acc = None
            for k in range(0, D, 8):
                xk = _lanes(xcol[k:k + 8], 2)
                p = jnp.concatenate([wg_v[t3, k:k + 8, cols].astype(f32) * xk,
                                     wu_v[t3, k:k + 8, cols].astype(f32) * xk], axis=1)
                if k % 64 == 0:
                    p = p + _lanes(q_gate((sb * D + k) / (nsb * D)), 4)
                acc = p if acc is None else acc + p
            pa_v[:, 512 * sb:512 * (sb + 1)] = acc

        put_cols(r_v, i, 0, jnp.where(i > 0, ln2(hprev, off[0], atts[0], 6), -jnp.inf))

        @pl.when(i > 0)
        def _():
            cp_out(q0).start()

        acc = _allred8(pa_v[pl.ds(pl.multiple_of(zs[3, 0].astype(i32) * 32, 32), 8), :], jnp.add)
        g_ = jnp.concatenate([acc[:, 512 * t:512 * t + 256] for t in range(nsb)], axis=1)
        u_ = jnp.concatenate([acc[:, 512 * t + 256:512 * t + 512] for t in range(nsb)], axis=1)
        a8 = g_ * jax.nn.sigmoid(g_) * u_
        ac = _col(jnp.concatenate([jnp.where(t3 == 2, 0.0, a8[:, 0:NDUP]), a8[:, NDUP:]], axis=1))
        for q in range(2):
            cols = slice(D // 2 * q, D // 2 * (q + 1))
            ysum = jnp.where(i > 1, y_v[:, cols], 0.0)
            for k in range(0, NA * 128, 8):
                p = wd_v[t3, k:k + 8, cols].astype(f32) * _lanes(ac[k:k + 8], 4)
                if k % 32 == 0:
                    p = p + _lanes(o_gate(64 + (q * NA * 128 + k) * 376 // (2 * NA * 128)), 4)
                ysum = ysum + p
            y_v[:, cols] = ysum

        for k in range(CPT):
            if k == NCAND:
                ok = (lane >= C // 8) & (lane < (NCAND + 1) * (C // 8))
                cm, cpos = _first_max(jnp.where(ok, r_v[0], -jnp.inf), pos)
                cand = token_at(cpos, C, (NCAND + 1) * C)
                ord_s[NC + 1] = cand
                sg_v[...] = jax.nn.sigmoid(jnp.broadcast_to(cm, (8, 128)))
                xc_v[...] = _col(token_row(cand))
            h = x_v[pl.ds(off[k + 1], C), :].astype(f32) + atts[k]
            if k == CPT - 1:
                hbuf[...] = h
            else:
                put_cols(r_v, i, (k + 1) * (C // 8), ln2(h, off[k + 1], atts[k + 1], 5 if k == CPT - 2 else 6))
                cp_out(q0 + k + 1).start()
        return carry

    lax.fori_loop(0, NT, phase2, 0)

    for q in range(1, NCAND + 1):
        cp_out(q).wait()
    fsem = new_sems(1)

    def patch(tok, y8, sg):
        rows, hit = slab_of(tok)
        cur = out_v[rows, :].astype(f32)
        fix_v[...] = jnp.where(hit, cur + _rows(y8 * _lanes(sg, D // 128), 2), cur).astype(bf16)
        return pltpu.make_async_copy(fix_v, out_hbm.at[0, rows], sems.at[fsem])

    cand = ord_s[NC + 1]
    cp_fix = patch(cand, _allred8(y_v[...], jnp.add), sg_v[...])
    cp_fix.start()
    last = pl.multiple_of(ord_s[NC], C)
    stats, cp_last = [], []
    for g in range(0, C, EG):
        h = hbuf[g:g + EG, :]
        s1 = h[:, 0:128]
        s2 = s1 * s1
        for j in range(128, D, 128):
            s1 = s1 + h[:, j:j + 128]
            s2 = s2 + h[:, j:j + 128] * h[:, j:j + 128]
        m = jnp.sum(s1, axis=-1, keepdims=True) * (1.0 / D)
        v = jnp.sum(s2, axis=-1, keepdims=True) * (1.0 / D) - m * m
        rs = lax.rsqrt(jnp.maximum(v, 0.0) + EPS)
        stats.append((m, rs))
        rows = pl.ds(pl.multiple_of(last + g, EG), EG)
        out_v[rows, :] = (h * (1.0 + rs) - m * rs).astype(bf16)
        cp_last.append(cp(out_v.at[rows], out_hbm.at[0, rows]))
        cp_last[-1].start()
    for q in range(NCAND + 1, NC - 1):
        cp_out(q).wait()
    pm, pi = _first_max(*_merge_max([(r_v[i], pos + float(i * T) if i else pos) for i in range(NT)]))
    wr = wr_row()
    wsum = jnp.sum(wr, axis=-1, keepdims=True)
    sub = lax.broadcasted_iota(i32, (8, 1), 0).astype(f32)
    cands = []
    for g, (m, rs) in zip(range(0, C, EG), stats):
        r = (jnp.sum(hbuf[g:g + EG, :] * wr, axis=-1, keepdims=True) - m * wsum) * rs
        cands += [(r[k:k + 8], sub + float(S + g + k)) for k in range(0, EG, 8)]
    while len(cands) > 1:
        cands = [_merge_max(cands[k:k + 2]) for k in range(0, len(cands), 2)]
    bv, bt = [jnp.broadcast_to(v, (8, 128)) for v in _merge_max([(pm, pi), cands[0]])]
    rmax = _allred8(bv, jnp.maximum)
    idx = token_at(_allred8(jnp.where(bv == rmax, bt, float(2 * S)), jnp.minimum), C, S + C)
    cp_out(NC - 1).wait()
    cp_fix.wait()
    for c in cp_last:
        c.wait()

    @pl.when(idx != cand)
    def _():
        rows, _ = slab_of(cand)
        undo = pltpu.make_async_copy(out_v.at[rows], out_hbm.at[0, rows], sems.at[fsem])
        undo.start()
        hn_v[pl.ds(last, C), :] = _ln(hbuf[...]).astype(bf16)
        xs = _rows(token_row(idx), 2).astype(bf16)

        def step(j, acc):
            t = lax.shift_right_logical(j, 1)
            cols = pl.ds(pl.multiple_of((j & 1) * (NA * 64), 128), NA * 64)
            g = _dot(xs, wg_v[t, :, cols])
            a = g * jax.nn.sigmoid(g) * _dot(xs, wu_v[t, :, cols])
            a = jnp.concatenate([jnp.where(j == 4, 0.0, a[:, 0:NDUP]), a[:, NDUP:]], axis=1)
            return acc + _dot(a.astype(bf16), wd_v[t, cols, :])[0:8]

        y8 = lax.fori_loop(0, 6, step, jnp.zeros((8, D), f32))
        undo.wait()
        redo = patch(idx, y8, jax.nn.sigmoid(rmax))
        redo.start()
        redo.wait()


@jax.jit
def pallas_sequential_preLN__linear_kernel_hedgehog__moe_arch_mod__prompt_kernel(
    A_x: jax.Array,
    A_wqkv: jax.Array,
    A_w_phi: jax.Array,
    A_wo: jax.Array,
    B_x: jax.Array,
    B_w_r: jax.Array,
    B_w_gate: jax.Array,
    B_w_up: jax.Array,
    B_w_down: jax.Array,
):
    del B_x
    any_spec = pl.BlockSpec(memory_space=pl.ANY)
    return pl.pallas_call(
        _kernel,
        out_shape=jax.ShapeDtypeStruct((1, S, D), bf16),
        in_specs=[any_spec] * 8,
        out_specs=any_spec,
        scratch_shapes=[
            pltpu.VMEM((S, D), bf16),
            pltpu.VMEM((D, 3 * D), bf16),
            pltpu.VMEM((D // 128, D, 128), bf16),
            pltpu.VMEM((H, DH, DH), bf16),
            pltpu.VMEM((N1 * GO, D, 128), bf16),
            pltpu.VMEM((N1 * GO, D // 2, 128), u32),
            pltpu.VMEM((D,), bf16),
            pltpu.VMEM((3, D, NA * 128), bf16),
            pltpu.VMEM((3, D, NA * 128), bf16),
            pltpu.VMEM((3, NA * 128, D), bf16),
            pltpu.VMEM((D, D), u32),
            pltpu.VMEM((D // 2, D), u32),
            pltpu.VMEM((8, 64, 128), u32),
            pltpu.VMEM((S + C, D), bf16),
            pltpu.VMEM((S + C, D), bf16),
            pltpu.VMEM((NP, 64, 128), f32),
            pltpu.VMEM((NP, 128, 128), f32),
            pltpu.VMEM((NP, 128, 128), f32),
            pltpu.VMEM((C, D), f32),
            pltpu.VMEM((S + C, D), bf16),
            pltpu.VMEM((8, 128), u32),
            pltpu.SMEM((8, 128), u32),
            pltpu.VMEM((1 + N1, 8, 128), f32),
            pltpu.VMEM((NT, 8, 128), f32),
            pltpu.VMEM((D, 128), f32),
            pltpu.VMEM((8, NA * 256), f32),
            pltpu.VMEM((8, D), f32),
            pltpu.VMEM((8, 128), f32),
            pltpu.VMEM((16, D), bf16),
            pltpu.SMEM((NC + 2,), i32),
            pltpu.SemaphoreType.DMA((64,)),
        ],
        compiler_params=pltpu.CompilerParams(vmem_limit_bytes=120 * 1024 * 1024,
                                             disable_bounds_checks=True,
                                             disable_semaphore_checks=True),
        name="hedgehog_mod",
    )(A_x, A_wqkv, A_w_phi, A_wo, B_w_r, B_w_gate, B_w_up, B_w_down)
```

```python
import jax
import jax.numpy as jnp
from jax import lax
import jax.experimental.pallas as pl
import jax.experimental.pallas.tpu as pltpu

S = 2048
D = 1024
H = 32
DH = 32
F = 3584
NP = H // 2
C = 128
NC = S // C
T = 512
NT = S // T
CPT = T // C
T1 = 512
N1 = (S - T) // T1
CP1 = T1 // C
GQ = 6 // N1
GO = -(-8 // N1)
SEGS = ((256, 256), (128, 256), (128, 512))
PHI = ((0, 512), (512, 512), (512, 1024))
KEEP = 256
DEFER = 2
NB = F // 128
NA = 10
B0 = (0, NA, NB - NA)
NDUP = (3 * NA - NB) * 128
NCAND = 2
EG = 32
LOG2E = 1.4426950408889634
EPS = 1e-5

f32 = jnp.float32
bf16 = jnp.bfloat16
u32 = jnp.uint32
i32 = jnp.int32


def _dot_nt(a, b):
    return lax.dot_general(a, b, (((1,), (1,)), ((), ())), preferred_element_type=f32)


def _dot(a, b):
    return jnp.dot(a, b, preferred_element_type=f32)


def _pk(x):
    return pltpu.bitcast(x, u32)


def _un(x):
    return pltpu.bitcast(x, bf16)


def _rcp(x):
    r = pl.reciprocal(x, approx=True)
    return r * (2.0 - x * r)


def _allred(v, op):
    v = op(v, pltpu.roll(v, 2, 0))
    return op(v, pltpu.roll(v, 4, 0))


def _allred8(v, op):
    return _allred(op(v, pltpu.roll(v, 1, 0)), op)


def _rows(v, n):
    return jnp.concatenate([v] * n, axis=0)


def _lanes(v, n):
    return jnp.concatenate([v] * n, axis=1)


def _zero_after(dep, zm):
    return pltpu.bitcast(pltpu.bitcast(dep, u32) & zm, f32)


def _exps(x):
    x3 = x.reshape(8, 8, x.shape[1])
    mx = _allred(jnp.max(x3, axis=0), jnp.maximum)
    mn = _allred(jnp.min(x3, axis=0), jnp.minimum)
    ep = jnp.exp2(x3 - mx[None])
    en = jnp.exp2(mn[None] - x3)
    rp = _rcp(_allred(jnp.sum(ep, axis=0), jnp.add))
    rn = _rcp(_allred(jnp.sum(en, axis=0), jnp.add))
    return ep, en, rp, rn


def _phi_k(x):
    L = x.shape[1]
    ep, en, rp, rn = _exps(x)
    return jnp.concatenate([(ep * rp[None]).reshape(64, L), (en * rn[None]).reshape(64, L)], axis=0)


def _phi_q(x, zb):
    L = x.shape[1]
    ep, en, rp, rn = _exps(x)
    zb = _lanes(zb, L // 128).reshape(16, 8, L)
    den = rp * jnp.sum(ep * zb[0:8], axis=0) + rn * jnp.sum(en * zb[8:16], axis=0)
    inv = _rcp(_allred(den, jnp.add) + 1e-6)
    cp = rp * inv
    cn = rn * inv
    phi = jnp.concatenate([(ep * cp[None]).reshape(64, L), (en * cn[None]).reshape(64, L)], axis=0)
    return phi.astype(bf16)


def _lane_blocks_sum(v, acc):
    for c in range(0, v.shape[1], 128):
        acc = acc + v[:, c:c + 128]
    return acc


def _row_sum(x, deps, zm):
    g = x.shape[0] // len(deps)
    gate = jnp.concatenate([jnp.zeros((8, 128), f32) if d is None else _zero_after(d, zm)
                            for d in deps for _ in range(g // 8)], axis=0)
    return jnp.sum(_lane_blocks_sum(x[:, 128:], x[:, 0:128] + gate), axis=-1, keepdims=True)


def _ln(x, deps=None, zm=None):
    tot = jnp.sum(x, axis=-1, keepdims=True) if deps is None else _row_sum(x, deps, zm)
    xc = x - tot * (1.0 / D)
    return xc * lax.rsqrt(jnp.sum(xc * xc, axis=-1, keepdims=True) * (1.0 / D) + EPS)


def _col(a8):
    return _rows(a8, 16).astype(bf16).T.astype(f32)


def _first_max(v, t):
    m = jnp.max(_allred8(v, jnp.maximum), axis=1, keepdims=True)
    return m, jnp.min(_allred8(jnp.where(v == m, t, float(2 * S)), jnp.minimum), axis=1, keepdims=True)


def _merge_max(cands):
    v, t = cands[0]
    for v2, t2 in cands[1:]:
        gt = v2 > v
        v, t = jnp.where(gt, v2, v), jnp.where(gt, t2, t)
    return v, t


def _scalar(v, lo, hi):
    return jnp.clip(jnp.broadcast_to(v, (8, 128)).astype(i32)[0, 0], lo, hi)


class _Group:
    def __init__(self, parts, dst, sem):
        self.parts, self.dst, self.sem = parts, dst, sem

    def start(self):
        for src, dst in self.parts:
            pltpu.make_async_copy(src, dst, self.sem).start()

    def wait(self):
        pltpu.make_async_copy(self.dst, self.dst, self.sem).wait()


def _kernel(x_hbm, wqkv_hbm, wphi_hbm, wo_hbm, wr_hbm, wg_hbm, wu_hbm, wd_hbm, out_hbm,
            x_v, wkv_v, wqb_v, wphi_v, wo_v, wo32, wr_v, wg_v, wu_v, wd_v,
            wt_v, wq_v, a_v, xn_v, hn_v, kv_acc, z_acc, zb_v, hbuf, out_v, zv, zs, p_v, r_v,
            xc_v, pa_v, y_v, sg_v, fix_v, ord_s, sems):
    nsem = [0]

    def new_sems(n):
        nsem[0] += n
        return nsem[0] - n

    def cp(src, dst):
        return pltpu.make_async_copy(src, dst, sems.at[new_sems(1)])

    def cp_w(lo, hi):
        return cp(wqkv_hbm.at[:, lo:hi], wkv_v.at[:, lo:hi])

    def cp_x(lo, hi):
        return cp(x_hbm.at[0, lo:hi], x_v.at[lo:hi])

    cp_wr = cp(wr_hbm, wr_v)
    kcum = [0]
    for _, dk in SEGS:
        kcum.append(kcum[-1] + dk)
    seg_cp = []
    x0 = 0
    for si, (dx, dk) in enumerate(SEGS):
        lo, hi = PHI[si][0] // DH, PHI[si][1] // DH
        ph = [cp(wphi_hbm.at[lo:hi], wphi_v.at[lo:hi])] if hi > lo else []
        seg_cp.append([cp_x(x0, x0 + dx)] + ph + [cp_w(D + kcum[si], D + kcum[si + 1])])
        x0 += dx
    cp_wv = cp_w(2 * D, 3 * D)
    cp_x1a = cp_x(T, T + C)
    cp_x1 = cp_x(T + C, S)
    cp_q0 = _Group([(wqkv_hbm.at[:, 128 * g:128 * (g + 1)], wqb_v.at[g]) for g in range(2)],
                   wqb_v.at[0:2], sems.at[new_sems(1)])
    qsem0 = new_sems(2 * N1)

    def cp_step(j):
        pq = po = None
        if isinstance(j, int):
            pq = [(wqkv_hbm.at[:, 128 * g:128 * (g + 1)], wqb_v.at[g]) for g in range(2 + GQ * j, 2 + GQ * (j + 1))]
            po = [(wo_hbm.at[:, 128 * min(g, 7):128 * (min(g, 7) + 1)], wo_v.at[g])
                  for g in range(GO * j, GO * (j + 1))]
        return [_Group(pq, wqb_v.at[pl.ds(2 + GQ * j, GQ)], sems.at[qsem0 + 2 * j]),
                _Group(po, wo_v.at[pl.ds(GO * j, GO)], sems.at[qsem0 + 2 * j + 1])]

    cp_ffn = []
    for t, b in enumerate(B0):
        cp_ffn += [cp(wg_hbm.at[:, b * 128:(b + NA) * 128], wg_v.at[t]),
                   cp(wu_hbm.at[:, b * 128:(b + NA) * 128], wu_v.at[t]),
                   cp(wd_hbm.at[b * 128:(b + NA) * 128], wd_v.at[t])]
    seg_cp[0] = seg_cp[0][1:] + seg_cp[0][0:1]
    for c in ([c for t in seg_cp for c in t] + [cp_wr, cp_wv, cp_x1a, cp_q0, cp_x1]
              + [c for j in range(N1) for c in cp_step(j)] + cp_ffn):
        c.start()
    osem0 = new_sems(NC + 1)

    def cp_out(q):
        rows = pl.ds(pl.multiple_of(ord_s[q], C), C)
        return pltpu.make_async_copy(out_v.at[rows], out_hbm.at[0, rows], sems.at[osem0 + q])

    def wr_row():
        return wr_v[...].reshape(1, D).astype(f32)

    def put_cols(ref, idx, col0, r):
        for k in range(0, r.shape[0], 8):
            ref[idx, :, col0 + k // 8:col0 + k // 8 + 1] = r[k:k + 8]

    def half(row0, n):
        if isinstance(row0, int):
            return pl.ds(row0 // 2, n // 2)
        return pl.ds(pl.multiple_of(lax.shift_right_logical(row0, 1), C // 2), n // 2)

    def ln1(src, dst, n, deps=None):
        xb = _pk(_ln(x_v[pl.ds(src, n), :].astype(f32), deps, None if deps is None else zv[...]).astype(bf16))
        xn_v[half(dst, n), :] = xb
        return _un(xb)

    def xn(row0, n):
        return _un(xn_v[half(row0, n), :])

    def predict(rows, t, c, deps):
        wr = wr_row()
        wc = wr - jnp.sum(wr, axis=-1, keepdims=True) * (1.0 / D)
        put_cols(p_v, t, c * (C // 8), _row_sum(x_v[rows, :].astype(f32) * wc, deps, zv[...]))

    def fold(dst, w, g):
        rows = pl.ds(64 * g if isinstance(g, int) else pl.multiple_of(64 * g, 64), 64)
        res = _dot_nt(_un(a_v[g]), w)
        dst[rows, :] = _pk((res * LOG2E).astype(bf16))
        return res

    def wt(lo, hi):
        return _un(wt_v[lo // 2:hi // 2, :])

    def kv_and_z(vt, phis, z_of, tail, zm):
        lag = 4
        kvs, zs_ = [], []
        for p in range(NP):
            kvs.append(_dot_nt(vt[64 * p:64 * (p + 1)].astype(bf16), phis[p].astype(bf16)))
            dep = kvs[p - lag][0:8] if p >= lag else tail[D - 64 * (lag - p):D - 64 * (lag - p) + 8]
            zs_.append(_lane_blocks_sum(phis[p], z_of(p, _rows(_zero_after(dep, zm), 16))))
        return kvs, zs_

    r_i = lax.broadcasted_iota(i32, (128, DH), 0)
    f_i = lax.broadcasted_iota(i32, (128, DH), 1)
    sel = jnp.where(f_i == (r_i % 64) // 2, 1.0, 0.0).astype(bf16)
    r_i = lax.broadcasted_iota(i32, (128, 128), 0)
    c_i = lax.broadcasted_iota(i32, (128, 128), 1)
    amask = jnp.where(c_i // 32 == 2 * (r_i // 64) + r_i % 2, jnp.uint32(0xFFFFFFFF), jnp.uint32(0))

    def build_a(lo, hi):
        a_full = _dot_nt(sel, wphi_v[lo // DH:hi // DH].reshape(hi - lo, DH))
        for g in range((hi - lo) // 128):
            blk = pltpu.bitcast(pltpu.bitcast(a_full[:, 128 * g:128 * (g + 1)], u32) & amask, f32)
            a_v[lo // 128 + g] = _pk(blk.astype(bf16))

    zv[...] = jnp.zeros((8, 128), u32)
    cp_z = cp(zv, zs)
    cp_z.start()
    hbuf[...] = jnp.zeros(hbuf.shape, f32)
    xc_v[...] = jnp.zeros(xc_v.shape, f32)
    y_v[...] = jnp.zeros(y_v.shape, f32)
    r_v[...] = jnp.full(r_v.shape, -jnp.inf, f32)
    p_v[...] = jnp.full(p_v.shape, -jnp.inf, f32)

    pieces = [[] for _ in range(NP)]
    pending = []

    def phi_piece(p, t0, yp, dep=None):
        if dep is not None:
            yp = jnp.concatenate([yp[0:8] + _zero_after(dep, zv[...]), yp[8:]], axis=0)
        pieces[p].append((t0, _phi_k(yp)))

    def k_block(klo, khi, t0, t1, defer=0):
        y = _dot_nt(wt(klo, khi), xn(t0, t1 - t0))
        npair = (khi - klo) // 64
        for p in range(npair):
            yp = y[64 * p:64 * (p + 1)]
            if p >= npair - defer:
                if t1 - t0 > C:
                    phi_piece(klo // 64 + p, t0, yp[:, 0:t1 - t0 - C])
                pending.append((klo // 64 + p, t1 - C, yp[:, t1 - t0 - C:]))
            else:
                phi_piece(klo // 64 + p, t0, yp)
        return y

    def flush(res):
        for k, (p, t0, yp) in enumerate(pending):
            phi_piece(p, t0, yp, res[32 * k:32 * k + 8, 0:128])
        del pending[:]

    x0 = 0
    for si, (dx, dk) in enumerate(SEGS):
        k0, k1 = kcum[si], kcum[si + 1]
        if si == 0:
            seg_cp[0][0].wait()
            build_a(*PHI[0])
            seg_cp[0][1].wait()
        else:
            for c in seg_cp[si]:
                c.wait()
            if PHI[si][1] > PHI[si][0]:
                build_a(*PHI[si])
        res = [fold(wt_v, wkv_v[:, D + 128 * g:D + 128 * (g + 1)], g) for g in range(k0 // 128, k1 // 128)]
        flush(res[0])
        if si == 0:
            seg_cp[0][2].wait()
        ln1(x0, x0, dx)
        if si:
            k_block(k0, k1, 0, x0)
        k_block(0, k1 - (KEEP if k1 == D else 0), x0, x0 + dx, DEFER)
        x0 += dx
    for c in (cp_wv, cp_x1a, cp_q0, cp_wr, cp_z):
        c.wait()
    for g in range(D // 128):
        wt_v[(D + 128 * g) // 2:(D + 128 * (g + 1)) // 2, :] = _pk(wkv_v[:, 2 * D + 128 * g:2 * D + 128 * (g + 1)].T)
    flush(k_block(D - KEEP, D, T - SEGS[-1][0], T))
    yv = _dot_nt(wt(D, 2 * D), xn(0, T))
    ln1(T, T, C, [yv[128 * k:128 * k + 8, 128:256] for k in range(8)])
    for c in range(CPT):
        predict(slice(C * c, C * (c + 1)), 0, c,
                [yv[256 * c + 32 * k:256 * c + 32 * k + 8, 256:384] for k in range(8)])
    phis = [jnp.concatenate([ph for _, ph in sorted(pieces[p], key=lambda tp: tp[0])], axis=1) for p in range(NP)]
    kvs, zs_ = kv_and_z(yv, phis, lambda p, zero: zero, yv[:, T - C:T], zv[...])
    for p in range(NP):
        kv_acc[p] = kvs[p]
        z_acc[p] = zs_[p]
    fold(wq_v, wqb_v[0], 0)
    fold(wq_v, wqb_v[1], 1)
    cp_x1.wait()

    def order_chunks():
        lane16 = lax.shift_right_logical(lax.broadcasted_iota(i32, (8, 128), 1), 4).astype(f32)
        vals = [p_v[t] for t in range(1 + N1)]
        cids = [lane16 + float(0 if t == 0 else CPT + CP1 * (t - 1)) for t in range(1 + N1)]
        b1 = _first_max(*_merge_max(list(zip(vals, cids))))[1]
        b2 = _first_max(*_merge_max([(jnp.where(c == b1, -jnp.inf, v), c) for v, c in zip(vals, cids)]))[1]
        c1, c2 = _scalar(b1, 0, NC - 1), _scalar(b2, 0, NC - 1)
        c2 = jnp.where(c2 == c1, (c1 + 1) & (NC - 1), c2)
        ord_s[0] = S
        for c in range(NC):
            ord_s[1 + c] = c * C
        ord_s[1 + c1] = 0
        ord_s[1] = c1 * C
        ord_s[1 + jnp.where(c2 == 0, c1, c2)] = jnp.where(c1 == 1, 0, C)
        ord_s[2] = c2 * C

    def phase1(j, carry):
        for c in cp_step(j):
            c.wait()
        zm = zv[...]
        s = pl.multiple_of(T + j * T1, C)
        nxt = pl.multiple_of(jnp.where(j + 1 < N1, s + T1, 0), C)
        xt = xn(s, C)
        ys, ph = [], []
        for n in range(CP1):
            if n + 1 < CP1:
                row0 = pl.multiple_of(s + C * (n + 1), C)
                xt1 = ln1(row0, row0, C)
                yn = _dot_nt(wt(0, 2 * D), xt)
                xt = xt1
            else:
                ya = _dot_nt(_un(wt_v[:, 0:D // 2]), xt[:, 0:D // 2])
                for c in range(CP1):
                    r0, st = 384 + 1280 * c // CP1 // 8 * 8, 1280 // CP1 // 64 * 8
                    predict(pl.ds(pl.multiple_of(s + C * c, C), C), 1 + j, c,
                            [ya[r0 + st * k:r0 + st * k + 8] for k in range(8)])
                order_chunks()
                yn = ya + _dot_nt(_un(wt_v[:, D // 2:D]), xt[:, D // 2:D])
            ys.append(yn)
            ph.append([_phi_k(yn[64 * p:64 * (p + 1)]) for p in range(NP)])
            if n == CP1 - 2:
                ln1(nxt, pl.multiple_of(s + T1, C), C,
                    [yn[1536 + 64 * k:1536 + 64 * k + 8] for k in range(8)])
        for t in range(GQ):
            fold(wq_v, wqb_v[2 + GQ * j + t], 2 + GQ * j + t)
        for e in range(4 * GO):
            row = 1408 + 640 * e // (4 * GO) // 8 * 8
            w = _pk(wo_v[GO * j + e // 4, 256 * (e % 4):256 * (e % 4 + 1), :])
            wo32[GO * j + e // 4, 128 * (e % 4):128 * (e % 4 + 1), :] = (
                w.reshape(16, 8, 128) | (_pk(ys[0][row:row + 8]) & zm)[None]).reshape(128, 128)
        vt = jnp.concatenate([yn[D:] for yn in ys], axis=1)
        phis = [jnp.concatenate([ph[n][p] for n in range(CP1)], axis=1) for p in range(NP)]
        kvs, zs_ = kv_and_z(vt, phis, lambda p, zero: z_acc[p] + zero, ys[-1][D:], zm)
        for p in range(NP):
            kv_acc[p] += kvs[p]
            z_acc[p] = zs_[p]
            zb_v[p] = jnp.broadcast_to(jnp.sum(zs_[p], axis=1, keepdims=True), (128, 128))
        return carry

    lax.fori_loop(0, N1, phase1, 0)
    for c in cp_ffn:
        c.wait()

    def ln2(h, row0, nx, nrel):
        deps = [None]
        for j in range(1, C // 8):
            t = (j * nrel * 2) // (C // 8) - 1
            r0 = (C - 8) * (t % 2)
            deps.append(nx[r0:r0 + 8, 128 * (t // 2):128 * (t // 2) + 128] if t >= 0 else None)
        hn = _ln(h, deps, zv[...])
        r = jnp.sum(hn * wr_row(), axis=-1, keepdims=True)
        hn_v[pl.ds(row0, C), :] = hn.astype(bf16)
        out_v[pl.ds(row0, C), :] = (h + hn).astype(bf16)
        return r

    lane = lax.broadcasted_iota(i32, (8, 128), 1)
    pos = (lane * 8 + lax.broadcasted_iota(i32, (8, 128), 0)).astype(f32)

    def token_at(posv, lo, hi):
        p = _scalar(posv, lo, hi - 1)
        return ord_s[lax.shift_right_logical(p, 7)] + (p & (C - 1))

    def slab_of(tok):
        base = pl.multiple_of(lax.shift_left(lax.shift_right_logical(tok, 4), 4), 16)
        return pl.ds(base, 16), lax.broadcasted_iota(i32, (16, D), 0) == tok - base

    def token_row(tok):
        rows, hit = slab_of(tok)
        slab = jnp.where(hit, hn_v[rows, :].astype(f32), 0.0)
        return _allred8(slab[0:8] + slab[8:16], jnp.add)

    def phase2(i, carry):
        q0 = CPT * i
        off = [pl.multiple_of(ord_s[q0 + k], C) for k in range(CPT + 1)]
        zm = zv[...]
        hprev = hbuf[...]
        kmask = lax.broadcasted_iota(i32, (64, 128), 0) // 32 == lax.broadcasted_iota(i32, (64, 128), 1) % 2

        def attend(y):
            os_ = []
            for p in range(NP):
                phi = _phi_q(y[64 * p:64 * (p + 1)], zb_v[p])
                os_.append(_dot(jnp.where(kmask, kv_acc[p], 0.0).astype(bf16), phi))
            return jnp.concatenate(os_, axis=0).astype(bf16).T

        ya, ys = [], []
        for n in range(CPT):
            xt = xn(off[n + 1], C)
            ya.append(_dot_nt(_un(wq_v[:, 0:D // 2]), xt[:, 0:D // 2]))
            if n == CPT - 1:
                o01 = attend(jnp.concatenate(ys[0:2], axis=1))
            ys.append(ya[n] + _dot_nt(_un(wq_v[:, D // 2:D]), xt[:, D // 2:D]))
        wo = jnp.concatenate([_un(wo32[j]) for j in range(D // 128)], axis=1)
        head = _dot(o01[0:C], wo[:, 0:256])
        o23 = attend(jnp.concatenate(ys[2:4], axis=1))
        atts = [jnp.concatenate([head, _dot(o01[0:C], wo[:, 256:])], axis=1),
                _dot(o01[C:2 * C], wo), _dot(o23[0:C], wo), _dot(o23[C:2 * C], wo)]

        def q_gate(v):
            lens = [128, 104, 104, 104]
            t, n = int(v * sum(lens)), 0
            while t >= lens[n]:
                t -= lens[n]
                n += 1
            r0 = 8 * (t + 128 - lens[n])
            return _zero_after(ya[n][r0:r0 + 8], zm)

        def o_gate(t):
            r0, j = 8 * (t % 16), (t % 128) // 16
            return _zero_after(atts[t // 128][r0:r0 + 8, 128 * j:128 * j + 128], zm)

        t3 = jnp.maximum(i - 1, 0)
        nsb = NA // 2
        for sb in range(nsb):
            cols = slice(256 * sb, 256 * (sb + 1))
            xcol = xc_v[...]
            acc = None
            for k in range(0, D, 8):
                xk = _lanes(xcol[k:k + 8], 2)
                p = jnp.concatenate([wg_v[t3, k:k + 8, cols].astype(f32) * xk,
                                     wu_v[t3, k:k + 8, cols].astype(f32) * xk], axis=1)
                if k % 64 == 0:
                    p = p + _lanes(q_gate((sb * D + k) / (nsb * D)), 4)
                acc = p if acc is None else acc + p
            pa_v[:, 512 * sb:512 * (sb + 1)] = acc

        put_cols(r_v, i, 0, jnp.where(i > 0, ln2(hprev, off[0], atts[0], 6), -jnp.inf))

        @pl.when(i > 0)
        def _():
            cp_out(q0).start()

        acc = _allred8(pa_v[pl.ds(pl.multiple_of(zs[3, 0].astype(i32) * 32, 32), 8), :], jnp.add)
        g_ = jnp.concatenate([acc[:, 512 * t:512 * t + 256] for t in range(nsb)], axis=1)
        u_ = jnp.concatenate([acc[:, 512 * t + 256:512 * t + 512] for t in range(nsb)], axis=1)
        a8 = g_ * jax.nn.sigmoid(g_) * u_
        ac = _col(jnp.concatenate([jnp.where(t3 == 2, 0.0, a8[:, 0:NDUP]), a8[:, NDUP:]], axis=1))
        for q in range(2):
            cols = slice(D // 2 * q, D // 2 * (q + 1))
            ysum = jnp.where(i > 1, y_v[:, cols], 0.0)
            for k in range(0, NA * 128, 8):
                p = wd_v[t3, k:k + 8, cols].astype(f32) * _lanes(ac[k:k + 8], 4)
                if k % 32 == 0:
                    p = p + _lanes(o_gate(64 + (q * NA * 128 + k) * 376 // (2 * NA * 128)), 4)
                ysum = ysum + p
            y_v[:, cols] = ysum

        for k in range(CPT):
            if k == NCAND:
                ok = (lane >= C // 8) & (lane < (NCAND + 1) * (C // 8))
                cm, cpos = _first_max(jnp.where(ok, r_v[0], -jnp.inf), pos)
                cand = token_at(cpos, C, (NCAND + 1) * C)
                ord_s[NC + 1] = cand
                sg_v[...] = jax.nn.sigmoid(jnp.broadcast_to(cm, (8, 128)))
                xc_v[...] = _col(token_row(cand))
            h = x_v[pl.ds(off[k + 1], C), :].astype(f32) + atts[k]
            if k == CPT - 1:
                hbuf[...] = h
            else:
                put_cols(r_v, i, (k + 1) * (C // 8), ln2(h, off[k + 1], atts[k + 1], 5 if k == CPT - 2 else 6))
                cp_out(q0 + k + 1).start()
        return carry

    lax.fori_loop(0, NT, phase2, 0)

    for q in range(1, NCAND + 1):
        cp_out(q).wait()
    fsem = new_sems(1)

    def patch(tok, y8, sg):
        rows, hit = slab_of(tok)
        cur = out_v[rows, :].astype(f32)
        fix_v[...] = jnp.where(hit, cur + _rows(y8 * _lanes(sg, D // 128), 2), cur).astype(bf16)
        return pltpu.make_async_copy(fix_v, out_hbm.at[0, rows], sems.at[fsem])

    cand = ord_s[NC + 1]
    cp_fix = patch(cand, _allred8(y_v[...], jnp.add), sg_v[...])
    cp_fix.start()
    last = pl.multiple_of(ord_s[NC], C)
    stats, cp_last = [], []
    for g in range(0, C, EG):
        h = hbuf[g:g + EG, :]
        s1 = h[:, 0:128]
        s2 = s1 * s1
        for j in range(128, D, 128):
            s1 = s1 + h[:, j:j + 128]
            s2 = s2 + h[:, j:j + 128] * h[:, j:j + 128]
        m = jnp.sum(s1, axis=-1, keepdims=True) * (1.0 / D)
        v = jnp.sum(s2, axis=-1, keepdims=True) * (1.0 / D) - m * m
        rs = lax.rsqrt(jnp.maximum(v, 0.0) + EPS)
        stats.append((m, rs))
        rows = pl.ds(pl.multiple_of(last + g, EG), EG)
        out_v[rows, :] = (h * (1.0 + rs) - m * rs).astype(bf16)
        cp_last.append(cp(out_v.at[rows], out_hbm.at[0, rows]))
        cp_last[-1].start()
    for q in range(NCAND + 1, NC - 1):
        cp_out(q).wait()
    pm, pi = _first_max(*_merge_max([(r_v[i], pos + float(i * T) if i else pos) for i in range(NT)]))
    wr = wr_row()
    wsum = jnp.sum(wr, axis=-1, keepdims=True)
    sub = lax.broadcasted_iota(i32, (8, 1), 0).astype(f32)
    cands = []
    for g, (m, rs) in zip(range(0, C, EG), stats):
        r = (jnp.sum(hbuf[g:g + EG, :] * wr, axis=-1, keepdims=True) - m * wsum) * rs
        cands += [(r[k:k + 8], sub + float(S + g + k)) for k in range(0, EG, 8)]
    while len(cands) > 1:
        cands = [_merge_max(cands[k:k + 2]) for k in range(0, len(cands), 2)]
    bv, bt = [jnp.broadcast_to(v, (8, 128)) for v in _merge_max([(pm, pi), cands[0]])]
    rmax = _allred8(bv, jnp.maximum)
    idx = token_at(_allred8(jnp.where(bv == rmax, bt, float(2 * S)), jnp.minimum), C, S + C)
    cp_out(NC - 1).wait()
    cp_fix.wait()
    for c in cp_last:
        c.wait()

    @pl.when(idx != cand)
    def _():
        rows, _ = slab_of(cand)
        undo = pltpu.make_async_copy(out_v.at[rows], out_hbm.at[0, rows], sems.at[fsem])
        undo.start()
        hn_v[pl.ds(last, C), :] = _ln(hbuf[...]).astype(bf16)
        xs = _rows(token_row(idx), 2).astype(bf16)

        def step(j, acc):
            t = lax.shift_right_logical(j, 1)
            cols = pl.ds(pl.multiple_of((j & 1) * (NA * 64), 128), NA * 64)
            g = _dot(xs, wg_v[t, :, cols])
            a = g * jax.nn.sigmoid(g) * _dot(xs, wu_v[t, :, cols])
            a = jnp.concatenate([jnp.where(j == 4, 0.0, a[:, 0:NDUP]), a[:, NDUP:]], axis=1)
            return acc + _dot(a.astype(bf16), wd_v[t, cols, :])[0:8]

        y8 = lax.fori_loop(0, 6, step, jnp.zeros((8, D), f32))
        undo.wait()
        redo = patch(idx, y8, jax.nn.sigmoid(rmax))
        redo.start()
        redo.wait()


@jax.jit
def pallas_sequential_preLN__linear_kernel_hedgehog__moe_arch_mod__prompt_kernel(
    A_x: jax.Array,
    A_wqkv: jax.Array,
    A_w_phi: jax.Array,
    A_wo: jax.Array,
    B_x: jax.Array,
    B_w_r: jax.Array,
    B_w_gate: jax.Array,
    B_w_up: jax.Array,
    B_w_down: jax.Array,
):
    del B_x
    any_spec = pl.BlockSpec(memory_space=pl.ANY)
    return pl.pallas_call(
        _kernel,
        out_shape=jax.ShapeDtypeStruct((1, S, D), bf16),
        in_specs=[any_spec] * 8,
        out_specs=any_spec,
        scratch_shapes=[
            pltpu.VMEM((S, D), bf16),
            pltpu.VMEM((D, 3 * D), bf16),
            pltpu.VMEM((D // 128, D, 128), bf16),
            pltpu.VMEM((H, DH, DH), bf16),
            pltpu.VMEM((N1 * GO, D, 128), bf16),
            pltpu.VMEM((N1 * GO, D // 2, 128), u32),
            pltpu.VMEM((D,), bf16),
            pltpu.VMEM((3, D, NA * 128), bf16),
            pltpu.VMEM((3, D, NA * 128), bf16),
            pltpu.VMEM((3, NA * 128, D), bf16),
            pltpu.VMEM((D, D), u32),
            pltpu.VMEM((D // 2, D), u32),
            pltpu.VMEM((8, 64, 128), u32),
            pltpu.VMEM(((S + C) // 2, D), u32),
            pltpu.VMEM((S + C, D), bf16),
            pltpu.VMEM((NP, 64, 128), f32),
            pltpu.VMEM((NP, 128, 128), f32),
            pltpu.VMEM((NP, 128, 128), f32),
            pltpu.VMEM((C, D), f32),
            pltpu.VMEM((S + C, D), bf16),
            pltpu.VMEM((8, 128), u32),
            pltpu.SMEM((8, 128), u32),
            pltpu.VMEM((1 + N1, 8, 128), f32),
            pltpu.VMEM((NT, 8, 128), f32),
            pltpu.VMEM((D, 128), f32),
            pltpu.VMEM((8, NA * 256), f32),
            pltpu.VMEM((8, D), f32),
            pltpu.VMEM((8, 128), f32),
            pltpu.VMEM((16, D), bf16),
            pltpu.SMEM((NC + 2,), i32),
            pltpu.SemaphoreType.DMA((64,)),
        ],
        compiler_params=pltpu.CompilerParams(vmem_limit_bytes=120 * 1024 * 1024,
                                             disable_bounds_checks=True,
                                             disable_semaphore_checks=True),
        name="hedgehog_mod",
    )(A_x, A_wqkv, A_w_phi, A_wo, B_w_r, B_w_gate, B_w_up, B_w_down)
```

```python
import jax
import jax.numpy as jnp
from jax import lax
import jax.experimental.pallas as pl
import jax.experimental.pallas.tpu as pltpu

S = 2048
D = 1024
H = 32
DH = 32
F = 3584
NP = H // 2
C = 128
NC = S // C
T = 512
NT = S // T
CPT = T // C
T1 = 512
N1 = (S - T) // T1
CP1 = T1 // C
KR = H * (DH - 1)
GO = -(-8 // N1)
SEGS = ((256, 256), (128, 256), (128, 512))
PHI = ((0, 512), (512, 512), (512, 1024))
DEFER = 2
NB = F // 128
NA = 10
B0 = (0, NA, NB - NA)
NDUP = (3 * NA - NB) * 128
NCAND = 2
EG = 32
LOG2E = 1.4426950408889634
EPS = 1e-5

f32 = jnp.float32
bf16 = jnp.bfloat16
u32 = jnp.uint32
i32 = jnp.int32


def _dot_nt(a, b):
    return lax.dot_general(a, b, (((1,), (1,)), ((), ())), preferred_element_type=f32)


def _dot(a, b):
    return jnp.dot(a, b, preferred_element_type=f32)


def _pk(x):
    return pltpu.bitcast(x, u32)


def _un(x):
    return pltpu.bitcast(x, bf16)


def _rcp(x):
    r = pl.reciprocal(x, approx=True)
    return r * (2.0 - x * r)


def _allred(v, op):
    v = op(v, pltpu.roll(v, 2, 0))
    return op(v, pltpu.roll(v, 4, 0))


def _allred8(v, op):
    return _allred(op(v, pltpu.roll(v, 1, 0)), op)


def _rows(v, n):
    return jnp.concatenate([v] * n, axis=0)


def _lanes(v, n):
    return jnp.concatenate([v] * n, axis=1)


def _zero_after(dep, zm):
    return pltpu.bitcast(pltpu.bitcast(dep, u32) & zm, f32)


def _exps(x):
    x3 = x.reshape(8, 8, x.shape[1])
    mx = _allred(jnp.max(x3, axis=0), jnp.maximum)
    mn = _allred(jnp.min(x3, axis=0), jnp.minimum)
    ep = jnp.exp2(x3 - mx[None])
    en = jnp.exp2(mn[None] - x3)
    rp = _rcp(_allred(jnp.sum(ep, axis=0), jnp.add))
    rn = _rcp(_allred(jnp.sum(en, axis=0), jnp.add))
    return ep, en, rp, rn


def _phi_k(x):
    L = x.shape[1]
    ep, en, rp, rn = _exps(x)
    return jnp.concatenate([(ep * rp[None]).reshape(64, L), (en * rn[None]).reshape(64, L)], axis=0)


def _phi_q(x, zb):
    L = x.shape[1]
    ep, en, rp, rn = _exps(x)
    zb = _lanes(zb, L // 128).reshape(16, 8, L)
    den = rp * jnp.sum(ep * zb[0:8], axis=0) + rn * jnp.sum(en * zb[8:16], axis=0)
    inv = _rcp(_allred(den, jnp.add) + 1e-6)
    cp = rp * inv
    cn = rn * inv
    phi = jnp.concatenate([(ep * cp[None]).reshape(64, L), (en * cn[None]).reshape(64, L)], axis=0)
    return phi.astype(bf16)


def _slot(n):
    return lax.shift_right_logical(lax.broadcasted_iota(i32, (8, n), 0), 1)


def _pair_logits(y, sgs):
    slot = _slot(y.shape[1])
    out, r, shared = {}, 0, None
    for k, sg in enumerate(sgs):
        if k == 0 or sg % 2 == 0:
            shared, r = y[r:r + 16], r + 16
        l0, l1, l2 = y[r:r + 8], y[r + 8:r + 16], shared[8 * (sg % 2):8 * (sg % 2) + 8]
        for q in range(4):
            x0 = jnp.where(slot == q, l0, jnp.where(slot == (q + 1) % 4, l1, jnp.where(slot == (q + 2) % 4, l2, 0.0)))
            out[4 * sg + q] = jnp.concatenate([x0, y[r + 16 + 56 * q:r + 72 + 56 * q]], axis=0)
        r += 240
    return out


def _lane_blocks_sum(v, acc):
    for c in range(0, v.shape[1], 128):
        acc = acc + v[:, c:c + 128]
    return acc


def _row_sum(x, deps, zm):
    g = x.shape[0] // len(deps)
    gate = jnp.concatenate([jnp.zeros((8, 128), f32) if d is None else _zero_after(d, zm)
                            for d in deps for _ in range(g // 8)], axis=0)
    return jnp.sum(_lane_blocks_sum(x[:, 128:], x[:, 0:128] + gate), axis=-1, keepdims=True)


def _ln(x, deps=None, zm=None):
    tot = jnp.sum(x, axis=-1, keepdims=True) if deps is None else _row_sum(x, deps, zm)
    xc = x - tot * (1.0 / D)
    return xc * lax.rsqrt(jnp.sum(xc * xc, axis=-1, keepdims=True) * (1.0 / D) + EPS)


def _col(a8):
    return _rows(a8, 16).astype(bf16).T.astype(f32)


def _first_max(v, t):
    m = jnp.max(_allred8(v, jnp.maximum), axis=1, keepdims=True)
    return m, jnp.min(_allred8(jnp.where(v == m, t, float(2 * S)), jnp.minimum), axis=1, keepdims=True)


def _merge_max(cands):
    v, t = cands[0]
    for v2, t2 in cands[1:]:
        gt = v2 > v
        v, t = jnp.where(gt, v2, v), jnp.where(gt, t2, t)
    return v, t


def _scalar(v, lo, hi):
    return jnp.clip(jnp.broadcast_to(v, (8, 128)).astype(i32)[0, 0], lo, hi)


class _Group:
    def __init__(self, parts, dst, sem):
        self.parts, self.dst, self.sem = parts, dst, sem

    def start(self):
        for src, dst in self.parts:
            pltpu.make_async_copy(src, dst, self.sem).start()

    def wait(self):
        pltpu.make_async_copy(self.dst, self.dst, self.sem).wait()


def _kernel(x_hbm, wqkv_hbm, wphi_hbm, wo_hbm, wr_hbm, wg_hbm, wu_hbm, wd_hbm, out_hbm,
            x_v, wkv_v, wqb_v, wphi_v, wo_v, wo32, wr_v, wg_v, wu_v, wd_v,
            wt_v, wq_v, a_v, xn_v, hn_v, kv_acc, z_acc, zb_v, hbuf, out_v, zv, zs, p_v, r_v,
            xc_v, pa_v, y_v, sg_v, fix_v, ord_s, sems):
    nsem = [0]

    def new_sems(n):
        nsem[0] += n
        return nsem[0] - n

    def cp(src, dst):
        return pltpu.make_async_copy(src, dst, sems.at[new_sems(1)])

    def cp_w(lo, hi):
        return cp(wqkv_hbm.at[:, lo:hi], wkv_v.at[:, lo:hi])

    def cp_x(lo, hi):
        return cp(x_hbm.at[0, lo:hi], x_v.at[lo:hi])

    cp_wr = cp(wr_hbm, wr_v)
    kcum = [0]
    for _, dk in SEGS:
        kcum.append(kcum[-1] + dk)
    seg_cp = []
    x0 = 0
    for si, (dx, dk) in enumerate(SEGS):
        lo, hi = PHI[si][0] // DH, PHI[si][1] // DH
        ph = [cp(wphi_hbm.at[lo:hi], wphi_v.at[lo:hi])] if hi > lo else []
        seg_cp.append([cp_x(x0, x0 + dx)] + ph + [cp_w(D + kcum[si], D + kcum[si + 1])])
        x0 += dx
    cp_wv = cp_w(2 * D, 3 * D)
    cp_x1a = cp_x(T, T + C)
    cp_x1 = cp_x(T + C, S)
    cp_q0 = _Group([(wqkv_hbm.at[:, 128 * g:128 * (g + 1)], wqb_v.at[g]) for g in range(2)],
                   wqb_v.at[0:2], sems.at[new_sems(1)])
    qsem0 = new_sems(2 * N1)

    def cp_step(j):
        pq = po = None
        if isinstance(j, int):
            pq = [(wqkv_hbm.at[:, 128 * g:128 * (g + 1)], wqb_v.at[g]) for g in range(2 + 2 * j, 4 + 2 * j)]
            po = [(wo_hbm.at[:, 128 * min(g, 7):128 * (min(g, 7) + 1)], wo_v.at[g])
                  for g in range(GO * j, GO * (j + 1))]
        return [_Group(pq, wqb_v.at[pl.ds(2 + 2 * j, 2)], sems.at[qsem0 + 2 * j]),
                _Group(po, wo_v.at[pl.ds(GO * j, GO)], sems.at[qsem0 + 2 * j + 1])]

    cp_ffn = []
    for t, b in enumerate(B0):
        cp_ffn += [cp(wg_hbm.at[:, b * 128:(b + NA) * 128], wg_v.at[t]),
                   cp(wu_hbm.at[:, b * 128:(b + NA) * 128], wu_v.at[t]),
                   cp(wd_hbm.at[b * 128:(b + NA) * 128], wd_v.at[t])]
    seg_cp[0] = seg_cp[0][1:] + seg_cp[0][0:1]
    for c in ([c for t in seg_cp for c in t] + [cp_wr, cp_wv, cp_x1a, cp_q0, cp_x1]
              + [c for j in range(N1) for c in cp_step(j)] + cp_ffn):
        c.start()
    osem0 = new_sems(NC + 1)

    def cp_out(q):
        rows = pl.ds(pl.multiple_of(ord_s[q], C), C)
        return pltpu.make_async_copy(out_v.at[rows], out_hbm.at[0, rows], sems.at[osem0 + q])

    def wr_row():
        return wr_v[...].reshape(1, D).astype(f32)

    def put_cols(ref, idx, col0, r):
        for k in range(0, r.shape[0], 8):
            ref[idx, :, col0 + k // 8:col0 + k // 8 + 1] = r[k:k + 8]

    def half(row0, n):
        if isinstance(row0, int):
            return pl.ds(row0 // 2, n // 2)
        return pl.ds(pl.multiple_of(lax.shift_right_logical(row0, 1), C // 2), n // 2)

    def ln1(src, dst, n, deps=None):
        xb = _pk(_ln(x_v[pl.ds(src, n), :].astype(f32), deps, None if deps is None else zv[...]).astype(bf16))
        xn_v[half(dst, n), :] = xb
        return _un(xb)

    def xn(row0, n):
        return _un(xn_v[half(row0, n), :])

    def predict(rows, t, c, deps):
        wr = wr_row()
        wc = wr - jnp.sum(wr, axis=-1, keepdims=True) * (1.0 / D)
        put_cols(p_v, t, c * (C // 8), _row_sum(x_v[rows, :].astype(f32) * wc, deps, zv[...]))

    def fold(dst, ws, sg):
        slot = _slot(D)
        res = [_dot_nt(_un(a_v[2 * sg + e]), ws[e]) for e in range(2)]
        main, e0, e1 = [], [], []
        for e in range(2):
            z = jnp.where(((slot + 3) % 4) // 2 == e, 0.0, res[e][0:8])
            b1 = z + pltpu.roll(z, 4, 0)
            b0 = pltpu.roll(b1, 2, 0)
            for pp in range(2):
                base = jnp.where(slot % 2 == pp, b0, b1)
                main.append((res[e][16 + 56 * pp:72 + 56 * pp].reshape(7, 8, D) - base[None]).reshape(56, D))
            e0.append(res[e][8:16] - b0)
            e1.append(res[e][0:8] - b1)
        rows = jnp.concatenate([jnp.where(slot < 2, e0[0], e0[1]), e1[0] + e1[1]] + main, axis=0)
        l2 = _pk((_rows(jnp.where(slot < 2, e0[1], e0[0]), 2) * LOG2E).astype(bf16))
        if isinstance(sg, int):
            r0, r1 = 248 * (sg // 2), 248 * (sg // 2) + 8 + 120 * (sg % 2)
        else:
            r0 = pl.multiple_of(248 * lax.shift_right_logical(sg, 1), 8)
            r1 = pl.multiple_of(r0 + 8 + 120 * (sg & 1), 8)
        dst[pl.ds(r1, 120), :] = _pk((rows * LOG2E).astype(bf16))
        dst[pl.ds(r0, 8), :] = jnp.where(slot // 2 == sg % 2, l2, dst[pl.ds(r0, 8), :])
        return res

    def wk(lo, hi):
        r0, r1 = 248 * (lo // 2), 248 * ((hi - 1) // 2) + 128 + 120 * ((hi - 1) % 2)
        if lo % 2:
            return _un(jnp.concatenate([wt_v[r0:r0 + 8, :], wt_v[r0 + 128:r1, :]], axis=0))
        return _un(wt_v[r0:r1, :])

    def kv_and_z(vt, phis, z_of, tail, zm):
        lag = 4
        kvs, zs_ = [], []
        for p in range(NP):
            kvs.append(_dot_nt(vt[64 * p:64 * (p + 1)].astype(bf16), phis[p].astype(bf16)))
            dep = kvs[p - lag][0:8] if p >= lag else tail[D - 64 * (lag - p):D - 64 * (lag - p) + 8]
            zs_.append(_lane_blocks_sum(phis[p], z_of(p, _rows(_zero_after(dep, zm), 16))))
        return kvs, zs_

    def a_row(r, e):
        s = (r & 7) >> 1
        f = jnp.where(r >= 72, (r - 64) >> 1, jnp.where(r >= 16, (r - 8) >> 1, jnp.where(
            r >= 8, jnp.where(s >> 1 == e, 1, 3), jnp.where(((s + 3) & 3) >> 1 == e, 2, 0))))
        pp = jnp.where(r >= 72, 1, jnp.where(r >= 16, 0, jnp.where(r >= 8, s, s + 1) & 1))
        return f, 2 * pp + (r & 1)

    f_i = lax.broadcasted_iota(i32, (128, DH), 1)
    sel = [jnp.where(f_i == a_row(lax.broadcasted_iota(i32, (128, DH), 0), e)[0], 1.0, 0.0).astype(bf16)
           for e in range(2)]
    amask = jnp.where(lax.broadcasted_iota(i32, (128, 128), 1) >> 5
                      == a_row(lax.broadcasted_iota(i32, (128, 128), 0), 0)[1], jnp.uint32(0xFFFFFFFF), jnp.uint32(0))

    def build_a(lo, hi):
        for g in range(lo // 128, hi // 128):
            blk = _dot_nt(sel[g % 2], wphi_v[4 * g:4 * (g + 1)].reshape(128, DH))
            a_v[g] = _pk(pltpu.bitcast(pltpu.bitcast(blk, u32) & amask, f32).astype(bf16))

    zv[...] = jnp.zeros((8, 128), u32)
    cp_z = cp(zv, zs)
    cp_z.start()
    for ref in (wt_v, wq_v):
        for r0 in (0, 248):
            ref[r0:r0 + 8, :] = jnp.zeros((8, D), u32)
    hbuf[...] = jnp.zeros(hbuf.shape, f32)
    xc_v[...] = jnp.zeros(xc_v.shape, f32)
    y_v[...] = jnp.zeros(y_v.shape, f32)
    r_v[...] = jnp.full(r_v.shape, -jnp.inf, f32)
    p_v[...] = jnp.full(p_v.shape, -jnp.inf, f32)

    pieces = [[] for _ in range(NP)]
    pending = []

    def phi_piece(p, t0, yp, dep=None):
        if dep is not None:
            yp = jnp.concatenate([yp[0:8] + _zero_after(dep, zv[...]), yp[8:]], axis=0)
        pieces[p].append((t0, _phi_k(yp)))

    def k_block(lo, hi, t0, t1, defer=0):
        y = _dot_nt(wk(lo, hi), xn(t0, t1 - t0))
        for p, yp in _pair_logits(y, range(lo, hi)).items():
            if p >= 4 * hi - defer:
                if t1 - t0 > C:
                    phi_piece(p, t0, yp[:, 0:t1 - t0 - C])
                pending.append((p, t1 - C, yp[:, t1 - t0 - C:]))
            else:
                phi_piece(p, t0, yp)
        return y

    def flush(res):
        for k, (p, t0, yp) in enumerate(pending):
            phi_piece(p, t0, yp, res[32 * k:32 * k + 8, 0:128])
        del pending[:]

    x0 = 0
    for si, (dx, dk) in enumerate(SEGS):
        k0, k1 = kcum[si] // 256, kcum[si + 1] // 256
        if si == 0:
            seg_cp[0][0].wait()
            build_a(*PHI[0])
            seg_cp[0][1].wait()
        else:
            for c in seg_cp[si]:
                c.wait()
            if PHI[si][1] > PHI[si][0]:
                build_a(*PHI[si])
        res = [fold(wt_v, [wkv_v[:, D + 128 * g:D + 128 * (g + 1)] for g in (2 * sg, 2 * sg + 1)], sg)
               for sg in range(k0, k1)]
        flush(res[0][0])
        if si == 0:
            seg_cp[0][2].wait()
        ln1(x0, x0, dx)
        if si:
            k_block(k0, k1, 0, x0)
        k_block(0, min(k1, 3), x0, x0 + dx, DEFER)
        x0 += dx
    for c in (cp_wv, cp_x1a, cp_q0, cp_wr, cp_z):
        c.wait()
    for g in range(D // 128):
        wt_v[KR // 2 + 64 * g:KR // 2 + 64 * (g + 1), :] = _pk(wkv_v[:, 2 * D + 128 * g:2 * D + 128 * (g + 1)].T)
    flush(k_block(3, 4, T - SEGS[-1][0], T))
    yv = _dot_nt(_un(wt_v[KR // 2:, :]), xn(0, T))
    ln1(T, T, C, [yv[128 * k:128 * k + 8, 128:256] for k in range(8)])
    for c in range(CPT):
        predict(slice(C * c, C * (c + 1)), 0, c,
                [yv[256 * c + 32 * k:256 * c + 32 * k + 8, 256:384] for k in range(8)])
    phis = [jnp.concatenate([ph for _, ph in sorted(pieces[p], key=lambda tp: tp[0])], axis=1) for p in range(NP)]
    kvs, zs_ = kv_and_z(yv, phis, lambda p, zero: zero, yv[:, T - C:T], zv[...])
    for p in range(NP):
        kv_acc[p] = kvs[p]
        z_acc[p] = zs_[p]
    fold(wq_v, [wqb_v[0], wqb_v[1]], 0)
    cp_x1.wait()

    def order_chunks():
        lane16 = lax.shift_right_logical(lax.broadcasted_iota(i32, (8, 128), 1), 4).astype(f32)
        vals = [p_v[t] for t in range(1 + N1)]
        cids = [lane16 + float(0 if t == 0 else CPT + CP1 * (t - 1)) for t in range(1 + N1)]
        b1 = _first_max(*_merge_max(list(zip(vals, cids))))[1]
        b2 = _first_max(*_merge_max([(jnp.where(c == b1, -jnp.inf, v), c) for v, c in zip(vals, cids)]))[1]
        c1, c2 = _scalar(b1, 0, NC - 1), _scalar(b2, 0, NC - 1)
        c2 = jnp.where(c2 == c1, (c1 + 1) & (NC - 1), c2)
        ord_s[0] = S
        for c in range(NC):
            ord_s[1 + c] = c * C
        ord_s[1 + c1] = 0
        ord_s[1] = c1 * C
        ord_s[1 + jnp.where(c2 == 0, c1, c2)] = jnp.where(c1 == 1, 0, C)
        ord_s[2] = c2 * C

    def phase1(j, carry):
        for c in cp_step(j):
            c.wait()
        zm = zv[...]
        s = pl.multiple_of(T + j * T1, C)
        nxt = pl.multiple_of(jnp.where(j + 1 < N1, s + T1, 0), C)
        xt = xn(s, C)
        ys, ph = [], []
        for n in range(CP1):
            if n + 1 < CP1:
                row0 = pl.multiple_of(s + C * (n + 1), C)
                xt1 = ln1(row0, row0, C)
                yn = _dot_nt(_un(wt_v[...]), xt)
                xt = xt1
            else:
                ya = _dot_nt(_un(wt_v[:, 0:D // 2]), xt[:, 0:D // 2])
                for c in range(CP1):
                    r0, st = 384 + 1280 * c // CP1 // 8 * 8, 1280 // CP1 // 64 * 8
                    predict(pl.ds(pl.multiple_of(s + C * c, C), C), 1 + j, c,
                            [ya[r0 + st * k:r0 + st * k + 8] for k in range(8)])
                order_chunks()
                yn = ya + _dot_nt(_un(wt_v[:, D // 2:D]), xt[:, D // 2:D])
            ys.append(yn)
            ph.append([_phi_k(yp) for yp in _pair_logits(yn[0:KR], range(4)).values()])
            if n == CP1 - 2:
                ln1(nxt, pl.multiple_of(s + T1, C), C,
                    [yn[KR + 512 + 64 * k:KR + 520 + 64 * k] for k in range(8)])
        fold(wq_v, [wqb_v[2 + 2 * j], wqb_v[3 + 2 * j]], 1 + j)
        for e in range(4 * GO):
            row = KR + 384 + 640 * e // (4 * GO) // 8 * 8
            w = _pk(wo_v[GO * j + e // 4, 256 * (e % 4):256 * (e % 4 + 1), :])
            wo32[GO * j + e // 4, 128 * (e % 4):128 * (e % 4 + 1), :] = (
                w.reshape(16, 8, 128) | (_pk(ys[0][row:row + 8]) & zm)[None]).reshape(128, 128)
        vt = jnp.concatenate([yn[KR:] for yn in ys], axis=1)
        phis = [jnp.concatenate([ph[n][p] for n in range(CP1)], axis=1) for p in range(NP)]
        kvs, zs_ = kv_and_z(vt, phis, lambda p, zero: z_acc[p] + zero, ys[-1][KR:], zm)
        for p in range(NP):
            kv_acc[p] += kvs[p]
            z_acc[p] = zs_[p]
            zb_v[p] = jnp.broadcast_to(jnp.sum(zs_[p], axis=1, keepdims=True), (128, 128))
        return carry

    lax.fori_loop(0, N1, phase1, 0)
    for c in cp_ffn:
        c.wait()

    def ln2(h, row0, nx, nrel):
        deps = [None]
        for j in range(1, C // 8):
            t = (j * nrel * 2) // (C // 8) - 1
            r0 = (C - 8) * (t % 2)
            deps.append(nx[r0:r0 + 8, 128 * (t // 2):128 * (t // 2) + 128] if t >= 0 else None)
        hn = _ln(h, deps, zv[...])
        r = jnp.sum(hn * wr_row(), axis=-1, keepdims=True)
        hn_v[pl.ds(row0, C), :] = hn.astype(bf16)
        out_v[pl.ds(row0, C), :] = (h + hn).astype(bf16)
        return r

    lane = lax.broadcasted_iota(i32, (8, 128), 1)
    pos = (lane * 8 + lax.broadcasted_iota(i32, (8, 128), 0)).astype(f32)

    def token_at(posv, lo, hi):
        p = _scalar(posv, lo, hi - 1)
        return ord_s[lax.shift_right_logical(p, 7)] + (p & (C - 1))

    def slab_of(tok):
        base = pl.multiple_of(lax.shift_left(lax.shift_right_logical(tok, 4), 4), 16)
        return pl.ds(base, 16), lax.broadcasted_iota(i32, (16, D), 0) == tok - base

    def token_row(tok):
        rows, hit = slab_of(tok)
        slab = jnp.where(hit, hn_v[rows, :].astype(f32), 0.0)
        return _allred8(slab[0:8] + slab[8:16], jnp.add)

    def phase2(i, carry):
        q0 = CPT * i
        off = [pl.multiple_of(ord_s[q0 + k], C) for k in range(CPT + 1)]
        zm = zv[...]
        hprev = hbuf[...]
        kmask = lax.broadcasted_iota(i32, (64, 128), 0) // 32 == lax.broadcasted_iota(i32, (64, 128), 1) % 2

        def attend(y):
            os_ = []
            for p, yp in _pair_logits(y, range(4)).items():
                os_.append(_dot(jnp.where(kmask, kv_acc[p], 0.0).astype(bf16), _phi_q(yp, zb_v[p])))
            return jnp.concatenate(os_, axis=0).astype(bf16).T

        ya, ys = [], []
        for n in range(CPT):
            xt = xn(off[n + 1], C)
            ya.append(_dot_nt(_un(wq_v[:, 0:D // 2]), xt[:, 0:D // 2]))
            if n == CPT - 1:
                o01 = attend(jnp.concatenate(ys[0:2], axis=1))
            ys.append(ya[n] + _dot_nt(_un(wq_v[:, D // 2:D]), xt[:, D // 2:D]))
        wo = jnp.concatenate([_un(wo32[j]) for j in range(D // 128)], axis=1)
        head = _dot(o01[0:C], wo[:, 0:256])
        o23 = attend(jnp.concatenate(ys[2:4], axis=1))
        atts = [jnp.concatenate([head, _dot(o01[0:C], wo[:, 256:])], axis=1),
                _dot(o01[C:2 * C], wo), _dot(o23[0:C], wo), _dot(o23[C:2 * C], wo)]

        def q_gate(v):
            lens = [KR // 8] + [KR // 8 - 24] * 3
            t, n = int(v * sum(lens)), 0
            while t >= lens[n]:
                t -= lens[n]
                n += 1
            r0 = 8 * (t + KR // 8 - lens[n])
            return _zero_after(ya[n][r0:r0 + 8], zm)

        def o_gate(t):
            r0, j = 8 * (t % 16), (t % 128) // 16
            return _zero_after(atts[t // 128][r0:r0 + 8, 128 * j:128 * j + 128], zm)

        t3 = jnp.maximum(i - 1, 0)
        nsb = NA // 2
        for sb in range(nsb):
            cols = slice(256 * sb, 256 * (sb + 1))
            xcol = xc_v[...]
            acc = None
            for k in range(0, D, 8):
                xk = _lanes(xcol[k:k + 8], 2)
                p = jnp.concatenate([wg_v[t3, k:k + 8, cols].astype(f32) * xk,
                                     wu_v[t3, k:k + 8, cols].astype(f32) * xk], axis=1)
                if k % 64 == 0:
                    p = p + _lanes(q_gate((sb * D + k) / (nsb * D)), 4)
                acc = p if acc is None else acc + p
            pa_v[:, 512 * sb:512 * (sb + 1)] = acc

        put_cols(r_v, i, 0, jnp.where(i > 0, ln2(hprev, off[0], atts[0], 6), -jnp.inf))

        @pl.when(i > 0)
        def _():
            cp_out(q0).start()

        acc = _allred8(pa_v[pl.ds(pl.multiple_of(zs[3, 0].astype(i32) * 32, 32), 8), :], jnp.add)
        g_ = jnp.concatenate([acc[:, 512 * t:512 * t + 256] for t in range(nsb)], axis=1)
        u_ = jnp.concatenate([acc[:, 512 * t + 256:512 * t + 512] for t in range(nsb)], axis=1)
        a8 = g_ * jax.nn.sigmoid(g_) * u_
        ac = _col(jnp.concatenate([jnp.where(t3 == 2, 0.0, a8[:, 0:NDUP]), a8[:, NDUP:]], axis=1))
        for q in range(2):
            cols = slice(D // 2 * q, D // 2 * (q + 1))
            ysum = jnp.where(i > 1, y_v[:, cols], 0.0)
            for k in range(0, NA * 128, 8):
                p = wd_v[t3, k:k + 8, cols].astype(f32) * _lanes(ac[k:k + 8], 4)
                if k % 32 == 0:
                    p = p + _lanes(o_gate(64 + (q * NA * 128 + k) * 376 // (2 * NA * 128)), 4)
                ysum = ysum + p
            y_v[:, cols] = ysum

        for k in range(CPT):
            if k == NCAND:
                ok = (lane >= C // 8) & (lane < (NCAND + 1) * (C // 8))
                cm, cpos = _first_max(jnp.where(ok, r_v[0], -jnp.inf), pos)
                cand = token_at(cpos, C, (NCAND + 1) * C)
                ord_s[NC + 1] = cand
                sg_v[...] = jax.nn.sigmoid(jnp.broadcast_to(cm, (8, 128)))
                xc_v[...] = _col(token_row(cand))
            h = x_v[pl.ds(off[k + 1], C), :].astype(f32) + atts[k]
            if k == CPT - 1:
                hbuf[...] = h
            else:
                put_cols(r_v, i, (k + 1) * (C // 8), ln2(h, off[k + 1], atts[k + 1], 5 if k == CPT - 2 else 6))
                cp_out(q0 + k + 1).start()
        return carry

    lax.fori_loop(0, NT, phase2, 0)

    for q in range(1, NCAND + 1):
        cp_out(q).wait()
    fsem = new_sems(1)

    def patch(tok, y8, sg):
        rows, hit = slab_of(tok)
        cur = out_v[rows, :].astype(f32)
        fix_v[...] = jnp.where(hit, cur + _rows(y8 * _lanes(sg, D // 128), 2), cur).astype(bf16)
        return pltpu.make_async_copy(fix_v, out_hbm.at[0, rows], sems.at[fsem])

    cand = ord_s[NC + 1]
    cp_fix = patch(cand, _allred8(y_v[...], jnp.add), sg_v[...])
    cp_fix.start()
    last = pl.multiple_of(ord_s[NC], C)
    stats, cp_last = [], []
    for g in range(0, C, EG):
        h = hbuf[g:g + EG, :]
        s1 = h[:, 0:128]
        s2 = s1 * s1
        for j in range(128, D, 128):
            s1 = s1 + h[:, j:j + 128]
            s2 = s2 + h[:, j:j + 128] * h[:, j:j + 128]
        m = jnp.sum(s1, axis=-1, keepdims=True) * (1.0 / D)
        v = jnp.sum(s2, axis=-1, keepdims=True) * (1.0 / D) - m * m
        rs = lax.rsqrt(jnp.maximum(v, 0.0) + EPS)
        stats.append((m, rs))
        rows = pl.ds(pl.multiple_of(last + g, EG), EG)
        out_v[rows, :] = (h * (1.0 + rs) - m * rs).astype(bf16)
        cp_last.append(cp(out_v.at[rows], out_hbm.at[0, rows]))
        cp_last[-1].start()
    for q in range(NCAND + 1, NC - 1):
        cp_out(q).wait()
    pm, pi = _first_max(*_merge_max([(r_v[i], pos + float(i * T) if i else pos) for i in range(NT)]))
    wr = wr_row()
    wsum = jnp.sum(wr, axis=-1, keepdims=True)
    sub = lax.broadcasted_iota(i32, (8, 1), 0).astype(f32)
    cands = []
    for g, (m, rs) in zip(range(0, C, EG), stats):
        r = (jnp.sum(hbuf[g:g + EG, :] * wr, axis=-1, keepdims=True) - m * wsum) * rs
        cands += [(r[k:k + 8], sub + float(S + g + k)) for k in range(0, EG, 8)]
    while len(cands) > 1:
        cands = [_merge_max(cands[k:k + 2]) for k in range(0, len(cands), 2)]
    bv, bt = [jnp.broadcast_to(v, (8, 128)) for v in _merge_max([(pm, pi), cands[0]])]
    rmax = _allred8(bv, jnp.maximum)
    idx = token_at(_allred8(jnp.where(bv == rmax, bt, float(2 * S)), jnp.minimum), C, S + C)
    cp_out(NC - 1).wait()
    cp_fix.wait()
    for c in cp_last:
        c.wait()

    @pl.when(idx != cand)
    def _():
        rows, _ = slab_of(cand)
        undo = pltpu.make_async_copy(out_v.at[rows], out_hbm.at[0, rows], sems.at[fsem])
        undo.start()
        hn_v[pl.ds(last, C), :] = _ln(hbuf[...]).astype(bf16)
        xs = _rows(token_row(idx), 2).astype(bf16)

        def step(j, acc):
            t = lax.shift_right_logical(j, 1)
            cols = pl.ds(pl.multiple_of((j & 1) * (NA * 64), 128), NA * 64)
            g = _dot(xs, wg_v[t, :, cols])
            a = g * jax.nn.sigmoid(g) * _dot(xs, wu_v[t, :, cols])
            a = jnp.concatenate([jnp.where(j == 4, 0.0, a[:, 0:NDUP]), a[:, NDUP:]], axis=1)
            return acc + _dot(a.astype(bf16), wd_v[t, cols, :])[0:8]

        y8 = lax.fori_loop(0, 6, step, jnp.zeros((8, D), f32))
        undo.wait()
        redo = patch(idx, y8, jax.nn.sigmoid(rmax))
        redo.start()
        redo.wait()


@jax.jit
def pallas_sequential_preLN__linear_kernel_hedgehog__moe_arch_mod__prompt_kernel(
    A_x: jax.Array,
    A_wqkv: jax.Array,
    A_w_phi: jax.Array,
    A_wo: jax.Array,
    B_x: jax.Array,
    B_w_r: jax.Array,
    B_w_gate: jax.Array,
    B_w_up: jax.Array,
    B_w_down: jax.Array,
):
    del B_x
    any_spec = pl.BlockSpec(memory_space=pl.ANY)
    return pl.pallas_call(
        _kernel,
        out_shape=jax.ShapeDtypeStruct((1, S, D), bf16),
        in_specs=[any_spec] * 8,
        out_specs=any_spec,
        scratch_shapes=[
            pltpu.VMEM((S, D), bf16),
            pltpu.VMEM((D, 3 * D), bf16),
            pltpu.VMEM((D // 128, D, 128), bf16),
            pltpu.VMEM((H, DH, DH), bf16),
            pltpu.VMEM((N1 * GO, D, 128), bf16),
            pltpu.VMEM((N1 * GO, D // 2, 128), u32),
            pltpu.VMEM((D,), bf16),
            pltpu.VMEM((3, D, NA * 128), bf16),
            pltpu.VMEM((3, D, NA * 128), bf16),
            pltpu.VMEM((3, NA * 128, D), bf16),
            pltpu.VMEM(((KR + D) // 2, D), u32),
            pltpu.VMEM((KR // 2, D), u32),
            pltpu.VMEM((8, 64, 128), u32),
            pltpu.VMEM(((S + C) // 2, D), u32),
            pltpu.VMEM((S + C, D), bf16),
            pltpu.VMEM((NP, 64, 128), f32),
            pltpu.VMEM((NP, 128, 128), f32),
            pltpu.VMEM((NP, 128, 128), f32),
            pltpu.VMEM((C, D), f32),
            pltpu.VMEM((S + C, D), bf16),
            pltpu.VMEM((8, 128), u32),
            pltpu.SMEM((8, 128), u32),
            pltpu.VMEM((1 + N1, 8, 128), f32),
            pltpu.VMEM((NT, 8, 128), f32),
            pltpu.VMEM((D, 128), f32),
            pltpu.VMEM((8, NA * 256), f32),
            pltpu.VMEM((8, D), f32),
            pltpu.VMEM((8, 128), f32),
            pltpu.VMEM((16, D), bf16),
            pltpu.SMEM((NC + 2,), i32),
            pltpu.SemaphoreType.DMA((64,)),
        ],
        compiler_params=pltpu.CompilerParams(vmem_limit_bytes=120 * 1024 * 1024,
                                             disable_bounds_checks=True,
                                             disable_semaphore_checks=True),
        name="hedgehog_mod",
    )(A_x, A_wqkv, A_w_phi, A_wo, B_w_r, B_w_gate, B_w_up, B_w_down)
```

```python
import jax
import jax.numpy as jnp
from jax import lax
import jax.experimental.pallas as pl
import jax.experimental.pallas.tpu as pltpu

S = 2048
D = 1024
H = 32
DH = 32
F = 3584
NP = H // 2
C = 128
NC = S // C
T = 512
NT = S // T
CPT = T // C
T1 = 512
N1 = (S - T) // T1
CP1 = T1 // C
KR = H * (DH - 1)
GO = -(-8 // N1)
SEGS = ((256, 256), (128, 256), (128, 512))
PHI = ((0, 512), (512, 512), (512, 1024))
DEFER = 2
NB = F // 128
NA = 10
B0 = (0, NA, NB - NA)
NDUP = (3 * NA - NB) * 128
NCAND = 2
EG = 16
LOG2E = 1.4426950408889634
EPS = 1e-5

f32 = jnp.float32
bf16 = jnp.bfloat16
u32 = jnp.uint32
i32 = jnp.int32


def _dot_nt(a, b):
    return lax.dot_general(a, b, (((1,), (1,)), ((), ())), preferred_element_type=f32)


def _dot(a, b):
    return jnp.dot(a, b, preferred_element_type=f32)


def _pk(x):
    return pltpu.bitcast(x, u32)


def _un(x):
    return pltpu.bitcast(x, bf16)


def _rcp(x):
    r = pl.reciprocal(x, approx=True)
    return r * (2.0 - x * r)


def _allred(v, op):
    v = op(v, pltpu.roll(v, 2, 0))
    return op(v, pltpu.roll(v, 4, 0))


def _allred8(v, op):
    return _allred(op(v, pltpu.roll(v, 1, 0)), op)


def _rows(v, n):
    return jnp.concatenate([v] * n, axis=0)


def _lanes(v, n):
    return jnp.concatenate([v] * n, axis=1)


def _zero_after(dep, zm):
    return pltpu.bitcast(pltpu.bitcast(dep, u32) & zm, f32)


def _exps(x):
    x3 = x.reshape(8, 8, x.shape[1])
    mx = _allred(jnp.max(x3, axis=0), jnp.maximum)
    mn = _allred(jnp.min(x3, axis=0), jnp.minimum)
    ep = jnp.exp2(x3 - mx[None])
    en = jnp.exp2(mn[None] - x3)
    rp = _rcp(_allred(jnp.sum(ep, axis=0), jnp.add))
    rn = _rcp(_allred(jnp.sum(en, axis=0), jnp.add))
    return ep, en, rp, rn


def _phi_k(x):
    L = x.shape[1]
    ep, en, rp, rn = _exps(x)
    return jnp.concatenate([(ep * rp[None]).reshape(64, L), (en * rn[None]).reshape(64, L)], axis=0)


def _phi_q(x, zb):
    L = x.shape[1]
    ep, en, rp, rn = _exps(x)
    zb = _lanes(zb, L // 128).reshape(16, 8, L)
    den = rp * jnp.sum(ep * zb[0:8], axis=0) + rn * jnp.sum(en * zb[8:16], axis=0)
    inv = _rcp(_allred(den, jnp.add) + 1e-6)
    cp = rp * inv
    cn = rn * inv
    phi = jnp.concatenate([(ep * cp[None]).reshape(64, L), (en * cn[None]).reshape(64, L)], axis=0)
    return phi.astype(bf16)


def _slot(n):
    return lax.shift_right_logical(lax.broadcasted_iota(i32, (8, n), 0), 1)


def _pair_logits(y, sgs):
    slot = _slot(y.shape[1])
    out, r, shared = {}, 0, None
    for k, sg in enumerate(sgs):
        if k == 0 or sg % 2 == 0:
            shared, r = y[r:r + 16], r + 16
        l0, l1, l2 = y[r:r + 8], y[r + 8:r + 16], shared[8 * (sg % 2):8 * (sg % 2) + 8]
        for q in range(4):
            x0 = jnp.where(slot == q, l0, jnp.where(slot == (q + 1) % 4, l1, jnp.where(slot == (q + 2) % 4, l2, 0.0)))
            out[4 * sg + q] = jnp.concatenate([x0, y[r + 16 + 56 * q:r + 72 + 56 * q]], axis=0)
        r += 240
    return out


def _lane_blocks_sum(v, acc):
    for c in range(0, v.shape[1], 128):
        acc = acc + v[:, c:c + 128]
    return acc


def _row_sum(x, deps, zm):
    g = x.shape[0] // len(deps)
    gate = jnp.concatenate([jnp.zeros((8, 128), f32) if d is None else _zero_after(d, zm)
                            for d in deps for _ in range(g // 8)], axis=0)
    return jnp.sum(_lane_blocks_sum(x[:, 128:], x[:, 0:128] + gate), axis=-1, keepdims=True)


def _ln(x, deps=None, zm=None):
    tot = jnp.sum(x, axis=-1, keepdims=True) if deps is None else _row_sum(x, deps, zm)
    xc = x - tot * (1.0 / D)
    return xc * lax.rsqrt(jnp.sum(xc * xc, axis=-1, keepdims=True) * (1.0 / D) + EPS)


def _col(a8):
    return _rows(a8, 16).astype(bf16).T.astype(f32)


def _first_max(v, t):
    m = jnp.max(_allred8(v, jnp.maximum), axis=1, keepdims=True)
    return m, jnp.min(_allred8(jnp.where(v == m, t, float(2 * S)), jnp.minimum), axis=1, keepdims=True)


def _merge_max(cands):
    v, t = cands[0]
    for v2, t2 in cands[1:]:
        gt = v2 > v
        v, t = jnp.where(gt, v2, v), jnp.where(gt, t2, t)
    return v, t


def _scalar(v, lo, hi):
    return jnp.clip(jnp.broadcast_to(v, (8, 128)).astype(i32)[0, 0], lo, hi)


class _Group:
    def __init__(self, parts, dst, sem):
        self.parts, self.dst, self.sem = parts, dst, sem

    def start(self):
        for src, dst in self.parts:
            pltpu.make_async_copy(src, dst, self.sem).start()

    def wait(self):
        pltpu.make_async_copy(self.dst, self.dst, self.sem).wait()


def _kernel(x_hbm, wqkv_hbm, wphi_hbm, wo_hbm, wr_hbm, wg_hbm, wu_hbm, wd_hbm, out_hbm,
            x_v, wkv_v, wqb_v, wphi_v, wo_v, wo32, wr_v, wg_v, wu_v, wd_v,
            wt_v, wq_v, a_v, xn_v, hn_v, kv_acc, z_acc, zb_v, hbuf, out_v, zv, zs, p_v, r_v,
            xc_v, pa_v, y_v, fix_v, ord_s, sems):
    nsem = [0]

    def new_sems(n):
        nsem[0] += n
        return nsem[0] - n

    def cp(src, dst):
        return pltpu.make_async_copy(src, dst, sems.at[new_sems(1)])

    def cp_w(lo, hi):
        return cp(wqkv_hbm.at[:, lo:hi], wkv_v.at[:, lo:hi])

    def cp_x(lo, hi):
        return cp(x_hbm.at[0, lo:hi], x_v.at[lo:hi])

    cp_wr = cp(wr_hbm, wr_v)
    kcum = [0]
    for _, dk in SEGS:
        kcum.append(kcum[-1] + dk)
    seg_cp = []
    x0 = 0
    for si, (dx, dk) in enumerate(SEGS):
        lo, hi = PHI[si][0] // DH, PHI[si][1] // DH
        ph = [cp(wphi_hbm.at[lo:hi], wphi_v.at[lo:hi])] if hi > lo else []
        seg_cp.append([cp_x(x0, x0 + dx)] + ph + [cp_w(D + kcum[si], D + kcum[si + 1])])
        x0 += dx
    cp_wv = cp_w(2 * D, 3 * D)
    cp_x1a = cp_x(T, T + C)
    cp_x1 = cp_x(T + C, S)
    cp_q0 = _Group([(wqkv_hbm.at[:, 128 * g:128 * (g + 1)], wqb_v.at[g]) for g in range(2)],
                   wqb_v.at[0:2], sems.at[new_sems(1)])
    qsem0 = new_sems(2 * N1)

    def cp_step(j):
        pq = po = None
        if isinstance(j, int):
            pq = [(wqkv_hbm.at[:, 128 * g:128 * (g + 1)], wqb_v.at[g]) for g in range(2 + 2 * j, 4 + 2 * j)]
            po = [(wo_hbm.at[:, 128 * min(g, 7):128 * (min(g, 7) + 1)], wo_v.at[g])
                  for g in range(GO * j, GO * (j + 1))]
        return [_Group(pq, wqb_v.at[pl.ds(2 + 2 * j, 2)], sems.at[qsem0 + 2 * j]),
                _Group(po, wo_v.at[pl.ds(GO * j, GO)], sems.at[qsem0 + 2 * j + 1])]

    cp_ffn = []
    for t, b in enumerate(B0):
        cp_ffn += [cp(wg_hbm.at[:, b * 128:(b + NA) * 128], wg_v.at[t]),
                   cp(wu_hbm.at[:, b * 128:(b + NA) * 128], wu_v.at[t]),
                   cp(wd_hbm.at[b * 128:(b + NA) * 128], wd_v.at[t])]
    seg_cp[0] = seg_cp[0][1:] + seg_cp[0][0:1]
    for c in ([c for t in seg_cp for c in t] + [cp_wr, cp_wv, cp_x1a, cp_q0, cp_x1]
              + [c for j in range(N1) for c in cp_step(j)] + cp_ffn):
        c.start()
    osem0 = new_sems(NC + 1)

    def cp_out(q):
        rows = pl.ds(pl.multiple_of(ord_s[q], C), C)
        return pltpu.make_async_copy(out_v.at[rows], out_hbm.at[0, rows], sems.at[osem0 + q])

    def wr_row():
        return wr_v[...].reshape(1, D).astype(f32)

    def put_cols(ref, idx, col0, r):
        for k in range(0, r.shape[0], 8):
            ref[idx, :, col0 + k // 8:col0 + k // 8 + 1] = r[k:k + 8]

    def half(row0, n):
        if isinstance(row0, int):
            return pl.ds(row0 // 2, n // 2)
        return pl.ds(pl.multiple_of(lax.shift_right_logical(row0, 1), C // 2), n // 2)

    def ln1(src, dst, n, deps=None):
        xb = _pk(_ln(x_v[pl.ds(src, n), :].astype(f32), deps, None if deps is None else zv[...]).astype(bf16))
        xn_v[half(dst, n), :] = xb
        return _un(xb)

    def xn(row0, n):
        return _un(xn_v[half(row0, n), :])

    def predict(rows, t, c, deps):
        wr = wr_row()
        wc = wr - jnp.sum(wr, axis=-1, keepdims=True) * (1.0 / D)
        put_cols(p_v, t, c * (C // 8), _row_sum(x_v[rows, :].astype(f32) * wc, deps, zv[...]))

    def fold(dst, ws, sg):
        slot = _slot(D)
        res = [_dot_nt(_un(a_v[2 * sg + e]), ws[e]) for e in range(2)]
        main, e0, e1 = [], [], []
        for e in range(2):
            z = jnp.where(((slot + 3) % 4) // 2 == e, 0.0, res[e][0:8])
            b1 = z + pltpu.roll(z, 4, 0)
            b0 = pltpu.roll(b1, 2, 0)
            for pp in range(2):
                base = jnp.where(slot % 2 == pp, b0, b1)
                main.append((res[e][16 + 56 * pp:72 + 56 * pp].reshape(7, 8, D) - base[None]).reshape(56, D))
            e0.append(res[e][8:16] - b0)
            e1.append(res[e][0:8] - b1)
        rows = jnp.concatenate([jnp.where(slot < 2, e0[0], e0[1]), e1[0] + e1[1]] + main, axis=0)
        l2 = _pk((_rows(jnp.where(slot < 2, e0[1], e0[0]), 2) * LOG2E).astype(bf16))
        if isinstance(sg, int):
            r0, r1 = 248 * (sg // 2), 248 * (sg // 2) + 8 + 120 * (sg % 2)
        else:
            r0 = pl.multiple_of(248 * lax.shift_right_logical(sg, 1), 8)
            r1 = pl.multiple_of(r0 + 8 + 120 * (sg & 1), 8)
        dst[pl.ds(r1, 120), :] = _pk((rows * LOG2E).astype(bf16))
        dst[pl.ds(r0, 8), :] = jnp.where(slot // 2 == sg % 2, l2, dst[pl.ds(r0, 8), :])
        return res

    def wk(lo, hi):
        r0, r1 = 248 * (lo // 2), 248 * ((hi - 1) // 2) + 128 + 120 * ((hi - 1) % 2)
        if lo % 2:
            return _un(jnp.concatenate([wt_v[r0:r0 + 8, :], wt_v[r0 + 128:r1, :]], axis=0))
        return _un(wt_v[r0:r1, :])

    def kv_and_z(vt, phis, z_of, tail, zm):
        lag = 4
        kvs, zs_ = [], []
        for p in range(NP):
            kvs.append(_dot_nt(vt[64 * p:64 * (p + 1)].astype(bf16), phis[p].astype(bf16)))
            dep = kvs[p - lag][0:8] if p >= lag else tail[D - 64 * (lag - p):D - 64 * (lag - p) + 8]
            zs_.append(_lane_blocks_sum(phis[p], z_of(p, _rows(_zero_after(dep, zm), 16))))
        return kvs, zs_

    def a_row(r, e):
        s = (r & 7) >> 1
        f = jnp.where(r >= 72, (r - 64) >> 1, jnp.where(r >= 16, (r - 8) >> 1, jnp.where(
            r >= 8, jnp.where(s >> 1 == e, 1, 3), jnp.where(((s + 3) & 3) >> 1 == e, 2, 0))))
        pp = jnp.where(r >= 72, 1, jnp.where(r >= 16, 0, jnp.where(r >= 8, s, s + 1) & 1))
        return f, 2 * pp + (r & 1)

    f_i = lax.broadcasted_iota(i32, (128, DH), 1)
    sel = [jnp.where(f_i == a_row(lax.broadcasted_iota(i32, (128, DH), 0), e)[0], 1.0, 0.0).astype(bf16)
           for e in range(2)]
    amask = jnp.where(lax.broadcasted_iota(i32, (128, 128), 1) >> 5
                      == a_row(lax.broadcasted_iota(i32, (128, 128), 0), 0)[1], jnp.uint32(0xFFFFFFFF), jnp.uint32(0))

    def build_a(lo, hi):
        for g in range(lo // 128, hi // 128):
            blk = _dot_nt(sel[g % 2], wphi_v[4 * g:4 * (g + 1)].reshape(128, DH))
            a_v[g] = _pk(pltpu.bitcast(pltpu.bitcast(blk, u32) & amask, f32).astype(bf16))

    zv[...] = jnp.zeros((8, 128), u32)
    cp_z = cp(zv, zs)
    cp_z.start()
    for ref in (wt_v, wq_v):
        for r0 in (0, 248):
            ref[r0:r0 + 8, :] = jnp.zeros((8, D), u32)
    hbuf[...] = jnp.zeros(hbuf.shape, f32)
    xc_v[...] = jnp.zeros(xc_v.shape, f32)
    y_v[...] = jnp.zeros(y_v.shape, f32)
    r_v[...] = jnp.full(r_v.shape, -jnp.inf, f32)
    p_v[...] = jnp.full(p_v.shape, -jnp.inf, f32)

    pieces = [[] for _ in range(NP)]
    pending = []

    def phi_piece(p, t0, yp, dep=None):
        if dep is not None:
            yp = jnp.concatenate([yp[0:8] + _zero_after(dep, zv[...]), yp[8:]], axis=0)
        pieces[p].append((t0, _phi_k(yp)))

    def k_block(lo, hi, t0, t1, defer=0):
        y = _dot_nt(wk(lo, hi), xn(t0, t1 - t0))
        for p, yp in _pair_logits(y, range(lo, hi)).items():
            if p >= 4 * hi - defer:
                if t1 - t0 > C:
                    phi_piece(p, t0, yp[:, 0:t1 - t0 - C])
                pending.append((p, t1 - C, yp[:, t1 - t0 - C:]))
            else:
                phi_piece(p, t0, yp)
        return y

    def flush(res):
        for k, (p, t0, yp) in enumerate(pending):
            phi_piece(p, t0, yp, res[32 * k:32 * k + 8, 0:128])
        del pending[:]

    x0 = 0
    for si, (dx, dk) in enumerate(SEGS):
        k0, k1 = kcum[si] // 256, kcum[si + 1] // 256
        if si == 0:
            seg_cp[0][0].wait()
            build_a(*PHI[0])
            seg_cp[0][1].wait()
        else:
            for c in seg_cp[si]:
                c.wait()
            if PHI[si][1] > PHI[si][0]:
                build_a(*PHI[si])
        res = [fold(wt_v, [wkv_v[:, D + 128 * g:D + 128 * (g + 1)] for g in (2 * sg, 2 * sg + 1)], sg)
               for sg in range(k0, k1)]
        flush(res[0][0])
        if si == 0:
            seg_cp[0][2].wait()
        ln1(x0, x0, dx)
        if si:
            k_block(k0, k1, 0, x0)
        k_block(0, k1, x0, x0 + dx, DEFER)
        x0 += dx
    for c in (cp_wv, cp_x1a, cp_q0, cp_wr, cp_z):
        c.wait()
    for g in range(D // 128):
        wt_v[KR // 2 + 64 * g:KR // 2 + 64 * (g + 1), :] = _pk(wkv_v[:, 2 * D + 128 * g:2 * D + 128 * (g + 1)].T)
    flush(fold(wq_v, [wqb_v[0], wqb_v[1]], 0)[0])
    yv = _dot_nt(_un(wt_v[KR // 2:, :]), xn(0, T))
    ln1(T, T, C, [yv[128 * k:128 * k + 8, 128:256] for k in range(8)])
    for c in range(CPT):
        predict(slice(C * c, C * (c + 1)), 0, c,
                [yv[256 * c + 32 * k:256 * c + 32 * k + 8, 256:384] for k in range(8)])
    phis = [jnp.concatenate([ph for _, ph in sorted(pieces[p], key=lambda tp: tp[0])], axis=1) for p in range(NP)]
    kvs, zs_ = kv_and_z(yv, phis, lambda p, zero: zero, yv[:, T - C:T], zv[...])
    for p in range(NP):
        kv_acc[p] = kvs[p]
        z_acc[p] = zs_[p]
    cp_x1.wait()

    def order_chunks():
        lane16 = lax.shift_right_logical(lax.broadcasted_iota(i32, (8, 128), 1), 4).astype(f32)
        vals = [p_v[t] for t in range(1 + N1)]
        cids = [lane16 + float(0 if t == 0 else CPT + CP1 * (t - 1)) for t in range(1 + N1)]
        b1 = _first_max(*_merge_max(list(zip(vals, cids))))[1]
        b2 = _first_max(*_merge_max([(jnp.where(c == b1, -jnp.inf, v), c) for v, c in zip(vals, cids)]))[1]
        c1, c2 = _scalar(b1, 0, NC - 1), _scalar(b2, 0, NC - 1)
        c2 = jnp.where(c2 == c1, (c1 + 1) & (NC - 1), c2)
        ord_s[0] = S
        for c in range(NC):
            ord_s[1 + c] = c * C
        ord_s[1 + c1] = 0
        ord_s[1] = c1 * C
        ord_s[1 + jnp.where(c2 == 0, c1, c2)] = jnp.where(c1 == 1, 0, C)
        ord_s[2] = c2 * C

    def phase1(j, carry):
        for c in cp_step(j):
            c.wait()
        zm = zv[...]
        s = pl.multiple_of(T + j * T1, C)
        nxt = pl.multiple_of(jnp.where(j + 1 < N1, s + T1, 0), C)
        xt = xn(s, C)
        ys, ph = [], []
        for n in range(CP1):
            if n + 1 < CP1:
                row0 = pl.multiple_of(s + C * (n + 1), C)
                xt1 = ln1(row0, row0, C)
                yn = _dot_nt(_un(wt_v[...]), xt)
                xt = xt1
            else:
                ya = _dot_nt(_un(wt_v[:, 0:D // 2]), xt[:, 0:D // 2])
                for c in range(CP1):
                    r0, st = 384 + 1280 * c // CP1 // 8 * 8, 1280 // CP1 // 64 * 8
                    predict(pl.ds(pl.multiple_of(s + C * c, C), C), 1 + j, c,
                            [ya[r0 + st * k:r0 + st * k + 8] for k in range(8)])
                order_chunks()
                yn = ya + _dot_nt(_un(wt_v[:, D // 2:D]), xt[:, D // 2:D])
            ys.append(yn)
            ph.append([_phi_k(yp) for yp in _pair_logits(yn[0:KR], range(4)).values()])
            if n == CP1 - 2:
                ln1(nxt, pl.multiple_of(s + T1, C), C,
                    [yn[KR + 512 + 64 * k:KR + 520 + 64 * k] for k in range(8)])
        fold(wq_v, [wqb_v[2 + 2 * j], wqb_v[3 + 2 * j]], 1 + j)
        for e in range(4 * GO):
            row = KR + 384 + 640 * e // (4 * GO) // 8 * 8
            w = _pk(wo_v[GO * j + e // 4, 256 * (e % 4):256 * (e % 4 + 1), :])
            wo32[GO * j + e // 4, 128 * (e % 4):128 * (e % 4 + 1), :] = (
                w.reshape(16, 8, 128) | (_pk(ys[0][row:row + 8]) & zm)[None]).reshape(128, 128)
        vt = jnp.concatenate([yn[KR:] for yn in ys], axis=1)
        phis = [jnp.concatenate([ph[n][p] for n in range(CP1)], axis=1) for p in range(NP)]
        kvs, zs_ = kv_and_z(vt, phis, lambda p, zero: z_acc[p] + zero, ys[-1][KR:], zm)
        for p in range(NP):
            kv_acc[p] += kvs[p]
            z_acc[p] = zs_[p]
            zb_v[p] = jnp.broadcast_to(jnp.sum(zs_[p], axis=1, keepdims=True), (128, 128))
        return carry

    lax.fori_loop(0, N1, phase1, 0)
    for c in cp_ffn:
        c.wait()

    def ln2(h, row0, nx, nrel):
        deps = [None]
        for j in range(1, C // 8):
            t = (j * nrel * 2) // (C // 8) - 1
            r0 = (C - 8) * (t % 2)
            deps.append(nx[r0:r0 + 8, 128 * (t // 2):128 * (t // 2) + 128] if t >= 0 else None)
        hn = _ln(h, deps, zv[...])
        r = jnp.sum(hn * wr_row(), axis=-1, keepdims=True)
        hn_v[pl.ds(row0, C), :] = hn.astype(bf16)
        out_v[pl.ds(row0, C), :] = (h + hn).astype(bf16)
        return r

    lane = lax.broadcasted_iota(i32, (8, 128), 1)
    pos = (lane * 8 + lax.broadcasted_iota(i32, (8, 128), 0)).astype(f32)

    def token_at(posv, lo, hi):
        p = _scalar(posv, lo, hi - 1)
        return ord_s[lax.shift_right_logical(p, 7)] + (p & (C - 1))

    def slab_of(tok):
        base = pl.multiple_of(lax.shift_left(lax.shift_right_logical(tok, 4), 4), 16)
        return pl.ds(base, 16), lax.broadcasted_iota(i32, (16, D), 0) == tok - base

    def token_row(tok):
        rows, hit = slab_of(tok)
        slab = jnp.where(hit, hn_v[rows, :].astype(f32), 0.0)
        return _allred8(slab[0:8] + slab[8:16], jnp.add)

    def patch(tok, y8, sg):
        rows, hit = slab_of(tok)
        cur = out_v[rows, :].astype(f32)
        fix_v[...] = jnp.where(hit, cur + _rows(y8 * _lanes(sg, D // 128), 2), cur).astype(bf16)

    def phase2(i, carry):
        q0 = CPT * i
        off = [pl.multiple_of(ord_s[q0 + k], C) for k in range(CPT + 1)]
        zm = zv[...]
        hprev = hbuf[...]
        kmask = lax.broadcasted_iota(i32, (64, 128), 0) // 32 == lax.broadcasted_iota(i32, (64, 128), 1) % 2

        def attend(y):
            os_ = []
            for p, yp in _pair_logits(y, range(4)).items():
                os_.append(_dot(jnp.where(kmask, kv_acc[p], 0.0).astype(bf16), _phi_q(yp, zb_v[p])))
            return jnp.concatenate(os_, axis=0).astype(bf16).T

        ya, ys = [], []
        for n in range(CPT):
            xt = xn(off[n + 1], C)
            ya.append(_dot_nt(_un(wq_v[:, 0:D // 2]), xt[:, 0:D // 2]))
            if n == CPT - 1:
                o01 = attend(jnp.concatenate(ys[0:2], axis=1))
            ys.append(ya[n] + _dot_nt(_un(wq_v[:, D // 2:D]), xt[:, D // 2:D]))
        wo = jnp.concatenate([_un(wo32[j]) for j in range(D // 128)], axis=1)
        head = _dot(o01[0:C], wo[:, 0:256])
        o23 = attend(jnp.concatenate(ys[2:4], axis=1))
        atts = [jnp.concatenate([head, _dot(o01[0:C], wo[:, 256:])], axis=1),
                _dot(o01[C:2 * C], wo), _dot(o23[0:C], wo), _dot(o23[C:2 * C], wo)]

        def q_gate(v):
            lens = [KR // 8] + [KR // 8 - 24] * 3
            t, n = int(v * sum(lens)), 0
            while t >= lens[n]:
                t -= lens[n]
                n += 1
            r0 = 8 * (t + KR // 8 - lens[n])
            return _zero_after(ya[n][r0:r0 + 8], zm)

        def o_gate(t):
            r0, j = 8 * (t % 16), (t % 128) // 16
            return _zero_after(atts[t // 128][r0:r0 + 8, 128 * j:128 * j + 128], zm)

        t3 = jnp.maximum(i - 1, 0)
        nsb = NA // 2
        for sb in range(nsb):
            cols = slice(256 * sb, 256 * (sb + 1))
            xcol = xc_v[...]
            acc = None
            for k in range(0, D, 8):
                xk = _lanes(xcol[k:k + 8], 2)
                p = jnp.concatenate([wg_v[t3, k:k + 8, cols].astype(f32) * xk,
                                     wu_v[t3, k:k + 8, cols].astype(f32) * xk], axis=1)
                if k % 64 == 0:
                    p = p + _lanes(q_gate((sb * D + k) / (nsb * D)), 4)
                acc = p if acc is None else acc + p
            pa_v[:, 512 * sb:512 * (sb + 1)] = acc

        put_cols(r_v, i, 0, jnp.where(i > 0, ln2(hprev, off[0], atts[0], 6), -jnp.inf))

        @pl.when(i > 0)
        def _():
            cp_out(q0).start()

        acc = _allred8(pa_v[pl.ds(pl.multiple_of(zs[3, 0].astype(i32) * 32, 32), 8), :], jnp.add)
        g_ = jnp.concatenate([acc[:, 512 * t:512 * t + 256] for t in range(nsb)], axis=1)
        u_ = jnp.concatenate([acc[:, 512 * t + 256:512 * t + 512] for t in range(nsb)], axis=1)
        a8 = g_ * jax.nn.sigmoid(g_) * u_
        ac = _col(jnp.concatenate([jnp.where(t3 == 2, 0.0, a8[:, 0:NDUP]), a8[:, NDUP:]], axis=1))
        ysums = []
        for q in range(2):
            cols = slice(D // 2 * q, D // 2 * (q + 1))
            ysum = jnp.where(i > 1, y_v[:, cols], 0.0)
            for k in range(0, NA * 128, 8):
                p = wd_v[t3, k:k + 8, cols].astype(f32) * _lanes(ac[k:k + 8], 4)
                if k % 32 == 0:
                    p = p + _lanes(o_gate(64 + (q * NA * 128 + k) * 376 // (2 * NA * 128)), 4)
                ysum = ysum + p
            y_v[:, cols] = ysum
            ysums.append(ysum)

        for k in range(CPT):
            if k == NCAND:
                ok = (lane >= C // 8) & (lane < (NCAND + 1) * (C // 8))
                cm, cpos = _first_max(jnp.where(ok, r_v[0], -jnp.inf), pos)
                cand = token_at(cpos, C, (NCAND + 1) * C)
                ord_s[NC + 1] = cand
                xc_v[...] = _col(token_row(cand))
                patch(cand, _allred8(jnp.concatenate(ysums, axis=1), jnp.add),
                      jax.nn.sigmoid(jnp.broadcast_to(cm, (8, 128))))
            h = x_v[pl.ds(off[k + 1], C), :].astype(f32) + atts[k]
            if k == CPT - 1:
                hbuf[...] = h
            else:
                put_cols(r_v, i, (k + 1) * (C // 8), ln2(h, off[k + 1], atts[k + 1], 5 if k == CPT - 2 else 6))
                cp_out(q0 + k + 1).start()
        return carry

    lax.fori_loop(0, NT, phase2, 0)

    for q in range(1, NCAND + 1):
        cp_out(q).wait()
    fsem = new_sems(1)

    cand = ord_s[NC + 1]

    def cp_patch(tok):
        return pltpu.make_async_copy(fix_v, out_hbm.at[0, slab_of(tok)[0]], sems.at[fsem])

    cp_fix = cp_patch(cand)
    cp_fix.start()
    cp_out(NCAND + 1).wait()
    last = pl.multiple_of(ord_s[NC], C)
    stats, cp_last = [], []
    for g in range(0, C, EG):
        h = hbuf[g:g + EG, :]
        s1 = h[:, 0:128]
        s2 = s1 * s1
        for j in range(128, D, 128):
            s1 = s1 + h[:, j:j + 128]
            s2 = s2 + h[:, j:j + 128] * h[:, j:j + 128]
        m = jnp.sum(s1, axis=-1, keepdims=True) * (1.0 / D)
        v = jnp.sum(s2, axis=-1, keepdims=True) * (1.0 / D) - m * m
        rs = lax.rsqrt(jnp.maximum(v, 0.0) + EPS)
        stats.append((m, rs))
        rows = pl.ds(pl.multiple_of(last + g, EG), EG)
        out_v[rows, :] = (h * (1.0 + rs) - m * rs).astype(bf16)
        cp_last.append(cp(out_v.at[rows], out_hbm.at[0, rows]))
        cp_last[-1].start()
    for q in range(NCAND + 2, NC - 1):
        cp_out(q).wait()
    pm, pi = _first_max(*_merge_max([(r_v[i], pos + float(i * T) if i else pos) for i in range(NT)]))
    wr = wr_row()
    wsum = jnp.sum(wr, axis=-1, keepdims=True)
    sub = lax.broadcasted_iota(i32, (8, 1), 0).astype(f32)
    cands = []
    for g, (m, rs) in zip(range(0, C, EG), stats):
        r = (jnp.sum(hbuf[g:g + EG, :] * wr, axis=-1, keepdims=True) - m * wsum) * rs
        cands += [(r[k:k + 8], sub + float(S + g + k)) for k in range(0, EG, 8)]
    while len(cands) > 1:
        cands = [_merge_max(cands[k:k + 2]) for k in range(0, len(cands), 2)]
    bv, bt = [jnp.broadcast_to(v, (8, 128)) for v in _merge_max([(pm, pi), cands[0]])]
    rmax = _allred8(bv, jnp.maximum)
    idx = token_at(_allred8(jnp.where(bv == rmax, bt, float(2 * S)), jnp.minimum), C, S + C)
    cp_out(NC - 1).wait()
    cp_fix.wait()
    for c in cp_last:
        c.wait()

    @pl.when(idx != cand)
    def _():
        rows, _ = slab_of(cand)
        undo = pltpu.make_async_copy(out_v.at[rows], out_hbm.at[0, rows], sems.at[fsem])
        undo.start()
        hn_v[pl.ds(last, C), :] = _ln(hbuf[...]).astype(bf16)
        xs = _rows(token_row(idx), 2).astype(bf16)

        def step(j, acc):
            t = lax.shift_right_logical(j, 1)
            cols = pl.ds(pl.multiple_of((j & 1) * (NA * 64), 128), NA * 64)
            g = _dot(xs, wg_v[t, :, cols])
            a = g * jax.nn.sigmoid(g) * _dot(xs, wu_v[t, :, cols])
            a = jnp.concatenate([jnp.where(j == 4, 0.0, a[:, 0:NDUP]), a[:, NDUP:]], axis=1)
            return acc + _dot(a.astype(bf16), wd_v[t, cols, :])[0:8]

        y8 = lax.fori_loop(0, 6, step, jnp.zeros((8, D), f32))
        undo.wait()
        patch(idx, y8, jax.nn.sigmoid(rmax))
        redo = cp_patch(idx)
        redo.start()
        redo.wait()


@jax.jit
def pallas_sequential_preLN__linear_kernel_hedgehog__moe_arch_mod__prompt_kernel(
    A_x: jax.Array,
    A_wqkv: jax.Array,
    A_w_phi: jax.Array,
    A_wo: jax.Array,
    B_x: jax.Array,
    B_w_r: jax.Array,
    B_w_gate: jax.Array,
    B_w_up: jax.Array,
    B_w_down: jax.Array,
):
    del B_x
    any_spec = pl.BlockSpec(memory_space=pl.ANY)
    return pl.pallas_call(
        _kernel,
        out_shape=jax.ShapeDtypeStruct((1, S, D), bf16),
        in_specs=[any_spec] * 8,
        out_specs=any_spec,
        scratch_shapes=[
            pltpu.VMEM((S, D), bf16),
            pltpu.VMEM((D, 3 * D), bf16),
            pltpu.VMEM((D // 128, D, 128), bf16),
            pltpu.VMEM((H, DH, DH), bf16),
            pltpu.VMEM((N1 * GO, D, 128), bf16),
            pltpu.VMEM((N1 * GO, D // 2, 128), u32),
            pltpu.VMEM((D,), bf16),
            pltpu.VMEM((3, D, NA * 128), bf16),
            pltpu.VMEM((3, D, NA * 128), bf16),
            pltpu.VMEM((3, NA * 128, D), bf16),
            pltpu.VMEM(((KR + D) // 2, D), u32),
            pltpu.VMEM((KR // 2, D), u32),
            pltpu.VMEM((8, 64, 128), u32),
            pltpu.VMEM(((S + C) // 2, D), u32),
            pltpu.VMEM((S + C, D), bf16),
            pltpu.VMEM((NP, 64, 128), f32),
            pltpu.VMEM((NP, 128, 128), f32),
            pltpu.VMEM((NP, 128, 128), f32),
            pltpu.VMEM((C, D), f32),
            pltpu.VMEM((S + C, D), bf16),
            pltpu.VMEM((8, 128), u32),
            pltpu.SMEM((8, 128), u32),
            pltpu.VMEM((1 + N1, 8, 128), f32),
            pltpu.VMEM((NT, 8, 128), f32),
            pltpu.VMEM((D, 128), f32),
            pltpu.VMEM((8, NA * 256), f32),
            pltpu.VMEM((8, D), f32),
            pltpu.VMEM((16, D), bf16),
            pltpu.SMEM((NC + 2,), i32),
            pltpu.SemaphoreType.DMA((64,)),
        ],
        compiler_params=pltpu.CompilerParams(vmem_limit_bytes=120 * 1024 * 1024,
                                             disable_bounds_checks=True,
                                             disable_semaphore_checks=True),
        name="hedgehog_mod",
    )(A_x, A_wqkv, A_w_phi, A_wo, B_w_r, B_w_gate, B_w_up, B_w_down)
```

```python
import jax
import jax.numpy as jnp
from jax import lax
import jax.experimental.pallas as pl
import jax.experimental.pallas.tpu as pltpu

S = 2048
D = 1024
H = 32
DH = 32
F = 3584
NP = H // 2
C = 128
NC = S // C
T = 512
NT = S // T
CPT = T // C
T1 = 512
N1 = (S - T) // T1
CP1 = T1 // C
KR = H * (DH - 1)
GO = -(-8 // N1)
SEGS = ((256, 256), (128, 256), (128, 512))
PHI = ((0, 512), (512, 512), (512, 1024))
DEFER = 2
NB = F // 128
NA = 10
B0 = (0, NA, NB - NA)
NDUP = (3 * NA - NB) * 128
NCAND = 2
EG = 16
LOG2E = 1.4426950408889634
EPS = 1e-5

f32 = jnp.float32
bf16 = jnp.bfloat16
u32 = jnp.uint32
i32 = jnp.int32


def _dot_nt(a, b):
    return lax.dot_general(a, b, (((1,), (1,)), ((), ())), preferred_element_type=f32)


def _dot(a, b):
    return jnp.dot(a, b, preferred_element_type=f32)


def _pk(x):
    return pltpu.bitcast(x, u32)


def _un(x):
    return pltpu.bitcast(x, bf16)


def _rcp(x):
    r = pl.reciprocal(x, approx=True)
    return r * (2.0 - x * r)


def _allred(v, op):
    v = op(v, pltpu.roll(v, 2, 0))
    return op(v, pltpu.roll(v, 4, 0))


def _allred8(v, op):
    return _allred(op(v, pltpu.roll(v, 1, 0)), op)


def _rows(v, n):
    return jnp.concatenate([v] * n, axis=0)


def _lanes(v, n):
    return jnp.concatenate([v] * n, axis=1)


def _zero_after(dep, zm):
    return pltpu.bitcast(pltpu.bitcast(dep, u32) & zm, f32)


def _exps(x):
    x3 = x.reshape(8, 8, x.shape[1])
    mx = _allred(jnp.max(x3, axis=0), jnp.maximum)
    mn = _allred(jnp.min(x3, axis=0), jnp.minimum)
    ep = jnp.exp2(x3 - mx[None])
    en = jnp.exp2(mn[None] - x3)
    rp = _rcp(_allred(jnp.sum(ep, axis=0), jnp.add))
    rn = _rcp(_allred(jnp.sum(en, axis=0), jnp.add))
    return ep, en, rp, rn


def _phi_k(x):
    L = x.shape[1]
    ep, en, rp, rn = _exps(x)
    return jnp.concatenate([(ep * rp[None]).reshape(64, L), (en * rn[None]).reshape(64, L)], axis=0)


def _phi_q(x, zb):
    L = x.shape[1]
    ep, en, rp, rn = _exps(x)
    zb = _lanes(zb, L // 128).reshape(16, 8, L)
    den = rp * jnp.sum(ep * zb[0:8], axis=0) + rn * jnp.sum(en * zb[8:16], axis=0)
    inv = _rcp(_allred(den, jnp.add) + 1e-6)
    cp = rp * inv
    cn = rn * inv
    phi = jnp.concatenate([(ep * cp[None]).reshape(64, L), (en * cn[None]).reshape(64, L)], axis=0)
    return phi.astype(bf16)


def _slot(n):
    return lax.shift_right_logical(lax.broadcasted_iota(i32, (8, n), 0), 1)


def _pair_logits(y, sgs):
    slot = _slot(y.shape[1])
    out, r, shared = {}, 0, None
    for k, sg in enumerate(sgs):
        if k == 0 or sg % 2 == 0:
            shared, r = y[r:r + 16], r + 16
        l0, l1, l2 = y[r:r + 8], y[r + 8:r + 16], shared[8 * (sg % 2):8 * (sg % 2) + 8]
        for q in range(4):
            x0 = jnp.where(slot == q, l0, jnp.where(slot == (q + 1) % 4, l1, jnp.where(slot == (q + 2) % 4, l2, 0.0)))
            out[4 * sg + q] = jnp.concatenate([x0, y[r + 16 + 56 * q:r + 72 + 56 * q]], axis=0)
        r += 240
    return out


def _lane_blocks_sum(v, acc):
    for c in range(0, v.shape[1], 128):
        acc = acc + v[:, c:c + 128]
    return acc


def _row_sum(x, deps, zm):
    g = x.shape[0] // len(deps)
    gate = jnp.concatenate([jnp.zeros((8, 128), f32) if d is None else _zero_after(d, zm)
                            for d in deps for _ in range(g // 8)], axis=0)
    return jnp.sum(_lane_blocks_sum(x[:, 128:], x[:, 0:128] + gate), axis=-1, keepdims=True)


def _ln(x, deps=None, zm=None):
    tot = jnp.sum(x, axis=-1, keepdims=True) if deps is None else _row_sum(x, deps, zm)
    xc = x - tot * (1.0 / D)
    return xc * lax.rsqrt(jnp.sum(xc * xc, axis=-1, keepdims=True) * (1.0 / D) + EPS)


def _col(a8):
    return _rows(a8, 16).astype(bf16).T.astype(f32)


def _first_max(v, t):
    m = jnp.max(_allred8(v, jnp.maximum), axis=1, keepdims=True)
    return m, jnp.min(_allred8(jnp.where(v == m, t, float(2 * S)), jnp.minimum), axis=1, keepdims=True)


def _merge_max(cands):
    v, t = cands[0]
    for v2, t2 in cands[1:]:
        gt = v2 > v
        v, t = jnp.where(gt, v2, v), jnp.where(gt, t2, t)
    return v, t


def _scalar(v, lo, hi):
    return jnp.clip(jnp.broadcast_to(v, (8, 128)).astype(i32)[0, 0], lo, hi)


class _Group:
    def __init__(self, parts, dst, sem):
        self.parts, self.dst, self.sem = parts, dst, sem

    def start(self):
        for src, dst in self.parts:
            pltpu.make_async_copy(src, dst, self.sem).start()

    def wait(self):
        pltpu.make_async_copy(self.dst, self.dst, self.sem).wait()


def _kernel(x_hbm, wqkv_hbm, wphi_hbm, wo_hbm, wr_hbm, wg_hbm, wu_hbm, wd_hbm, out_hbm,
            x_v, wkv_v, wqb_v, wphi_v, wo_v, wo32, wr_v, wg_v, wu_v, wd_v,
            wt_v, wq_v, a_v, xn_v, xk_v, xq_v, hn_v, kv_acc, z_acc, zb_v, hbuf, out_v, zv, zs, p_v, r_v,
            xc_v, pa_v, y_v, fix_v, ord_s, sems):
    nsem = [0]

    def new_sems(n):
        nsem[0] += n
        return nsem[0] - n

    def cp(src, dst):
        return pltpu.make_async_copy(src, dst, sems.at[new_sems(1)])

    def cp_w(lo, hi):
        return cp(wqkv_hbm.at[:, lo:hi], wkv_v.at[:, lo:hi])

    def cp_x(lo, hi):
        return cp(x_hbm.at[0, lo:hi], x_v.at[lo:hi])

    cp_wr = cp(wr_hbm, wr_v)
    kcum = [0]
    for _, dk in SEGS:
        kcum.append(kcum[-1] + dk)
    seg_cp = []
    x0 = 0
    for si, (dx, dk) in enumerate(SEGS):
        lo, hi = PHI[si][0] // DH, PHI[si][1] // DH
        ph = [cp(wphi_hbm.at[lo:hi], wphi_v.at[lo:hi])] if hi > lo else []
        seg_cp.append([cp_x(x0, x0 + dx)] + ph + [cp_w(D + kcum[si], D + kcum[si + 1])])
        x0 += dx
    cp_wv = cp_w(2 * D, 3 * D)
    cp_x1a = cp_x(T, T + C)
    cp_x1 = cp_x(T + C, S)
    cp_q0 = _Group([(wqkv_hbm.at[:, 128 * g:128 * (g + 1)], wqb_v.at[g]) for g in range(2)],
                   wqb_v.at[0:2], sems.at[new_sems(1)])
    qsem0 = new_sems(2 * N1)

    def cp_step(j):
        pq = po = None
        if isinstance(j, int):
            pq = [(wqkv_hbm.at[:, 128 * g:128 * (g + 1)], wqb_v.at[g]) for g in range(2 + 2 * j, 4 + 2 * j)]
            po = [(wo_hbm.at[:, 128 * min(g, 7):128 * (min(g, 7) + 1)], wo_v.at[g])
                  for g in range(GO * j, GO * (j + 1))]
        return [_Group(pq, wqb_v.at[pl.ds(2 + 2 * j, 2)], sems.at[qsem0 + 2 * j]),
                _Group(po, wo_v.at[pl.ds(GO * j, GO)], sems.at[qsem0 + 2 * j + 1])]

    cp_ffn = []
    for t, b in enumerate(B0):
        cp_ffn += [cp(wg_hbm.at[:, b * 128:(b + NA) * 128], wg_v.at[t]),
                   cp(wu_hbm.at[:, b * 128:(b + NA) * 128], wu_v.at[t]),
                   cp(wd_hbm.at[b * 128:(b + NA) * 128], wd_v.at[t])]
    seg_cp[0] = seg_cp[0][1:] + seg_cp[0][0:1]
    for c in ([c for t in seg_cp for c in t] + [cp_wr, cp_wv, cp_x1a, cp_q0, cp_x1]
              + [c for j in range(N1) for c in cp_step(j)] + cp_ffn):
        c.start()
    osem0 = new_sems(NC + 1)

    def cp_out(q):
        rows = pl.ds(pl.multiple_of(ord_s[q], C), C)
        return pltpu.make_async_copy(out_v.at[rows], out_hbm.at[0, rows], sems.at[osem0 + q])

    def wr_row():
        return wr_v[...].reshape(1, D).astype(f32)

    def put_cols(ref, idx, col0, r):
        for k in range(0, r.shape[0], 8):
            ref[idx, :, col0 + k // 8:col0 + k // 8 + 1] = r[k:k + 8]

    def half(row0, n):
        if isinstance(row0, int):
            return pl.ds(row0 // 2, n // 2)
        return pl.ds(pl.multiple_of(lax.shift_right_logical(row0, 1), C // 2), n // 2)

    def ln1(src, dst, n, deps=None):
        xb = _pk(_ln(x_v[pl.ds(src, n), :].astype(f32), deps, None if deps is None else zv[...]).astype(bf16))
        xn_v[half(dst, n), :] = xb
        return _un(xb)

    def xn(row0, n):
        return _un(xn_v[half(row0, n), :])

    def predict(rows, t, c, deps):
        wr = wr_row()
        wc = wr - jnp.sum(wr, axis=-1, keepdims=True) * (1.0 / D)
        put_cols(p_v, t, c * (C // 8), _row_sum(x_v[rows, :].astype(f32) * wc, deps, zv[...]))

    def fold(dst, ws, sg):
        slot = _slot(D)
        res = [_dot_nt(_un(a_v[2 * sg + e]), ws[e]) for e in range(2)]
        main, e0, e1 = [], [], []
        for e in range(2):
            z = jnp.where(((slot + 3) % 4) // 2 == e, 0.0, res[e][0:8])
            b1 = z + pltpu.roll(z, 4, 0)
            b0 = pltpu.roll(b1, 2, 0)
            for pp in range(2):
                base = jnp.where(slot % 2 == pp, b0, b1)
                main.append((res[e][16 + 56 * pp:72 + 56 * pp].reshape(7, 8, D) - base[None]).reshape(56, D))
            e0.append(res[e][8:16] - b0)
            e1.append(res[e][0:8] - b1)
        rows = jnp.concatenate([jnp.where(slot < 2, e0[0], e0[1]), e1[0] + e1[1]] + main, axis=0)
        l2 = _pk((_rows(jnp.where(slot < 2, e0[1], e0[0]), 2) * LOG2E).astype(bf16))
        if isinstance(sg, int):
            r0, r1 = 248 * (sg // 2), 248 * (sg // 2) + 8 + 120 * (sg % 2)
        else:
            r0 = pl.multiple_of(248 * lax.shift_right_logical(sg, 1), 8)
            r1 = pl.multiple_of(r0 + 8 + 120 * (sg & 1), 8)
        dst[pl.ds(r1, 120), :] = _pk((rows * LOG2E).astype(bf16))
        dst[pl.ds(r0, 8), :] = jnp.where(slot // 2 == sg % 2, l2, dst[pl.ds(r0, 8), :])
        return res

    def wk(lo, hi):
        r0, r1 = 248 * (lo // 2), 248 * ((hi - 1) // 2) + 128 + 120 * ((hi - 1) % 2)
        if lo % 2:
            return _un(jnp.concatenate([wt_v[r0:r0 + 8, :], wt_v[r0 + 128:r1, :]], axis=0))
        return _un(wt_v[r0:r1, :])

    def kv_and_z(vt, phis, z_of, tail, zm):
        lag = 4
        kvs, zs_ = [], []
        for p in range(NP):
            kvs.append(_dot_nt(vt[64 * p:64 * (p + 1)].astype(bf16), phis[p].astype(bf16)))
            dep = kvs[p - lag][0:8] if p >= lag else tail[D - 64 * (lag - p):D - 64 * (lag - p) + 8]
            zs_.append(_lane_blocks_sum(phis[p], z_of(p, _rows(_zero_after(dep, zm), 16))))
        return kvs, zs_

    def a_row(r, e):
        s = (r & 7) >> 1
        f = jnp.where(r >= 72, (r - 64) >> 1, jnp.where(r >= 16, (r - 8) >> 1, jnp.where(
            r >= 8, jnp.where(s >> 1 == e, 1, 3), jnp.where(((s + 3) & 3) >> 1 == e, 2, 0))))
        pp = jnp.where(r >= 72, 1, jnp.where(r >= 16, 0, jnp.where(r >= 8, s, s + 1) & 1))
        return f, 2 * pp + (r & 1)

    f_i = lax.broadcasted_iota(i32, (128, DH), 1)
    sel = [jnp.where(f_i == a_row(lax.broadcasted_iota(i32, (128, DH), 0), e)[0], 1.0, 0.0).astype(bf16)
           for e in range(2)]
    amask = jnp.where(lax.broadcasted_iota(i32, (128, 128), 1) >> 5
                      == a_row(lax.broadcasted_iota(i32, (128, 128), 0), 0)[1], jnp.uint32(0xFFFFFFFF), jnp.uint32(0))

    def build_a(lo, hi):
        for g in range(lo // 128, hi // 128):
            blk = _dot_nt(sel[g % 2], wphi_v[4 * g:4 * (g + 1)].reshape(128, DH))
            a_v[g] = _pk(pltpu.bitcast(pltpu.bitcast(blk, u32) & amask, f32).astype(bf16))

    zv[...] = jnp.zeros((8, 128), u32)
    cp_z = cp(zv, zs)
    cp_z.start()
    for ref in (wt_v, wq_v):
        for r0 in (0, 248):
            ref[r0:r0 + 8, :] = jnp.zeros((8, D), u32)
    hbuf[...] = jnp.zeros(hbuf.shape, f32)
    xc_v[...] = jnp.zeros(xc_v.shape, f32)
    y_v[...] = jnp.zeros(y_v.shape, f32)
    r_v[...] = jnp.full(r_v.shape, -jnp.inf, f32)
    p_v[...] = jnp.full(p_v.shape, -jnp.inf, f32)

    pieces = [[] for _ in range(NP)]
    pending = []

    def phi_piece(p, t0, yp, dep=None):
        if dep is not None:
            yp = jnp.concatenate([yp[0:8] + _zero_after(dep, zv[...]), yp[8:]], axis=0)
        pieces[p].append((t0, _phi_k(yp)))

    def k_block(lo, hi, t0, t1, defer=0):
        y = _dot_nt(wk(lo, hi), xn(t0, t1 - t0))
        for p, yp in _pair_logits(y, range(lo, hi)).items():
            if p >= 4 * hi - defer:
                if t1 - t0 > C:
                    phi_piece(p, t0, yp[:, 0:t1 - t0 - C])
                pending.append((p, t1 - C, yp[:, t1 - t0 - C:]))
            else:
                phi_piece(p, t0, yp)
        return y

    def flush(res):
        for k, (p, t0, yp) in enumerate(pending):
            phi_piece(p, t0, yp, res[32 * k:32 * k + 8, 0:128])
        del pending[:]

    x0 = 0
    for si, (dx, dk) in enumerate(SEGS):
        k0, k1 = kcum[si] // 256, kcum[si + 1] // 256
        if si == 0:
            seg_cp[0][0].wait()
            build_a(*PHI[0])
            seg_cp[0][1].wait()
        else:
            for c in seg_cp[si]:
                c.wait()
            if PHI[si][1] > PHI[si][0]:
                build_a(*PHI[si])
        res = [fold(wt_v, [wkv_v[:, D + 128 * g:D + 128 * (g + 1)] for g in (2 * sg, 2 * sg + 1)], sg)
               for sg in range(k0, k1)]
        flush(res[0][0])
        if si == 0:
            seg_cp[0][2].wait()
        ln1(x0, x0, dx)
        if si:
            k_block(k0, k1, 0, x0)
        k_block(0, k1, x0, x0 + dx, DEFER)
        x0 += dx
    for c in (cp_wv, cp_x1a, cp_q0, cp_wr, cp_z):
        c.wait()
    for g in range(D // 128):
        wt_v[KR // 2 + 64 * g:KR // 2 + 64 * (g + 1), :] = _pk(wkv_v[:, 2 * D + 128 * g:2 * D + 128 * (g + 1)].T)
    flush(fold(wq_v, [wqb_v[0], wqb_v[1]], 0)[0])
    yv = _dot_nt(_un(wt_v[KR // 2:, :]), xn(0, T))
    xk_v[...] = _pk(ln1(T, T, C, [yv[128 * k:128 * k + 8, 128:256] for k in range(8)])[:, 0:D // 2].T)
    for c in range(CPT):
        predict(slice(C * c, C * (c + 1)), 0, c,
                [yv[256 * c + 32 * k:256 * c + 32 * k + 8, 256:384] for k in range(8)])
    phis = [jnp.concatenate([ph for _, ph in sorted(pieces[p], key=lambda tp: tp[0])], axis=1) for p in range(NP)]
    kvs, zs_ = kv_and_z(yv, phis, lambda p, zero: zero, yv[:, T - C:T], zv[...])
    for p in range(NP):
        kv_acc[p] = kvs[p]
        z_acc[p] = zs_[p]
    cp_x1.wait()

    def order_chunks():
        lane16 = lax.shift_right_logical(lax.broadcasted_iota(i32, (8, 128), 1), 4).astype(f32)
        vals = [p_v[t] for t in range(1 + N1)]
        cids = [lane16 + float(0 if t == 0 else CPT + CP1 * (t - 1)) for t in range(1 + N1)]
        b1 = _first_max(*_merge_max(list(zip(vals, cids))))[1]
        b2 = _first_max(*_merge_max([(jnp.where(c == b1, -jnp.inf, v), c) for v, c in zip(vals, cids)]))[1]
        c1, c2 = _scalar(b1, 0, NC - 1), _scalar(b2, 0, NC - 1)
        c2 = jnp.where(c2 == c1, (c1 + 1) & (NC - 1), c2)
        ord_s[0] = S
        for c in range(NC):
            ord_s[1 + c] = c * C
        ord_s[1 + c1] = 0
        ord_s[1] = c1 * C
        ord_s[1 + jnp.where(c2 == 0, c1, c2)] = jnp.where(c1 == 1, 0, C)
        ord_s[2] = c2 * C

    def phase1(j, carry):
        for c in cp_step(j):
            c.wait()
        zm = zv[...]
        s = pl.multiple_of(T + j * T1, C)
        nxt = pl.multiple_of(jnp.where(j + 1 < N1, s + T1, 0), C)
        xt = xn(s, C)
        ys, ph = [], []
        for n in range(CP1):
            if n + 1 < CP1:
                row0 = pl.multiple_of(s + C * (n + 1), C)
                xt1 = ln1(row0, row0, C)
                if n == 0:
                    y0 = _dot(_un(wt_v[:, 0:D // 2]), _un(xk_v[...]))
                    yn = _dot_nt(_un(wt_v[:, D // 2:D]), xt[:, D // 2:D]) + y0
                else:
                    yn = _dot_nt(_un(wt_v[...]), xt)
                xt = xt1
            else:
                ya = _dot_nt(_un(wt_v[:, 0:D // 2]), xt[:, 0:D // 2])
                for c in range(CP1):
                    r0, st = 384 + 1280 * c // CP1 // 8 * 8, 1280 // CP1 // 64 * 8
                    predict(pl.ds(pl.multiple_of(s + C * c, C), C), 1 + j, c,
                            [ya[r0 + st * k:r0 + st * k + 8] for k in range(8)])
                order_chunks()
                xq_v[...] = _pk(xn(pl.multiple_of(ord_s[1], C), C)[:, 0:D // 2].T)
                yn = ya + _dot_nt(_un(wt_v[:, D // 2:D]), xt[:, D // 2:D])
            ys.append(yn)
            ph.append([_phi_k(yp) for yp in _pair_logits(yn[0:KR], range(4)).values()])
            if n == CP1 - 2:
                xk_v[...] = _pk(ln1(nxt, pl.multiple_of(s + T1, C), C,
                                    [yn[KR + 512 + 64 * k:KR + 520 + 64 * k] for k in range(8)])[:, 0:D // 2].T)
        fold(wq_v, [wqb_v[2 + 2 * j], wqb_v[3 + 2 * j]], 1 + j)
        for e in range(4 * GO):
            row = KR + 384 + 640 * e // (4 * GO) // 8 * 8
            w = _pk(wo_v[GO * j + e // 4, 256 * (e % 4):256 * (e % 4 + 1), :])
            wo32[GO * j + e // 4, 128 * (e % 4):128 * (e % 4 + 1), :] = (
                w.reshape(16, 8, 128) | (_pk(ys[0][row:row + 8]) & zm)[None]).reshape(128, 128)
        vt = jnp.concatenate([yn[KR:] for yn in ys], axis=1)
        phis = [jnp.concatenate([ph[n][p] for n in range(CP1)], axis=1) for p in range(NP)]
        kvs, zs_ = kv_and_z(vt, phis, lambda p, zero: z_acc[p] + zero, ys[-1][KR:], zm)
        for p in range(NP):
            kv_acc[p] += kvs[p]
            z_acc[p] = zs_[p]
            zb_v[p] = jnp.broadcast_to(jnp.sum(zs_[p], axis=1, keepdims=True), (128, 128))
        return carry

    lax.fori_loop(0, N1, phase1, 0)
    for c in cp_ffn:
        c.wait()

    def ln2(h, row0, nx, nrel):
        deps = [None]
        for j in range(1, C // 8):
            t = (j * nrel * 2) // (C // 8) - 1
            r0 = (C - 8) * (t % 2)
            deps.append(nx[r0:r0 + 8, 128 * (t // 2):128 * (t // 2) + 128] if t >= 0 else None)
        hn = _ln(h, deps, zv[...])
        r = jnp.sum(hn * wr_row(), axis=-1, keepdims=True)
        hn_v[pl.ds(row0, C), :] = hn.astype(bf16)
        out_v[pl.ds(row0, C), :] = (h + hn).astype(bf16)
        return r

    lane = lax.broadcasted_iota(i32, (8, 128), 1)
    pos = (lane * 8 + lax.broadcasted_iota(i32, (8, 128), 0)).astype(f32)

    def token_at(posv, lo, hi):
        p = _scalar(posv, lo, hi - 1)
        return ord_s[lax.shift_right_logical(p, 7)] + (p & (C - 1))

    def slab_of(tok):
        base = pl.multiple_of(lax.shift_left(lax.shift_right_logical(tok, 4), 4), 16)
        return pl.ds(base, 16), lax.broadcasted_iota(i32, (16, D), 0) == tok - base

    def token_row(tok):
        rows, hit = slab_of(tok)
        slab = jnp.where(hit, hn_v[rows, :].astype(f32), 0.0)
        return _allred8(slab[0:8] + slab[8:16], jnp.add)

    def patch(tok, y8, sg):
        rows, hit = slab_of(tok)
        cur = out_v[rows, :].astype(f32)
        fix_v[...] = jnp.where(hit, cur + _rows(y8 * _lanes(sg, D // 128), 2), cur).astype(bf16)

    def phase2(i, carry):
        q0 = CPT * i
        off = [pl.multiple_of(ord_s[q0 + k], C) for k in range(CPT + 1)]
        zm = zv[...]
        hprev = hbuf[...]
        kmask = lax.broadcasted_iota(i32, (64, 128), 0) // 32 == lax.broadcasted_iota(i32, (64, 128), 1) % 2

        def attend(y):
            os_ = []
            for p, yp in _pair_logits(y, range(4)).items():
                os_.append(_dot(jnp.where(kmask, kv_acc[p], 0.0).astype(bf16), _phi_q(yp, zb_v[p])))
            return jnp.concatenate(os_, axis=0).astype(bf16).T

        ya, ys = [], []
        for n in range(CPT):
            xt = xn(off[n + 1], C)
            ya.append(_dot_nt(_un(wq_v[:, 0:D // 2]), xt[:, 0:D // 2]) if n else
                      _dot(_un(wq_v[:, 0:D // 2]), _un(xq_v[...])))
            if n == CPT - 1:
                o01 = attend(jnp.concatenate(ys[0:2], axis=1))
            ys.append(ya[n] + _dot_nt(_un(wq_v[:, D // 2:D]), xt[:, D // 2:D]))
        wo = jnp.concatenate([_un(wo32[j]) for j in range(D // 128)], axis=1)
        head = _dot(o01[0:C], wo[:, 0:256])
        o23 = attend(jnp.concatenate(ys[2:4], axis=1))
        atts = [jnp.concatenate([head, _dot(o01[0:C], wo[:, 256:])], axis=1),
                _dot(o01[C:2 * C], wo), _dot(o23[0:C], wo), _dot(o23[C:2 * C], wo)]

        xq_v[...] = _pk(xn(pl.multiple_of(ord_s[jnp.minimum(q0 + CPT + 1, NC)], C), C)[:, 0:D // 2].T)

        def q_gate(v):
            lens = [KR // 8] + [KR // 8 - 24] * 3
            t, n = int(v * sum(lens)), 0
            while t >= lens[n]:
                t -= lens[n]
                n += 1
            r0 = 8 * (t + KR // 8 - lens[n])
            return _zero_after(ya[n][r0:r0 + 8], zm)

        def o_gate(t):
            r0, j = 8 * (t % 16), (t % 128) // 16
            return _zero_after(atts[t // 128][r0:r0 + 8, 128 * j:128 * j + 128], zm)

        t3 = jnp.maximum(i - 1, 0)
        nsb = NA // 2
        for sb in range(nsb):
            cols = slice(256 * sb, 256 * (sb + 1))
            xcol = xc_v[...]
            acc = None
            for k in range(0, D, 8):
                xk = _lanes(xcol[k:k + 8], 2)
                p = jnp.concatenate([wg_v[t3, k:k + 8, cols].astype(f32) * xk,
                                     wu_v[t3, k:k + 8, cols].astype(f32) * xk], axis=1)
                if k % 64 == 0:
                    p = p + _lanes(q_gate((sb * D + k) / (nsb * D)), 4)
                acc = p if acc is None else acc + p
            pa_v[:, 512 * sb:512 * (sb + 1)] = acc

        put_cols(r_v, i, 0, jnp.where(i > 0, ln2(hprev, off[0], atts[0], 6), -jnp.inf))

        @pl.when(i > 0)
        def _():
            cp_out(q0).start()

        acc = _allred8(pa_v[pl.ds(pl.multiple_of(zs[3, 0].astype(i32) * 32, 32), 8), :], jnp.add)
        g_ = jnp.concatenate([acc[:, 512 * t:512 * t + 256] for t in range(nsb)], axis=1)
        u_ = jnp.concatenate([acc[:, 512 * t + 256:512 * t + 512] for t in range(nsb)], axis=1)
        a8 = g_ * jax.nn.sigmoid(g_) * u_
        ac = _col(jnp.concatenate([jnp.where(t3 == 2, 0.0, a8[:, 0:NDUP]), a8[:, NDUP:]], axis=1))
        ysums = []
        for q in range(2):
            cols = slice(D // 2 * q, D // 2 * (q + 1))
            ysum = jnp.where(i > 1, y_v[:, cols], 0.0)
            for k in range(0, NA * 128, 8):
                p = wd_v[t3, k:k + 8, cols].astype(f32) * _lanes(ac[k:k + 8], 4)
                if k % 32 == 0:
                    p = p + _lanes(o_gate(64 + (q * NA * 128 + k) * 376 // (2 * NA * 128)), 4)
                ysum = ysum + p
            y_v[:, cols] = ysum
            ysums.append(ysum)

        for k in range(CPT):
            if k == NCAND:
                ok = (lane >= C // 8) & (lane < (NCAND + 1) * (C // 8))
                cm, cpos = _first_max(jnp.where(ok, r_v[0], -jnp.inf), pos)
                cand = token_at(cpos, C, (NCAND + 1) * C)
                ord_s[NC + 1] = cand
                xc_v[...] = _col(token_row(cand))
                patch(cand, _allred8(jnp.concatenate(ysums, axis=1), jnp.add),
                      jax.nn.sigmoid(jnp.broadcast_to(cm, (8, 128))))
            h = x_v[pl.ds(off[k + 1], C), :].astype(f32) + atts[k]
            if k == CPT - 1:
                hbuf[...] = h
            else:
                put_cols(r_v, i, (k + 1) * (C // 8), ln2(h, off[k + 1], atts[k + 1], 5 if k == CPT - 2 else 6))
                cp_out(q0 + k + 1).start()
        return carry

    lax.fori_loop(0, NT, phase2, 0)

    for q in range(1, NCAND + 1):
        cp_out(q).wait()
    fsem = new_sems(1)

    cand = ord_s[NC + 1]

    def cp_patch(tok):
        return pltpu.make_async_copy(fix_v, out_hbm.at[0, slab_of(tok)[0]], sems.at[fsem])

    cp_fix = cp_patch(cand)
    cp_fix.start()
    cp_out(NCAND + 1).wait()
    last = pl.multiple_of(ord_s[NC], C)
    stats, cp_last = [], []
    for g in range(0, C, EG):
        h = hbuf[g:g + EG, :]
        s1 = h[:, 0:128]
        s2 = s1 * s1
        for j in range(128, D, 128):
            s1 = s1 + h[:, j:j + 128]
            s2 = s2 + h[:, j:j + 128] * h[:, j:j + 128]
        m = jnp.sum(s1, axis=-1, keepdims=True) * (1.0 / D)
        v = jnp.sum(s2, axis=-1, keepdims=True) * (1.0 / D) - m * m
        rs = lax.rsqrt(jnp.maximum(v, 0.0) + EPS)
        stats.append((m, rs))
        rows = pl.ds(pl.multiple_of(last + g, EG), EG)
        out_v[rows, :] = (h * (1.0 + rs) - m * rs).astype(bf16)
        cp_last.append(cp(out_v.at[rows], out_hbm.at[0, rows]))
        cp_last[-1].start()
    for q in range(NCAND + 2, NC - 1):
        cp_out(q).wait()
    pm, pi = _first_max(*_merge_max([(r_v[i], pos + float(i * T) if i else pos) for i in range(NT)]))
    wr = wr_row()
    wsum = jnp.sum(wr, axis=-1, keepdims=True)
    sub = lax.broadcasted_iota(i32, (8, 1), 0).astype(f32)
    cands = []
    for g, (m, rs) in zip(range(0, C, EG), stats):
        r = (jnp.sum(hbuf[g:g + EG, :] * wr, axis=-1, keepdims=True) - m * wsum) * rs
        cands += [(r[k:k + 8], sub + float(S + g + k)) for k in range(0, EG, 8)]
    while len(cands) > 1:
        cands = [_merge_max(cands[k:k + 2]) for k in range(0, len(cands), 2)]
    bv, bt = [jnp.broadcast_to(v, (8, 128)) for v in _merge_max([(pm, pi), cands[0]])]
    rmax = _allred8(bv, jnp.maximum)
    idx = token_at(_allred8(jnp.where(bv == rmax, bt, float(2 * S)), jnp.minimum), C, S + C)
    cp_out(NC - 1).wait()
    cp_fix.wait()
    for c in cp_last:
        c.wait()

    @pl.when(idx != cand)
    def _():
        rows, _ = slab_of(cand)
        undo = pltpu.make_async_copy(out_v.at[rows], out_hbm.at[0, rows], sems.at[fsem])
        undo.start()
        hn_v[pl.ds(last, C), :] = _ln(hbuf[...]).astype(bf16)
        xs = _rows(token_row(idx), 2).astype(bf16)

        def step(j, acc):
            t = lax.shift_right_logical(j, 1)
            cols = pl.ds(pl.multiple_of((j & 1) * (NA * 64), 128), NA * 64)
            g = _dot(xs, wg_v[t, :, cols])
            a = g * jax.nn.sigmoid(g) * _dot(xs, wu_v[t, :, cols])
            a = jnp.concatenate([jnp.where(j == 4, 0.0, a[:, 0:NDUP]), a[:, NDUP:]], axis=1)
            return acc + _dot(a.astype(bf16), wd_v[t, cols, :])[0:8]

        y8 = lax.fori_loop(0, 6, step, jnp.zeros((8, D), f32))
        undo.wait()
        patch(idx, y8, jax.nn.sigmoid(rmax))
        redo = cp_patch(idx)
        redo.start()
        redo.wait()


@jax.jit
def pallas_sequential_preLN__linear_kernel_hedgehog__moe_arch_mod__prompt_kernel(
    A_x: jax.Array,
    A_wqkv: jax.Array,
    A_w_phi: jax.Array,
    A_wo: jax.Array,
    B_x: jax.Array,
    B_w_r: jax.Array,
    B_w_gate: jax.Array,
    B_w_up: jax.Array,
    B_w_down: jax.Array,
):
    del B_x
    any_spec = pl.BlockSpec(memory_space=pl.ANY)
    return pl.pallas_call(
        _kernel,
        out_shape=jax.ShapeDtypeStruct((1, S, D), bf16),
        in_specs=[any_spec] * 8,
        out_specs=any_spec,
        scratch_shapes=[
            pltpu.VMEM((S, D), bf16),
            pltpu.VMEM((D, 3 * D), bf16),
            pltpu.VMEM((D // 128, D, 128), bf16),
            pltpu.VMEM((H, DH, DH), bf16),
            pltpu.VMEM((N1 * GO, D, 128), bf16),
            pltpu.VMEM((N1 * GO, D // 2, 128), u32),
            pltpu.VMEM((D,), bf16),
            pltpu.VMEM((3, D, NA * 128), bf16),
            pltpu.VMEM((3, D, NA * 128), bf16),
            pltpu.VMEM((3, NA * 128, D), bf16),
            pltpu.VMEM(((KR + D) // 2, D), u32),
            pltpu.VMEM((KR // 2, D), u32),
            pltpu.VMEM((8, 64, 128), u32),
            pltpu.VMEM(((S + C) // 2, D), u32),
            pltpu.VMEM((D // 4, C), u32),
            pltpu.VMEM((D // 4, C), u32),
            pltpu.VMEM((S + C, D), bf16),
            pltpu.VMEM((NP, 64, 128), f32),
            pltpu.VMEM((NP, 128, 128), f32),
            pltpu.VMEM((NP, 128, 128), f32),
            pltpu.VMEM((C, D), f32),
            pltpu.VMEM((S + C, D), bf16),
            pltpu.VMEM((8, 128), u32),
            pltpu.SMEM((8, 128), u32),
            pltpu.VMEM((1 + N1, 8, 128), f32),
            pltpu.VMEM((NT, 8, 128), f32),
            pltpu.VMEM((D, 128), f32),
            pltpu.VMEM((8, NA * 256), f32),
            pltpu.VMEM((8, D), f32),
            pltpu.VMEM((16, D), bf16),
            pltpu.SMEM((NC + 2,), i32),
            pltpu.SemaphoreType.DMA((64,)),
        ],
        compiler_params=pltpu.CompilerParams(vmem_limit_bytes=120 * 1024 * 1024,
                                             disable_bounds_checks=True,
                                             disable_semaphore_checks=True),
        name="hedgehog_mod",
    )(A_x, A_wqkv, A_w_phi, A_wo, B_w_r, B_w_gate, B_w_up, B_w_down)
```

```python
import jax
import jax.numpy as jnp
from jax import lax
import jax.experimental.pallas as pl
import jax.experimental.pallas.tpu as pltpu

S = 2048
D = 1024
H = 32
DH = 32
F = 3584
NP = H // 2
C = 128
NC = S // C
T = 512
NT = S // T
CPT = T // C
T1 = 512
N1 = (S - T) // T1
CP1 = T1 // C
KR = H * (DH - 1)
GO = -(-8 // N1)
SEGS = ((256, 256), (128, 256), (128, 512))
PHI = ((0, 512), (512, 512), (512, 1024))
DEFER = 2
NB = F // 128
NA = 10
B0 = (0, NA, NB - NA)
NDUP = (3 * NA - NB) * 128
NCAND = 2
EG = 16
LOG2E = 1.4426950408889634
EPS = 1e-5

f32 = jnp.float32
bf16 = jnp.bfloat16
u32 = jnp.uint32
i32 = jnp.int32


def _dot_nt(a, b):
    return lax.dot_general(a, b, (((1,), (1,)), ((), ())), preferred_element_type=f32)


def _dot(a, b):
    return jnp.dot(a, b, preferred_element_type=f32)


def _pk(x):
    return pltpu.bitcast(x, u32)


def _un(x):
    return pltpu.bitcast(x, bf16)


def _rcp(x):
    r = pl.reciprocal(x, approx=True)
    return r * (2.0 - x * r)


def _allred(v, op):
    v = op(v, pltpu.roll(v, 2, 0))
    return op(v, pltpu.roll(v, 4, 0))


def _allred8(v, op):
    return _allred(op(v, pltpu.roll(v, 1, 0)), op)


def _rows(v, n):
    return jnp.concatenate([v] * n, axis=0)


def _lanes(v, n):
    return jnp.concatenate([v] * n, axis=1)


def _zero_after(dep, zm):
    return pltpu.bitcast(pltpu.bitcast(dep, u32) & zm, f32)


def _exps(x):
    x3 = x.reshape(8, 8, x.shape[1])
    mx = _allred(jnp.max(x3, axis=0), jnp.maximum)
    mn = _allred(jnp.min(x3, axis=0), jnp.minimum)
    ep = jnp.exp2(x3 - mx[None])
    en = jnp.exp2(mn[None] - x3)
    rp = _rcp(_allred(jnp.sum(ep, axis=0), jnp.add))
    rn = _rcp(_allred(jnp.sum(en, axis=0), jnp.add))
    return ep, en, rp, rn


def _phi_k(x):
    L = x.shape[1]
    ep, en, rp, rn = _exps(x)
    return jnp.concatenate([(ep * rp[None]).reshape(64, L), (en * rn[None]).reshape(64, L)], axis=0)


def _phi_q(x, zb):
    L = x.shape[1]
    ep, en, rp, rn = _exps(x)
    zb = _lanes(zb, L // 128).reshape(16, 8, L)
    den = rp * jnp.sum(ep * zb[0:8], axis=0) + rn * jnp.sum(en * zb[8:16], axis=0)
    inv = _rcp(_allred(den, jnp.add) + 1e-6)
    cp = rp * inv
    cn = rn * inv
    phi = jnp.concatenate([(ep * cp[None]).reshape(64, L), (en * cn[None]).reshape(64, L)], axis=0)
    return phi.astype(bf16)


def _slot(n):
    return lax.shift_right_logical(lax.broadcasted_iota(i32, (8, n), 0), 1)


def _pair_logits(y, sgs):
    slot = _slot(y.shape[1])
    out, r, shared = {}, 0, None
    for k, sg in enumerate(sgs):
        if k == 0 or sg % 2 == 0:
            shared, r = y[r:r + 16], r + 16
        l0, l1, l2 = y[r:r + 8], y[r + 8:r + 16], shared[8 * (sg % 2):8 * (sg % 2) + 8]
        for q in range(4):
            x0 = jnp.where(slot == q, l0, jnp.where(slot == (q + 1) % 4, l1, jnp.where(slot == (q + 2) % 4, l2, 0.0)))
            out[4 * sg + q] = jnp.concatenate([x0, y[r + 16 + 56 * q:r + 72 + 56 * q]], axis=0)
        r += 240
    return out


def _lane_blocks_sum(v, acc):
    for c in range(0, v.shape[1], 128):
        acc = acc + v[:, c:c + 128]
    return acc


def _row_sum(x, deps, zm):
    g = x.shape[0] // len(deps)
    gate = jnp.concatenate([jnp.zeros((8, 128), f32) if d is None else _zero_after(d, zm)
                            for d in deps for _ in range(g // 8)], axis=0)
    return jnp.sum(_lane_blocks_sum(x[:, 128:], x[:, 0:128] + gate), axis=-1, keepdims=True)


def _ln(x, deps=None, zm=None):
    tot = jnp.sum(x, axis=-1, keepdims=True) if deps is None else _row_sum(x, deps, zm)
    xc = x - tot * (1.0 / D)
    return xc * lax.rsqrt(jnp.sum(xc * xc, axis=-1, keepdims=True) * (1.0 / D) + EPS)


def _col(a8):
    return _rows(a8, 16).astype(bf16).T.astype(f32)


def _first_max(v, t):
    m = jnp.max(_allred8(v, jnp.maximum), axis=1, keepdims=True)
    return m, jnp.min(_allred8(jnp.where(v == m, t, float(2 * S)), jnp.minimum), axis=1, keepdims=True)


def _merge_max(cands):
    v, t = cands[0]
    for v2, t2 in cands[1:]:
        gt = v2 > v
        v, t = jnp.where(gt, v2, v), jnp.where(gt, t2, t)
    return v, t


def _scalar(v, lo, hi):
    return jnp.clip(jnp.broadcast_to(v, (8, 128)).astype(i32)[0, 0], lo, hi)


class _Group:
    def __init__(self, parts, dst, sem):
        self.parts, self.dst, self.sem = parts, dst, sem

    def start(self):
        for src, dst in self.parts:
            pltpu.make_async_copy(src, dst, self.sem).start()

    def wait(self):
        pltpu.make_async_copy(self.dst, self.dst, self.sem).wait()


def _kernel(x_hbm, wqkv_hbm, wphi_hbm, wo_hbm, wr_hbm, wg_hbm, wu_hbm, wd_hbm, out_hbm,
            x_v, wkv_v, wqb_v, wphi_v, wo_v, wo32, wr_v, wg_v, wu_v, wd_v,
            wt_v, wq_v, a_v, xn_v, xk_v, xq_v, hn_v, kv_acc, z_acc, zb_v, hbuf, out_v, zv, zs, p_v, r_v,
            xc_v, pa_v, y_v, fix_v, ord_s, sems):
    nsem = [0]

    def new_sems(n):
        nsem[0] += n
        return nsem[0] - n

    def cp(src, dst):
        return pltpu.make_async_copy(src, dst, sems.at[new_sems(1)])

    def cp_w(lo, hi):
        return cp(wqkv_hbm.at[:, lo:hi], wkv_v.at[:, lo:hi])

    def cp_x(lo, hi):
        return cp(x_hbm.at[0, lo:hi], x_v.at[lo:hi])

    cp_wr = cp(wr_hbm, wr_v)
    kcum = [0]
    for _, dk in SEGS:
        kcum.append(kcum[-1] + dk)
    seg_cp = []
    x0 = 0
    for si, (dx, dk) in enumerate(SEGS):
        lo, hi = PHI[si][0] // DH, PHI[si][1] // DH
        ph = [cp(wphi_hbm.at[lo:hi], wphi_v.at[lo:hi])] if hi > lo else []
        seg_cp.append([cp_x(x0, x0 + dx)] + ph + [cp_w(D + kcum[si], D + kcum[si + 1])])
        x0 += dx
    cp_wv = cp_w(2 * D, 3 * D)
    cp_x1a = cp_x(T, T + C)
    cp_x1 = cp_x(T + C, S)
    cp_q0 = _Group([(wqkv_hbm.at[:, 128 * g:128 * (g + 1)], wqb_v.at[g]) for g in range(2)],
                   wqb_v.at[0:2], sems.at[new_sems(1)])
    qsem0 = new_sems(2 * N1)

    def cp_step(j):
        pq = po = None
        if isinstance(j, int):
            pq = [(wqkv_hbm.at[:, 128 * g:128 * (g + 1)], wqb_v.at[g]) for g in range(2 + 2 * j, 4 + 2 * j)]
            po = [(wo_hbm.at[:, 128 * min(g, 7):128 * (min(g, 7) + 1)], wo_v.at[g])
                  for g in range(GO * j, GO * (j + 1))]
        return [_Group(pq, wqb_v.at[pl.ds(2 + 2 * j, 2)], sems.at[qsem0 + 2 * j]),
                _Group(po, wo_v.at[pl.ds(GO * j, GO)], sems.at[qsem0 + 2 * j + 1])]

    cp_ffn = []
    for t, b in enumerate(B0):
        cp_ffn += [cp(wg_hbm.at[:, b * 128:(b + NA) * 128], wg_v.at[t]),
                   cp(wu_hbm.at[:, b * 128:(b + NA) * 128], wu_v.at[t]),
                   cp(wd_hbm.at[b * 128:(b + NA) * 128], wd_v.at[t])]
    seg_cp[0] = seg_cp[0][1:] + seg_cp[0][0:1]
    for c in ([c for t in seg_cp for c in t] + [cp_wr, cp_wv, cp_x1a, cp_q0, cp_x1]
              + [c for j in range(N1) for c in cp_step(j)] + cp_ffn):
        c.start()
    osem0 = new_sems(NC + 1)

    def cp_out(q):
        rows = pl.ds(pl.multiple_of(ord_s[q], C), C)
        return pltpu.make_async_copy(out_v.at[rows], out_hbm.at[0, rows], sems.at[osem0 + q])

    def wr_row():
        return wr_v[...].reshape(1, D).astype(f32)

    def put_cols(ref, idx, col0, r):
        for k in range(0, r.shape[0], 8):
            ref[idx, :, col0 + k // 8:col0 + k // 8 + 1] = r[k:k + 8]

    def half(row0, n):
        if isinstance(row0, int):
            return pl.ds(row0 // 2, n // 2)
        return pl.ds(pl.multiple_of(lax.shift_right_logical(row0, 1), C // 2), n // 2)

    def ln1(src, dst, n, deps=None):
        xb = _pk(_ln(x_v[pl.ds(src, n), :].astype(f32), deps, None if deps is None else zv[...]).astype(bf16))
        xn_v[half(dst, n), :] = xb
        return _un(xb)

    def xn(row0, n):
        return _un(xn_v[half(row0, n), :])

    def predict(rows, t, c, deps):
        wr = wr_row()
        wc = wr - jnp.sum(wr, axis=-1, keepdims=True) * (1.0 / D)
        put_cols(p_v, t, c * (C // 8), _row_sum(x_v[rows, :].astype(f32) * wc, deps, zv[...]))

    def fold(dst, ws, sg):
        slot = _slot(D)
        res = [_dot_nt(_un(a_v[2 * sg + e]), ws[e]) for e in range(2)]
        main, e0, e1 = [], [], []
        for e in range(2):
            z = jnp.where(((slot + 3) % 4) // 2 == e, 0.0, res[e][0:8])
            b1 = z + pltpu.roll(z, 4, 0)
            b0 = pltpu.roll(b1, 2, 0)
            for pp in range(2):
                base = jnp.where(slot % 2 == pp, b0, b1)
                main.append((res[e][16 + 56 * pp:72 + 56 * pp].reshape(7, 8, D) - base[None]).reshape(56, D))
            e0.append(res[e][8:16] - b0)
            e1.append(res[e][0:8] - b1)
        rows = jnp.concatenate([jnp.where(slot < 2, e0[0], e0[1]), e1[0] + e1[1]] + main, axis=0)
        l2 = _pk((_rows(jnp.where(slot < 2, e0[1], e0[0]), 2) * LOG2E).astype(bf16))
        if isinstance(sg, int):
            r0, r1 = 248 * (sg // 2), 248 * (sg // 2) + 8 + 120 * (sg % 2)
        else:
            r0 = pl.multiple_of(248 * lax.shift_right_logical(sg, 1), 8)
            r1 = pl.multiple_of(r0 + 8 + 120 * (sg & 1), 8)
        dst[pl.ds(r1, 120), :] = _pk((rows * LOG2E).astype(bf16))
        dst[pl.ds(r0, 8), :] = jnp.where(slot // 2 == sg % 2, l2, dst[pl.ds(r0, 8), :])
        return res

    def wk(lo, hi):
        r0, r1 = 248 * (lo // 2), 248 * ((hi - 1) // 2) + 128 + 120 * ((hi - 1) % 2)
        if lo % 2:
            return _un(jnp.concatenate([wt_v[r0:r0 + 8, :], wt_v[r0 + 128:r1, :]], axis=0))
        return _un(wt_v[r0:r1, :])

    def kv_and_z(vt, phis, z_of, tail, zm):
        lag = 4
        kvs, zs_ = [], []
        for p in range(NP):
            kvs.append(_dot_nt(vt[64 * p:64 * (p + 1)].astype(bf16), phis[p].astype(bf16)))
            dep = kvs[p - lag][0:8] if p >= lag else tail[D - 64 * (lag - p):D - 64 * (lag - p) + 8]
            zs_.append(_lane_blocks_sum(phis[p], z_of(p, _rows(_zero_after(dep, zm), 16))))
        return kvs, zs_

    def a_row(r, e):
        s = (r & 7) >> 1
        f = jnp.where(r >= 72, (r - 64) >> 1, jnp.where(r >= 16, (r - 8) >> 1, jnp.where(
            r >= 8, jnp.where(s >> 1 == e, 1, 3), jnp.where(((s + 3) & 3) >> 1 == e, 2, 0))))
        pp = jnp.where(r >= 72, 1, jnp.where(r >= 16, 0, jnp.where(r >= 8, s, s + 1) & 1))
        return f, 2 * pp + (r & 1)

    f_i = lax.broadcasted_iota(i32, (128, DH), 1)
    sel = [jnp.where(f_i == a_row(lax.broadcasted_iota(i32, (128, DH), 0), e)[0], 1.0, 0.0).astype(bf16)
           for e in range(2)]
    amask = jnp.where(lax.broadcasted_iota(i32, (128, 128), 1) >> 5
                      == a_row(lax.broadcasted_iota(i32, (128, 128), 0), 0)[1], jnp.uint32(0xFFFFFFFF), jnp.uint32(0))

    def build_a(lo, hi):
        for g in range(lo // 128, hi // 128):
            blk = _dot_nt(sel[g % 2], wphi_v[4 * g:4 * (g + 1)].reshape(128, DH))
            a_v[g] = _pk(pltpu.bitcast(pltpu.bitcast(blk, u32) & amask, f32).astype(bf16))

    zv[...] = jnp.zeros((8, 128), u32)
    cp_z = cp(zv, zs)
    cp_z.start()
    for ref in (wt_v, wq_v):
        for r0 in (0, 248):
            ref[r0:r0 + 8, :] = jnp.zeros((8, D), u32)
    hbuf[...] = jnp.zeros(hbuf.shape, f32)
    xc_v[...] = jnp.zeros(xc_v.shape, f32)
    y_v[...] = jnp.zeros(y_v.shape, f32)
    r_v[...] = jnp.full(r_v.shape, -jnp.inf, f32)
    p_v[...] = jnp.full(p_v.shape, -jnp.inf, f32)

    pieces = [[] for _ in range(NP)]
    pending = []

    def phi_piece(p, t0, yp, dep=None):
        if dep is not None:
            yp = jnp.concatenate([yp[0:8] + _zero_after(dep, zv[...]), yp[8:]], axis=0)
        pieces[p].append((t0, _phi_k(yp)))

    def k_block(lo, hi, t0, t1, defer=0):
        y = _dot_nt(wk(lo, hi), xn(t0, t1 - t0))
        for p, yp in _pair_logits(y, range(lo, hi)).items():
            if p >= 4 * hi - defer:
                if t1 - t0 > C:
                    phi_piece(p, t0, yp[:, 0:t1 - t0 - C])
                pending.append((p, t1 - C, yp[:, t1 - t0 - C:]))
            else:
                phi_piece(p, t0, yp)
        return y

    def flush(res):
        for k, (p, t0, yp) in enumerate(pending):
            phi_piece(p, t0, yp, res[32 * k:32 * k + 8, 0:128])
        del pending[:]

    x0 = 0
    for si, (dx, dk) in enumerate(SEGS):
        k0, k1 = kcum[si] // 256, kcum[si + 1] // 256
        if si == 0:
            seg_cp[0][0].wait()
            build_a(*PHI[0])
            seg_cp[0][1].wait()
        else:
            for c in seg_cp[si]:
                c.wait()
            if PHI[si][1] > PHI[si][0]:
                build_a(*PHI[si])
        res = [fold(wt_v, [wkv_v[:, D + 128 * g:D + 128 * (g + 1)] for g in (2 * sg, 2 * sg + 1)], sg)
               for sg in range(k0, k1)]
        flush(res[0][0])
        if si == 0:
            seg_cp[0][2].wait()
        ln1(x0, x0, dx)
        if si:
            k_block(k0, k1, 0, x0)
        k_block(0, k1, x0, x0 + dx, DEFER)
        x0 += dx
    for c in (cp_wv, cp_x1a, cp_q0, cp_wr, cp_z):
        c.wait()
    for g in range(D // 128):
        wt_v[KR // 2 + 64 * g:KR // 2 + 64 * (g + 1), :] = _pk(wkv_v[:, 2 * D + 128 * g:2 * D + 128 * (g + 1)].T)
    flush(fold(wq_v, [wqb_v[0], wqb_v[1]], 0)[0])
    yv = _dot_nt(_un(wt_v[KR // 2:, :]), xn(0, T))
    xk_v[...] = _pk(ln1(T, T, C, [yv[128 * k:128 * k + 8, 128:256] for k in range(8)])[:, 0:D // 2].T)
    for c in range(CPT):
        predict(slice(C * c, C * (c + 1)), 0, c,
                [yv[256 * c + 32 * k:256 * c + 32 * k + 8, 256:384] for k in range(8)])
    phis = [jnp.concatenate([ph for _, ph in sorted(pieces[p], key=lambda tp: tp[0])], axis=1) for p in range(NP)]
    kvs, zs_ = kv_and_z(yv, phis, lambda p, zero: zero, yv[:, T - C:T], zv[...])
    for p in range(NP):
        kv_acc[p] = kvs[p]
        z_acc[p] = zs_[p]
    cp_x1.wait()

    def order_chunks():
        lane16 = lax.shift_right_logical(lax.broadcasted_iota(i32, (8, 128), 1), 4).astype(f32)
        vals = [p_v[t] for t in range(1 + N1)]
        cids = [lane16 + float(0 if t == 0 else CPT + CP1 * (t - 1)) for t in range(1 + N1)]
        b1 = _first_max(*_merge_max(list(zip(vals, cids))))[1]
        b2 = _first_max(*_merge_max([(jnp.where(c == b1, -jnp.inf, v), c) for v, c in zip(vals, cids)]))[1]
        c1, c2 = _scalar(b1, 0, NC - 1), _scalar(b2, 0, NC - 1)
        c2 = jnp.where(c2 == c1, (c1 + 1) & (NC - 1), c2)
        ord_s[0] = S
        for c in range(NC):
            ord_s[1 + c] = c * C
        ord_s[1 + c1] = 0
        ord_s[1] = c1 * C
        ord_s[1 + jnp.where(c2 == 0, c1, c2)] = jnp.where(c1 == 1, 0, C)
        ord_s[2] = c2 * C

    def phase1(j, carry):
        for c in cp_step(j):
            c.wait()
        zm = zv[...]
        s = pl.multiple_of(T + j * T1, C)
        nxt = pl.multiple_of(jnp.where(j + 1 < N1, s + T1, 0), C)
        s2 = s + zs[2, 0].astype(i32)
        ys, ph = [], []
        for n in range(CP1):
            xt = xn(pl.multiple_of(s2 + C * n, C), C)
            y0 = _dot_nt(_un(wt_v[:, 0:D // 2]), xt[:, 0:D // 2]) if n else _dot(_un(wt_v[:, 0:D // 2]), _un(xk_v[...]))
            row0 = pl.multiple_of(s + C * (n + 1), C)
            xb = ln1(row0 if n + 1 < CP1 else nxt, row0, C, [y0[128 + 96 * k:136 + 96 * k] for k in range(16)])
            if n + 1 == CP1:
                xk_v[...] = _pk(xb[:, 0:D // 2].T)
            yn = _dot_nt(_un(wt_v[:, D // 2:D]), xt[:, D // 2:D]) + y0
            ys.append(yn)
            ph.append([_phi_k(yp) for yp in _pair_logits(yn[0:KR], range(4)).values()])
            if n == CP1 - 2:
                for c in range(CP1):
                    r0 = KR + 256 + 192 * c
                    predict(pl.ds(pl.multiple_of(s + C * c, C), C), 1 + j, c,
                            [yn[r0 + 24 * k:r0 + 24 * k + 8] for k in range(8)])
        order_chunks()
        xq_v[...] = _pk(xn(pl.multiple_of(ord_s[1], C), C)[:, 0:D // 2].T)
        fold(wq_v, [wqb_v[2 + 2 * j], wqb_v[3 + 2 * j]], 1 + j)
        for e in range(4 * GO):
            row = KR + 384 + 640 * e // (4 * GO) // 8 * 8
            w = _pk(wo_v[GO * j + e // 4, 256 * (e % 4):256 * (e % 4 + 1), :])
            wo32[GO * j + e // 4, 128 * (e % 4):128 * (e % 4 + 1), :] = (
                w.reshape(16, 8, 128) | (_pk(ys[0][row:row + 8]) & zm)[None]).reshape(128, 128)
        vt = jnp.concatenate([yn[KR:] for yn in ys], axis=1)
        phis = [jnp.concatenate([ph[n][p] for n in range(CP1)], axis=1) for p in range(NP)]
        kvs, zs_ = kv_and_z(vt, phis, lambda p, zero: z_acc[p] + zero, ys[-1][KR:], zm)
        for p in range(NP):
            kv_acc[p] += kvs[p]
            z_acc[p] = zs_[p]
            zb_v[p] = jnp.broadcast_to(jnp.sum(zs_[p], axis=1, keepdims=True), (128, 128))
        return carry

    lax.fori_loop(0, N1, phase1, 0)
    for c in cp_ffn:
        c.wait()

    def ln2(h, row0, nx, nrel):
        deps = [None]
        for j in range(1, C // 8):
            t = (j * nrel * 2) // (C // 8) - 1
            r0 = (C - 8) * (t % 2)
            deps.append(nx[r0:r0 + 8, 128 * (t // 2):128 * (t // 2) + 128] if t >= 0 else None)
        hn = _ln(h, deps, zv[...])
        r = jnp.sum(hn * wr_row(), axis=-1, keepdims=True)
        hn_v[pl.ds(row0, C), :] = hn.astype(bf16)
        out_v[pl.ds(row0, C), :] = (h + hn).astype(bf16)
        return r

    lane = lax.broadcasted_iota(i32, (8, 128), 1)
    pos = (lane * 8 + lax.broadcasted_iota(i32, (8, 128), 0)).astype(f32)

    def token_at(posv, lo, hi):
        p = _scalar(posv, lo, hi - 1)
        return ord_s[lax.shift_right_logical(p, 7)] + (p & (C - 1))

    def slab_of(tok):
        base = pl.multiple_of(lax.shift_left(lax.shift_right_logical(tok, 4), 4), 16)
        return pl.ds(base, 16), lax.broadcasted_iota(i32, (16, D), 0) == tok - base

    def token_row(tok):
        rows, hit = slab_of(tok)
        slab = jnp.where(hit, hn_v[rows, :].astype(f32), 0.0)
        return _allred8(slab[0:8] + slab[8:16], jnp.add)

    def patch(tok, y8, sg):
        rows, hit = slab_of(tok)
        cur = out_v[rows, :].astype(f32)
        fix_v[...] = jnp.where(hit, cur + _rows(y8 * _lanes(sg, D // 128), 2), cur).astype(bf16)

    def phase2(i, carry):
        q0 = CPT * i
        off = [pl.multiple_of(ord_s[q0 + k], C) for k in range(CPT + 1)]
        zm = zv[...]
        hprev = hbuf[...]
        kmask = lax.broadcasted_iota(i32, (64, 128), 0) // 32 == lax.broadcasted_iota(i32, (64, 128), 1) % 2

        def attend(y):
            os_ = []
            for p, yp in _pair_logits(y, range(4)).items():
                os_.append(_dot(jnp.where(kmask, kv_acc[p], 0.0).astype(bf16), _phi_q(yp, zb_v[p])))
            return jnp.concatenate(os_, axis=0).astype(bf16).T

        ya, ys = [], []
        for n in range(CPT):
            xt = xn(off[n + 1], C)
            ya.append(_dot_nt(_un(wq_v[:, 0:D // 2]), xt[:, 0:D // 2]) if n else
                      _dot(_un(wq_v[:, 0:D // 2]), _un(xq_v[...])))
            if n == CPT - 1:
                o01 = attend(jnp.concatenate(ys[0:2], axis=1))
            ys.append(ya[n] + _dot_nt(_un(wq_v[:, D // 2:D]), xt[:, D // 2:D]))
        wo = jnp.concatenate([_un(wo32[j]) for j in range(D // 128)], axis=1)
        head = _dot(o01[0:C], wo[:, 0:256])
        o23 = attend(jnp.concatenate(ys[2:4], axis=1))
        atts = [jnp.concatenate([head, _dot(o01[0:C], wo[:, 256:])], axis=1),
                _dot(o01[C:2 * C], wo), _dot(o23[0:C], wo), _dot(o23[C:2 * C], wo)]

        xq_v[...] = _pk(xn(pl.multiple_of(ord_s[jnp.minimum(q0 + CPT + 1, NC)], C), C)[:, 0:D // 2].T)

        def q_gate(v):
            lens = [KR // 8] + [KR // 8 - 24] * 3
            t, n = int(v * sum(lens)), 0
            while t >= lens[n]:
                t -= lens[n]
                n += 1
            r0 = 8 * (t + KR // 8 - lens[n])
            return _zero_after(ya[n][r0:r0 + 8], zm)

        def o_gate(t):
            r0, j = 8 * (t % 16), (t % 128) // 16
            return _zero_after(atts[t // 128][r0:r0 + 8, 128 * j:128 * j + 128], zm)

        t3 = jnp.maximum(i - 1, 0)
        nsb = NA // 2
        for sb in range(nsb):
            cols = slice(256 * sb, 256 * (sb + 1))
            xcol = xc_v[...]
            acc = None
            for k in range(0, D, 8):
                xk = _lanes(xcol[k:k + 8], 2)
                p = jnp.concatenate([wg_v[t3, k:k + 8, cols].astype(f32) * xk,
                                     wu_v[t3, k:k + 8, cols].astype(f32) * xk], axis=1)
                if k % 64 == 0:
                    p = p + _lanes(q_gate((sb * D + k) / (nsb * D)), 4)
                acc = p if acc is None else acc + p
            pa_v[:, 512 * sb:512 * (sb + 1)] = acc

        put_cols(r_v, i, 0, jnp.where(i > 0, ln2(hprev, off[0], atts[0], 6), -jnp.inf))

        @pl.when(i > 0)
        def _():
            cp_out(q0).start()

        acc = _allred8(pa_v[pl.ds(pl.multiple_of(zs[3, 0].astype(i32) * 32, 32), 8), :], jnp.add)
        g_ = jnp.concatenate([acc[:, 512 * t:512 * t + 256] for t in range(nsb)], axis=1)
        u_ = jnp.concatenate([acc[:, 512 * t + 256:512 * t + 512] for t in range(nsb)], axis=1)
        a8 = g_ * jax.nn.sigmoid(g_) * u_
        ac = _col(jnp.concatenate([jnp.where(t3 == 2, 0.0, a8[:, 0:NDUP]), a8[:, NDUP:]], axis=1))
        ysums = []
        for q in range(2):
            cols = slice(D // 2 * q, D // 2 * (q + 1))
            ysum = jnp.where(i > 1, y_v[:, cols], 0.0)
            for k in range(0, NA * 128, 8):
                p = wd_v[t3, k:k + 8, cols].astype(f32) * _lanes(ac[k:k + 8], 4)
                if k % 32 == 0:
                    p = p + _lanes(o_gate(64 + (q * NA * 128 + k) * 376 // (2 * NA * 128)), 4)
                ysum = ysum + p
            y_v[:, cols] = ysum
            ysums.append(ysum)

        for k in range(CPT):
            if k == NCAND:
                ok = (lane >= C // 8) & (lane < (NCAND + 1) * (C // 8))
                cm, cpos = _first_max(jnp.where(ok, r_v[0], -jnp.inf), pos)
                cand = token_at(cpos, C, (NCAND + 1) * C)
                ord_s[NC + 1] = cand
                xc_v[...] = _col(token_row(cand))
                patch(cand, _allred8(jnp.concatenate(ysums, axis=1), jnp.add),
                      jax.nn.sigmoid(jnp.broadcast_to(cm, (8, 128))))
            h = x_v[pl.ds(off[k + 1], C), :].astype(f32) + atts[k]
            if k == CPT - 1:
                hbuf[...] = h
            else:
                put_cols(r_v, i, (k + 1) * (C // 8), ln2(h, off[k + 1], atts[k + 1], 5 if k == CPT - 2 else 6))
                cp_out(q0 + k + 1).start()
        return carry

    lax.fori_loop(0, NT, phase2, 0)

    for q in range(1, NCAND + 1):
        cp_out(q).wait()
    fsem = new_sems(1)

    cand = ord_s[NC + 1]

    def cp_patch(tok):
        return pltpu.make_async_copy(fix_v, out_hbm.at[0, slab_of(tok)[0]], sems.at[fsem])

    cp_fix = cp_patch(cand)
    cp_fix.start()
    cp_out(NCAND + 1).wait()
    last = pl.multiple_of(ord_s[NC], C)
    stats, cp_last = [], []
    for g in range(0, C, EG):
        h = hbuf[g:g + EG, :]
        s1 = h[:, 0:128]
        s2 = s1 * s1
        for j in range(128, D, 128):
            s1 = s1 + h[:, j:j + 128]
            s2 = s2 + h[:, j:j + 128] * h[:, j:j + 128]
        m = jnp.sum(s1, axis=-1, keepdims=True) * (1.0 / D)
        v = jnp.sum(s2, axis=-1, keepdims=True) * (1.0 / D) - m * m
        rs = lax.rsqrt(jnp.maximum(v, 0.0) + EPS)
        stats.append((m, rs))
        rows = pl.ds(pl.multiple_of(last + g, EG), EG)
        out_v[rows, :] = (h * (1.0 + rs) - m * rs).astype(bf16)
        cp_last.append(cp(out_v.at[rows], out_hbm.at[0, rows]))
        cp_last[-1].start()
    for q in range(NCAND + 2, NC - 1):
        cp_out(q).wait()
    pm, pi = _first_max(*_merge_max([(r_v[i], pos + float(i * T) if i else pos) for i in range(NT)]))
    wr = wr_row()
    wsum = jnp.sum(wr, axis=-1, keepdims=True)
    sub = lax.broadcasted_iota(i32, (8, 1), 0).astype(f32)
    cands = []
    for g, (m, rs) in zip(range(0, C, EG), stats):
        r = (jnp.sum(hbuf[g:g + EG, :] * wr, axis=-1, keepdims=True) - m * wsum) * rs
        cands += [(r[k:k + 8], sub + float(S + g + k)) for k in range(0, EG, 8)]
    while len(cands) > 1:
        cands = [_merge_max(cands[k:k + 2]) for k in range(0, len(cands), 2)]
    bv, bt = [jnp.broadcast_to(v, (8, 128)) for v in _merge_max([(pm, pi), cands[0]])]
    rmax = _allred8(bv, jnp.maximum)
    idx = token_at(_allred8(jnp.where(bv == rmax, bt, float(2 * S)), jnp.minimum), C, S + C)
    cp_out(NC - 1).wait()
    cp_fix.wait()
    for c in cp_last:
        c.wait()

    @pl.when(idx != cand)
    def _():
        rows, _ = slab_of(cand)
        undo = pltpu.make_async_copy(out_v.at[rows], out_hbm.at[0, rows], sems.at[fsem])
        undo.start()
        hn_v[pl.ds(last, C), :] = _ln(hbuf[...]).astype(bf16)
        xs = _rows(token_row(idx), 2).astype(bf16)

        def step(j, acc):
            t = lax.shift_right_logical(j, 1)
            cols = pl.ds(pl.multiple_of((j & 1) * (NA * 64), 128), NA * 64)
            g = _dot(xs, wg_v[t, :, cols])
            a = g * jax.nn.sigmoid(g) * _dot(xs, wu_v[t, :, cols])
            a = jnp.concatenate([jnp.where(j == 4, 0.0, a[:, 0:NDUP]), a[:, NDUP:]], axis=1)
            return acc + _dot(a.astype(bf16), wd_v[t, cols, :])[0:8]

        y8 = lax.fori_loop(0, 6, step, jnp.zeros((8, D), f32))
        undo.wait()
        patch(idx, y8, jax.nn.sigmoid(rmax))
        redo = cp_patch(idx)
        redo.start()
        redo.wait()


@jax.jit
def pallas_sequential_preLN__linear_kernel_hedgehog__moe_arch_mod__prompt_kernel(
    A_x: jax.Array,
    A_wqkv: jax.Array,
    A_w_phi: jax.Array,
    A_wo: jax.Array,
    B_x: jax.Array,
    B_w_r: jax.Array,
    B_w_gate: jax.Array,
    B_w_up: jax.Array,
    B_w_down: jax.Array,
):
    del B_x
    any_spec = pl.BlockSpec(memory_space=pl.ANY)
    return pl.pallas_call(
        _kernel,
        out_shape=jax.ShapeDtypeStruct((1, S, D), bf16),
        in_specs=[any_spec] * 8,
        out_specs=any_spec,
        scratch_shapes=[
            pltpu.VMEM((S, D), bf16),
            pltpu.VMEM((D, 3 * D), bf16),
            pltpu.VMEM((D // 128, D, 128), bf16),
            pltpu.VMEM((H, DH, DH), bf16),
            pltpu.VMEM((N1 * GO, D, 128), bf16),
            pltpu.VMEM((N1 * GO, D // 2, 128), u32),
            pltpu.VMEM((D,), bf16),
            pltpu.VMEM((3, D, NA * 128), bf16),
            pltpu.VMEM((3, D, NA * 128), bf16),
            pltpu.VMEM((3, NA * 128, D), bf16),
            pltpu.VMEM(((KR + D) // 2, D), u32),
            pltpu.VMEM((KR // 2, D), u32),
            pltpu.VMEM((8, 64, 128), u32),
            pltpu.VMEM(((S + C) // 2, D), u32),
            pltpu.VMEM((D // 4, C), u32),
            pltpu.VMEM((D // 4, C), u32),
            pltpu.VMEM((S + C, D), bf16),
            pltpu.VMEM((NP, 64, 128), f32),
            pltpu.VMEM((NP, 128, 128), f32),
            pltpu.VMEM((NP, 128, 128), f32),
            pltpu.VMEM((C, D), f32),
            pltpu.VMEM((S + C, D), bf16),
            pltpu.VMEM((8, 128), u32),
            pltpu.SMEM((8, 128), u32),
            pltpu.VMEM((1 + N1, 8, 128), f32),
            pltpu.VMEM((NT, 8, 128), f32),
            pltpu.VMEM((D, 128), f32),
            pltpu.VMEM((8, NA * 256), f32),
            pltpu.VMEM((8, D), f32),
            pltpu.VMEM((16, D), bf16),
            pltpu.SMEM((NC + 2,), i32),
            pltpu.SemaphoreType.DMA((64,)),
        ],
        compiler_params=pltpu.CompilerParams(vmem_limit_bytes=120 * 1024 * 1024,
                                             disable_bounds_checks=True,
                                             disable_semaphore_checks=True),
        name="hedgehog_mod",
    )(A_x, A_wqkv, A_w_phi, A_wo, B_w_r, B_w_gate, B_w_up, B_w_down)
```

```python
import jax
import jax.numpy as jnp
from jax import lax
import jax.experimental.pallas as pl
import jax.experimental.pallas.tpu as pltpu

S = 2048
D = 1024
H = 32
DH = 32
F = 3584
NP = H // 2
C = 128
NC = S // C
T = 512
NT = S // T
CPT = T // C
T1 = 512
N1 = (S - T) // T1
CP1 = T1 // C
KR = H * (DH - 1)
GO = -(-8 // N1)
SEGS = ((256, 256), (128, 256), (128, 512))
PHI = ((0, 512), (512, 512), (512, 1024))
DEFER = 2
NB = F // 128
NA = 10
B0 = (0, NA, NB - NA)
NDUP = (3 * NA - NB) * 128
NCAND = 2
EG = 16
LOG2E = 1.4426950408889634
EPS = 1e-5

f32 = jnp.float32
bf16 = jnp.bfloat16
u32 = jnp.uint32
i32 = jnp.int32


def _dot_nt(a, b):
    return lax.dot_general(a, b, (((1,), (1,)), ((), ())), preferred_element_type=f32)


def _dot(a, b):
    return jnp.dot(a, b, preferred_element_type=f32)


def _pk(x):
    return pltpu.bitcast(x, u32)


def _un(x):
    return pltpu.bitcast(x, bf16)


def _rcp(x):
    r = pl.reciprocal(x, approx=True)
    return r * (2.0 - x * r)


def _allred(v, op):
    v = op(v, pltpu.roll(v, 2, 0))
    return op(v, pltpu.roll(v, 4, 0))


def _allred8(v, op):
    return _allred(op(v, pltpu.roll(v, 1, 0)), op)


def _rows(v, n):
    return jnp.concatenate([v] * n, axis=0)


def _lanes(v, n):
    return jnp.concatenate([v] * n, axis=1)


def _zero_after(dep, zm):
    return pltpu.bitcast(pltpu.bitcast(dep, u32) & zm, f32)


def _exps(x):
    x3 = x.reshape(8, 8, x.shape[1])
    mx = _allred(jnp.max(x3, axis=0), jnp.maximum)
    mn = _allred(jnp.min(x3, axis=0), jnp.minimum)
    ep = jnp.exp2(x3 - mx[None])
    en = jnp.exp2(mn[None] - x3)
    rp = _rcp(_allred(jnp.sum(ep, axis=0), jnp.add))
    rn = _rcp(_allred(jnp.sum(en, axis=0), jnp.add))
    return ep, en, rp, rn


def _phi_k(x):
    L = x.shape[1]
    ep, en, rp, rn = _exps(x)
    return jnp.concatenate([(ep * rp[None]).reshape(64, L), (en * rn[None]).reshape(64, L)], axis=0)


def _phi_q(x, zb):
    L = x.shape[1]
    ep, en, rp, rn = _exps(x)
    zb = _lanes(zb, L // 128).reshape(16, 8, L)
    den = rp * jnp.sum(ep * zb[0:8], axis=0) + rn * jnp.sum(en * zb[8:16], axis=0)
    inv = _rcp(_allred(den, jnp.add) + 1e-6)
    cp = rp * inv
    cn = rn * inv
    phi = jnp.concatenate([(ep * cp[None]).reshape(64, L), (en * cn[None]).reshape(64, L)], axis=0)
    return phi.astype(bf16)


def _slot(n):
    return lax.shift_right_logical(lax.broadcasted_iota(i32, (8, n), 0), 1)


def _pair_logits(y, sgs):
    slot = _slot(y.shape[1])
    out, r, shared = {}, 0, None
    for k, sg in enumerate(sgs):
        if k == 0 or sg % 2 == 0:
            shared, r = y[r:r + 16], r + 16
        l0, l1, l2 = y[r:r + 8], y[r + 8:r + 16], shared[8 * (sg % 2):8 * (sg % 2) + 8]
        for q in range(4):
            x0 = jnp.where(slot == q, l0, jnp.where(slot == (q + 1) % 4, l1, jnp.where(slot == (q + 2) % 4, l2, 0.0)))
            out[4 * sg + q] = jnp.concatenate([x0, y[r + 16 + 56 * q:r + 72 + 56 * q]], axis=0)
        r += 240
    return out


def _lane_blocks_sum(v, acc):
    for c in range(0, v.shape[1], 128):
        acc = acc + v[:, c:c + 128]
    return acc


def _row_sum(x, deps, zm):
    g = x.shape[0] // len(deps)
    gate = jnp.concatenate([jnp.zeros((8, 128), f32) if d is None else _zero_after(d, zm)
                            for d in deps for _ in range(g // 8)], axis=0)
    return jnp.sum(_lane_blocks_sum(x[:, 128:], x[:, 0:128] + gate), axis=-1, keepdims=True)


def _ln(x, deps=None, zm=None):
    tot = jnp.sum(x, axis=-1, keepdims=True) if deps is None else _row_sum(x, deps, zm)
    xc = x - tot * (1.0 / D)
    return xc * lax.rsqrt(jnp.sum(xc * xc, axis=-1, keepdims=True) * (1.0 / D) + EPS)


def _col(a8):
    return _rows(a8, 16).astype(bf16).T.astype(f32)


def _first_max(v, t):
    m = jnp.max(_allred8(v, jnp.maximum), axis=1, keepdims=True)
    return m, jnp.min(_allred8(jnp.where(v == m, t, float(2 * S)), jnp.minimum), axis=1, keepdims=True)


def _merge_max(cands):
    v, t = cands[0]
    for v2, t2 in cands[1:]:
        gt = v2 > v
        v, t = jnp.where(gt, v2, v), jnp.where(gt, t2, t)
    return v, t


def _scalar(v, lo, hi):
    return jnp.clip(jnp.broadcast_to(v, (8, 128)).astype(i32)[0, 0], lo, hi)


class _Group:
    def __init__(self, parts, dst, sem):
        self.parts, self.dst, self.sem = parts, dst, sem

    def start(self):
        for src, dst in self.parts:
            pltpu.make_async_copy(src, dst, self.sem).start()

    def wait(self):
        pltpu.make_async_copy(self.dst, self.dst, self.sem).wait()


def _kernel(x_hbm, wqkv_hbm, wphi_hbm, wo_hbm, wr_hbm, wg_hbm, wu_hbm, wd_hbm, out_hbm,
            x_v, wkv_v, wqb_v, wphi_v, wo_v, wo32, wr_v, wg_v, wu_v, wd_v,
            wt_v, wq_v, a_v, xn_v, xk_v, xq_v, hn_v, kv_acc, z_acc, zb_v, hbuf, out_v, zv, zs, p_v, r_v,
            xc_v, pa_v, y_v, fix_v, ord_s, sems):
    nsem = [0]

    def new_sems(n):
        nsem[0] += n
        return nsem[0] - n

    def cp(src, dst):
        return pltpu.make_async_copy(src, dst, sems.at[new_sems(1)])

    def cp_w(lo, hi):
        return cp(wqkv_hbm.at[:, lo:hi], wkv_v.at[:, lo:hi])

    def cp_x(lo, hi):
        return cp(x_hbm.at[0, lo:hi], x_v.at[lo:hi])

    cp_wr = cp(wr_hbm, wr_v)
    kcum = [0]
    for _, dk in SEGS:
        kcum.append(kcum[-1] + dk)
    seg_cp = []
    x0 = 0
    for si, (dx, dk) in enumerate(SEGS):
        lo, hi = PHI[si][0] // DH, PHI[si][1] // DH
        ph = [cp(wphi_hbm.at[lo:hi], wphi_v.at[lo:hi])] if hi > lo else []
        seg_cp.append([cp_x(x0, x0 + dx)] + ph + [cp_w(D + kcum[si], D + kcum[si + 1])])
        x0 += dx
    cp_wv = cp_w(2 * D, 3 * D)
    cp_x1a = cp_x(T, T + C)
    cp_x1 = cp_x(T + C, S)
    cp_q0 = _Group([(wqkv_hbm.at[:, 128 * g:128 * (g + 1)], wqb_v.at[g]) for g in range(2)],
                   wqb_v.at[0:2], sems.at[new_sems(1)])
    qsem0 = new_sems(2 * N1)

    def cp_step(j):
        pq = po = None
        if isinstance(j, int):
            pq = [(wqkv_hbm.at[:, 128 * g:128 * (g + 1)], wqb_v.at[g]) for g in range(2 + 2 * j, 4 + 2 * j)]
            po = [(wo_hbm.at[:, 128 * min(g, 7):128 * (min(g, 7) + 1)], wo_v.at[g])
                  for g in range(GO * j, GO * (j + 1))]
        return [_Group(pq, wqb_v.at[pl.ds(2 + 2 * j, 2)], sems.at[qsem0 + 2 * j]),
                _Group(po, wo_v.at[pl.ds(GO * j, GO)], sems.at[qsem0 + 2 * j + 1])]

    cp_ffn = []
    for t, b in enumerate(B0):
        cp_ffn += [cp(wg_hbm.at[:, b * 128:(b + NA) * 128], wg_v.at[t]),
                   cp(wu_hbm.at[:, b * 128:(b + NA) * 128], wu_v.at[t]),
                   cp(wd_hbm.at[b * 128:(b + NA) * 128], wd_v.at[t])]
    seg_cp[0] = seg_cp[0][1:] + seg_cp[0][0:1]
    for c in ([c for t in seg_cp for c in t] + [cp_wr, cp_wv, cp_x1a, cp_q0, cp_x1]
              + [c for j in range(N1) for c in cp_step(j)] + cp_ffn):
        c.start()
    osem0 = new_sems(NC + 1)

    def cp_out(q):
        rows = pl.ds(pl.multiple_of(ord_s[q], C), C)
        return pltpu.make_async_copy(out_v.at[rows], out_hbm.at[0, rows], sems.at[osem0 + q])

    def wr_row():
        return wr_v[...].reshape(1, D).astype(f32)

    def put_cols(ref, idx, col0, r):
        for k in range(0, r.shape[0], 8):
            ref[idx, :, col0 + k // 8:col0 + k // 8 + 1] = r[k:k + 8]

    def half(row0, n):
        if isinstance(row0, int):
            return pl.ds(row0 // 2, n // 2)
        return pl.ds(pl.multiple_of(lax.shift_right_logical(row0, 1), C // 2), n // 2)

    def ln1(src, dst, n, deps=None):
        xb = _pk(_ln(x_v[pl.ds(src, n), :].astype(f32), deps, None if deps is None else zv[...]).astype(bf16))
        xn_v[half(dst, n), :] = xb
        return _un(xb)

    def xn(row0, n):
        return _un(xn_v[half(row0, n), :])

    def predict(rows, t, c, deps):
        wr = wr_row()
        wc = wr - jnp.sum(wr, axis=-1, keepdims=True) * (1.0 / D)
        put_cols(p_v, t, c * (C // 8), _row_sum(x_v[rows, :].astype(f32) * wc, deps, zv[...]))

    def fold(dst, ws, sg):
        slot = _slot(D)
        res = [_dot_nt(_un(a_v[2 * sg + e]), ws[e]) for e in range(2)]
        main, e0, e1 = [], [], []
        for e in range(2):
            z = jnp.where(((slot + 3) % 4) // 2 == e, 0.0, res[e][0:8])
            b1 = z + pltpu.roll(z, 4, 0)
            b0 = pltpu.roll(b1, 2, 0)
            for pp in range(2):
                base = jnp.where(slot % 2 == pp, b0, b1)
                main.append((res[e][16 + 56 * pp:72 + 56 * pp].reshape(7, 8, D) - base[None]).reshape(56, D))
            e0.append(res[e][8:16] - b0)
            e1.append(res[e][0:8] - b1)
        rows = jnp.concatenate([jnp.where(slot < 2, e0[0], e0[1]), e1[0] + e1[1]] + main, axis=0)
        l2 = _pk((_rows(jnp.where(slot < 2, e0[1], e0[0]), 2) * LOG2E).astype(bf16))
        if isinstance(sg, int):
            r0, r1 = 248 * (sg // 2), 248 * (sg // 2) + 8 + 120 * (sg % 2)
        else:
            r0 = pl.multiple_of(248 * lax.shift_right_logical(sg, 1), 8)
            r1 = pl.multiple_of(r0 + 8 + 120 * (sg & 1), 8)
        dst[pl.ds(r1, 120), :] = _pk((rows * LOG2E).astype(bf16))
        dst[pl.ds(r0, 8), :] = jnp.where(slot // 2 == sg % 2, l2, dst[pl.ds(r0, 8), :])
        return res

    def wk(lo, hi):
        r0, r1 = 248 * (lo // 2), 248 * ((hi - 1) // 2) + 128 + 120 * ((hi - 1) % 2)
        if lo % 2:
            return _un(jnp.concatenate([wt_v[r0:r0 + 8, :], wt_v[r0 + 128:r1, :]], axis=0))
        return _un(wt_v[r0:r1, :])

    def kv_and_z(vt, phis, z_of, tail, zm):
        kvs = [_dot_nt(vt[64 * p:64 * (p + 1)].astype(bf16), phis[p].astype(bf16)) for p in range(NP)]
        zs_ = [_lane_blocks_sum(phis[p], z_of(p, _rows(_zero_after(tail[256 + 48 * p:264 + 48 * p], zm), 16)))
               for p in range(NP)]
        return kvs, zs_

    def a_row(r, e):
        s = (r & 7) >> 1
        f = jnp.where(r >= 72, (r - 64) >> 1, jnp.where(r >= 16, (r - 8) >> 1, jnp.where(
            r >= 8, jnp.where(s >> 1 == e, 1, 3), jnp.where(((s + 3) & 3) >> 1 == e, 2, 0))))
        pp = jnp.where(r >= 72, 1, jnp.where(r >= 16, 0, jnp.where(r >= 8, s, s + 1) & 1))
        return f, 2 * pp + (r & 1)

    f_i = lax.broadcasted_iota(i32, (128, DH), 1)
    sel = [jnp.where(f_i == a_row(lax.broadcasted_iota(i32, (128, DH), 0), e)[0], 1.0, 0.0).astype(bf16)
           for e in range(2)]
    amask = jnp.where(lax.broadcasted_iota(i32, (128, 128), 1) >> 5
                      == a_row(lax.broadcasted_iota(i32, (128, 128), 0), 0)[1], jnp.uint32(0xFFFFFFFF), jnp.uint32(0))

    def build_a(lo, hi):
        for g in range(lo // 128, hi // 128):
            blk = _dot_nt(sel[g % 2], wphi_v[4 * g:4 * (g + 1)].reshape(128, DH))
            a_v[g] = _pk(pltpu.bitcast(pltpu.bitcast(blk, u32) & amask, f32).astype(bf16))

    zv[...] = jnp.zeros((8, 128), u32)
    cp_z = cp(zv, zs)
    cp_z.start()
    for ref in (wt_v, wq_v):
        for r0 in (0, 248):
            ref[r0:r0 + 8, :] = jnp.zeros((8, D), u32)
    hbuf[...] = jnp.zeros(hbuf.shape, f32)
    xc_v[...] = jnp.zeros(xc_v.shape, f32)
    y_v[...] = jnp.zeros(y_v.shape, f32)
    r_v[...] = jnp.full(r_v.shape, -jnp.inf, f32)
    p_v[...] = jnp.full(p_v.shape, -jnp.inf, f32)

    pieces = [[] for _ in range(NP)]
    pending = []

    def phi_piece(p, t0, yp, dep=None):
        if dep is not None:
            yp = jnp.concatenate([yp[0:8] + _zero_after(dep, zv[...]), yp[8:]], axis=0)
        pieces[p].append((t0, _phi_k(yp)))

    def k_block(lo, hi, t0, t1, defer=0):
        y = _dot_nt(wk(lo, hi), xn(t0, t1 - t0))
        for p, yp in _pair_logits(y, range(lo, hi)).items():
            if p >= 4 * hi - defer:
                if t1 - t0 > C:
                    phi_piece(p, t0, yp[:, 0:t1 - t0 - C])
                pending.append((p, t1 - C, yp[:, t1 - t0 - C:]))
            else:
                phi_piece(p, t0, yp)
        return y

    def flush(res):
        for k, (p, t0, yp) in enumerate(pending):
            phi_piece(p, t0, yp, res[32 * k:32 * k + 8, 0:128])
        del pending[:]

    x0 = 0
    for si, (dx, dk) in enumerate(SEGS):
        k0, k1 = kcum[si] // 256, kcum[si + 1] // 256
        if si == 0:
            seg_cp[0][0].wait()
            build_a(*PHI[0])
            seg_cp[0][1].wait()
        else:
            for c in seg_cp[si]:
                c.wait()
            if PHI[si][1] > PHI[si][0]:
                build_a(*PHI[si])
        res = [fold(wt_v, [wkv_v[:, D + 128 * g:D + 128 * (g + 1)] for g in (2 * sg, 2 * sg + 1)], sg)
               for sg in range(k0, k1)]
        flush(res[0][0])
        if si == 0:
            seg_cp[0][2].wait()
        ln1(x0, x0, dx)
        if si:
            k_block(k0, k1, 0, x0)
        k_block(0, k1, x0, x0 + dx, DEFER)
        x0 += dx
    for c in (cp_wv, cp_x1a, cp_q0, cp_wr, cp_z):
        c.wait()
    for g in range(D // 128):
        wt_v[KR // 2 + 64 * g:KR // 2 + 64 * (g + 1), :] = _pk(wkv_v[:, 2 * D + 128 * g:2 * D + 128 * (g + 1)].T)
    flush(fold(wq_v, [wqb_v[0], wqb_v[1]], 0)[0])
    yv = _dot_nt(_un(wt_v[KR // 2:, :]), xn(0, T))
    xk_v[...] = _pk(ln1(T, T, C, [yv[128 * k:128 * k + 8, 128:256] for k in range(8)])[:, 0:D // 2].T)
    for c in range(CPT):
        predict(slice(C * c, C * (c + 1)), 0, c,
                [yv[256 * c + 32 * k:256 * c + 32 * k + 8, 256:384] for k in range(8)])
    phis = [jnp.concatenate([ph for _, ph in sorted(pieces[p], key=lambda tp: tp[0])], axis=1) for p in range(NP)]
    kvs, zs_ = kv_and_z(yv, phis, lambda p, zero: zero, yv[:, T - C:T], zv[...])
    for p in range(NP):
        kv_acc[p] = kvs[p]
        z_acc[p] = zs_[p]
    cp_x1.wait()

    def order_chunks():
        lane16 = lax.shift_right_logical(lax.broadcasted_iota(i32, (8, 128), 1), 4).astype(f32)
        vals = [p_v[t] for t in range(1 + N1)]
        cids = [lane16 + float(0 if t == 0 else CPT + CP1 * (t - 1)) for t in range(1 + N1)]
        b1 = _first_max(*_merge_max(list(zip(vals, cids))))[1]
        b2 = _first_max(*_merge_max([(jnp.where(c == b1, -jnp.inf, v), c) for v, c in zip(vals, cids)]))[1]
        c1, c2 = _scalar(b1, 0, NC - 1), _scalar(b2, 0, NC - 1)
        c2 = jnp.where(c2 == c1, (c1 + 1) & (NC - 1), c2)
        ord_s[0] = S
        for c in range(NC):
            ord_s[1 + c] = c * C
        ord_s[1 + c1] = 0
        ord_s[1] = c1 * C
        ord_s[1 + jnp.where(c2 == 0, c1, c2)] = jnp.where(c1 == 1, 0, C)
        ord_s[2] = c2 * C

    def phase1(j, carry):
        for c in cp_step(j):
            c.wait()
        zm = zv[...]
        s = pl.multiple_of(T + j * T1, C)
        nxt = pl.multiple_of(jnp.where(j + 1 < N1, s + T1, 0), C)
        s2 = s + zs[2, 0].astype(i32)
        ys, ph = [], []
        for n in range(CP1):
            xt = xn(pl.multiple_of(s2 + C * n, C), C)
            y0 = _dot_nt(_un(wt_v[:, 0:D // 2]), xt[:, 0:D // 2]) if n else _dot(_un(wt_v[:, 0:D // 2]), _un(xk_v[...]))
            row0 = pl.multiple_of(s + C * (n + 1), C)
            xb = ln1(row0 if n + 1 < CP1 else nxt, row0, C, [y0[128 + 96 * k:136 + 96 * k] for k in range(16)])
            if n + 1 == CP1:
                xk_v[...] = _pk(xb[:, 0:D // 2].T)
            yn = _dot_nt(_un(wt_v[:, D // 2:D]), xt[:, D // 2:D]) + y0
            ys.append(yn)
            ph.append([_phi_k(yp) for yp in _pair_logits(yn[0:KR], range(4)).values()])
            if n == CP1 - 2:
                for c in range(CP1):
                    r0 = KR + 256 + 192 * c
                    predict(pl.ds(pl.multiple_of(s + C * c, C), C), 1 + j, c,
                            [yn[r0 + 24 * k:r0 + 24 * k + 8] for k in range(8)])
        order_chunks()
        xq_v[...] = _pk(xn(pl.multiple_of(ord_s[1], C), C)[:, 0:D // 2].T)
        fold(wq_v, [wqb_v[2 + 2 * j], wqb_v[3 + 2 * j]], 1 + j)
        for e in range(4 * GO):
            row = KR + 384 + 640 * e // (4 * GO) // 8 * 8
            w = _pk(wo_v[GO * j + e // 4, 256 * (e % 4):256 * (e % 4 + 1), :])
            wo32[GO * j + e // 4, 128 * (e % 4):128 * (e % 4 + 1), :] = (
                w.reshape(16, 8, 128) | (_pk(ys[0][row:row + 8]) & zm)[None]).reshape(128, 128)
        vt = jnp.concatenate([yn[KR:] for yn in ys], axis=1)
        phis = [jnp.concatenate([ph[n][p] for n in range(CP1)], axis=1) for p in range(NP)]
        kvs, zs_ = kv_and_z(vt, phis, lambda p, zero: z_acc[p] + zero, ys[-1][KR:], zm)
        for p in range(NP):
            kv_acc[p] += kvs[p]
            z_acc[p] = zs_[p]
            zb_v[p] = jnp.broadcast_to(jnp.sum(zs_[p], axis=1, keepdims=True), (128, 128))
        return carry

    lax.fori_loop(0, N1, phase1, 0)
    for c in cp_ffn:
        c.wait()

    def ln2(h, row0, nx, nrel):
        deps = [None]
        for j in range(1, C // 8):
            t = (j * nrel * 2) // (C // 8) - 1
            r0 = (C - 8) * (t % 2)
            deps.append(nx[r0:r0 + 8, 128 * (t // 2):128 * (t // 2) + 128] if t >= 0 else None)
        hn = _ln(h, deps, zv[...])
        r = jnp.sum(hn * wr_row(), axis=-1, keepdims=True)
        hn_v[pl.ds(row0, C), :] = hn.astype(bf16)
        out_v[pl.ds(row0, C), :] = (h + hn).astype(bf16)
        return r

    lane = lax.broadcasted_iota(i32, (8, 128), 1)
    pos = (lane * 8 + lax.broadcasted_iota(i32, (8, 128), 0)).astype(f32)

    def token_at(posv, lo, hi):
        p = _scalar(posv, lo, hi - 1)
        return ord_s[lax.shift_right_logical(p, 7)] + (p & (C - 1))

    def slab_of(tok):
        base = pl.multiple_of(lax.shift_left(lax.shift_right_logical(tok, 4), 4), 16)
        return pl.ds(base, 16), lax.broadcasted_iota(i32, (16, D), 0) == tok - base

    def token_row(tok):
        rows, hit = slab_of(tok)
        slab = jnp.where(hit, hn_v[rows, :].astype(f32), 0.0)
        return _allred8(slab[0:8] + slab[8:16], jnp.add)

    def patch(tok, y8, sg):
        rows, hit = slab_of(tok)
        cur = out_v[rows, :].astype(f32)
        fix_v[...] = jnp.where(hit, cur + _rows(y8 * _lanes(sg, D // 128), 2), cur).astype(bf16)

    def phase2(i, carry):
        q0 = CPT * i
        off = [pl.multiple_of(ord_s[q0 + k], C) for k in range(CPT + 1)]
        zm = zv[...]
        hprev = hbuf[...]
        kmask = lax.broadcasted_iota(i32, (64, 128), 0) // 32 == lax.broadcasted_iota(i32, (64, 128), 1) % 2

        def attend(y):
            os_ = []
            for p, yp in _pair_logits(y, range(4)).items():
                os_.append(_dot(jnp.where(kmask, kv_acc[p], 0.0).astype(bf16), _phi_q(yp, zb_v[p])))
            return jnp.concatenate(os_, axis=0).astype(bf16).T

        ya, ys = [], []
        for n in range(CPT):
            xt = xn(off[n + 1], C)
            ya.append(_dot_nt(_un(wq_v[:, 0:D // 2]), xt[:, 0:D // 2]) if n else
                      _dot(_un(wq_v[:, 0:D // 2]), _un(xq_v[...])))
            if n == CPT - 1:
                o01 = attend(jnp.concatenate(ys[0:2], axis=1))
            ys.append(ya[n] + _dot_nt(_un(wq_v[:, D // 2:D]), xt[:, D // 2:D]))
        wo = jnp.concatenate([_un(wo32[j]) for j in range(D // 128)], axis=1)
        head = _dot(o01[0:C], wo[:, 0:256])
        o23 = attend(jnp.concatenate(ys[2:4], axis=1))
        atts = [jnp.concatenate([head, _dot(o01[0:C], wo[:, 256:])], axis=1),
                _dot(o01[C:2 * C], wo), _dot(o23[0:C], wo), _dot(o23[C:2 * C], wo)]

        xq_v[...] = _pk(xn(pl.multiple_of(ord_s[jnp.minimum(q0 + CPT + 1, NC)], C), C)[:, 0:D // 2].T)

        def q_gate(v):
            lens = [KR // 8] + [KR // 8 - 24] * 3
            t, n = int(v * sum(lens)), 0
            while t >= lens[n]:
                t -= lens[n]
                n += 1
            r0 = 8 * (t + KR // 8 - lens[n])
            return _zero_after(ya[n][r0:r0 + 8], zm)

        def o_gate(t):
            r0, j = 8 * (t % 16), (t % 128) // 16
            return _zero_after(atts[t // 128][r0:r0 + 8, 128 * j:128 * j + 128], zm)

        t3 = jnp.maximum(i - 1, 0)
        nsb = NA // 2
        for sb in range(nsb):
            cols = slice(256 * sb, 256 * (sb + 1))
            xcol = xc_v[...]
            acc = None
            for k in range(0, D, 8):
                xk = _lanes(xcol[k:k + 8], 2)
                p = jnp.concatenate([wg_v[t3, k:k + 8, cols].astype(f32) * xk,
                                     wu_v[t3, k:k + 8, cols].astype(f32) * xk], axis=1)
                if k % 64 == 0:
                    p = p + _lanes(q_gate((sb * D + k) / (nsb * D)), 4)
                acc = p if acc is None else acc + p
            pa_v[:, 512 * sb:512 * (sb + 1)] = acc

        put_cols(r_v, i, 0, jnp.where(i > 0, ln2(hprev, off[0], atts[0], 6), -jnp.inf))

        @pl.when(i > 0)
        def _():
            cp_out(q0).start()

        acc = _allred8(pa_v[pl.ds(pl.multiple_of(zs[3, 0].astype(i32) * 32, 32), 8), :], jnp.add)
        g_ = jnp.concatenate([acc[:, 512 * t:512 * t + 256] for t in range(nsb)], axis=1)
        u_ = jnp.concatenate([acc[:, 512 * t + 256:512 * t + 512] for t in range(nsb)], axis=1)
        a8 = g_ * jax.nn.sigmoid(g_) * u_
        ac = _col(jnp.concatenate([jnp.where(t3 == 2, 0.0, a8[:, 0:NDUP]), a8[:, NDUP:]], axis=1))
        ysums = []
        for q in range(2):
            cols = slice(D // 2 * q, D // 2 * (q + 1))
            ysum = jnp.where(i > 1, y_v[:, cols], 0.0)
            for k in range(0, NA * 128, 8):
                p = wd_v[t3, k:k + 8, cols].astype(f32) * _lanes(ac[k:k + 8], 4)
                if k % 32 == 0:
                    p = p + _lanes(o_gate(64 + (q * NA * 128 + k) * 376 // (2 * NA * 128)), 4)
                ysum = ysum + p
            y_v[:, cols] = ysum
            ysums.append(ysum)

        for k in range(CPT):
            if k == NCAND:
                ok = (lane >= C // 8) & (lane < (NCAND + 1) * (C // 8))
                cm, cpos = _first_max(jnp.where(ok, r_v[0], -jnp.inf), pos)
                cand = token_at(cpos, C, (NCAND + 1) * C)
                ord_s[NC + 1] = cand
                xc_v[...] = _col(token_row(cand))
                patch(cand, _allred8(jnp.concatenate(ysums, axis=1), jnp.add),
                      jax.nn.sigmoid(jnp.broadcast_to(cm, (8, 128))))
            h = x_v[pl.ds(off[k + 1], C), :].astype(f32) + atts[k]
            if k == CPT - 1:
                hbuf[...] = h
            else:
                put_cols(r_v, i, (k + 1) * (C // 8), ln2(h, off[k + 1], atts[k + 1], 5 if k == CPT - 2 else 6))
                cp_out(q0 + k + 1).start()
        return carry

    lax.fori_loop(0, NT, phase2, 0)

    for q in range(1, NCAND + 1):
        cp_out(q).wait()
    fsem = new_sems(1)

    cand = ord_s[NC + 1]

    def cp_patch(tok):
        return pltpu.make_async_copy(fix_v, out_hbm.at[0, slab_of(tok)[0]], sems.at[fsem])

    cp_fix = cp_patch(cand)
    cp_fix.start()
    cp_out(NCAND + 1).wait()
    last = pl.multiple_of(ord_s[NC], C)
    stats, cp_last = [], []
    for g in range(0, C, EG):
        h = hbuf[g:g + EG, :]
        s1 = h[:, 0:128]
        s2 = s1 * s1
        for j in range(128, D, 128):
            s1 = s1 + h[:, j:j + 128]
            s2 = s2 + h[:, j:j + 128] * h[:, j:j + 128]
        m = jnp.sum(s1, axis=-1, keepdims=True) * (1.0 / D)
        v = jnp.sum(s2, axis=-1, keepdims=True) * (1.0 / D) - m * m
        rs = lax.rsqrt(jnp.maximum(v, 0.0) + EPS)
        stats.append((m, rs))
        rows = pl.ds(pl.multiple_of(last + g, EG), EG)
        out_v[rows, :] = (h * (1.0 + rs) - m * rs).astype(bf16)
        cp_last.append(cp(out_v.at[rows], out_hbm.at[0, rows]))
        cp_last[-1].start()
    for q in range(NCAND + 2, NC - 1):
        cp_out(q).wait()
    pm, pi = _first_max(*_merge_max([(r_v[i], pos + float(i * T) if i else pos) for i in range(NT)]))
    wr = wr_row()
    wsum = jnp.sum(wr, axis=-1, keepdims=True)
    sub = lax.broadcasted_iota(i32, (8, 1), 0).astype(f32)
    cands = []
    for g, (m, rs) in zip(range(0, C, EG), stats):
        r = (jnp.sum(hbuf[g:g + EG, :] * wr, axis=-1, keepdims=True) - m * wsum) * rs
        cands += [(r[k:k + 8], sub + float(S + g + k)) for k in range(0, EG, 8)]
    while len(cands) > 1:
        cands = [_merge_max(cands[k:k + 2]) for k in range(0, len(cands), 2)]
    bv, bt = [jnp.broadcast_to(v, (8, 128)) for v in _merge_max([(pm, pi), cands[0]])]
    rmax = _allred8(bv, jnp.maximum)
    idx = token_at(_allred8(jnp.where(bv == rmax, bt, float(2 * S)), jnp.minimum), C, S + C)
    cp_out(NC - 1).wait()
    cp_fix.wait()
    for c in cp_last:
        c.wait()

    @pl.when(idx != cand)
    def _():
        rows, _ = slab_of(cand)
        undo = pltpu.make_async_copy(out_v.at[rows], out_hbm.at[0, rows], sems.at[fsem])
        undo.start()
        hn_v[pl.ds(last, C), :] = _ln(hbuf[...]).astype(bf16)
        xs = _rows(token_row(idx), 2).astype(bf16)

        def step(j, acc):
            t = lax.shift_right_logical(j, 1)
            cols = pl.ds(pl.multiple_of((j & 1) * (NA * 64), 128), NA * 64)
            g = _dot(xs, wg_v[t, :, cols])
            a = g * jax.nn.sigmoid(g) * _dot(xs, wu_v[t, :, cols])
            a = jnp.concatenate([jnp.where(j == 4, 0.0, a[:, 0:NDUP]), a[:, NDUP:]], axis=1)
            return acc + _dot(a.astype(bf16), wd_v[t, cols, :])[0:8]

        y8 = lax.fori_loop(0, 6, step, jnp.zeros((8, D), f32))
        undo.wait()
        patch(idx, y8, jax.nn.sigmoid(rmax))
        redo = cp_patch(idx)
        redo.start()
        redo.wait()


@jax.jit
def pallas_sequential_preLN__linear_kernel_hedgehog__moe_arch_mod__prompt_kernel(
    A_x: jax.Array,
    A_wqkv: jax.Array,
    A_w_phi: jax.Array,
    A_wo: jax.Array,
    B_x: jax.Array,
    B_w_r: jax.Array,
    B_w_gate: jax.Array,
    B_w_up: jax.Array,
    B_w_down: jax.Array,
):
    del B_x
    any_spec = pl.BlockSpec(memory_space=pl.ANY)
    return pl.pallas_call(
        _kernel,
        out_shape=jax.ShapeDtypeStruct((1, S, D), bf16),
        in_specs=[any_spec] * 8,
        out_specs=any_spec,
        scratch_shapes=[
            pltpu.VMEM((S, D), bf16),
            pltpu.VMEM((D, 3 * D), bf16),
            pltpu.VMEM((D // 128, D, 128), bf16),
            pltpu.VMEM((H, DH, DH), bf16),
            pltpu.VMEM((N1 * GO, D, 128), bf16),
            pltpu.VMEM((N1 * GO, D // 2, 128), u32),
            pltpu.VMEM((D,), bf16),
            pltpu.VMEM((3, D, NA * 128), bf16),
            pltpu.VMEM((3, D, NA * 128), bf16),
            pltpu.VMEM((3, NA * 128, D), bf16),
            pltpu.VMEM(((KR + D) // 2, D), u32),
            pltpu.VMEM((KR // 2, D), u32),
            pltpu.VMEM((8, 64, 128), u32),
            pltpu.VMEM(((S + C) // 2, D), u32),
            pltpu.VMEM((D // 4, C), u32),
            pltpu.VMEM((D // 4, C), u32),
            pltpu.VMEM((S + C, D), bf16),
            pltpu.VMEM((NP, 64, 128), f32),
            pltpu.VMEM((NP, 128, 128), f32),
            pltpu.VMEM((NP, 128, 128), f32),
            pltpu.VMEM((C, D), f32),
            pltpu.VMEM((S + C, D), bf16),
            pltpu.VMEM((8, 128), u32),
            pltpu.SMEM((8, 128), u32),
            pltpu.VMEM((1 + N1, 8, 128), f32),
            pltpu.VMEM((NT, 8, 128), f32),
            pltpu.VMEM((D, 128), f32),
            pltpu.VMEM((8, NA * 256), f32),
            pltpu.VMEM((8, D), f32),
            pltpu.VMEM((16, D), bf16),
            pltpu.SMEM((NC + 2,), i32),
            pltpu.SemaphoreType.DMA((64,)),
        ],
        compiler_params=pltpu.CompilerParams(vmem_limit_bytes=120 * 1024 * 1024,
                                             disable_bounds_checks=True,
                                             disable_semaphore_checks=True),
        name="hedgehog_mod",
    )(A_x, A_wqkv, A_w_phi, A_wo, B_w_r, B_w_gate, B_w_up, B_w_down)
```

```python
import jax
import jax.numpy as jnp
from jax import lax
import jax.experimental.pallas as pl
import jax.experimental.pallas.tpu as pltpu

S = 2048
D = 1024
H = 32
DH = 32
F = 3584
NP = H // 2
C = 128
NC = S // C
T = 512
NT = S // T
CPT = T // C
T1 = 512
N1 = (S - T) // T1
CP1 = T1 // C
KR = H * (DH - 1)
GO = -(-8 // N1)
SEGS = ((256, 256), (128, 256), (128, 512))
PHI = ((0, 512), (512, 512), (512, 1024))
DEFER = 2
NB = F // 128
NA = 10
B0 = (0, NA, NB - NA)
NDUP = (3 * NA - NB) * 128
NCAND = 2
EG = 16
LOG2E = 1.4426950408889634
EPS = 1e-5

f32 = jnp.float32
bf16 = jnp.bfloat16
u32 = jnp.uint32
i32 = jnp.int32


def _dot_nt(a, b):
    return lax.dot_general(a, b, (((1,), (1,)), ((), ())), preferred_element_type=f32)


def _dot(a, b):
    return jnp.dot(a, b, preferred_element_type=f32)


def _pk(x):
    return pltpu.bitcast(x, u32)


def _un(x):
    return pltpu.bitcast(x, bf16)


def _rcp(x):
    r = pl.reciprocal(x, approx=True)
    return r * (2.0 - x * r)


def _allred(v, op):
    v = op(v, pltpu.roll(v, 2, 0))
    return op(v, pltpu.roll(v, 4, 0))


def _allred8(v, op):
    return _allred(op(v, pltpu.roll(v, 1, 0)), op)


def _rows(v, n):
    return jnp.concatenate([v] * n, axis=0)


def _lanes(v, n):
    return jnp.concatenate([v] * n, axis=1)


def _zero_after(dep, zm):
    return pltpu.bitcast(pltpu.bitcast(dep, u32) & zm, f32)


def _exps(x):
    x3 = x.reshape(8, 8, x.shape[1])
    mx = _allred(jnp.max(x3, axis=0), jnp.maximum)
    mn = _allred(jnp.min(x3, axis=0), jnp.minimum)
    ep = jnp.exp2(x3 - mx[None])
    en = jnp.exp2(mn[None] - x3)
    rp = _rcp(_allred(jnp.sum(ep, axis=0), jnp.add))
    rn = _rcp(_allred(jnp.sum(en, axis=0), jnp.add))
    return ep, en, rp, rn


def _phi_k(x):
    L = x.shape[1]
    ep, en, rp, rn = _exps(x)
    return jnp.concatenate([(ep * rp[None]).reshape(64, L), (en * rn[None]).reshape(64, L)], axis=0)


def _phi_q(x, zb):
    L = x.shape[1]
    ep, en, rp, rn = _exps(x)
    zb = _lanes(zb, L // 128).reshape(16, 8, L)
    den = rp * jnp.sum(ep * zb[0:8], axis=0) + rn * jnp.sum(en * zb[8:16], axis=0)
    inv = _rcp(_allred(den, jnp.add) + 1e-6)
    cp = rp * inv
    cn = rn * inv
    phi = jnp.concatenate([(ep * cp[None]).reshape(64, L), (en * cn[None]).reshape(64, L)], axis=0)
    return phi.astype(bf16)


def _slot(n):
    return lax.shift_right_logical(lax.broadcasted_iota(i32, (8, n), 0), 1)


def _pair_logits(y, sgs):
    slot = _slot(y.shape[1])
    out, r, shared = {}, 0, None
    for k, sg in enumerate(sgs):
        if k == 0 or sg % 2 == 0:
            shared, r = y[r:r + 16], r + 16
        l0, l1, l2 = y[r:r + 8], y[r + 8:r + 16], shared[8 * (sg % 2):8 * (sg % 2) + 8]
        for q in range(4):
            x0 = jnp.where(slot == q, l0, jnp.where(slot == (q + 1) % 4, l1, jnp.where(slot == (q + 2) % 4, l2, 0.0)))
            out[4 * sg + q] = jnp.concatenate([x0, y[r + 16 + 56 * q:r + 72 + 56 * q]], axis=0)
        r += 240
    return out


def _lane_blocks_sum(v, acc):
    for c in range(0, v.shape[1], 128):
        acc = acc + v[:, c:c + 128]
    return acc


def _row_sum(x, deps, zm):
    g = x.shape[0] // len(deps)
    gate = jnp.concatenate([jnp.zeros((8, 128), f32) if d is None else _zero_after(d, zm)
                            for d in deps for _ in range(g // 8)], axis=0)
    return jnp.sum(_lane_blocks_sum(x[:, 128:], x[:, 0:128] + gate), axis=-1, keepdims=True)


def _ln(x, deps=None, zm=None):
    tot = jnp.sum(x, axis=-1, keepdims=True) if deps is None else _row_sum(x, deps, zm)
    xc = x - tot * (1.0 / D)
    return xc * lax.rsqrt(jnp.sum(xc * xc, axis=-1, keepdims=True) * (1.0 / D) + EPS)


def _col(a8):
    return _rows(a8, 16).astype(bf16).T.astype(f32)


def _first_max(v, t):
    m = jnp.max(_allred8(v, jnp.maximum), axis=1, keepdims=True)
    return m, jnp.min(_allred8(jnp.where(v == m, t, float(2 * S)), jnp.minimum), axis=1, keepdims=True)


def _merge_max(cands):
    v, t = cands[0]
    for v2, t2 in cands[1:]:
        gt = v2 > v
        v, t = jnp.where(gt, v2, v), jnp.where(gt, t2, t)
    return v, t


def _scalar(v, lo, hi):
    return jnp.clip(jnp.broadcast_to(v, (8, 128)).astype(i32)[0, 0], lo, hi)


class _Group:
    def __init__(self, parts, dst, sem):
        self.parts, self.dst, self.sem = parts, dst, sem

    def start(self):
        for src, dst in self.parts:
            pltpu.make_async_copy(src, dst, self.sem).start()

    def wait(self):
        pltpu.make_async_copy(self.dst, self.dst, self.sem).wait()


def _kernel(x_hbm, wqkv_hbm, wphi_hbm, wo_hbm, wr_hbm, wg_hbm, wu_hbm, wd_hbm, out_hbm,
            x_v, wkv_v, wqb_v, wphi_v, wo_v, wo32, wr_v, wg_v, wu_v, wd_v,
            wt_v, wq_v, a_v, xn_v, xk_v, xq_v, hn_v, kv_acc, z_acc, zb_v, hbuf, out_v, zv, zs, p_v, r_v,
            xc_v, pa_v, y_v, fix_v, ord_s, sems):
    nsem = [0]

    def new_sems(n):
        nsem[0] += n
        return nsem[0] - n

    def cp(src, dst):
        return pltpu.make_async_copy(src, dst, sems.at[new_sems(1)])

    def cp_w(lo, hi):
        return cp(wqkv_hbm.at[:, lo:hi], wkv_v.at[:, lo:hi])

    def cp_x(lo, hi):
        return cp(x_hbm.at[0, lo:hi], x_v.at[lo:hi])

    cp_wr = cp(wr_hbm, wr_v)
    kcum = [0]
    for _, dk in SEGS:
        kcum.append(kcum[-1] + dk)
    seg_cp = []
    x0 = 0
    for si, (dx, dk) in enumerate(SEGS):
        lo, hi = PHI[si][0] // DH, PHI[si][1] // DH
        ph = [cp(wphi_hbm.at[lo:hi], wphi_v.at[lo:hi])] if hi > lo else []
        seg_cp.append([cp_x(x0, x0 + dx)] + ph + [cp_w(D + kcum[si], D + kcum[si + 1])])
        x0 += dx
    cp_wv = cp_w(2 * D, 3 * D)
    cp_x1a = cp_x(T, T + C)
    cp_x1 = cp_x(T + C, T + T1 + C)
    cp_x2 = cp_x(T + T1 + C, S)
    cp_q0 = _Group([(wqkv_hbm.at[:, 128 * g:128 * (g + 1)], wqb_v.at[g]) for g in range(2)],
                   wqb_v.at[0:2], sems.at[new_sems(1)])
    cp_q1 = _Group([(wqkv_hbm.at[:, 128 * g:128 * (g + 1)], wqb_v.at[g]) for g in range(2, 8)],
                   wqb_v.at[2:8], sems.at[new_sems(1)])
    cp_wo = _Group([(wo_hbm.at[:, 128 * g:128 * (g + 1)], wo_v.at[g]) for g in range(8)], wo_v, sems.at[new_sems(1)])
    cp_ffn = [_Group([(wg_hbm.at[:, b * 128:(b + NA) * 128], wg_v.at[t]) for t, b in enumerate(B0)],
                     wg_v, sems.at[new_sems(1)]),
              _Group([(wu_hbm.at[:, b * 128:(b + NA) * 128], wu_v.at[t]) for t, b in enumerate(B0)],
                     wu_v, sems.at[new_sems(1)]),
              _Group([(wd_hbm.at[b * 128:(b + NA) * 128], wd_v.at[t]) for t, b in enumerate(B0)],
                     wd_v, sems.at[new_sems(1)])]
    seg_cp[0] = seg_cp[0][1:] + seg_cp[0][0:1]
    for c in [c for t in seg_cp for c in t] + [cp_wr, cp_wv, cp_x1a, cp_q0, cp_x1, cp_q1, cp_wo, cp_x2] + cp_ffn:
        c.start()
    osem0 = new_sems(NC + 1)

    def cp_out(q):
        rows = pl.ds(pl.multiple_of(ord_s[q], C), C)
        return pltpu.make_async_copy(out_v.at[rows], out_hbm.at[0, rows], sems.at[osem0 + q])

    def wr_row():
        return wr_v[...].reshape(1, D).astype(f32)

    def put_cols(ref, idx, col0, r):
        for k in range(0, r.shape[0], 8):
            ref[idx, :, col0 + k // 8:col0 + k // 8 + 1] = r[k:k + 8]

    def half(row0, n):
        if isinstance(row0, int):
            return pl.ds(row0 // 2, n // 2)
        return pl.ds(pl.multiple_of(lax.shift_right_logical(row0, 1), C // 2), n // 2)

    def ln1(src, dst, n, deps=None):
        xb = _pk(_ln(x_v[pl.ds(src, n), :].astype(f32), deps, None if deps is None else zv[...]).astype(bf16))
        xn_v[half(dst, n), :] = xb
        return _un(xb)

    def xn(row0, n):
        return _un(xn_v[half(row0, n), :])

    def predict(rows, t, c, deps):
        wr = wr_row()
        wc = wr - jnp.sum(wr, axis=-1, keepdims=True) * (1.0 / D)
        put_cols(p_v, t, c * (C // 8), _row_sum(x_v[rows, :].astype(f32) * wc, deps, zv[...]))

    def fold(dst, ws, sg):
        slot = _slot(D)
        res = [_dot_nt(_un(a_v[2 * sg + e]), ws[e]) for e in range(2)]
        main, e0, e1 = [], [], []
        for e in range(2):
            z = jnp.where(((slot + 3) % 4) // 2 == e, 0.0, res[e][0:8])
            b1 = z + pltpu.roll(z, 4, 0)
            b0 = pltpu.roll(b1, 2, 0)
            for pp in range(2):
                base = jnp.where(slot % 2 == pp, b0, b1)
                main.append((res[e][16 + 56 * pp:72 + 56 * pp].reshape(7, 8, D) - base[None]).reshape(56, D))
            e0.append(res[e][8:16] - b0)
            e1.append(res[e][0:8] - b1)
        rows = jnp.concatenate([jnp.where(slot < 2, e0[0], e0[1]), e1[0] + e1[1]] + main, axis=0)
        l2 = _pk((_rows(jnp.where(slot < 2, e0[1], e0[0]), 2) * LOG2E).astype(bf16))
        if isinstance(sg, int):
            r0, r1 = 248 * (sg // 2), 248 * (sg // 2) + 8 + 120 * (sg % 2)
        else:
            r0 = pl.multiple_of(248 * lax.shift_right_logical(sg, 1), 8)
            r1 = pl.multiple_of(r0 + 8 + 120 * (sg & 1), 8)
        dst[pl.ds(r1, 120), :] = _pk((rows * LOG2E).astype(bf16))
        dst[pl.ds(r0, 8), :] = jnp.where(slot // 2 == sg % 2, l2, dst[pl.ds(r0, 8), :])
        return res

    def wk(lo, hi):
        r0, r1 = 248 * (lo // 2), 248 * ((hi - 1) // 2) + 128 + 120 * ((hi - 1) % 2)
        if lo % 2:
            return _un(jnp.concatenate([wt_v[r0:r0 + 8, :], wt_v[r0 + 128:r1, :]], axis=0))
        return _un(wt_v[r0:r1, :])

    def kv_and_z(vt, phis, z_of, tail, zm):
        kvs = [_dot_nt(vt[64 * p:64 * (p + 1)].astype(bf16), phis[p].astype(bf16)) for p in range(NP)]
        zs_ = [_lane_blocks_sum(phis[p], z_of(p, _rows(_zero_after(tail[256 + 48 * p:264 + 48 * p], zm), 16)))
               for p in range(NP)]
        return kvs, zs_

    def a_row(r, e):
        s = (r & 7) >> 1
        f = jnp.where(r >= 72, (r - 64) >> 1, jnp.where(r >= 16, (r - 8) >> 1, jnp.where(
            r >= 8, jnp.where(s >> 1 == e, 1, 3), jnp.where(((s + 3) & 3) >> 1 == e, 2, 0))))
        pp = jnp.where(r >= 72, 1, jnp.where(r >= 16, 0, jnp.where(r >= 8, s, s + 1) & 1))
        return f, 2 * pp + (r & 1)

    f_i = lax.broadcasted_iota(i32, (128, DH), 1)
    sel = [jnp.where(f_i == a_row(lax.broadcasted_iota(i32, (128, DH), 0), e)[0], 1.0, 0.0).astype(bf16)
           for e in range(2)]
    amask = jnp.where(lax.broadcasted_iota(i32, (128, 128), 1) >> 5
                      == a_row(lax.broadcasted_iota(i32, (128, 128), 0), 0)[1], jnp.uint32(0xFFFFFFFF), jnp.uint32(0))

    def build_a(lo, hi):
        for g in range(lo // 128, hi // 128):
            blk = _dot_nt(sel[g % 2], wphi_v[4 * g:4 * (g + 1)].reshape(128, DH))
            a_v[g] = _pk(pltpu.bitcast(pltpu.bitcast(blk, u32) & amask, f32).astype(bf16))

    zv[...] = jnp.zeros((8, 128), u32)
    cp_z = cp(zv, zs)
    cp_z.start()
    for ref in (wt_v, wq_v):
        for r0 in (0, 248):
            ref[r0:r0 + 8, :] = jnp.zeros((8, D), u32)
    hbuf[...] = jnp.zeros(hbuf.shape, f32)
    xc_v[...] = jnp.zeros(xc_v.shape, f32)
    y_v[...] = jnp.zeros(y_v.shape, f32)
    r_v[...] = jnp.full(r_v.shape, -jnp.inf, f32)
    p_v[...] = jnp.full(p_v.shape, -jnp.inf, f32)

    pieces = [[] for _ in range(NP)]
    pending = []

    def phi_piece(p, t0, yp, dep=None):
        if dep is not None:
            yp = jnp.concatenate([yp[0:8] + _zero_after(dep, zv[...]), yp[8:]], axis=0)
        pieces[p].append((t0, _phi_k(yp)))

    def k_block(lo, hi, t0, t1, defer=0):
        y = _dot_nt(wk(lo, hi), xn(t0, t1 - t0))
        for p, yp in _pair_logits(y, range(lo, hi)).items():
            if p >= 4 * hi - defer:
                if t1 - t0 > C:
                    phi_piece(p, t0, yp[:, 0:t1 - t0 - C])
                pending.append((p, t1 - C, yp[:, t1 - t0 - C:]))
            else:
                phi_piece(p, t0, yp)
        return y

    def flush(res):
        for k, (p, t0, yp) in enumerate(pending):
            phi_piece(p, t0, yp, res[32 * k:32 * k + 8, 0:128])
        del pending[:]

    x0 = 0
    for si, (dx, dk) in enumerate(SEGS):
        k0, k1 = kcum[si] // 256, kcum[si + 1] // 256
        if si == 0:
            seg_cp[0][0].wait()
            build_a(*PHI[0])
            seg_cp[0][1].wait()
        else:
            for c in seg_cp[si]:
                c.wait()
            if PHI[si][1] > PHI[si][0]:
                build_a(*PHI[si])
        res = [fold(wt_v, [wkv_v[:, D + 128 * g:D + 128 * (g + 1)] for g in (2 * sg, 2 * sg + 1)], sg)
               for sg in range(k0, k1)]
        flush(res[0][0])
        if si == 0:
            seg_cp[0][2].wait()
        ln1(x0, x0, dx)
        if si:
            k_block(k0, k1, 0, x0)
        k_block(0, k1, x0, x0 + dx, DEFER)
        x0 += dx
    for c in (cp_wv, cp_x1a, cp_q0, cp_wr, cp_z):
        c.wait()
    for g in range(D // 128):
        wt_v[KR // 2 + 64 * g:KR // 2 + 64 * (g + 1), :] = _pk(wkv_v[:, 2 * D + 128 * g:2 * D + 128 * (g + 1)].T)
    flush(fold(wq_v, [wqb_v[0], wqb_v[1]], 0)[0])
    yv = _dot_nt(_un(wt_v[KR // 2:, :]), xn(0, T))
    xk_v[...] = _pk(ln1(T, T, C, [yv[128 * k:128 * k + 8, 128:256] for k in range(8)])[:, 0:D // 2].T)
    for c in range(CPT):
        predict(slice(C * c, C * (c + 1)), 0, c,
                [yv[256 * c + 32 * k:256 * c + 32 * k + 8, 256:384] for k in range(8)])
    phis = [jnp.concatenate([ph for _, ph in sorted(pieces[p], key=lambda tp: tp[0])], axis=1) for p in range(NP)]
    kvs, zs_ = kv_and_z(yv, phis, lambda p, zero: zero, yv[:, T - C:T], zv[...])
    for p in range(NP):
        kv_acc[p] = kvs[p]
        z_acc[p] = zs_[p]
    for c in (cp_x1, cp_q1, cp_wo):
        c.wait()

    def order_chunks():
        lane16 = lax.shift_right_logical(lax.broadcasted_iota(i32, (8, 128), 1), 4).astype(f32)
        vals = [p_v[t] for t in range(1 + N1)]
        cids = [lane16 + float(0 if t == 0 else CPT + CP1 * (t - 1)) for t in range(1 + N1)]
        b1 = _first_max(*_merge_max(list(zip(vals, cids))))[1]
        b2 = _first_max(*_merge_max([(jnp.where(c == b1, -jnp.inf, v), c) for v, c in zip(vals, cids)]))[1]
        both = _scalar(b1 * float(NC) + b2, 0, NC * NC - 1)
        c1, c2 = lax.shift_right_logical(both, 4), both & (NC - 1)
        c2 = jnp.where(c2 == c1, (c1 + 1) & (NC - 1), c2)
        ord_s[0] = S
        for c in range(NC):
            ord_s[1 + c] = c * C
        ord_s[1 + c1] = 0
        ord_s[1] = c1 * C
        ord_s[1 + jnp.where(c2 == 0, c1, c2)] = jnp.where(c1 == 1, 0, C)
        ord_s[2] = c2 * C

    def phase1(j, carry):
        @pl.when(j == 1)
        def _():
            cp_x2.wait()

        zm = zv[...]
        s = pl.multiple_of(T + j * T1, C)
        nxt = pl.multiple_of(jnp.where(j + 1 < N1, s + T1, 0), C)
        s2 = s + zs[2, 0].astype(i32)
        ys, ph = [], []
        for n in range(CP1):
            xt = xn(pl.multiple_of(s2 + C * n, C), C)
            y0 = _dot_nt(_un(wt_v[:, 0:D // 2]), xt[:, 0:D // 2]) if n else _dot(_un(wt_v[:, 0:D // 2]), _un(xk_v[...]))
            row0 = pl.multiple_of(s + C * (n + 1), C)
            xb = ln1(row0 if n + 1 < CP1 else nxt, row0, C, [y0[128 + 96 * k:136 + 96 * k] for k in range(16)])
            if n + 1 == CP1:
                xk_v[...] = _pk(xb[:, 0:D // 2].T)
            yn = _dot_nt(_un(wt_v[:, D // 2:D]), xt[:, D // 2:D]) + y0
            ys.append(yn)
            ph.append([_phi_k(yp) for yp in _pair_logits(yn[0:KR], range(4)).values()])
            if n == CP1 - 2:
                for c in range(CP1):
                    r0 = KR + 256 + 192 * c
                    predict(pl.ds(pl.multiple_of(s + C * c, C), C), 1 + j, c,
                            [yn[r0 + 24 * k:r0 + 24 * k + 8] for k in range(8)])
        order_chunks()
        xq_v[...] = _pk(xn(pl.multiple_of(ord_s[1], C), C)[:, 0:D // 2].T)
        fold(wq_v, [wqb_v[2 + 2 * j], wqb_v[3 + 2 * j]], 1 + j)
        for e in range(4 * GO):
            row = KR + 384 + 640 * e // (4 * GO) // 8 * 8
            blk = jnp.minimum(GO * j + e // 4, D // 128 - 1)
            w = _pk(wo_v[blk, 256 * (e % 4):256 * (e % 4 + 1), :])
            wo32[blk, 128 * (e % 4):128 * (e % 4 + 1), :] = (
                w.reshape(16, 8, 128) | (_pk(ys[0][row:row + 8]) & zm)[None]).reshape(128, 128)
        vt = jnp.concatenate([yn[KR:] for yn in ys], axis=1)
        phis = [jnp.concatenate([ph[n][p] for n in range(CP1)], axis=1) for p in range(NP)]
        kvs, zs_ = kv_and_z(vt, phis, lambda p, zero: z_acc[p] + zero, ys[-1][KR:], zm)
        for p in range(NP):
            kv_acc[p] += kvs[p]
            z_acc[p] = zs_[p]
            zb_v[p] = jnp.broadcast_to(jnp.sum(zs_[p], axis=1, keepdims=True), (128, 128))
        return carry

    lax.fori_loop(0, N1, phase1, 0)
    for c in cp_ffn:
        c.wait()

    def ln2(h, row0, nx, nrel):
        deps = [None]
        for j in range(1, C // 8):
            t = (j * nrel * 2) // (C // 8) - 1
            r0 = (C - 8) * (t % 2)
            deps.append(nx[r0:r0 + 8, 128 * (t // 2):128 * (t // 2) + 128] if t >= 0 else None)
        hn = _ln(h, deps, zv[...])
        r = jnp.sum(hn * wr_row(), axis=-1, keepdims=True)
        hn_v[pl.ds(row0, C), :] = hn.astype(bf16)
        out_v[pl.ds(row0, C), :] = (h + hn).astype(bf16)
        return r

    lane = lax.broadcasted_iota(i32, (8, 128), 1)
    pos = (lane * 8 + lax.broadcasted_iota(i32, (8, 128), 0)).astype(f32)

    def token_at(posv, lo, hi):
        p = _scalar(posv, lo, hi - 1)
        return ord_s[lax.shift_right_logical(p, 7)] + (p & (C - 1))

    def slab_of(tok):
        base = pl.multiple_of(lax.shift_left(lax.shift_right_logical(tok, 4), 4), 16)
        return pl.ds(base, 16), lax.broadcasted_iota(i32, (16, D), 0) == tok - base

    def token_row(tok):
        rows, hit = slab_of(tok)
        slab = jnp.where(hit, hn_v[rows, :].astype(f32), 0.0)
        return _allred8(slab[0:8] + slab[8:16], jnp.add)

    def patch(tok, y8, sg):
        rows, hit = slab_of(tok)
        cur = out_v[rows, :].astype(f32)
        fix_v[...] = jnp.where(hit, cur + _rows(y8 * _lanes(sg, D // 128), 2), cur).astype(bf16)

    def phase2(i, carry):
        q0 = CPT * i
        off = [pl.multiple_of(ord_s[q0 + k], C) for k in range(CPT + 1)]
        zm = zv[...]
        hprev = hbuf[...]
        kmask = lax.broadcasted_iota(i32, (64, 128), 0) // 32 == lax.broadcasted_iota(i32, (64, 128), 1) % 2

        def attend(y):
            os_ = []
            for p, yp in _pair_logits(y, range(4)).items():
                os_.append(_dot(jnp.where(kmask, kv_acc[p], 0.0).astype(bf16), _phi_q(yp, zb_v[p])))
            return jnp.concatenate(os_, axis=0).astype(bf16).T

        ya, ys = [], []
        for n in range(CPT):
            xt = xn(off[n + 1], C)
            ya.append(_dot_nt(_un(wq_v[:, 0:D // 2]), xt[:, 0:D // 2]) if n else
                      _dot(_un(wq_v[:, 0:D // 2]), _un(xq_v[...])))
            if n == CPT - 1:
                o01 = attend(jnp.concatenate(ys[0:2], axis=1))
            ys.append(ya[n] + _dot_nt(_un(wq_v[:, D // 2:D]), xt[:, D // 2:D]))
        wo = jnp.concatenate([_un(wo32[j]) for j in range(D // 128)], axis=1)
        head = _dot(o01[0:C], wo[:, 0:256])
        o23 = attend(jnp.concatenate(ys[2:4], axis=1))
        atts = [jnp.concatenate([head, _dot(o01[0:C], wo[:, 256:])], axis=1),
                _dot(o01[C:2 * C], wo), _dot(o23[0:C], wo), _dot(o23[C:2 * C], wo)]

        xq_v[...] = _pk(xn(pl.multiple_of(ord_s[jnp.minimum(q0 + CPT + 1, NC)], C), C)[:, 0:D // 2].T)

        def q_gate(v):
            lens = [KR // 8] + [KR // 8 - 24] * 3
            t, n = int(v * sum(lens)), 0
            while t >= lens[n]:
                t -= lens[n]
                n += 1
            r0 = 8 * (t + KR // 8 - lens[n])
            return _zero_after(ya[n][r0:r0 + 8], zm)

        def o_gate(t):
            r0, j = 8 * (t % 16), (t % 128) // 16
            return _zero_after(atts[t // 128][r0:r0 + 8, 128 * j:128 * j + 128], zm)

        t3 = jnp.maximum(i - 1, 0)
        nsb = NA // 2
        for sb in range(nsb):
            cols = slice(256 * sb, 256 * (sb + 1))
            xcol = xc_v[...]
            acc = None
            for k in range(0, D, 8):
                xk = _lanes(xcol[k:k + 8], 2)
                p = jnp.concatenate([wg_v[t3, k:k + 8, cols].astype(f32) * xk,
                                     wu_v[t3, k:k + 8, cols].astype(f32) * xk], axis=1)
                if k % 64 == 0:
                    p = p + _lanes(q_gate((sb * D + k) / (nsb * D)), 4)
                acc = p if acc is None else acc + p
            pa_v[:, 512 * sb:512 * (sb + 1)] = acc

        put_cols(r_v, i, 0, jnp.where(i > 0, ln2(hprev, off[0], atts[0], 6), -jnp.inf))

        @pl.when(i > 0)
        def _():
            cp_out(q0).start()

        acc = _allred8(pa_v[pl.ds(pl.multiple_of(zs[3, 0].astype(i32) * 32, 32), 8), :], jnp.add)
        g_ = jnp.concatenate([acc[:, 512 * t:512 * t + 256] for t in range(nsb)], axis=1)
        u_ = jnp.concatenate([acc[:, 512 * t + 256:512 * t + 512] for t in range(nsb)], axis=1)
        a8 = g_ * jax.nn.sigmoid(g_) * u_
        ac = _col(jnp.concatenate([jnp.where(t3 == 2, 0.0, a8[:, 0:NDUP]), a8[:, NDUP:]], axis=1))
        ysums = []
        for q in range(2):
            cols = slice(D // 2 * q, D // 2 * (q + 1))
            ysum = jnp.where(i > 1, y_v[:, cols], 0.0)
            for k in range(0, NA * 128, 8):
                p = wd_v[t3, k:k + 8, cols].astype(f32) * _lanes(ac[k:k + 8], 4)
                if k % 32 == 0:
                    p = p + _lanes(o_gate(64 + (q * NA * 128 + k) * 376 // (2 * NA * 128)), 4)
                ysum = ysum + p
            y_v[:, cols] = ysum
            ysums.append(ysum)

        for k in range(CPT):
            if k == NCAND:
                ok = (lane >= C // 8) & (lane < (NCAND + 1) * (C // 8))
                cm, cpos = _first_max(jnp.where(ok, r_v[0], -jnp.inf), pos)
                cand = token_at(cpos, C, (NCAND + 1) * C)
                ord_s[NC + 1] = cand
                xc_v[...] = _col(token_row(cand))
                patch(cand, _allred8(jnp.concatenate(ysums, axis=1), jnp.add),
                      jax.nn.sigmoid(jnp.broadcast_to(cm, (8, 128))))
            h = x_v[pl.ds(off[k + 1], C), :].astype(f32) + atts[k]
            if k == CPT - 1:
                hbuf[...] = h
            else:
                put_cols(r_v, i, (k + 1) * (C // 8), ln2(h, off[k + 1], atts[k + 1], 5 if k == CPT - 2 else 6))
                cp_out(q0 + k + 1).start()
        return carry

    lax.fori_loop(0, NT, phase2, 0)

    for q in range(1, NCAND + 1):
        cp_out(q).wait()
    fsem = new_sems(1)

    cand = ord_s[NC + 1]

    def cp_patch(tok):
        return pltpu.make_async_copy(fix_v, out_hbm.at[0, slab_of(tok)[0]], sems.at[fsem])

    cp_fix = cp_patch(cand)
    cp_fix.start()
    cp_out(NCAND + 1).wait()
    last = pl.multiple_of(ord_s[NC], C)
    stats, cp_last = [], []
    for g in range(0, C, EG):
        h = hbuf[g:g + EG, :]
        s1 = h[:, 0:128]
        s2 = s1 * s1
        for j in range(128, D, 128):
            s1 = s1 + h[:, j:j + 128]
            s2 = s2 + h[:, j:j + 128] * h[:, j:j + 128]
        m = jnp.sum(s1, axis=-1, keepdims=True) * (1.0 / D)
        v = jnp.sum(s2, axis=-1, keepdims=True) * (1.0 / D) - m * m
        rs = lax.rsqrt(jnp.maximum(v, 0.0) + EPS)
        stats.append((m, rs))
        rows = pl.ds(pl.multiple_of(last + g, EG), EG)
        out_v[rows, :] = (h * (1.0 + rs) - m * rs).astype(bf16)
        cp_last.append(cp(out_v.at[rows], out_hbm.at[0, rows]))
        cp_last[-1].start()
    for q in range(NCAND + 2, NC - 1):
        cp_out(q).wait()
    pm, pi = _first_max(*_merge_max([(r_v[i], pos + float(i * T) if i else pos) for i in range(NT)]))
    wr = wr_row()
    wsum = jnp.sum(wr, axis=-1, keepdims=True)
    sub = lax.broadcasted_iota(i32, (8, 1), 0).astype(f32)
    cands = []
    for g, (m, rs) in zip(range(0, C, EG), stats):
        r = (jnp.sum(hbuf[g:g + EG, :] * wr, axis=-1, keepdims=True) - m * wsum) * rs
        cands += [(r[k:k + 8], sub + float(S + g + k)) for k in range(0, EG, 8)]
    while len(cands) > 1:
        cands = [_merge_max(cands[k:k + 2]) for k in range(0, len(cands), 2)]
    bv, bt = [jnp.broadcast_to(v, (8, 128)) for v in _merge_max([(pm, pi), cands[0]])]
    rmax = _allred8(bv, jnp.maximum)
    idx = token_at(_allred8(jnp.where(bv == rmax, bt, float(2 * S)), jnp.minimum), C, S + C)
    cp_out(NC - 1).wait()
    cp_fix.wait()
    for c in cp_last:
        c.wait()

    @pl.when(idx != cand)
    def _():
        rows, _ = slab_of(cand)
        undo = pltpu.make_async_copy(out_v.at[rows], out_hbm.at[0, rows], sems.at[fsem])
        undo.start()
        hn_v[pl.ds(last, C), :] = _ln(hbuf[...]).astype(bf16)
        xs = _rows(token_row(idx), 2).astype(bf16)

        def step(j, acc):
            t = lax.shift_right_logical(j, 1)
            cols = pl.ds(pl.multiple_of((j & 1) * (NA * 64), 128), NA * 64)
            g = _dot(xs, wg_v[t, :, cols])
            a = g * jax.nn.sigmoid(g) * _dot(xs, wu_v[t, :, cols])
            a = jnp.concatenate([jnp.where(j == 4, 0.0, a[:, 0:NDUP]), a[:, NDUP:]], axis=1)
            return acc + _dot(a.astype(bf16), wd_v[t, cols, :])[0:8]

        y8 = lax.fori_loop(0, 6, step, jnp.zeros((8, D), f32))
        undo.wait()
        patch(idx, y8, jax.nn.sigmoid(rmax))
        redo = cp_patch(idx)
        redo.start()
        redo.wait()


@jax.jit
def pallas_sequential_preLN__linear_kernel_hedgehog__moe_arch_mod__prompt_kernel(
    A_x: jax.Array,
    A_wqkv: jax.Array,
    A_w_phi: jax.Array,
    A_wo: jax.Array,
    B_x: jax.Array,
    B_w_r: jax.Array,
    B_w_gate: jax.Array,
    B_w_up: jax.Array,
    B_w_down: jax.Array,
):
    del B_x
    any_spec = pl.BlockSpec(memory_space=pl.ANY)
    return pl.pallas_call(
        _kernel,
        out_shape=jax.ShapeDtypeStruct((1, S, D), bf16),
        in_specs=[any_spec] * 8,
        out_specs=any_spec,
        scratch_shapes=[
            pltpu.VMEM((S, D), bf16),
            pltpu.VMEM((D, 3 * D), bf16),
            pltpu.VMEM((D // 128, D, 128), bf16),
            pltpu.VMEM((H, DH, DH), bf16),
            pltpu.VMEM((D // 128, D, 128), bf16),
            pltpu.VMEM((D // 128, D // 2, 128), u32),
            pltpu.VMEM((D,), bf16),
            pltpu.VMEM((3, D, NA * 128), bf16),
            pltpu.VMEM((3, D, NA * 128), bf16),
            pltpu.VMEM((3, NA * 128, D), bf16),
            pltpu.VMEM(((KR + D) // 2, D), u32),
            pltpu.VMEM((KR // 2, D), u32),
            pltpu.VMEM((8, 64, 128), u32),
            pltpu.VMEM(((S + C) // 2, D), u32),
            pltpu.VMEM((D // 4, C), u32),
            pltpu.VMEM((D // 4, C), u32),
            pltpu.VMEM((S + C, D), bf16),
            pltpu.VMEM((NP, 64, 128), f32),
            pltpu.VMEM((NP, 128, 128), f32),
            pltpu.VMEM((NP, 128, 128), f32),
            pltpu.VMEM((C, D), f32),
            pltpu.VMEM((S + C, D), bf16),
            pltpu.VMEM((8, 128), u32),
            pltpu.SMEM((8, 128), u32),
            pltpu.VMEM((1 + N1, 8, 128), f32),
            pltpu.VMEM((NT, 8, 128), f32),
            pltpu.VMEM((D, 128), f32),
            pltpu.VMEM((8, NA * 256), f32),
            pltpu.VMEM((8, D), f32),
            pltpu.VMEM((16, D), bf16),
            pltpu.SMEM((NC + 2,), i32),
            pltpu.SemaphoreType.DMA((64,)),
        ],
        compiler_params=pltpu.CompilerParams(vmem_limit_bytes=120 * 1024 * 1024,
                                             disable_bounds_checks=True,
                                             disable_semaphore_checks=True),
        name="hedgehog_mod",
    )(A_x, A_wqkv, A_w_phi, A_wo, B_w_r, B_w_gate, B_w_up, B_w_down)
```

```python
import jax
import jax.numpy as jnp
from jax import lax
import jax.experimental.pallas as pl
import jax.experimental.pallas.tpu as pltpu

S = 2048
D = 1024
H = 32
DH = 32
F = 3584
NP = H // 2
C = 128
NC = S // C
U = 64
NU = S // U
T = 512
NT = S // T
CPT = T // C
T1 = 512
N1 = (S - T) // T1
CP1 = T1 // C
KR = H * (DH - 1)
GO = -(-8 // N1)
SEGS = ((256, 256), (128, 256), (128, 512))
PHI = ((0, 512), (512, 512), (512, 1024))
DEFER = 2
NB = F // 128
NA = 10
B0 = (0, NA, NB - NA)
NDUP = (3 * NA - NB) * 128
NCAND = 2
EG = 16
LOG2E = 1.4426950408889634
EPS = 1e-5

f32 = jnp.float32
bf16 = jnp.bfloat16
u32 = jnp.uint32
i32 = jnp.int32


def _dot_nt(a, b):
    return lax.dot_general(a, b, (((1,), (1,)), ((), ())), preferred_element_type=f32)


def _dot(a, b):
    return jnp.dot(a, b, preferred_element_type=f32)


def _pk(x):
    return pltpu.bitcast(x, u32)


def _un(x):
    return pltpu.bitcast(x, bf16)


def _rcp(x):
    r = pl.reciprocal(x, approx=True)
    return r * (2.0 - x * r)


def _allred(v, op):
    v = op(v, pltpu.roll(v, 2, 0))
    return op(v, pltpu.roll(v, 4, 0))


def _allred8(v, op):
    return _allred(op(v, pltpu.roll(v, 1, 0)), op)


def _rows(v, n):
    return jnp.concatenate([v] * n, axis=0)


def _lanes(v, n):
    return jnp.concatenate([v] * n, axis=1)


def _zero_after(dep, zm):
    return pltpu.bitcast(pltpu.bitcast(dep, u32) & zm, f32)


def _exps(x):
    x3 = x.reshape(8, 8, x.shape[1])
    mx = _allred(jnp.max(x3, axis=0), jnp.maximum)
    mn = _allred(jnp.min(x3, axis=0), jnp.minimum)
    ep = jnp.exp2(x3 - mx[None])
    en = jnp.exp2(mn[None] - x3)
    rp = _rcp(_allred(jnp.sum(ep, axis=0), jnp.add))
    rn = _rcp(_allred(jnp.sum(en, axis=0), jnp.add))
    return ep, en, rp, rn


def _phi_k(x):
    L = x.shape[1]
    ep, en, rp, rn = _exps(x)
    return jnp.concatenate([(ep * rp[None]).reshape(64, L), (en * rn[None]).reshape(64, L)], axis=0)


def _phi_q(x, zb):
    L = x.shape[1]
    ep, en, rp, rn = _exps(x)
    zb = _lanes(zb, L // 128).reshape(16, 8, L)
    den = rp * jnp.sum(ep * zb[0:8], axis=0) + rn * jnp.sum(en * zb[8:16], axis=0)
    inv = _rcp(_allred(den, jnp.add) + 1e-6)
    cp = rp * inv
    cn = rn * inv
    phi = jnp.concatenate([(ep * cp[None]).reshape(64, L), (en * cn[None]).reshape(64, L)], axis=0)
    return phi.astype(bf16)


def _slot(n):
    return lax.shift_right_logical(lax.broadcasted_iota(i32, (8, n), 0), 1)


def _pair_logits(y, sgs):
    slot = _slot(y.shape[1])
    out, r, shared = {}, 0, None
    for k, sg in enumerate(sgs):
        if k == 0 or sg % 2 == 0:
            shared, r = y[r:r + 16], r + 16
        l0, l1, l2 = y[r:r + 8], y[r + 8:r + 16], shared[8 * (sg % 2):8 * (sg % 2) + 8]
        for q in range(4):
            x0 = jnp.where(slot == q, l0, jnp.where(slot == (q + 1) % 4, l1, jnp.where(slot == (q + 2) % 4, l2, 0.0)))
            out[4 * sg + q] = jnp.concatenate([x0, y[r + 16 + 56 * q:r + 72 + 56 * q]], axis=0)
        r += 240
    return out


def _lane_blocks_sum(v, acc):
    for c in range(0, v.shape[1], 128):
        acc = acc + v[:, c:c + 128]
    return acc


def _row_sum(x, deps, zm):
    g = x.shape[0] // len(deps)
    gate = jnp.concatenate([jnp.zeros((8, 128), f32) if d is None else _zero_after(d, zm)
                            for d in deps for _ in range(g // 8)], axis=0)
    return jnp.sum(_lane_blocks_sum(x[:, 128:], x[:, 0:128] + gate), axis=-1, keepdims=True)


def _ln(x, deps=None, zm=None):
    tot = jnp.sum(x, axis=-1, keepdims=True) if deps is None else _row_sum(x, deps, zm)
    xc = x - tot * (1.0 / D)
    return xc * lax.rsqrt(jnp.sum(xc * xc, axis=-1, keepdims=True) * (1.0 / D) + EPS)


def _col(a8):
    return _rows(a8, 16).astype(bf16).T.astype(f32)


def _first_max(v, t):
    m = jnp.max(_allred8(v, jnp.maximum), axis=1, keepdims=True)
    return m, jnp.min(_allred8(jnp.where(v == m, t, float(2 * S)), jnp.minimum), axis=1, keepdims=True)


def _merge_max(cands):
    v, t = cands[0]
    for v2, t2 in cands[1:]:
        gt = v2 > v
        v, t = jnp.where(gt, v2, v), jnp.where(gt, t2, t)
    return v, t


def _scalar(v, lo, hi):
    return jnp.clip(jnp.broadcast_to(v, (8, 128)).astype(i32)[0, 0], lo, hi)


class _Group:
    def __init__(self, parts, dst, sem):
        self.parts, self.dst, self.sem = parts, dst, sem

    def start(self):
        for src, dst in self.parts:
            pltpu.make_async_copy(src, dst, self.sem).start()

    def wait(self):
        pltpu.make_async_copy(self.dst, self.dst, self.sem).wait()


def _kernel(x_hbm, wqkv_hbm, wphi_hbm, wo_hbm, wr_hbm, wg_hbm, wu_hbm, wd_hbm, out_hbm,
            x_v, wkv_v, wqb_v, wphi_v, wo_v, wo32, wr_v, wg_v, wu_v, wd_v,
            wt_v, wq_v, a_v, xn_v, xk_v, xq_v, hn_v, kv_acc, z_acc, zb_v, hbuf, out_v, zv, zs, p_v, r_v,
            xc_v, pa_v, y_v, fix_v, ord_s, sems):
    nsem = [0]

    def new_sems(n):
        nsem[0] += n
        return nsem[0] - n

    def cp(src, dst):
        return pltpu.make_async_copy(src, dst, sems.at[new_sems(1)])

    def cp_w(lo, hi):
        return cp(wqkv_hbm.at[:, lo:hi], wkv_v.at[:, lo:hi])

    def cp_x(lo, hi):
        return cp(x_hbm.at[0, lo:hi], x_v.at[lo:hi])

    cp_wr = cp(wr_hbm, wr_v)
    kcum = [0]
    for _, dk in SEGS:
        kcum.append(kcum[-1] + dk)
    seg_cp = []
    x0 = 0
    for si, (dx, dk) in enumerate(SEGS):
        lo, hi = PHI[si][0] // DH, PHI[si][1] // DH
        ph = [cp(wphi_hbm.at[lo:hi], wphi_v.at[lo:hi])] if hi > lo else []
        seg_cp.append([cp_x(x0, x0 + dx)] + ph + [cp_w(D + kcum[si], D + kcum[si + 1])])
        x0 += dx
    cp_wv = cp_w(2 * D, 3 * D)
    cp_x1a = cp_x(T, T + C)
    cp_x1 = cp_x(T + C, T + T1 + C)
    cp_x2 = cp_x(T + T1 + C, S)
    cp_q0 = _Group([(wqkv_hbm.at[:, 128 * g:128 * (g + 1)], wqb_v.at[g]) for g in range(2)],
                   wqb_v.at[0:2], sems.at[new_sems(1)])
    cp_q1 = _Group([(wqkv_hbm.at[:, 128 * g:128 * (g + 1)], wqb_v.at[g]) for g in range(2, 8)],
                   wqb_v.at[2:8], sems.at[new_sems(1)])
    cp_wo = _Group([(wo_hbm.at[:, 128 * g:128 * (g + 1)], wo_v.at[g]) for g in range(8)], wo_v, sems.at[new_sems(1)])
    cp_ffn = [_Group([(wg_hbm.at[:, b * 128:(b + NA) * 128], wg_v.at[t]) for t, b in enumerate(B0)],
                     wg_v, sems.at[new_sems(1)]),
              _Group([(wu_hbm.at[:, b * 128:(b + NA) * 128], wu_v.at[t]) for t, b in enumerate(B0)],
                     wu_v, sems.at[new_sems(1)]),
              _Group([(wd_hbm.at[b * 128:(b + NA) * 128], wd_v.at[t]) for t, b in enumerate(B0)],
                     wd_v, sems.at[new_sems(1)])]
    seg_cp[0] = seg_cp[0][1:] + seg_cp[0][0:1]
    for c in [c for t in seg_cp for c in t] + [cp_wr, cp_wv, cp_x1a, cp_q0, cp_x1, cp_q1, cp_wo, cp_x2] + cp_ffn:
        c.start()
    osem0 = new_sems(NU)

    def cp_out(u):
        rows = pl.ds(pl.multiple_of(ord_s[u], U), U)
        return pltpu.make_async_copy(out_v.at[rows], out_hbm.at[0, rows], sems.at[osem0 + u])

    def wr_row():
        return wr_v[...].reshape(1, D).astype(f32)

    def put_cols(ref, idx, col0, r):
        for k in range(0, r.shape[0], 8):
            ref[idx, :, col0 + k // 8:col0 + k // 8 + 1] = r[k:k + 8]

    def half(row0, n):
        if isinstance(row0, int):
            return pl.ds(row0 // 2, n // 2)
        return pl.ds(pl.multiple_of(lax.shift_right_logical(row0, 1), U // 2), n // 2)

    def ln1(src, dst, n, deps=None):
        xb = _pk(_ln(x_v[pl.ds(src, n), :].astype(f32), deps, None if deps is None else zv[...]).astype(bf16))
        xn_v[half(dst, n), :] = xb
        return _un(xb)

    def xn(row0, n):
        return _un(xn_v[half(row0, n), :])

    def units(q):
        return [pl.multiple_of(ord_s[2 * q + t], U) for t in range(2)]

    def xn_units(offs):
        return _un(jnp.concatenate([xn_v[half(o, U), :] for o in offs], axis=0))

    def predict(rows, t, c, deps):
        wr = wr_row()
        wc = wr - jnp.sum(wr, axis=-1, keepdims=True) * (1.0 / D)
        put_cols(p_v, t, c * (C // 8), _row_sum(x_v[rows, :].astype(f32) * wc, deps, zv[...]))

    def fold(dst, ws, sg):
        slot = _slot(D)
        res = [_dot_nt(_un(a_v[2 * sg + e]), ws[e]) for e in range(2)]
        main, e0, e1 = [], [], []
        for e in range(2):
            z = jnp.where(((slot + 3) % 4) // 2 == e, 0.0, res[e][0:8])
            b1 = z + pltpu.roll(z, 4, 0)
            b0 = pltpu.roll(b1, 2, 0)
            for pp in range(2):
                base = jnp.where(slot % 2 == pp, b0, b1)
                main.append((res[e][16 + 56 * pp:72 + 56 * pp].reshape(7, 8, D) - base[None]).reshape(56, D))
            e0.append(res[e][8:16] - b0)
            e1.append(res[e][0:8] - b1)
        rows = jnp.concatenate([jnp.where(slot < 2, e0[0], e0[1]), e1[0] + e1[1]] + main, axis=0)
        l2 = _pk((_rows(jnp.where(slot < 2, e0[1], e0[0]), 2) * LOG2E).astype(bf16))
        if isinstance(sg, int):
            r0, r1 = 248 * (sg // 2), 248 * (sg // 2) + 8 + 120 * (sg % 2)
        else:
            r0 = pl.multiple_of(248 * lax.shift_right_logical(sg, 1), 8)
            r1 = pl.multiple_of(r0 + 8 + 120 * (sg & 1), 8)
        dst[pl.ds(r1, 120), :] = _pk((rows * LOG2E).astype(bf16))
        dst[pl.ds(r0, 8), :] = jnp.where(slot // 2 == sg % 2, l2, dst[pl.ds(r0, 8), :])
        return res

    def wk(lo, hi):
        r0, r1 = 248 * (lo // 2), 248 * ((hi - 1) // 2) + 128 + 120 * ((hi - 1) % 2)
        if lo % 2:
            return _un(jnp.concatenate([wt_v[r0:r0 + 8, :], wt_v[r0 + 128:r1, :]], axis=0))
        return _un(wt_v[r0:r1, :])

    def kv_and_z(vt, phis, z_of, tail, zm):
        kvs = [_dot_nt(vt[64 * p:64 * (p + 1)].astype(bf16), phis[p].astype(bf16)) for p in range(NP)]
        zs_ = [_lane_blocks_sum(phis[p], z_of(p, _rows(_zero_after(tail[256 + 48 * p:264 + 48 * p], zm), 16)))
               for p in range(NP)]
        return kvs, zs_

    def a_row(r, e):
        s = (r & 7) >> 1
        f = jnp.where(r >= 72, (r - 64) >> 1, jnp.where(r >= 16, (r - 8) >> 1, jnp.where(
            r >= 8, jnp.where(s >> 1 == e, 1, 3), jnp.where(((s + 3) & 3) >> 1 == e, 2, 0))))
        pp = jnp.where(r >= 72, 1, jnp.where(r >= 16, 0, jnp.where(r >= 8, s, s + 1) & 1))
        return f, 2 * pp + (r & 1)

    f_i = lax.broadcasted_iota(i32, (128, DH), 1)
    sel = [jnp.where(f_i == a_row(lax.broadcasted_iota(i32, (128, DH), 0), e)[0], 1.0, 0.0).astype(bf16)
           for e in range(2)]
    amask = jnp.where(lax.broadcasted_iota(i32, (128, 128), 1) >> 5
                      == a_row(lax.broadcasted_iota(i32, (128, 128), 0), 0)[1], jnp.uint32(0xFFFFFFFF), jnp.uint32(0))

    def build_a(lo, hi):
        for g in range(lo // 128, hi // 128):
            blk = _dot_nt(sel[g % 2], wphi_v[4 * g:4 * (g + 1)].reshape(128, DH))
            a_v[g] = _pk(pltpu.bitcast(pltpu.bitcast(blk, u32) & amask, f32).astype(bf16))

    zv[...] = jnp.zeros((8, 128), u32)
    cp_z = cp(zv, zs)
    cp_z.start()
    for ref in (wt_v, wq_v):
        for r0 in (0, 248):
            ref[r0:r0 + 8, :] = jnp.zeros((8, D), u32)
    hbuf[...] = jnp.zeros(hbuf.shape, f32)
    xc_v[...] = jnp.zeros(xc_v.shape, f32)
    y_v[...] = jnp.zeros(y_v.shape, f32)
    r_v[...] = jnp.full(r_v.shape, -jnp.inf, f32)
    p_v[...] = jnp.full(p_v.shape, -jnp.inf, f32)

    pieces = [[] for _ in range(NP)]
    pending = []

    def phi_piece(p, t0, yp, dep=None):
        if dep is not None:
            yp = jnp.concatenate([yp[0:8] + _zero_after(dep, zv[...]), yp[8:]], axis=0)
        pieces[p].append((t0, _phi_k(yp)))

    def k_block(lo, hi, t0, t1, defer=0):
        y = _dot_nt(wk(lo, hi), xn(t0, t1 - t0))
        for p, yp in _pair_logits(y, range(lo, hi)).items():
            if p >= 4 * hi - defer:
                if t1 - t0 > C:
                    phi_piece(p, t0, yp[:, 0:t1 - t0 - C])
                pending.append((p, t1 - C, yp[:, t1 - t0 - C:]))
            else:
                phi_piece(p, t0, yp)
        return y

    def flush(res):
        for k, (p, t0, yp) in enumerate(pending):
            phi_piece(p, t0, yp, res[32 * k:32 * k + 8, 0:128])
        del pending[:]

    x0 = 0
    for si, (dx, dk) in enumerate(SEGS):
        k0, k1 = kcum[si] // 256, kcum[si + 1] // 256
        if si == 0:
            seg_cp[0][0].wait()
            build_a(*PHI[0])
            seg_cp[0][1].wait()
        else:
            for c in seg_cp[si]:
                c.wait()
            if PHI[si][1] > PHI[si][0]:
                build_a(*PHI[si])
        res = [fold(wt_v, [wkv_v[:, D + 128 * g:D + 128 * (g + 1)] for g in (2 * sg, 2 * sg + 1)], sg)
               for sg in range(k0, k1)]
        flush(res[0][0])
        if si == 0:
            seg_cp[0][2].wait()
        ln1(x0, x0, dx)
        if si:
            k_block(k0, k1, 0, x0)
        k_block(0, k1, x0, x0 + dx, DEFER)
        x0 += dx
    for c in (cp_wv, cp_x1a, cp_q0, cp_wr, cp_z):
        c.wait()
    for g in range(D // 128):
        wt_v[KR // 2 + 64 * g:KR // 2 + 64 * (g + 1), :] = _pk(wkv_v[:, 2 * D + 128 * g:2 * D + 128 * (g + 1)].T)
    flush(fold(wq_v, [wqb_v[0], wqb_v[1]], 0)[0])
    yv = _dot_nt(_un(wt_v[KR // 2:, :]), xn(0, T))
    xk_v[...] = _pk(ln1(T, T, C, [yv[128 * k:128 * k + 8, 128:256] for k in range(8)])[:, 0:D // 2].T)
    for c in range(CPT):
        predict(slice(C * c, C * (c + 1)), 0, c,
                [yv[256 * c + 32 * k:256 * c + 32 * k + 8, 256:384] for k in range(8)])
    phis = [jnp.concatenate([ph for _, ph in sorted(pieces[p], key=lambda tp: tp[0])], axis=1) for p in range(NP)]
    kvs, zs_ = kv_and_z(yv, phis, lambda p, zero: zero, yv[:, T - C:T], zv[...])
    for p in range(NP):
        kv_acc[p] = kvs[p]
        z_acc[p] = zs_[p]
    for c in (cp_x1, cp_q1, cp_wo):
        c.wait()

    def order_units():
        lane8 = lax.shift_right_logical(lax.broadcasted_iota(i32, (8, 128), 1), 3).astype(f32)
        vals = [p_v[t] for t in range(1 + N1)]
        uids = [lane8 + float(0 if t == 0 else (T + T1 * (t - 1)) // U) for t in range(1 + N1)]
        code = None
        for r in range(2 * NCAND):
            best = _first_max(*_merge_max(list(zip(vals, uids))))[1]
            vals = [jnp.where(u == best, -jnp.inf, v) for v, u in zip(vals, uids)]
            code = best if code is None else code * float(NU) + best
        code = _scalar(code, 0, NU ** (2 * NCAND) - 1)
        for u in range(NU + 2):
            ord_s[u] = (S + u * U) if u < 2 else (u - 2) * U
        swaps = []
        for r in range(2 * NCAND):
            p = lax.shift_right_logical(code, 5 * (2 * NCAND - 1 - r)) & (NU - 1)
            for lo, hi in swaps:
                p = jnp.where(p == lo, hi, jnp.where(p == hi, lo, p))
            swaps.append((r, p))
            here, there = ord_s[2 + r], ord_s[2 + p]
            ord_s[2 + r] = there
            ord_s[2 + p] = here

    def phase1(j, carry):
        @pl.when(j == 1)
        def _():
            cp_x2.wait()

        zm = zv[...]
        s = pl.multiple_of(T + j * T1, C)
        nxt = pl.multiple_of(jnp.where(j + 1 < N1, s + T1, 0), C)
        s2 = s + zs[2, 0].astype(i32)
        ys, ph = [], []
        for n in range(CP1):
            xt = xn(pl.multiple_of(s2 + C * n, C), C)
            y0 = _dot_nt(_un(wt_v[:, 0:D // 2]), xt[:, 0:D // 2]) if n else _dot(_un(wt_v[:, 0:D // 2]), _un(xk_v[...]))
            row0 = pl.multiple_of(s + C * (n + 1), C)
            xb = ln1(row0 if n + 1 < CP1 else nxt, row0, C, [y0[128 + 96 * k:136 + 96 * k] for k in range(16)])
            if n + 1 == CP1:
                xk_v[...] = _pk(xb[:, 0:D // 2].T)
            yn = _dot_nt(_un(wt_v[:, D // 2:D]), xt[:, D // 2:D]) + y0
            ys.append(yn)
            ph.append([_phi_k(yp) for yp in _pair_logits(yn[0:KR], range(4)).values()])
            if n == CP1 - 2:
                for c in range(CP1):
                    r0 = KR + 256 + 192 * c
                    predict(pl.ds(pl.multiple_of(s + C * c, C), C), 1 + j, c,
                            [yn[r0 + 24 * k:r0 + 24 * k + 8] for k in range(8)])
        order_units()
        xq_v[...] = _pk(xn_units(units(1))[:, 0:D // 2].T)
        fold(wq_v, [wqb_v[2 + 2 * j], wqb_v[3 + 2 * j]], 1 + j)
        for e in range(4 * GO):
            row = KR + 384 + 640 * e // (4 * GO) // 8 * 8
            blk = jnp.minimum(GO * j + e // 4, D // 128 - 1)
            w = _pk(wo_v[blk, 256 * (e % 4):256 * (e % 4 + 1), :])
            wo32[blk, 128 * (e % 4):128 * (e % 4 + 1), :] = (
                w.reshape(16, 8, 128) | (_pk(ys[0][row:row + 8]) & zm)[None]).reshape(128, 128)
        vt = jnp.concatenate([yn[KR:] for yn in ys], axis=1)
        phis = [jnp.concatenate([ph[n][p] for n in range(CP1)], axis=1) for p in range(NP)]
        kvs, zs_ = kv_and_z(vt, phis, lambda p, zero: z_acc[p] + zero, ys[-1][KR:], zm)
        for p in range(NP):
            kv_acc[p] += kvs[p]
            z_acc[p] = zs_[p]
            zb_v[p] = jnp.broadcast_to(jnp.sum(zs_[p], axis=1, keepdims=True), (128, 128))
        return carry

    lax.fori_loop(0, N1, phase1, 0)
    for c in cp_ffn:
        c.wait()

    def ln2(h, offs, nx, nrel):
        deps = [None]
        for j in range(1, C // 8):
            t = (j * nrel * 2) // (C // 8) - 1
            r0 = (C - 8) * (t % 2)
            deps.append(nx[r0:r0 + 8, 128 * (t // 2):128 * (t // 2) + 128] if t >= 0 else None)
        hn = _ln(h, deps, zv[...])
        r = jnp.sum(hn * wr_row(), axis=-1, keepdims=True)
        for t, o in enumerate(offs):
            hn_v[pl.ds(o, U), :] = hn[U * t:U * (t + 1)].astype(bf16)
            out_v[pl.ds(o, U), :] = (h + hn)[U * t:U * (t + 1)].astype(bf16)
        return r

    lane = lax.broadcasted_iota(i32, (8, 128), 1)
    pos = (lane * 8 + lax.broadcasted_iota(i32, (8, 128), 0)).astype(f32)

    def token_at(posv, lo, hi):
        p = _scalar(posv, lo, hi - 1)
        u = lax.shift_right_logical(p, 6)
        return ord_s[u] + (p & (U - 1)), u

    def slab_of(tok):
        base = pl.multiple_of(lax.shift_left(lax.shift_right_logical(tok, 4), 4), 16)
        return pl.ds(base, 16), lax.broadcasted_iota(i32, (16, D), 0) == tok - base

    def token_row(tok):
        rows, hit = slab_of(tok)
        slab = jnp.where(hit, hn_v[rows, :].astype(f32), 0.0)
        return _allred8(slab[0:8] + slab[8:16], jnp.add)

    def patch(tok, y8, sg):
        rows, hit = slab_of(tok)
        cur = out_v[rows, :].astype(f32)
        fix_v[...] = jnp.where(hit, cur + _rows(y8 * _lanes(sg, D // 128), 2), cur).astype(bf16)

    def phase2(i, carry):
        q0 = CPT * i
        off = [units(q0 + k) for k in range(CPT + 1)]
        zm = zv[...]
        hprev = hbuf[...]
        kmask = lax.broadcasted_iota(i32, (64, 128), 0) // 32 == lax.broadcasted_iota(i32, (64, 128), 1) % 2

        def attend(y):
            os_ = []
            for p, yp in _pair_logits(y, range(4)).items():
                os_.append(_dot(jnp.where(kmask, kv_acc[p], 0.0).astype(bf16), _phi_q(yp, zb_v[p])))
            return jnp.concatenate(os_, axis=0).astype(bf16).T

        ya, ys = [], []
        for n in range(CPT):
            xt = xn_units(off[n + 1])
            ya.append(_dot_nt(_un(wq_v[:, 0:D // 2]), xt[:, 0:D // 2]) if n else
                      _dot(_un(wq_v[:, 0:D // 2]), _un(xq_v[...])))
            if n == CPT - 1:
                o01 = attend(jnp.concatenate(ys[0:2], axis=1))
            ys.append(ya[n] + _dot_nt(_un(wq_v[:, D // 2:D]), xt[:, D // 2:D]))
        wo = jnp.concatenate([_un(wo32[j]) for j in range(D // 128)], axis=1)
        head = _dot(o01[0:C], wo[:, 0:256])
        o23 = attend(jnp.concatenate(ys[2:4], axis=1))
        atts = [jnp.concatenate([head, _dot(o01[0:C], wo[:, 256:])], axis=1),
                _dot(o01[C:2 * C], wo), _dot(o23[0:C], wo), _dot(o23[C:2 * C], wo)]

        xq_v[...] = _pk(xn_units(units(jnp.minimum(q0 + CPT + 1, NC)))[:, 0:D // 2].T)

        def q_gate(v):
            lens = [KR // 8] + [KR // 8 - 24] * 3
            t, n = int(v * sum(lens)), 0
            while t >= lens[n]:
                t -= lens[n]
                n += 1
            r0 = 8 * (t + KR // 8 - lens[n])
            return _zero_after(ya[n][r0:r0 + 8], zm)

        def o_gate(t):
            r0, j = 8 * (t % 16), (t % 128) // 16
            return _zero_after(atts[t // 128][r0:r0 + 8, 128 * j:128 * j + 128], zm)

        t3 = jnp.maximum(i - 1, 0)
        nsb = NA // 2
        for sb in range(nsb):
            cols = slice(256 * sb, 256 * (sb + 1))
            xcol = xc_v[...]
            acc = None
            for k in range(0, D, 8):
                xk = _lanes(xcol[k:k + 8], 2)
                p = jnp.concatenate([wg_v[t3, k:k + 8, cols].astype(f32) * xk,
                                     wu_v[t3, k:k + 8, cols].astype(f32) * xk], axis=1)
                if k % 64 == 0:
                    p = p + _lanes(q_gate((sb * D + k) / (nsb * D)), 4)
                acc = p if acc is None else acc + p
            pa_v[:, 512 * sb:512 * (sb + 1)] = acc

        put_cols(r_v, i, 0, jnp.where(i > 0, ln2(hprev, off[0], atts[0], 6), -jnp.inf))

        @pl.when(i > 0)
        def _():
            cp_out(2 * q0).start()
            cp_out(2 * q0 + 1).start()

        acc = _allred8(pa_v[pl.ds(pl.multiple_of(zs[3, 0].astype(i32) * 32, 32), 8), :], jnp.add)
        g_ = jnp.concatenate([acc[:, 512 * t:512 * t + 256] for t in range(nsb)], axis=1)
        u_ = jnp.concatenate([acc[:, 512 * t + 256:512 * t + 512] for t in range(nsb)], axis=1)
        a8 = g_ * jax.nn.sigmoid(g_) * u_
        ac = _col(jnp.concatenate([jnp.where(t3 == 2, 0.0, a8[:, 0:NDUP]), a8[:, NDUP:]], axis=1))
        ysums = []
        for q in range(2):
            cols = slice(D // 2 * q, D // 2 * (q + 1))
            ysum = jnp.where(i > 1, y_v[:, cols], 0.0)
            for k in range(0, NA * 128, 8):
                p = wd_v[t3, k:k + 8, cols].astype(f32) * _lanes(ac[k:k + 8], 4)
                if k % 32 == 0:
                    p = p + _lanes(o_gate(64 + (q * NA * 128 + k) * 376 // (2 * NA * 128)), 4)
                ysum = ysum + p
            y_v[:, cols] = ysum
            ysums.append(ysum)

        for k in range(CPT):
            if k == NCAND:
                ok = (lane >= C // 8) & (lane < (NCAND + 1) * (C // 8))
                cm, cpos = _first_max(jnp.where(ok, r_v[0], -jnp.inf), pos)
                cand, cand_u = token_at(cpos, C, (NCAND + 1) * C)
                ord_s[NU + 2] = cand
                ord_s[NU + 3] = cand_u
                xc_v[...] = _col(token_row(cand))
                patch(cand, _allred8(jnp.concatenate(ysums, axis=1), jnp.add),
                      jax.nn.sigmoid(jnp.broadcast_to(cm, (8, 128))))
            h = jnp.concatenate([x_v[pl.ds(o, U), :].astype(f32) for o in off[k + 1]], axis=0) + atts[k]
            if k == CPT - 1:
                hbuf[...] = h
            else:
                put_cols(r_v, i, (k + 1) * (C // 8), ln2(h, off[k + 1], atts[k + 1], 5 if k == CPT - 2 else 6))
                cp_out(2 * (q0 + k + 1)).start()
                cp_out(2 * (q0 + k + 1) + 1).start()
        return carry

    lax.fori_loop(0, NT, phase2, 0)

    cand_u = ord_s[NU + 3]
    cp_out(cand_u).wait()
    fsem = new_sems(1)

    cand = ord_s[NU + 2]

    def cp_patch(tok):
        return pltpu.make_async_copy(fix_v, out_hbm.at[0, slab_of(tok)[0]], sems.at[fsem])

    cp_fix = cp_patch(cand)
    cp_fix.start()
    cp_out(2 * NCAND + 2).wait()
    last = units(NC)
    stats, cp_last = [], []
    for g in range(0, C, EG):
        h = hbuf[g:g + EG, :]
        s1 = h[:, 0:128]
        s2 = s1 * s1
        for j in range(128, D, 128):
            s1 = s1 + h[:, j:j + 128]
            s2 = s2 + h[:, j:j + 128] * h[:, j:j + 128]
        m = jnp.sum(s1, axis=-1, keepdims=True) * (1.0 / D)
        v = jnp.sum(s2, axis=-1, keepdims=True) * (1.0 / D) - m * m
        rs = lax.rsqrt(jnp.maximum(v, 0.0) + EPS)
        stats.append((m, rs))
        rows = pl.ds(pl.multiple_of(last[g // U] + g % U, EG), EG)
        out_v[rows, :] = (h * (1.0 + rs) - m * rs).astype(bf16)
        cp_last.append(cp(out_v.at[rows], out_hbm.at[0, rows]))
        cp_last[-1].start()
    for u in range(2, 2 * NCAND + 2):
        pl.when(cand_u != u)(cp_out(u).wait)
    for u in range(2 * NCAND + 3, NU - 2):
        cp_out(u).wait()
    pm, pi = _first_max(*_merge_max([(r_v[i], pos + float(i * T) if i else pos) for i in range(NT)]))
    wr = wr_row()
    wsum = jnp.sum(wr, axis=-1, keepdims=True)
    sub = lax.broadcasted_iota(i32, (8, 1), 0).astype(f32)
    cands = []
    for g, (m, rs) in zip(range(0, C, EG), stats):
        r = (jnp.sum(hbuf[g:g + EG, :] * wr, axis=-1, keepdims=True) - m * wsum) * rs
        cands += [(r[k:k + 8], sub + float(S + g + k)) for k in range(0, EG, 8)]
    while len(cands) > 1:
        cands = [_merge_max(cands[k:k + 2]) for k in range(0, len(cands), 2)]
    bv, bt = [jnp.broadcast_to(v, (8, 128)) for v in _merge_max([(pm, pi), cands[0]])]
    rmax = _allred8(bv, jnp.maximum)
    idx, _ = token_at(_allred8(jnp.where(bv == rmax, bt, float(2 * S)), jnp.minimum), C, S + C)
    cp_out(NU - 2).wait()
    cp_out(NU - 1).wait()
    cp_fix.wait()
    for c in cp_last:
        c.wait()

    @pl.when(idx != cand)
    def _():
        rows, _ = slab_of(cand)
        undo = pltpu.make_async_copy(out_v.at[rows], out_hbm.at[0, rows], sems.at[fsem])
        undo.start()
        for t, o in enumerate(last):
            hn_v[pl.ds(o, U), :] = _ln(hbuf[U * t:U * (t + 1), :]).astype(bf16)
        xs = _rows(token_row(idx), 2).astype(bf16)

        def step(j, acc):
            t = lax.shift_right_logical(j, 1)
            cols = pl.ds(pl.multiple_of((j & 1) * (NA * 64), 128), NA * 64)
            g = _dot(xs, wg_v[t, :, cols])
            a = g * jax.nn.sigmoid(g) * _dot(xs, wu_v[t, :, cols])
            a = jnp.concatenate([jnp.where(j == 4, 0.0, a[:, 0:NDUP]), a[:, NDUP:]], axis=1)
            return acc + _dot(a.astype(bf16), wd_v[t, cols, :])[0:8]

        y8 = lax.fori_loop(0, 6, step, jnp.zeros((8, D), f32))
        undo.wait()
        patch(idx, y8, jax.nn.sigmoid(rmax))
        redo = cp_patch(idx)
        redo.start()
        redo.wait()


@jax.jit
def pallas_sequential_preLN__linear_kernel_hedgehog__moe_arch_mod__prompt_kernel(
    A_x: jax.Array,
    A_wqkv: jax.Array,
    A_w_phi: jax.Array,
    A_wo: jax.Array,
    B_x: jax.Array,
    B_w_r: jax.Array,
    B_w_gate: jax.Array,
    B_w_up: jax.Array,
    B_w_down: jax.Array,
):
    del B_x
    any_spec = pl.BlockSpec(memory_space=pl.ANY)
    return pl.pallas_call(
        _kernel,
        out_shape=jax.ShapeDtypeStruct((1, S, D), bf16),
        in_specs=[any_spec] * 8,
        out_specs=any_spec,
        scratch_shapes=[
            pltpu.VMEM((S, D), bf16),
            pltpu.VMEM((D, 3 * D), bf16),
            pltpu.VMEM((D // 128, D, 128), bf16),
            pltpu.VMEM((H, DH, DH), bf16),
            pltpu.VMEM((D // 128, D, 128), bf16),
            pltpu.VMEM((D // 128, D // 2, 128), u32),
            pltpu.VMEM((D,), bf16),
            pltpu.VMEM((3, D, NA * 128), bf16),
            pltpu.VMEM((3, D, NA * 128), bf16),
            pltpu.VMEM((3, NA * 128, D), bf16),
            pltpu.VMEM(((KR + D) // 2, D), u32),
            pltpu.VMEM((KR // 2, D), u32),
            pltpu.VMEM((8, 64, 128), u32),
            pltpu.VMEM(((S + C) // 2, D), u32),
            pltpu.VMEM((D // 4, C), u32),
            pltpu.VMEM((D // 4, C), u32),
            pltpu.VMEM((S + C, D), bf16),
            pltpu.VMEM((NP, 64, 128), f32),
            pltpu.VMEM((NP, 128, 128), f32),
            pltpu.VMEM((NP, 128, 128), f32),
            pltpu.VMEM((C, D), f32),
            pltpu.VMEM((S + C, D), bf16),
            pltpu.VMEM((8, 128), u32),
            pltpu.SMEM((8, 128), u32),
            pltpu.VMEM((1 + N1, 8, 128), f32),
            pltpu.VMEM((NT, 8, 128), f32),
            pltpu.VMEM((D, 128), f32),
            pltpu.VMEM((8, NA * 256), f32),
            pltpu.VMEM((8, D), f32),
            pltpu.VMEM((16, D), bf16),
            pltpu.SMEM((NU + 4,), i32),
            pltpu.SemaphoreType.DMA((72,)),
        ],
        compiler_params=pltpu.CompilerParams(vmem_limit_bytes=120 * 1024 * 1024,
                                             disable_bounds_checks=True,
                                             disable_semaphore_checks=True),
        name="hedgehog_mod",
    )(A_x, A_wqkv, A_w_phi, A_wo, B_w_r, B_w_gate, B_w_up, B_w_down)
```

```python
import jax
import jax.numpy as jnp
from jax import lax
import jax.experimental.pallas as pl
import jax.experimental.pallas.tpu as pltpu

S = 2048
D = 1024
H = 32
DH = 32
F = 3584
NP = H // 2
C = 128
NC = S // C
U = 64
NU = S // U
T = 512
NT = S // T
CPT = T // C
T1 = 512
N1 = (S - T) // T1
CP1 = T1 // C
KR = H * (DH - 1)
GO = -(-8 // N1)
SEGS = ((256, 256), (128, 256), (128, 512))
PHI = ((0, 512), (512, 512), (512, 1024))
DEFER = 2
NB = F // 128
NA = 10
B0 = (0, NA, NB - NA)
NDUP = (3 * NA - NB) * 128
NCAND = 2
EG = 16
LOG2E = 1.4426950408889634
EPS = 1e-5

f32 = jnp.float32
bf16 = jnp.bfloat16
u32 = jnp.uint32
i32 = jnp.int32


def _dot_nt(a, b):
    return lax.dot_general(a, b, (((1,), (1,)), ((), ())), preferred_element_type=f32)


def _dot(a, b):
    return jnp.dot(a, b, preferred_element_type=f32)


def _pk(x):
    return pltpu.bitcast(x, u32)


def _un(x):
    return pltpu.bitcast(x, bf16)


def _rcp(x):
    r = pl.reciprocal(x, approx=True)
    return r * (2.0 - x * r)


def _allred(v, op):
    v = op(v, pltpu.roll(v, 2, 0))
    return op(v, pltpu.roll(v, 4, 0))


def _allred8(v, op):
    return _allred(op(v, pltpu.roll(v, 1, 0)), op)


def _rows(v, n):
    return jnp.concatenate([v] * n, axis=0)


def _lanes(v, n):
    return jnp.concatenate([v] * n, axis=1)


def _zero_after(dep, zm):
    return pltpu.bitcast(pltpu.bitcast(dep, u32) & zm, f32)


def _exps(x):
    x3 = x.reshape(8, 8, x.shape[1])
    mx = _allred(jnp.max(x3, axis=0), jnp.maximum)
    mn = _allred(jnp.min(x3, axis=0), jnp.minimum)
    ep = jnp.exp2(x3 - mx[None])
    en = jnp.exp2(mn[None] - x3)
    rp = _rcp(_allred(jnp.sum(ep, axis=0), jnp.add))
    rn = _rcp(_allred(jnp.sum(en, axis=0), jnp.add))
    return ep, en, rp, rn


def _phi_k(x):
    L = x.shape[1]
    ep, en, rp, rn = _exps(x)
    return jnp.concatenate([(ep * rp[None]).reshape(64, L), (en * rn[None]).reshape(64, L)], axis=0)


def _phi_q(x, zb):
    L = x.shape[1]
    ep, en, rp, rn = _exps(x)
    zb = _lanes(zb, L // 128).reshape(16, 8, L)
    den = rp * jnp.sum(ep * zb[0:8], axis=0) + rn * jnp.sum(en * zb[8:16], axis=0)
    inv = _rcp(_allred(den, jnp.add) + 1e-6)
    cp = rp * inv
    cn = rn * inv
    phi = jnp.concatenate([(ep * cp[None]).reshape(64, L), (en * cn[None]).reshape(64, L)], axis=0)
    return phi.astype(bf16)


def _slot(n):
    return lax.shift_right_logical(lax.broadcasted_iota(i32, (8, n), 0), 1)


def _pair_logits(y, sgs):
    slot = _slot(y.shape[1])
    out, r, shared = {}, 0, None
    for k, sg in enumerate(sgs):
        if k == 0 or sg % 2 == 0:
            shared, r = y[r:r + 16], r + 16
        l0, l1, l2 = y[r:r + 8], y[r + 8:r + 16], shared[8 * (sg % 2):8 * (sg % 2) + 8]
        for q in range(4):
            x0 = jnp.where(slot == q, l0, jnp.where(slot == (q + 1) % 4, l1, jnp.where(slot == (q + 2) % 4, l2, 0.0)))
            out[4 * sg + q] = jnp.concatenate([x0, y[r + 16 + 56 * q:r + 72 + 56 * q]], axis=0)
        r += 240
    return out


def _lane_blocks_sum(v, acc):
    for c in range(0, v.shape[1], 128):
        acc = acc + v[:, c:c + 128]
    return acc


def _row_sum(x, deps, zm):
    g = x.shape[0] // len(deps)
    gate = jnp.concatenate([jnp.zeros((8, 128), f32) if d is None else _zero_after(d, zm)
                            for d in deps for _ in range(g // 8)], axis=0)
    return jnp.sum(_lane_blocks_sum(x[:, 128:], x[:, 0:128] + gate), axis=-1, keepdims=True)


def _ln(x, deps=None, zm=None):
    tot = jnp.sum(x, axis=-1, keepdims=True) if deps is None else _row_sum(x, deps, zm)
    xc = x - tot * (1.0 / D)
    return xc * lax.rsqrt(jnp.sum(xc * xc, axis=-1, keepdims=True) * (1.0 / D) + EPS)


def _col(a8):
    return _rows(a8, 16).astype(bf16).T.astype(f32)


def _first_max(v, t):
    m = jnp.max(_allred8(v, jnp.maximum), axis=1, keepdims=True)
    return m, jnp.min(_allred8(jnp.where(v == m, t, float(2 * S)), jnp.minimum), axis=1, keepdims=True)


def _merge_max(cands):
    v, t = cands[0]
    for v2, t2 in cands[1:]:
        gt = v2 > v
        v, t = jnp.where(gt, v2, v), jnp.where(gt, t2, t)
    return v, t


def _scalar(v, lo, hi):
    return jnp.clip(jnp.broadcast_to(v, (8, 128)).astype(i32)[0, 0], lo, hi)


class _Group:
    def __init__(self, parts, dst, sem):
        self.parts, self.dst, self.sem = parts, dst, sem

    def start(self):
        for src, dst in self.parts:
            pltpu.make_async_copy(src, dst, self.sem).start()

    def wait(self):
        pltpu.make_async_copy(self.dst, self.dst, self.sem).wait()


def _kernel(x_hbm, wqkv_hbm, wphi_hbm, wo_hbm, wr_hbm, wg_hbm, wu_hbm, wd_hbm, out_hbm,
            x_v, wkv_v, wqb_v, wphi_v, wo_v, wo32, wr_v, wg_v, wu_v, wd_v,
            wt_v, wq_v, a_v, xn_v, xk_v, xq_v, hn_v, kv_acc, z_acc, zb_v, hbuf, out_v, zv, zs, p_v, r_v,
            xc_v, pa_v, y_v, fix_v, ord_s, sems):
    nsem = [0]

    def new_sems(n):
        nsem[0] += n
        return nsem[0] - n

    def cp(src, dst):
        return pltpu.make_async_copy(src, dst, sems.at[new_sems(1)])

    def cp_w(lo, hi):
        return cp(wqkv_hbm.at[:, lo:hi], wkv_v.at[:, lo:hi])

    def cp_x(lo, hi):
        return cp(x_hbm.at[0, lo:hi], x_v.at[lo:hi])

    cp_wr = cp(wr_hbm, wr_v)
    kcum = [0]
    for _, dk in SEGS:
        kcum.append(kcum[-1] + dk)
    seg_cp = []
    x0 = 0
    for si, (dx, dk) in enumerate(SEGS):
        lo, hi = PHI[si][0] // DH, PHI[si][1] // DH
        ph = [cp(wphi_hbm.at[lo:hi], wphi_v.at[lo:hi])] if hi > lo else []
        seg_cp.append([cp_x(x0, x0 + dx)] + ph + [cp_w(D + kcum[si], D + kcum[si + 1])])
        x0 += dx
    cp_wv = cp_w(2 * D, 3 * D)
    cp_x1a = cp_x(T, T + C)
    cp_x1 = cp_x(T + C, T + T1 + C)
    cp_x2 = cp_x(T + T1 + C, S)
    cp_q0 = _Group([(wqkv_hbm.at[:, 128 * g:128 * (g + 1)], wqb_v.at[g]) for g in range(2)],
                   wqb_v.at[0:2], sems.at[new_sems(1)])
    cp_q1 = _Group([(wqkv_hbm.at[:, 128 * g:128 * (g + 1)], wqb_v.at[g]) for g in range(2, 8)],
                   wqb_v.at[2:8], sems.at[new_sems(1)])
    cp_wo = _Group([(wo_hbm.at[:, 128 * g:128 * (g + 1)], wo_v.at[g]) for g in range(8)], wo_v, sems.at[new_sems(1)])
    cp_ffn = [_Group([(wg_hbm.at[:, b * 128:(b + NA) * 128], wg_v.at[t]) for t, b in enumerate(B0)],
                     wg_v, sems.at[new_sems(1)]),
              _Group([(wu_hbm.at[:, b * 128:(b + NA) * 128], wu_v.at[t]) for t, b in enumerate(B0)],
                     wu_v, sems.at[new_sems(1)]),
              _Group([(wd_hbm.at[b * 128:(b + NA) * 128], wd_v.at[t]) for t, b in enumerate(B0)],
                     wd_v, sems.at[new_sems(1)])]
    seg_cp[0] = seg_cp[0][1:] + seg_cp[0][0:1]
    for c in [c for t in seg_cp for c in t] + [cp_wr, cp_wv, cp_x1a, cp_q0, cp_x1, cp_q1, cp_wo, cp_x2] + cp_ffn:
        c.start()
    osem0 = new_sems(NU)

    def cp_out(u):
        rows = pl.ds(pl.multiple_of(ord_s[u], U), U)
        return pltpu.make_async_copy(out_v.at[rows], out_hbm.at[0, rows], sems.at[osem0 + u])

    def wr_row():
        return wr_v[...].reshape(1, D).astype(f32)

    def put_cols(ref, idx, col0, r):
        for k in range(0, r.shape[0], 8):
            ref[idx, :, col0 + k // 8:col0 + k // 8 + 1] = r[k:k + 8]

    def half(row0, n):
        if isinstance(row0, int):
            return pl.ds(row0 // 2, n // 2)
        return pl.ds(pl.multiple_of(lax.shift_right_logical(row0, 1), U // 2), n // 2)

    def ln1(src, dst, n, deps=None):
        xb = _pk(_ln(x_v[pl.ds(src, n), :].astype(f32), deps, None if deps is None else zv[...]).astype(bf16))
        xn_v[half(dst, n), :] = xb
        return _un(xb)

    def xn(row0, n):
        return _un(xn_v[half(row0, n), :])

    def units(q):
        return [pl.multiple_of(ord_s[2 * q + t], U) for t in range(2)]

    def xn_units(offs):
        return _un(jnp.concatenate([xn_v[half(o, U), :] for o in offs], axis=0))

    def predict(rows, t, c, deps):
        wr = wr_row()
        wc = wr - jnp.sum(wr, axis=-1, keepdims=True) * (1.0 / D)
        put_cols(p_v, t, c * (C // 8), _row_sum(x_v[rows, :].astype(f32) * wc, deps, zv[...]))

    def fold(dst, ws, sg):
        slot = _slot(D)
        res = [_dot_nt(_un(a_v[2 * sg + e]), ws[e]) for e in range(2)]
        main, e0, e1 = [], [], []
        for e in range(2):
            z = jnp.where(((slot + 3) % 4) // 2 == e, 0.0, res[e][0:8])
            b1 = z + pltpu.roll(z, 4, 0)
            b0 = pltpu.roll(b1, 2, 0)
            for pp in range(2):
                base = jnp.where(slot % 2 == pp, b0, b1)
                main.append((res[e][16 + 56 * pp:72 + 56 * pp].reshape(7, 8, D) - base[None]).reshape(56, D))
            e0.append(res[e][8:16] - b0)
            e1.append(res[e][0:8] - b1)
        rows = jnp.concatenate([jnp.where(slot < 2, e0[0], e0[1]), e1[0] + e1[1]] + main, axis=0)
        l2 = _pk((_rows(jnp.where(slot < 2, e0[1], e0[0]), 2) * LOG2E).astype(bf16))
        if isinstance(sg, int):
            r0, r1 = 248 * (sg // 2), 248 * (sg // 2) + 8 + 120 * (sg % 2)
        else:
            r0 = pl.multiple_of(248 * lax.shift_right_logical(sg, 1), 8)
            r1 = pl.multiple_of(r0 + 8 + 120 * (sg & 1), 8)
        dst[pl.ds(r1, 120), :] = _pk((rows * LOG2E).astype(bf16))
        dst[pl.ds(r0, 8), :] = jnp.where(slot // 2 == sg % 2, l2, dst[pl.ds(r0, 8), :])
        return res

    def wk(lo, hi):
        r0, r1 = 248 * (lo // 2), 248 * ((hi - 1) // 2) + 128 + 120 * ((hi - 1) % 2)
        if lo % 2:
            return _un(jnp.concatenate([wt_v[r0:r0 + 8, :], wt_v[r0 + 128:r1, :]], axis=0))
        return _un(wt_v[r0:r1, :])

    def kv_and_z(vt, phis, z_of, tail, zm):
        kvs = [_dot_nt(vt[64 * p:64 * (p + 1)].astype(bf16), phis[p].astype(bf16)) for p in range(NP)]
        zs_ = [_lane_blocks_sum(phis[p], z_of(p, _rows(_zero_after(tail[256 + 48 * p:264 + 48 * p], zm), 16)))
               for p in range(NP)]
        return kvs, zs_

    def a_row(r, e):
        s = (r & 7) >> 1
        f = jnp.where(r >= 72, (r - 64) >> 1, jnp.where(r >= 16, (r - 8) >> 1, jnp.where(
            r >= 8, jnp.where(s >> 1 == e, 1, 3), jnp.where(((s + 3) & 3) >> 1 == e, 2, 0))))
        pp = jnp.where(r >= 72, 1, jnp.where(r >= 16, 0, jnp.where(r >= 8, s, s + 1) & 1))
        return f, 2 * pp + (r & 1)

    f_i = lax.broadcasted_iota(i32, (128, DH), 1)
    sel = [jnp.where(f_i == a_row(lax.broadcasted_iota(i32, (128, DH), 0), e)[0], 1.0, 0.0).astype(bf16)
           for e in range(2)]
    amask = jnp.where(lax.broadcasted_iota(i32, (128, 128), 1) >> 5
                      == a_row(lax.broadcasted_iota(i32, (128, 128), 0), 0)[1], jnp.uint32(0xFFFFFFFF), jnp.uint32(0))

    def build_a(lo, hi):
        for g in range(lo // 128, hi // 128):
            blk = _dot_nt(sel[g % 2], wphi_v[4 * g:4 * (g + 1)].reshape(128, DH))
            a_v[g] = _pk(pltpu.bitcast(pltpu.bitcast(blk, u32) & amask, f32).astype(bf16))

    zv[...] = jnp.zeros((8, 128), u32)
    cp_z = cp(zv, zs)
    cp_z.start()
    for ref in (wt_v, wq_v):
        for r0 in (0, 248):
            ref[r0:r0 + 8, :] = jnp.zeros((8, D), u32)
    hbuf[...] = jnp.zeros(hbuf.shape, f32)
    xc_v[...] = jnp.zeros(xc_v.shape, f32)
    y_v[...] = jnp.zeros(y_v.shape, f32)
    r_v[...] = jnp.full(r_v.shape, -jnp.inf, f32)
    p_v[...] = jnp.full(p_v.shape, -jnp.inf, f32)

    pieces = [[] for _ in range(NP)]
    pending = []

    def phi_piece(p, t0, yp, dep=None):
        if dep is not None:
            yp = jnp.concatenate([yp[0:8] + _zero_after(dep, zv[...]), yp[8:]], axis=0)
        pieces[p].append((t0, _phi_k(yp)))

    def k_block(lo, hi, t0, t1, defer=0):
        y = _dot_nt(wk(lo, hi), xn(t0, t1 - t0))
        for p, yp in _pair_logits(y, range(lo, hi)).items():
            if p >= 4 * hi - defer:
                if t1 - t0 > C:
                    phi_piece(p, t0, yp[:, 0:t1 - t0 - C])
                pending.append((p, t1 - C, yp[:, t1 - t0 - C:]))
            else:
                phi_piece(p, t0, yp)
        return y

    def flush(res):
        for k, (p, t0, yp) in enumerate(pending):
            phi_piece(p, t0, yp, res[32 * k:32 * k + 8, 0:128])
        del pending[:]

    x0 = 0
    for si, (dx, dk) in enumerate(SEGS):
        k0, k1 = kcum[si] // 256, kcum[si + 1] // 256
        if si == 0:
            seg_cp[0][0].wait()
            build_a(*PHI[0])
            seg_cp[0][1].wait()
        else:
            for c in seg_cp[si]:
                c.wait()
            if PHI[si][1] > PHI[si][0]:
                build_a(*PHI[si])
        res = [fold(wt_v, [wkv_v[:, D + 128 * g:D + 128 * (g + 1)] for g in (2 * sg, 2 * sg + 1)], sg)
               for sg in range(k0, k1)]
        flush(res[0][0])
        if si == 0:
            seg_cp[0][2].wait()
        ln1(x0, x0, dx)
        if si:
            k_block(k0, k1, 0, x0)
        k_block(0, k1, x0, x0 + dx, DEFER)
        x0 += dx
    for c in (cp_wv, cp_x1a, cp_q0, cp_wr, cp_z):
        c.wait()
    for g in range(D // 128):
        wt_v[KR // 2 + 64 * g:KR // 2 + 64 * (g + 1), :] = _pk(wkv_v[:, 2 * D + 128 * g:2 * D + 128 * (g + 1)].T)
    flush(fold(wq_v, [wqb_v[0], wqb_v[1]], 0)[0])
    yv = _dot_nt(_un(wt_v[KR // 2:, :]), xn(0, T))
    xk_v[...] = _pk(ln1(T, T, C, [yv[128 * k:128 * k + 8, 128:256] for k in range(8)])[:, 0:D // 2].T)
    for c in range(CPT):
        predict(slice(C * c, C * (c + 1)), 0, c,
                [yv[256 * c + 32 * k:256 * c + 32 * k + 8, 256:384] for k in range(8)])
    phis = [jnp.concatenate([ph for _, ph in sorted(pieces[p], key=lambda tp: tp[0])], axis=1) for p in range(NP)]
    kvs, zs_ = kv_and_z(yv, phis, lambda p, zero: zero, yv[:, T - C:T], zv[...])
    for p in range(NP):
        kv_acc[p] = kvs[p]
        z_acc[p] = zs_[p]
    for c in (cp_x1, cp_q1, cp_wo):
        c.wait()

    def order_units():
        lane8 = lax.shift_right_logical(lax.broadcasted_iota(i32, (8, 128), 1), 3).astype(f32)
        vals = [p_v[t] for t in range(1 + N1)]
        uids = [lane8 + float(0 if t == 0 else (T + T1 * (t - 1)) // U) for t in range(1 + N1)]
        code = None
        for r in range(2 * NCAND):
            best = _first_max(*_merge_max(list(zip(vals, uids))))[1]
            vals = [jnp.where(u == best, -jnp.inf, v) for v, u in zip(vals, uids)]
            code = best if code is None else code * float(NU) + best
        code = _scalar(code, 0, NU ** (2 * NCAND) - 1)
        for u in range(NU + 2):
            ord_s[u] = (S + u * U) if u < 2 else (u - 2) * U
        swaps = []
        for r in range(2 * NCAND):
            p = lax.shift_right_logical(code, 5 * (2 * NCAND - 1 - r)) & (NU - 1)
            for lo, hi in swaps:
                p = jnp.where(p == lo, hi, jnp.where(p == hi, lo, p))
            swaps.append((r, p))
            here, there = ord_s[2 + r], ord_s[2 + p]
            ord_s[2 + r] = there
            ord_s[2 + p] = here

    def phase1(j, carry):
        @pl.when(j == 1)
        def _():
            cp_x2.wait()

        zm = zv[...]
        s = pl.multiple_of(T + j * T1, C)
        nxt = pl.multiple_of(jnp.where(j + 1 < N1, s + T1, 0), C)
        s2 = s + zs[2, 0].astype(i32)
        ys, ph = [], []
        for n in range(CP1):
            xt = xn(pl.multiple_of(s2 + C * n, C), C)
            y0 = _dot_nt(_un(wt_v[:, 0:D // 2]), xt[:, 0:D // 2]) if n else _dot(_un(wt_v[:, 0:D // 2]), _un(xk_v[...]))
            row0 = pl.multiple_of(s + C * (n + 1), C)
            xb = ln1(row0 if n + 1 < CP1 else nxt, row0, C, [y0[128 + 96 * k:136 + 96 * k] for k in range(16)])
            if n + 1 == CP1:
                xk_v[...] = _pk(xb[:, 0:D // 2].T)
            yn = _dot_nt(_un(wt_v[:, D // 2:D]), xt[:, D // 2:D]) + y0
            ys.append(yn)
            ph.append([_phi_k(yp) for yp in _pair_logits(yn[0:KR], range(4)).values()])
            if n == CP1 - 2:
                for c in range(CP1):
                    r0 = KR + 256 + 192 * c
                    predict(pl.ds(pl.multiple_of(s + C * c, C), C), 1 + j, c,
                            [yn[r0 + 24 * k:r0 + 24 * k + 8] for k in range(8)])
        order_units()
        xq_v[...] = _pk(xn_units(units(1))[:, 0:D // 2].T)
        fold(wq_v, [wqb_v[2 + 2 * j], wqb_v[3 + 2 * j]], 1 + j)
        for e in range(4 * GO):
            row = KR + 384 + 640 * e // (4 * GO) // 8 * 8
            blk = jnp.minimum(GO * j + e // 4, D // 128 - 1)
            w = _pk(wo_v[blk, 256 * (e % 4):256 * (e % 4 + 1), :])
            wo32[blk, 128 * (e % 4):128 * (e % 4 + 1), :] = (
                w.reshape(16, 8, 128) | (_pk(ys[0][row:row + 8]) & zm)[None]).reshape(128, 128)
        vt = jnp.concatenate([yn[KR:] for yn in ys], axis=1)
        phis = [jnp.concatenate([ph[n][p] for n in range(CP1)], axis=1) for p in range(NP)]
        kvs, zs_ = kv_and_z(vt, phis, lambda p, zero: z_acc[p] + zero, ys[-1][KR:], zm)
        for p in range(NP):
            kv_acc[p] += kvs[p]
            z_acc[p] = zs_[p]
            zb_v[p] = jnp.broadcast_to(jnp.sum(zs_[p], axis=1, keepdims=True), (128, 128))
        return carry

    lax.fori_loop(0, N1, phase1, 0)
    for c in cp_ffn:
        c.wait()

    def ln2(h, offs, nx, nrel):
        deps = [None]
        for j in range(1, C // 8):
            t = (j * nrel * 2) // (C // 8) - 1
            r0 = (C - 8) * (t % 2)
            deps.append(nx[r0:r0 + 8, 128 * (t // 2):128 * (t // 2) + 128] if t >= 0 else None)
        hn = _ln(h, deps, zv[...])
        r = jnp.sum(hn * wr_row(), axis=-1, keepdims=True)
        for t, o in enumerate(offs):
            hn_v[pl.ds(o, U), :] = hn[U * t:U * (t + 1)].astype(bf16)
            out_v[pl.ds(o, U), :] = (h + hn)[U * t:U * (t + 1)].astype(bf16)
        return r

    lane = lax.broadcasted_iota(i32, (8, 128), 1)
    pos = (lane * 8 + lax.broadcasted_iota(i32, (8, 128), 0)).astype(f32)

    def token_at(posv, lo, hi):
        p = _scalar(posv, lo, hi - 1)
        u = lax.shift_right_logical(p, 6)
        return ord_s[u] + (p & (U - 1)), u

    def slab_of(tok):
        base = pl.multiple_of(lax.shift_left(lax.shift_right_logical(tok, 4), 4), 16)
        return pl.ds(base, 16), lax.broadcasted_iota(i32, (16, D), 0) == tok - base

    def token_row(tok):
        rows, hit = slab_of(tok)
        slab = jnp.where(hit, hn_v[rows, :].astype(f32), 0.0)
        return _allred8(slab[0:8] + slab[8:16], jnp.add)

    def patch(tok, y8, sg):
        rows, hit = slab_of(tok)
        cur = out_v[rows, :].astype(f32)
        fix_v[...] = jnp.where(hit, cur + _rows(y8 * _lanes(sg, D // 128), 2), cur).astype(bf16)

    def phase2(i, carry):
        q0 = CPT * i
        off = [units(q0 + k) for k in range(CPT + 1)]
        zm = zv[...]
        hprev = hbuf[...]
        kmask = lax.broadcasted_iota(i32, (64, 128), 0) // 32 == lax.broadcasted_iota(i32, (64, 128), 1) % 2

        def attend(y):
            os_ = []
            for p, yp in _pair_logits(y, range(4)).items():
                os_.append(_dot(jnp.where(kmask, kv_acc[p], 0.0).astype(bf16), _phi_q(yp, zb_v[p])))
            return jnp.concatenate(os_, axis=0).astype(bf16).T

        ya, ys = [], []
        for n in range(CPT):
            xt = xn_units(off[n + 1])
            ya.append(_dot_nt(_un(wq_v[:, 0:D // 2]), xt[:, 0:D // 2]) if n else
                      _dot(_un(wq_v[:, 0:D // 2]), _un(xq_v[...])))
            if n == CPT - 1:
                o01 = attend(jnp.concatenate(ys[0:2], axis=1))
            ys.append(ya[n] + _dot_nt(_un(wq_v[:, D // 2:D]), xt[:, D // 2:D]))
        wo = jnp.concatenate([_un(wo32[j]) for j in range(D // 128)], axis=1)
        head = _dot(o01[0:C], wo[:, 0:256])
        o23 = attend(jnp.concatenate(ys[2:4], axis=1))
        atts = [jnp.concatenate([head, _dot(o01[0:C], wo[:, 256:])], axis=1),
                _dot(o01[C:2 * C], wo), _dot(o23[0:C], wo), _dot(o23[C:2 * C], wo)]

        xq_v[...] = _pk(xn_units(units(jnp.minimum(q0 + CPT + 1, NC)))[:, 0:D // 2].T)

        def q_gate(v):
            lens = [KR // 8] + [KR // 8 - 24] * 3
            t, n = int(v * sum(lens)), 0
            while t >= lens[n]:
                t -= lens[n]
                n += 1
            r0 = 8 * (t + KR // 8 - lens[n])
            return _zero_after(ya[n][r0:r0 + 8], zm)

        def o_gate(t):
            r0, j = 8 * (t % 16), (t % 128) // 16
            return _zero_after(atts[t // 128][r0:r0 + 8, 128 * j:128 * j + 128], zm)

        t3 = jnp.maximum(i - 1, 0)
        nsb = NA // 2
        for sb in range(nsb):
            cols = slice(256 * sb, 256 * (sb + 1))
            xcol = xc_v[...]
            acc = None
            for k in range(0, D, 8):
                xk = _lanes(xcol[k:k + 8], 2)
                p = jnp.concatenate([wg_v[t3, k:k + 8, cols].astype(f32) * xk,
                                     wu_v[t3, k:k + 8, cols].astype(f32) * xk], axis=1)
                if k % 64 == 0:
                    p = p + _lanes(q_gate((sb * D + k) / (nsb * D)), 4)
                acc = p if acc is None else acc + p
                if (k + 8) % (D // 2) == 0:
                    pa_v[8 * (2 * k // D):8 * (2 * k // D) + 8, 512 * sb:512 * (sb + 1)] = acc
                    acc = None

        put_cols(r_v, i, 0, jnp.where(i > 0, ln2(hprev, off[0], atts[0], 7), -jnp.inf))

        @pl.when(i > 0)
        def _():
            cp_out(2 * q0).start()
            cp_out(2 * q0 + 1).start()

        acc = pa_v[pl.ds(pl.multiple_of(zs[3, 0].astype(i32) * 32, 32), 16), :]
        acc = _allred8(acc[0:8] + acc[8:16], jnp.add)
        g_ = jnp.concatenate([acc[:, 512 * t:512 * t + 256] for t in range(nsb)], axis=1)
        u_ = jnp.concatenate([acc[:, 512 * t + 256:512 * t + 512] for t in range(nsb)], axis=1)
        a8 = g_ * jax.nn.sigmoid(g_) * u_
        ac = _col(jnp.concatenate([jnp.where(t3 == 2, 0.0, a8[:, 0:NDUP]), a8[:, NDUP:]], axis=1))
        ysums = []
        for q in range(2):
            cols = slice(D // 2 * q, D // 2 * (q + 1))
            ysum = jnp.where(i > 1, y_v[:, cols], 0.0)
            for k in range(0, NA * 128, 8):
                p = wd_v[t3, k:k + 8, cols].astype(f32) * _lanes(ac[k:k + 8], 4)
                if k % 32 == 0:
                    p = p + _lanes(o_gate(64 + (q * NA * 128 + k) * 376 // (2 * NA * 128)), 4)
                ysum = ysum + p
            y_v[:, cols] = ysum
            ysums.append(ysum)

        for k in range(CPT):
            if k == NCAND:
                ok = (lane >= C // 8) & (lane < (NCAND + 1) * (C // 8))
                cm, cpos = _first_max(jnp.where(ok, r_v[0], -jnp.inf), pos)
                cand, cand_u = token_at(cpos, C, (NCAND + 1) * C)
                ord_s[NU + 2] = cand
                ord_s[NU + 3] = cand_u
                xc_v[...] = _col(token_row(cand))
                patch(cand, _allred8(jnp.concatenate(ysums, axis=1), jnp.add),
                      jax.nn.sigmoid(jnp.broadcast_to(cm, (8, 128))))
            h = jnp.concatenate([x_v[pl.ds(o, U), :].astype(f32) for o in off[k + 1]], axis=0) + atts[k]
            if k == CPT - 1:
                hbuf[...] = h
            else:
                put_cols(r_v, i, (k + 1) * (C // 8), ln2(h, off[k + 1], atts[k + 1], 5 if k == CPT - 2 else 7))
                cp_out(2 * (q0 + k + 1)).start()
                cp_out(2 * (q0 + k + 1) + 1).start()
        return carry

    lax.fori_loop(0, NT, phase2, 0)

    cand_u = ord_s[NU + 3]
    cp_out(cand_u).wait()
    fsem = new_sems(1)

    cand = ord_s[NU + 2]

    def cp_patch(tok):
        return pltpu.make_async_copy(fix_v, out_hbm.at[0, slab_of(tok)[0]], sems.at[fsem])

    cp_fix = cp_patch(cand)
    cp_fix.start()
    cp_out(2 * NCAND + 2).wait()
    last = units(NC)
    stats, cp_last = [], []
    for g in range(0, C, EG):
        h = hbuf[g:g + EG, :]
        s1 = h[:, 0:128]
        s2 = s1 * s1
        for j in range(128, D, 128):
            s1 = s1 + h[:, j:j + 128]
            s2 = s2 + h[:, j:j + 128] * h[:, j:j + 128]
        m = jnp.sum(s1, axis=-1, keepdims=True) * (1.0 / D)
        v = jnp.sum(s2, axis=-1, keepdims=True) * (1.0 / D) - m * m
        rs = lax.rsqrt(jnp.maximum(v, 0.0) + EPS)
        stats.append((m, rs))
        rows = pl.ds(pl.multiple_of(last[g // U] + g % U, EG), EG)
        out_v[rows, :] = (h * (1.0 + rs) - m * rs).astype(bf16)
        cp_last.append(cp(out_v.at[rows], out_hbm.at[0, rows]))
        cp_last[-1].start()
    for u in range(2, 2 * NCAND + 2):
        pl.when(cand_u != u)(cp_out(u).wait)
    for u in range(2 * NCAND + 3, NU - 2):
        cp_out(u).wait()
    pm, pi = _first_max(*_merge_max([(r_v[i], pos + float(i * T) if i else pos) for i in range(NT)]))
    wr = wr_row()
    wsum = jnp.sum(wr, axis=-1, keepdims=True)
    sub = lax.broadcasted_iota(i32, (8, 1), 0).astype(f32)
    cands = []
    for g, (m, rs) in zip(range(0, C, EG), stats):
        r = (jnp.sum(hbuf[g:g + EG, :] * wr, axis=-1, keepdims=True) - m * wsum) * rs
        cands += [(r[k:k + 8], sub + float(S + g + k)) for k in range(0, EG, 8)]
    while len(cands) > 1:
        cands = [_merge_max(cands[k:k + 2]) for k in range(0, len(cands), 2)]
    bv, bt = [jnp.broadcast_to(v, (8, 128)) for v in _merge_max([(pm, pi), cands[0]])]
    rmax = _allred8(bv, jnp.maximum)
    idx, _ = token_at(_allred8(jnp.where(bv == rmax, bt, float(2 * S)), jnp.minimum), C, S + C)
    cp_out(NU - 2).wait()
    cp_out(NU - 1).wait()
    cp_fix.wait()
    for c in cp_last:
        c.wait()

    @pl.when(idx != cand)
    def _():
        rows, _ = slab_of(cand)
        undo = pltpu.make_async_copy(out_v.at[rows], out_hbm.at[0, rows], sems.at[fsem])
        undo.start()
        for t, o in enumerate(last):
            hn_v[pl.ds(o, U), :] = _ln(hbuf[U * t:U * (t + 1), :]).astype(bf16)
        xs = _rows(token_row(idx), 2).astype(bf16)

        def step(j, acc):
            t = lax.shift_right_logical(j, 1)
            cols = pl.ds(pl.multiple_of((j & 1) * (NA * 64), 128), NA * 64)
            g = _dot(xs, wg_v[t, :, cols])
            a = g * jax.nn.sigmoid(g) * _dot(xs, wu_v[t, :, cols])
            a = jnp.concatenate([jnp.where(j == 4, 0.0, a[:, 0:NDUP]), a[:, NDUP:]], axis=1)
            return acc + _dot(a.astype(bf16), wd_v[t, cols, :])[0:8]

        y8 = lax.fori_loop(0, 6, step, jnp.zeros((8, D), f32))
        undo.wait()
        patch(idx, y8, jax.nn.sigmoid(rmax))
        redo = cp_patch(idx)
        redo.start()
        redo.wait()


@jax.jit
def pallas_sequential_preLN__linear_kernel_hedgehog__moe_arch_mod__prompt_kernel(
    A_x: jax.Array,
    A_wqkv: jax.Array,
    A_w_phi: jax.Array,
    A_wo: jax.Array,
    B_x: jax.Array,
    B_w_r: jax.Array,
    B_w_gate: jax.Array,
    B_w_up: jax.Array,
    B_w_down: jax.Array,
):
    del B_x
    any_spec = pl.BlockSpec(memory_space=pl.ANY)
    return pl.pallas_call(
        _kernel,
        out_shape=jax.ShapeDtypeStruct((1, S, D), bf16),
        in_specs=[any_spec] * 8,
        out_specs=any_spec,
        scratch_shapes=[
            pltpu.VMEM((S, D), bf16),
            pltpu.VMEM((D, 3 * D), bf16),
            pltpu.VMEM((D // 128, D, 128), bf16),
            pltpu.VMEM((H, DH, DH), bf16),
            pltpu.VMEM((D // 128, D, 128), bf16),
            pltpu.VMEM((D // 128, D // 2, 128), u32),
            pltpu.VMEM((D,), bf16),
            pltpu.VMEM((3, D, NA * 128), bf16),
            pltpu.VMEM((3, D, NA * 128), bf16),
            pltpu.VMEM((3, NA * 128, D), bf16),
            pltpu.VMEM(((KR + D) // 2, D), u32),
            pltpu.VMEM((KR // 2, D), u32),
            pltpu.VMEM((8, 64, 128), u32),
            pltpu.VMEM(((S + C) // 2, D), u32),
            pltpu.VMEM((D // 4, C), u32),
            pltpu.VMEM((D // 4, C), u32),
            pltpu.VMEM((S + C, D), bf16),
            pltpu.VMEM((NP, 64, 128), f32),
            pltpu.VMEM((NP, 128, 128), f32),
            pltpu.VMEM((NP, 128, 128), f32),
            pltpu.VMEM((C, D), f32),
            pltpu.VMEM((S + C, D), bf16),
            pltpu.VMEM((8, 128), u32),
            pltpu.SMEM((8, 128), u32),
            pltpu.VMEM((1 + N1, 8, 128), f32),
            pltpu.VMEM((NT, 8, 128), f32),
            pltpu.VMEM((D, 128), f32),
            pltpu.VMEM((16, NA * 256), f32),
            pltpu.VMEM((8, D), f32),
            pltpu.VMEM((16, D), bf16),
            pltpu.SMEM((NU + 4,), i32),
            pltpu.SemaphoreType.DMA((72,)),
        ],
        compiler_params=pltpu.CompilerParams(vmem_limit_bytes=100 * 1024 * 1024,
                                             disable_bounds_checks=True,
                                             disable_semaphore_checks=True),
        name="hedgehog_mod",
    )(A_x, A_wqkv, A_w_phi, A_wo, B_w_r, B_w_gate, B_w_up, B_w_down)
```
